```python
import jax
import jax.numpy as jnp

def _softmax(x, axis=-1):
    return jax.nn.softmax(x, axis=axis)

def _gelu(x):
    return jax.nn.gelu(x, approximate=True)

def _silu(x):
    return jax.nn.silu(x)

def _sigmoid(x):
    return jax.nn.sigmoid(x)

def _layernorm(x, axis=-1, eps=1e-05):
    m = jnp.mean(x, axis=axis, keepdims=True)
    v = jnp.var(x, axis=axis, keepdims=True)
    return (x - m) / jnp.sqrt(v + eps)

def _scatter_add(tgt, idx, src, axis=0):
    return tgt.at[idx].add(src)

def _segment_sum(src, seg, n):
    return jax.ops.segment_sum(src, seg, n)

class _Rng:

    def __init__(self, key):
        self._k = key

    def _next(self):
        self._k, sub = jax.random.split(self._k)
        return sub

    def normal(self, shape):
        return jax.random.normal(self._next(), shape, dtype=jnp.bfloat16)

    def randint(self, lo, hi, shape):
        return jax.random.randint(self._next(), shape, lo, hi, dtype=jnp.int32)

    def uniform(self, shape, lo=0.0, hi=1.0):
        return jax.random.uniform(self._next(), shape, jnp.bfloat16, lo, hi)

    def permutation(self, n):
        return jax.random.permutation(self._next(), n)
kernel_name = 'gated_mix__sliding_local_dilated__memory_aug_recurrent_mem_tr__prompt'

def setup_inputs():
    _rng = _Rng(jax.random.key(int.from_bytes(__import__("os").urandom(4), "little")))
    _w = lambda a: (lambda t: t.astype(jnp.bfloat16) if jnp.issubdtype(t.dtype, jnp.floating) else t)(jnp.asarray(a))

    def _A_setup():
        B, S, D = (1, 2048, 576)
        return {'x': _w((lambda *s: _rng.normal(s) * 0.05)(B, S, D)), 'wqkv': _w((lambda *s: _rng.normal(s) * 0.05)(D, 3 * D)), 'wo': _w((lambda *s: _rng.normal(s) * 0.05)(D, D))}
    _A_in = _A_setup()

    def _B_setup():
        B, S, Dm = (1, 2048, 576)
        H, Dh = (32, 128)
        M, seg = (8, 32)
        seg = min(seg, S)
        S = S // seg * seg
        return {'x': _w((lambda *s: _rng.normal(s) * 0.05)(B, S, Dm)), 'mem0': _w((lambda *s: _rng.normal(s) * 0.05)(B, M, Dm)), 'Wq': _w((lambda *s: _rng.normal(s) * 0.05)(Dm, H, Dh) * Dm ** (-0.5)), 'Wk': _w((lambda *s: _rng.normal(s) * 0.05)(Dm, H, Dh) * Dm ** (-0.5)), 'Wv': _w((lambda *s: _rng.normal(s) * 0.05)(Dm, H, Dh) * Dm ** (-0.5)), 'Wo': _w((lambda *s: _rng.normal(s) * 0.05)(H, Dh, Dm) * (H * Dh) ** (-0.5)), 'seg_len': seg}
    _B_in = _B_setup()
    return {'A_x': _A_in['x'], 'A_wqkv': _A_in['wqkv'], 'A_wo': _A_in['wo'], 'B_x': _B_in['x'], 'B_mem0': _B_in['mem0'], 'B_Wq': _B_in['Wq'], 'B_Wk': _B_in['Wk'], 'B_Wv': _B_in['Wv'], 'B_Wo': _B_in['Wo'], 'B_seg_len': _B_in['seg_len'], 'gate_w': _w((lambda *s: _rng.normal(s) * 0.05)(576))}

def reference(A_x, A_wqkv, A_wo, B_x, B_mem0, B_Wq, B_Wk, B_Wv, B_Wo, B_seg_len, gate_w):

    def _A_ref(x, wqkv, wo):
        B, S, D = x.shape
        H = 32
        Dh = D // H
        W, dil = (8, 2)
        qkv = (lambda x, *d: x.transpose(*d))((x @ wqkv).reshape(B, S, 3, H, Dh), 2, 0, 3, 1, 4)
        q, k, v = (qkv[0], qkv[1], qkv[2])
        scale = Dh ** (-0.5)
        pos = jnp.arange(S)
        off = jnp.arange(W) * dil
        idx = pos[:, None] - off[None, :]
        mask = idx >= 0
        idx_c = jnp.where(mask, idx, 0).reshape(-1)
        kg = k[:, :, idx_c, :].reshape(B, H, S, W, Dh)
        vg = v[:, :, idx_c, :].reshape(B, H, S, W, Dh)
        logits = jnp.einsum('bhsd,bhswd->bhsw', q, kg) * scale
        logits = jnp.where(mask[None, None, :, :], logits, -1000000000.0)
        attn = _softmax(logits, axis=-1)
        o = jnp.einsum('bhsw,bhswd->bhsd', attn, vg)
        return (lambda x, *d: x.transpose(*d))(o, 0, 2, 1, 3).reshape(B, S, D) @ wo

    def _B_ref(x, mem0, Wq, Wk, Wv, Wo, seg_len):
        B, S, Dm = x.shape
        H, Dh = (Wq.shape[1], Wq.shape[2])
        M = mem0.shape[1]
        scale = Dh ** (-0.5)
        n_seg = S // seg_len
        L = M + seg_len
        idx = jnp.arange(L)
        mask = (idx[:, None] < M) | (idx[:, None] >= idx[None, :])
        mem = mem0
        outs = []
        for s in range(n_seg):
            xs = x[:, s * seg_len:(s + 1) * seg_len, :].copy()
            h = jnp.concatenate([mem, xs], axis=1)
            q = jnp.einsum('btd,dhe->bhte', h, Wq)
            k = jnp.einsum('btd,dhe->bhte', h, Wk)
            v = jnp.einsum('btd,dhe->bhte', h, Wv)
            scores = jnp.einsum('bhqe,bhke->bhqk', q, k) * scale
            scores = jnp.where(mask[None, None], scores, -1000000000.0)
            p = _softmax(scores, axis=-1)
            o = jnp.einsum('bhqk,bhke->bhqe', p, v)
            o = jnp.einsum('bhte,hed->btd', o, Wo)
            mem = o[:, :M, :].copy()
            outs.append(o[:, M:, :])
        return jnp.concatenate(outs, axis=1)
    x = A_x
    g = _sigmoid((x * gate_w).sum(-1, keepdims=True))
    a = _A_ref(x, A_wqkv, A_wo)
    b = _B_ref(x, B_mem0, B_Wq, B_Wk, B_Wv, B_Wo, B_seg_len)
    return g * a + (1 - g) * b
```

```python
import functools

import jax
import jax.numpy as jnp
from jax import lax
import jax.experimental.pallas as pl
import jax.experimental.pallas.tpu as pltpu

F32, BF16, I32 = jnp.float32, jnp.bfloat16, jnp.int32

S, D = 2048, 576
NB = S // 128
HA, DA, WIN, DIL = 32, 18, 8, 2
H, DH, M, SEG = 32, 128, 8, 32
L = M + SEG
NP = H // 2
U = 128 // SEG
NEG = -1000000000.0

QA = 0
KA = QA + 576
K2 = KA + 512
VA = K2 + 64
PV = VA + 512
OA = PV + 128
PSTRIDE = OA + 640 + 8
HS = NP * PSTRIDE
GS = HS + U * 200
GT = GS + 64
QS = GT + 64
KS = QS + H * 40
RE = KS + NP * 64
PS = RE + H * 40
RS = PS + NP * 40
OS = RS + NP * 40
XN = OS + H * 40
BO = XN + 320
B_ROWS = BO + 640

WT = 0
GW = WT + 5 * 1728
WOT = GW + 40
AQ = WOT + 5 * 288
AK = AQ + 3 * 576
AV = AK + 3 * 288
AG = AV + 3 * 288
A_ROWS = AG + 24


def _dot(a, b):
    return lax.dot_general(a, b, (((1,), (0,)), ((), ())), preferred_element_type=F32)


class _Arena:
    def __init__(self, ref):
        self.r = ref

    def ldi(self, o, n):
        return self.r[o:o + n, :]

    def ldf(self, o, n):
        return pltpu.bitcast(self.r[o:o + n, :], F32)

    def ldb(self, o, n):
        return pltpu.bitcast(self.r[o:o + n, :], BF16)

    def stf(self, o, v):
        self.r[o:o + v.shape[0], :] = pltpu.bitcast(v, I32)

    def stb(self, o, v):
        self.r[o:o + v.shape[0] // 2, :] = pltpu.bitcast(v.astype(BF16), I32)


def _pad2(t, rows, cols):
    r, c = t.shape
    if c < cols:
        t = jnp.concatenate([t, jnp.zeros((r, cols - c), t.dtype)], 1)
    if r < rows:
        t = jnp.concatenate([t, jnp.zeros((rows - r, cols), t.dtype)], 0)
    return t


def _a_transpose_w(A, w_ref, cblocks):
    for c in cblocks:
        nc = min(128, 3 * D - 128 * c)
        for k in range(5):
            nk = min(128, D - 128 * k)
            t = _pad2(w_ref[128 * k:128 * k + nk, 128 * c:128 * c + nc], 128, 128).T
            A.stf(WT + 1728 * k + 128 * c, t[:nc].astype(F32))


def _a_transpose_wo(A, w_ref):
    for c in range(5):
        nc = min(128, D - 128 * c)
        for k in range(5):
            nk = min(128, D - 128 * k)
            t = _pad2(w_ref[128 * k:128 * k + nk, 128 * c:128 * c + nc], 128, 128).T
            A.stb(WOT + 288 * k + 64 * c, t[:nc])


def _a_qkv(A, xb, slot):
    def lhs(rows_of_k):
        ch = [rows_of_k(k) for k in range(5)]
        return jnp.concatenate(ch[:4] + [ch[4][:, :64]], 1)

    for part in (1, 0, 2):
        for d0 in range(0, DA, 3):
            w = lhs(lambda k: jnp.concatenate([
                pltpu.bitcast(A.r[pl.ds(WT + 1728 * k + D * part + d, HA, stride=DA), :], F32)
                for d in range(d0, d0 + 3)], 0))
            r = _dot(w, xb)
            if part == 0:
                A.stf(AQ + 576 * slot + 32 * d0, r)
            else:
                A.stb((AK if part == 1 else AV) + 288 * slot + 16 * d0, r)
    A.stf(AG + 8 * slot, jax.nn.sigmoid(_dot(lhs(lambda k: A.ldf(GW + 8 * k, 8)), xb)))


def _a_attend(A, j, slot, prev, o_ref, omg_ref):
    lane = lax.broadcasted_iota(I32, (8, 128), 1)
    pos = j * 128 + lax.broadcasted_iota(I32, (16, 128), 1)
    g = A.ldf(AG + 8 * slot, 8)
    omg_ref[j] = 1.0 - g
    g2 = jnp.concatenate([g, g], 0)

    def window(base, d, hg):
        cur = A.ldi(base + 288 * slot + 16 * d + 8 * hg, 8)
        old = A.ldi(base + 288 * prev + 16 * d + 8 * hg, 8)
        out = []
        for w in range(WIN):
            sh = DIL * w
            t = cur if w == 0 else pltpu.roll(jnp.where(lane >= 128 - sh, old, cur), sh, 1)
            out.append(pltpu.bitcast(t, BF16).astype(F32))
        return out

    for hg in range(2):
        lg = None
        for d in range(DA):
            q = A.ldf(AQ + 576 * slot + 32 * d + 16 * hg, 16)
            pr = [q * kw for kw in window(AK, d, hg)]
            lg = pr if d == 0 else [a + b for a, b in zip(lg, pr)]
        lg = [jnp.where(pos >= DIL * w, t * DA ** -0.5, NEG) for w, t in enumerate(lg)]
        mx = functools.reduce(jnp.maximum, lg)
        e = [jnp.exp(t - mx) for t in lg]
        r = g2 / functools.reduce(jnp.add, e)
        p = [t * r for t in e]
        for d in range(DA):
            o = functools.reduce(jnp.add, [a * b for a, b in zip(p, window(AV, d, hg))])
            o_ref[pl.ds(16 * DA * hg + d, 16, stride=DA), :] = o


def _a_out(A, o_ref, ga_ref):
    ob = o_ref[...].astype(BF16)
    for r0 in range(0, D, 96):
        ch = [A.ldb(WOT + 288 * k + r0 // 2, 48) for k in range(5)]
        ga_ref[r0:r0 + 96, :] = _dot(jnp.concatenate(ch[:4] + [ch[4][:, :64]], 1), ob)


def _b_split_heads(raw, dst, offs):
    for r in range(32):
        e = pltpu.bitcast(raw[64 * r:64 * r + 32, :], I32)
        o = pltpu.bitcast(raw[64 * r + 32:64 * r + 64, :], I32)
        dst[pl.ds(offs[0] + r, NP, stride=PSTRIDE), :] = (e & 0xFFFF) | (o << 16)
        dst[pl.ds(offs[1] + r, NP, stride=PSTRIDE), :] = lax.shift_right_logical(e, 16) | (o & -65536)


def _b_transpose_wo(wot, dst):
    for h in range(8):
        for n in range(5):
            if n < 4:
                t = wot[h, 128 * n:128 * n + 128, :]
            else:
                t = jnp.concatenate([wot[h, 512:576, :]] * 2, 0)
            o = PSTRIDE * (h // 2) + OA + 320 * (h % 2) + 64 * n
            dst[o:o + 64, :] = pltpu.bitcast(t.T, I32)


def _b_step(B, u, extra):
    hs, hs_next = HS + 200 * u, HS + 200 * ((u + 1) % U)
    row = lax.broadcasted_iota(I32, (L, 128), 0)
    lane = lax.broadcasted_iota(I32, (L, 128), 1)
    lo = lane < 64
    lo64 = lax.broadcasted_iota(I32, (64, 128), 1) < 64
    col = lane & 63
    mask = (col < L) & ((row < M) | (row >= col))
    fill = jnp.where(col < L, NEG, -jnp.inf).astype(F32)
    z24 = jnp.zeros((24, 128), F32)
    z8 = jnp.zeros((8, 128), F32)

    def w(base, size, h):
        return PSTRIDE * (h // 2) + base + size * (h % 2)

    def h1():
        return jnp.concatenate([B.ldf(hs + 40 * n, 40) for n in range(4)], 1)

    def t_g():
        c4 = B.ldf(hs + 160, 40)
        g = jnp.concatenate([jnp.where(lo, 0.0, c4), z24, jnp.where(lo, c4, 0.0), z24], 0)
        B.stb(GS, g)
        B.stb(GT, g.T)

    k1 = {}

    def t_k(h):
        k1[h] = _dot(h1(), B.ldb(w(KA, 256, h), 256))
        if h % 2:
            B.stb(KS + 64 * (h // 2), jnp.concatenate([k1[h - 1], z24, k1[h], z24], 0).astype(BF16).T)

    def t_q(h):
        o = w(QA, 288, h)
        B.stf(QS + 40 * h, _dot(h1(), B.ldb(o, 256)) + _dot(B.ldf(hs + 160, 40)[:, :64], B.ldb(o + 256, 32)))

    def t_s(h):
        kt, w2 = B.ldi(KS + 64 * (h // 2), 64), B.ldi(w(K2, 0, h), 64)
        rhs = jnp.where(lo64, w2, kt) if h % 2 else jnp.where(lo64, kt, w2)
        B.stf(RE + 40 * h, _dot(B.ldf(QS + 40 * h, 40), pltpu.bitcast(rhs, BF16)))

    def t_s2(j):
        a, b = B.ldf(RE + 80 * j, 40), B.ldf(RE + 80 * j + 40, 40)
        s = jnp.where(lo, a, b) + _dot(jnp.where(lo, b, a), B.ldb(GT, 64))
        s = jnp.where(mask, s * DH ** -0.5, fill)
        ma = jnp.max(jnp.where(lo, s, -jnp.inf), axis=1, keepdims=True)
        mb = jnp.max(jnp.where(lo, -jnp.inf, s), axis=1, keepdims=True)
        e = jnp.exp(s - jnp.where(lo, ma, mb))
        la = jnp.sum(jnp.where(lo, e, 0.0), axis=1, keepdims=True)
        lb = jnp.sum(jnp.where(lo, 0.0, e), axis=1, keepdims=True)
        B.stf(PS + 40 * j, e / jnp.where(lo, la, lb))

    def t_r(j):
        B.stf(RS + 40 * j, _dot(B.ldf(PS + 40 * j, 40), B.ldb(GS, 64)))

    def t_v(h):
        v = _dot(h1(), B.ldb(w(VA, 256, h), 256))
        B.stb(w(PV, 96, h), jnp.concatenate([v, z8], 0))

    def t_pv(h):
        p, r = B.ldf(PS + 40 * (h // 2), 40), B.ldf(RS + 40 * (h // 2), 40)
        lhs = jnp.where(lo, r, p) if h % 2 else jnp.where(lo, p, r)
        B.stf(OS + 40 * h, _dot(lhs, B.ldb(w(PV, 64, h), 64)))

    d_s, d_s2, d_r, d_pv, ahead = 20, 18, 64, 22, 7
    big = [("k", h) for h in range(ahead)] + [("g",)]
    for h in range(H):
        if h + ahead < H:
            big.append(("k", h + ahead))
        big.append(("q", h))
    big += [("v", h) for h in range(H)]
    big += [("o", n, h) for n in range(5) for h in range(H)]
    small = {"pv": t_pv, "r": t_r, "s2": t_s2, "s": t_s}
    nxt = dict.fromkeys(small, 0)
    done = {}
    now = 0

    def old(key, dist):
        return key in done and now - done[key] >= dist

    def ready(kind, i):
        if kind == "s":
            return old(("q", i), d_s)
        if kind == "s2":
            return old(("s", 2 * i + 1), d_s2)
        if kind == "r":
            return old(("s2", i), d_r)
        return old(("r", i // 2), d_s2) and old(("v", i), d_pv)

    acc = None
    for t in big:
        for kind, fn in small.items():
            if ready(kind, nxt[kind]):
                fn(nxt[kind])
                now += 1
                done[kind, nxt[kind]] = now
                nxt[kind] += 1
        if t in extra:
            extra[t]()
        if t[0] == "k":
            t_k(t[1])
            now += 4
        elif t[0] == "g":
            t_g()
        elif t[0] == "q":
            t_q(t[1])
            now += 5
        elif t[0] == "v":
            t_v(t[1])
            now += 4
        else:
            _, n, h = t
            assert ("pv", h) in done
            y = _dot(B.ldf(OS + 40 * h, 40), B.ldb(w(OA, 320, h) + 64 * n, 64))
            acc = y if h == 0 else acc + y
            if h == H - 1:
                B.stf(hs_next + 40 * n, acc[:M])
                B.stf(BO + 128 * n + SEG * u, acc[M:])
            now += 1
        done[t] = now


def _kernel(xt_hbm, wqkv_hbm, wo_hbm, mem_ref, gate_ref, wq_hbm, wk_hbm, wv_hbm, wot_hbm,
            out_hbm,
            xt, wqkv, wo, raw_q, raw_k, raw_v, raw_o, a_ref, b_ref, o_all, ga_all, omg, out_buf,
            sem_in, sem_w, sem_out):
    A, B = _Arena(a_ref), _Arena(b_ref)
    raws = ((wq_hbm, raw_q), (wk_hbm, raw_k), (wv_hbm, raw_v))

    x_first = pltpu.make_async_copy(xt_hbm.at[:, pl.ds(0, 512)], xt.at[:, pl.ds(0, 512)], sem_in.at[0])
    x_rest = pltpu.make_async_copy(xt_hbm.at[:, pl.ds(512, S - 512)], xt.at[:, pl.ds(512, S - 512)], sem_in.at[1])
    w_copy = pltpu.make_async_copy(wqkv_hbm, wqkv, sem_in.at[2])
    wo_copy = pltpu.make_async_copy(wo_hbm, wo, sem_in.at[3])

    def quarter(i):
        rows = pl.ds(pl.multiple_of(i * 4096, 4096), 4096)
        cps = [pltpu.make_async_copy(s.at[rows], d.at[rows], sem_w.at[i]) for s, d in raws]
        heads = pl.ds(i * 8, 8)
        return cps + [pltpu.make_async_copy(wot_hbm.at[heads], raw_o.at[heads], sem_w.at[i])]

    tail = [pltpu.make_async_copy(s.at[pl.ds(16384, 2048)], d.at[pl.ds(16384, 2048)], sem_in.at[4])
            for s, d in raws]

    def xblock(j):
        return xt[:, pl.ds(pl.multiple_of(j * 128, 128), 128)]

    w_copy.start()
    x_first.start()

    gate = jnp.broadcast_to(gate_ref[...].astype(F32), (8, D))
    mem0 = mem_ref[...].astype(F32)
    for k in range(4):
        A.stf(GW + 8 * k, gate[:, 128 * k:128 * k + 128])
        B.stf(HS + 40 * k, mem0[:, 128 * k:128 * k + 128])
    A.stf(GW + 32, jnp.concatenate([gate[:, 512:]] * 2, 1))
    B.stf(HS + 160, jnp.concatenate([mem0[:, 512:]] * 2, 1))
    for j in range(NP):
        B.stf(PSTRIDE * j + PV + 24, jnp.zeros((8, 128), F32))
        B.stf(PSTRIDE * j + PV + 120, jnp.zeros((8, 128), F32))
    B.stf(BO, jnp.zeros((640, 128), F32))

    w_copy.wait()
    x_rest.start()
    wo_copy.start()
    for c in tail:
        c.start()
    _a_transpose_w(A, wqkv, range(14))
    x_first.wait()
    _a_qkv(A, xblock(0), 0)
    for base in (AK, AV):
        a_ref[base + 576:base + 864, :] = jnp.broadcast_to(A.ldi(base, 288)[:, :1], (288, 128))

    def a_body(t, carry):
        @pl.when(t < 4)
        def _():
            for c in quarter(t):
                c.start()

        @pl.when(t == 1)
        def _():
            x_rest.wait()

        for i in range(3):
            j = 3 * t + i
            _a_attend(A, j, i, (i + 2) % 3, o_all.at[j], omg)
            _a_qkv(A, xblock(j + 1), (i + 1) % 3)
        return carry

    lax.fori_loop(0, 5, a_body, 0)

    def b_prepare(i):
        for c in range(2):
            src = pl.ds(pl.multiple_of((2 * i + c) * 2048, 2048), 2048)
            dst = b_ref.at[pl.ds(pl.multiple_of((2 * i + c) * 32, 32), NP * PSTRIDE), :]
            _b_split_heads(raw_q.at[src], dst, (QA, QA + 288))
            _b_split_heads(raw_k.at[src], dst, (KA, KA + 256))
            _b_split_heads(raw_v.at[src], dst, (VA, VA + 256))
        _b_transpose_wo(raw_o.at[pl.ds(i * 8, 8)],
                        b_ref.at[pl.ds(pl.multiple_of(i * 4 * PSTRIDE, 8), 4 * PSTRIDE), :])

    wo_copy.wait()
    for c in tail:
        c.wait()
    _a_transpose_wo(A, wo)
    _a_attend(A, NB - 1, 0, 2, o_all.at[NB - 1], omg)
    src = pl.ds(16384, 2048)
    _b_split_heads(raw_q.at[src], b_ref, (QA + 256, QA + 544))
    _b_split_heads(raw_k.at[src], b_ref, (K2 + 32, K2))
    _b_split_heads(raw_v.at[src], b_ref, (PV + 32, PV + 64))
    for j in range(NP):
        B.stb(PSTRIDE * j + K2, B.ldb(PSTRIDE * j + K2, 64).T)

    def out_body(i, carry):
        for c in quarter(i):
            c.wait()
        for b in range(4):
            _a_out(A, o_all.at[4 * i + b], ga_all.at[4 * i + b])
        b_prepare(i)
        return carry

    lax.fori_loop(0, 4, out_body, 0)

    def x_transpose(j, n):
        cols = pl.ds(pl.multiple_of(j * 128, 128), 128)
        if n < 4:
            t = xt[128 * n:128 * n + 128, cols]
        else:
            t = jnp.concatenate([xt[512:576, cols]] * 2, 0)
        B.stb(XN + 64 * n, t.T)

    def x_place(u):
        for n in range(5):
            B.stf(HS + 200 * u + 40 * n + M, B.ldb(XN + 64 * n + 16 * u, 16).astype(F32))

    def mix(j, n):
        rows = min(128, D - 128 * n)
        bt = B.ldf(BO + 128 * n, 128).T[:rows]
        w = jnp.concatenate([omg[j]] * (rows // 8), 0)
        out_buf[j, 128 * n:128 * n + rows, :] = (
            ga_all[j, 128 * n:128 * n + rows, :] + w * bt).astype(BF16)

    def out_copy(j):
        return pltpu.make_async_copy(
            out_buf.at[j], out_hbm.at[:, pl.ds(pl.multiple_of(j * 128, 128), 128)], sem_out)

    for n in range(5):
        x_transpose(0, n)
    for u in range(U):
        x_place(u)

    def b_body(g, carry):
        jn, jp = jnp.minimum(g + 1, NB - 1), jnp.maximum(g - 1, 0)
        for u in range(U):
            extra = {("o", 3, 0): functools.partial(x_place, u)}
            if u == 0:
                for n in range(5):
                    extra["v", 20 + 2 * n] = functools.partial(mix, jp, n)
                    extra["o", 0, 6 * n] = functools.partial(x_transpose, jn, n)
            _b_step(B, u, extra)

        @pl.when(g > 0)
        def _():
            out_copy(jp).start()

        return carry

    lax.fori_loop(0, NB, b_body, 0)
    for n in range(5):
        mix(NB - 1, n)
    out_copy(NB - 1).start()
    for j in range(NB):
        out_copy(j).wait()


@functools.partial(jax.jit, static_argnames=("B_seg_len",))
def pallas_gated_mix__sliding_local_dilated__memory_aug_recurrent_mem_tr__prompt_kernel(
    A_x: jax.Array,
    A_wqkv: jax.Array,
    A_wo: jax.Array,
    B_x: jax.Array,
    B_mem0: jax.Array,
    B_Wq: jax.Array,
    B_Wk: jax.Array,
    B_Wv: jax.Array,
    B_Wo: jax.Array,
    B_seg_len: int,
    gate_w: jax.Array,
):
    del B_x
    assert A_x.shape == (1, S, D) and B_mem0.shape == (1, M, D) and B_Wq.shape == (D, H, DH)
    assert B_seg_len == SEG
    hbm = pl.BlockSpec(memory_space=pl.ANY)
    vmem = pl.BlockSpec(memory_space=pltpu.VMEM)
    out_t = pl.pallas_call(
        _kernel,
        out_shape=jax.ShapeDtypeStruct((D, S), BF16),
        in_specs=[hbm, hbm, hbm, vmem, vmem, hbm, hbm, hbm, hbm],
        out_specs=hbm,
        scratch_shapes=[
            pltpu.VMEM((D, S), BF16),
            pltpu.VMEM((D, 3 * D), BF16),
            pltpu.VMEM((D, D), BF16),
            pltpu.VMEM((D * H, DH), BF16),
            pltpu.VMEM((D * H, DH), BF16),
            pltpu.VMEM((D * H, DH), BF16),
            pltpu.VMEM((H, D, DH), BF16),
            pltpu.VMEM((A_ROWS, 128), I32),
            pltpu.VMEM((B_ROWS, 128), I32),
            pltpu.VMEM((NB, D, 128), F32),
            pltpu.VMEM((NB, D, 128), F32),
            pltpu.VMEM((NB, 8, 128), F32),
            pltpu.VMEM((NB, D, 128), BF16),
            pltpu.SemaphoreType.DMA((5,)),
            pltpu.SemaphoreType.DMA((4,)),
            pltpu.SemaphoreType.DMA,
        ],
        compiler_params=pltpu.CompilerParams(vmem_limit_bytes=100 * 1024 * 1024),
    )(
        A_x.reshape(S, D).T, A_wqkv, A_wo, B_mem0.reshape(M, D), gate_w.reshape(1, D),
        B_Wq.reshape(D * H, DH), B_Wk.reshape(D * H, DH), B_Wv.reshape(D * H, DH),
        B_Wo.transpose(0, 2, 1),
    )
    return out_t.T.reshape(1, S, D)
```

```python
import functools

import jax
import jax.numpy as jnp
from jax import lax
import jax.experimental.pallas as pl
import jax.experimental.pallas.tpu as pltpu

F32, BF16, I32 = jnp.float32, jnp.bfloat16, jnp.int32

S, D = 2048, 576
NB = S // 128
HA, DA, WIN, DIL = 32, 18, 8, 2
H, DH, M, SEG = 32, 128, 8, 32
L = M + SEG
NP = H // 2
U = 128 // SEG
NEG = -1000000000.0

QA = 0
KA = QA + 576
K2 = KA + 512
VA = K2 + 64
PV = VA + 512
PSTRIDE = PV + 128 + 4
OA = NP * PSTRIDE
HS = OA + H * 320
GS = HS + U * 200
GT = GS + 64
QS = GT + 64
KS = QS + H * 40
RE = KS + NP * 64
PS = RE + H * 40
RS = PS + NP * 40
OS = RS + NP * 40
XN = OS + H * 40
BO = XN + 320
B_ROWS = BO + 640

PART = 3 * 2048 + 4 * D + 16
RAW_TICK = 4 * PART - 16

WT = 0
GW = WT + 5 * 1728
WOT = GW + 40
AX = WOT + 5 * 288
AO = AX + 2 * 288
A_ROWS = AO + 2 * 288
AQ, AK, AV, AG, TICK, SLOT = 0, 576, 864, 1152, 1160, 1168


def _dot(a, b):
    return lax.dot_general(a, b, (((1,), (0,)), ((), ())), preferred_element_type=F32)


class _Arena:
    def __init__(self, ref):
        self.r = ref

    def ldi(self, o, n):
        return self.r[o:o + n, :]

    def ldf(self, o, n):
        return pltpu.bitcast(self.r[o:o + n, :], F32)

    def ldb(self, o, n):
        return pltpu.bitcast(self.r[o:o + n, :], BF16)

    def stf(self, o, v):
        self.r[o:o + v.shape[0], :] = pltpu.bitcast(v, I32)

    def stb(self, o, v):
        self.r[o:o + v.shape[0] // 2, :] = pltpu.bitcast(v.astype(BF16), I32)


def _pad2(t, rows, cols):
    r, c = t.shape
    if c < cols:
        t = jnp.concatenate([t, jnp.zeros((r, cols - c), t.dtype)], 1)
    if r < rows:
        t = jnp.concatenate([t, jnp.zeros((rows - r, cols), t.dtype)], 0)
    return t


def _interleave(main, *side, span=(0.0, 0.9)):
    jobs = (main,) + side
    order = [((i + 1) / main[0], 0) for i in range(main[0])]
    order += [(span[0] + (span[1] - span[0]) * i / n, k + 1) for k, (n, _) in enumerate(side) for i in range(n)]
    for _, k in sorted(order):
        next(jobs[k][1])
    for _, gen in jobs:
        assert next(gen, "end") == "end"


def _chain(*jobs):
    def gen():
        for _, g in jobs:
            yield from g
    return sum(n for n, _ in jobs), gen()


def _a_transpose_w(A, w_ref, cblocks):
    for c in cblocks:
        nc = min(128, 3 * D - 128 * c)
        for k in range(5):
            nk = min(128, D - 128 * k)
            t = _pad2(w_ref[128 * k:128 * k + nk, 128 * c:128 * c + nc], 128, 128).T
            A.stf(WT + 1728 * k + 128 * c, t[:nc].astype(F32))


def _a_transpose_wo(A, w_ref):
    def gen():
        for c in range(5):
            nc = min(128, D - 128 * c)
            for k in range(5):
                nk = min(128, D - 128 * k)
                t = _pad2(w_ref[128 * k:128 * k + nk, 128 * c:128 * c + nc], 128, 128).T
                A.stb(WOT + 288 * k + 64 * c, t[:nc])
                yield
    return 25, gen()


def _a_qkv(A, x_off, dst, tick, parts=(3, 1, 0, 2)):
    def proj(rows_of_k):
        ch = [rows_of_k(k) for k in range(5)]
        return _dot(jnp.concatenate(ch[:4] + [ch[4][:, :64]], 1), A.ldb(x_off, 288))

    def gen():
        for part in parts:
            if part == 3:
                dst.stf(AG, jax.nn.sigmoid(proj(lambda k: A.ldf(GW + 8 * k, 8))))
                continue
            for d0 in range(0, DA, 2):
                r = proj(lambda k: jnp.concatenate([
                    pltpu.bitcast(A.r[pl.ds(WT + 1728 * k + D * part + 8 * DA * hg + d, 8, stride=DA), :], F32)
                    for hg in range(4) for d in (d0, d0 + 1)], 0))
                tick(r)
                if part == 0:
                    dst.stf(AQ + 32 * d0, r)
                else:
                    dst.stb((AK if part == 1 else AV) + 16 * d0, r)
                yield
    return sum(DA // 2 for p in parts if p < 3), gen()


def _a_attend(j, cur, old, o_ref, omg_ref):
    def window(o):
        lane = lax.broadcasted_iota(I32, (8, 128), 1)
        c, p = cur.ldi(o, 8), old.ldi(o, 8)
        out = []
        for w in range(WIN):
            sh = DIL * w
            t = c if w == 0 else pltpu.roll(jnp.where(lane >= 128 - sh, p, c), sh, 1)
            out.append(pltpu.bitcast(t, BF16).astype(F32))
        return out

    def gen():
        pos = j * 128 + lax.broadcasted_iota(I32, (8, 128), 1)
        for hg in range(4):
            lg = None
            for d in range(0, DA, 2):
                q = cur.ldf(AQ + 32 * d + 16 * hg, 16)
                pr = [q * kw for kw in window(AK + 16 * d + 8 * hg)]
                pr = [t[:8] + t[8:] for t in pr]
                lg = pr if d == 0 else [a + b for a, b in zip(lg, pr)]
                yield
            lg = [jnp.where(pos >= DIL * w, t * DA ** -0.5, NEG) for w, t in enumerate(lg)]
            mx = functools.reduce(jnp.maximum, lg)
            e = [jnp.exp(t - mx) for t in lg]
            g = cur.ldf(AG, 8)
            if hg == 0:
                omg_ref[j] = 1.0 - g
            r = g / functools.reduce(jnp.add, e)
            p = [jnp.concatenate([t * r] * 2, 0) for t in e]
            yield
            for d in range(0, DA, 2):
                o = functools.reduce(jnp.add, [a * b for a, b in zip(p, window(AV + 16 * d + 8 * hg))])
                o_ref[pl.ds(8 * DA * hg + d, 8, stride=DA), :] = o[:8]
                o_ref[pl.ds(8 * DA * hg + d + 1, 8, stride=DA), :] = o[8:]
                yield
    return 4 * DA + 4, gen()


def _a_out(A, o_off, ga_ref, tick):
    def gen():
        for r0 in range(0, D, 64):
            ch = [A.ldb(WOT + 288 * k + r0 // 2, 32) for k in range(5)]
            r = _dot(jnp.concatenate(ch[:4] + [ch[4][:, :64]], 1), A.ldb(o_off, 288))
            tick(r)
            ga_ref[r0:r0 + 64, :] = r
            yield
    return D // 64, gen()


def _b_split_heads(raw, dst, offs):
    def gen():
        for r in range(32):
            e = pltpu.bitcast(raw[64 * r:64 * r + 32, :], I32)
            o = pltpu.bitcast(raw[64 * r + 32:64 * r + 64, :], I32)
            dst[pl.ds(offs[0] + r, NP, stride=PSTRIDE), :] = (e & 0xFFFF) | (o << 16)
            dst[pl.ds(offs[1] + r, NP, stride=PSTRIDE), :] = lax.shift_right_logical(e, 16) | (o & -65536)
            yield
    return 32, gen()


def _b_transpose_wo(wot, dst):
    def gen():
        for h in range(4):
            for n in range(5):
                if n < 4:
                    t = wot[D * h + 128 * n:D * h + 128 * n + 128, :]
                else:
                    t = jnp.concatenate([wot[D * h + 512:D * h + 576, :]] * 2, 0)
                t = pltpu.bitcast(t.T, I32)
                o = OA + 512 * (5 * h + n)
                dst[o:o + 32, :] = t[:32]
                dst[o + 256:o + 288, :] = t[32:]
                yield
    return 20, gen()


def _b_step(B, u, extra):
    hs, hs_next = HS + 200 * u, HS + 200 * ((u + 1) % U)
    row = lax.broadcasted_iota(I32, (L, 128), 0)
    lane = lax.broadcasted_iota(I32, (L, 128), 1)
    lo = lane < 64
    lo64 = lax.broadcasted_iota(I32, (64, 128), 1) < 64
    col = lane & 63
    mask = (col < L) & ((row < M) | (row >= col))
    fill = jnp.where(col < L, NEG, -jnp.inf).astype(F32)
    z24 = jnp.zeros((24, 128), F32)
    z8 = jnp.zeros((8, 128), F32)

    def w(base, size, h):
        return PSTRIDE * (h // 2) + base + size * (h % 2)

    def h1():
        return jnp.concatenate([B.ldf(hs + 40 * n, 40) for n in range(4)], 1)

    def t_g():
        c4 = B.ldf(hs + 160, 40)
        g = jnp.concatenate([jnp.where(lo, 0.0, c4), z24, jnp.where(lo, c4, 0.0), z24], 0)
        B.stb(GS, g)
        B.stb(GT, g.T)

    k1 = {}

    def t_k(h):
        k1[h] = _dot(h1(), B.ldb(w(KA, 256, h), 256))
        if h % 2:
            B.stb(KS + 64 * (h // 2), jnp.concatenate([k1[h - 1], z24, k1[h], z24], 0).astype(BF16).T)

    def t_q(h):
        o = w(QA, 288, h)
        B.stf(QS + 40 * h, _dot(h1(), B.ldb(o, 256)) + _dot(B.ldf(hs + 160, 40)[:, :64], B.ldb(o + 256, 32)))

    def t_s(h):
        kt, w2 = B.ldi(KS + 64 * (h // 2), 64), B.ldi(w(K2, 0, h), 64)
        rhs = jnp.where(lo64, w2, kt) if h % 2 else jnp.where(lo64, kt, w2)
        B.stf(RE + 40 * h, _dot(B.ldf(QS + 40 * h, 40), pltpu.bitcast(rhs, BF16)))

    def t_s2(j):
        a, b = B.ldf(RE + 80 * j, 40), B.ldf(RE + 80 * j + 40, 40)
        s = jnp.where(lo, a, b) + _dot(jnp.where(lo, b, a), B.ldb(GT, 64))
        s = jnp.where(mask, s * DH ** -0.5, fill)
        ma = jnp.max(jnp.where(lo, s, -jnp.inf), axis=1, keepdims=True)
        mb = jnp.max(jnp.where(lo, -jnp.inf, s), axis=1, keepdims=True)
        e = jnp.exp(s - jnp.where(lo, ma, mb))
        la = jnp.sum(jnp.where(lo, e, 0.0), axis=1, keepdims=True)
        lb = jnp.sum(jnp.where(lo, 0.0, e), axis=1, keepdims=True)
        B.stf(PS + 40 * j, e / jnp.where(lo, la, lb))

    def t_r(j):
        B.stf(RS + 40 * j, _dot(B.ldf(PS + 40 * j, 40), B.ldb(GS, 64)))

    def t_v(h):
        v = _dot(h1(), B.ldb(w(VA, 256, h), 256))
        B.stb(w(PV, 96, h), jnp.concatenate([v, z8], 0))

    def t_pv(h):
        p, r = B.ldf(PS + 40 * (h // 2), 40), B.ldf(RS + 40 * (h // 2), 40)
        lhs = jnp.where(lo, r, p) if h % 2 else jnp.where(lo, p, r)
        B.stf(OS + 40 * h, _dot(lhs, B.ldb(w(PV, 64, h), 64)))

    d_s, d_s2, d_r, d_pv, ahead = 20, 18, 64, 22, 7
    big = [("k", h) for h in range(ahead)] + [("g",)]
    for h in range(H):
        if h + ahead < H:
            big.append(("k", h + ahead))
        big.append(("q", h))
    big += [("v", h) for h in range(H)]
    big += [("o", n, h) for n in range(5) for h in range(H)]
    small = {"pv": t_pv, "r": t_r, "s2": t_s2, "s": t_s}
    nxt = dict.fromkeys(small, 0)
    done = {}
    now = 0

    def old(key, dist):
        return key in done and now - done[key] >= dist

    def ready(kind, i):
        if kind == "s":
            return old(("q", i), d_s)
        if kind == "s2":
            return old(("s", 2 * i + 1), d_s2)
        if kind == "r":
            return old(("s2", i), d_r)
        return old(("r", i // 2), d_s2) and old(("v", i), d_pv)

    acc = None
    for t in big:
        for kind, fn in small.items():
            if ready(kind, nxt[kind]):
                fn(nxt[kind])
                now += 1
                done[kind, nxt[kind]] = now
                nxt[kind] += 1
        if t in extra:
            extra[t]()
        if t[0] == "k":
            t_k(t[1])
            now += 4
        elif t[0] == "g":
            t_g()
        elif t[0] == "q":
            t_q(t[1])
            now += 5
        elif t[0] == "v":
            t_v(t[1])
            now += 4
        else:
            _, n, h = t
            assert ("pv", h) in done
            o = OA + 512 * (5 * (h % 4) + n) + 32 * (h // 4)
            wo = jnp.concatenate([B.ldi(o, 32), B.ldi(o + 256, 32)], 0)
            y = _dot(B.ldf(OS + 40 * h, 40), pltpu.bitcast(wo, BF16))
            acc = y if h == 0 else acc + y
            if h == H - 1:
                B.stf(hs_next + 40 * n, acc[:M])
                B.stf(BO + 128 * n + SEG * u, acc[M:])
            now += 1
        done[t] = now


def _kernel(xt_hbm, wqkv_hbm, wo_hbm, mem_hbm, gate_hbm, wq_hbm, wk_hbm, wv_hbm, wot_hbm,
            out_hbm,
            xt, wqkv, wo, mem_ref, gate_ref, raw, a_ref, b_ref, qkv_all, o_all, ga_all, omg, out_buf,
            offs, sem_in, sem_w, sem_out):
    A, B = _Arena(a_ref), _Arena(b_ref)

    def cols(src, dst, c0, c1, sem):
        return pltpu.make_async_copy(src.at[:, pl.ds(c0, c1 - c0)], dst.at[:, pl.ds(c0, c1 - c0)], sem_in.at[sem])

    x_copy = [cols(xt_hbm, xt, 0, 256, 0), cols(xt_hbm, xt, 256, 896, 1), cols(xt_hbm, xt, 896, S, 2)]
    w_copy = [cols(wqkv_hbm, wqkv, 512, 1152, 4), cols(wqkv_hbm, wqkv, 0, 512, 5),
              cols(wqkv_hbm, wqkv, 1152, 3 * D, 6)]
    wo_copy = pltpu.make_async_copy(wo_hbm, wo, sem_in.at[3])
    mem_copy = pltpu.make_async_copy(mem_hbm, mem_ref, sem_in.at[7])
    gate_copy = pltpu.make_async_copy(gate_hbm, gate_ref, sem_in.at[8])

    def b_start(i):
        srcs = [w.at[pl.ds(2048 * i, 2048)] for w in (wq_hbm, wk_hbm, wv_hbm)]
        if i < 8:
            srcs.append(wot_hbm.at[pl.ds(4 * D * i, 4 * D)])
        for m, src in enumerate(srcs):
            pltpu.make_async_copy(src, raw.at[pl.ds(i * PART + 2048 * m, src.shape[0])], sem_w.at[i]).start()

    def b_wait(i, rows):
        part = raw.at[pl.ds(pl.multiple_of(i * PART, 16), rows)]
        pltpu.make_async_copy(part, part, sem_w.at[i]).wait()

    def x_stage(j, slot):
        A.stb(AX + 288 * slot, xt[:, pl.ds(pl.multiple_of(j * 128, 128), 128)])

    def proj(j):
        if isinstance(j, int):
            return _Arena(qkv_all.at[pl.ds(((j + 1) & 3) * SLOT, SLOT)])
        return _Arena(qkv_all.at[pl.ds(pl.multiple_of(offs[(j + 1) & 3], 8), SLOT)])

    def no_tick(r):
        pass

    for c in (gate_copy, mem_copy, w_copy[0], x_copy[0], w_copy[1], w_copy[2], wo_copy, x_copy[1], x_copy[2]):
        c.start()

    for i in range(4):
        offs[i] = i * SLOT
    for i in range(8):
        offs[4 + i] = i * PART
    for j in range(NP):
        B.stf(PSTRIDE * j + PV + 24, jnp.zeros((8, 128), F32))
        B.stf(PSTRIDE * j + PV + 120, jnp.zeros((8, 128), F32))
    B.stf(BO, jnp.zeros((640, 128), F32))
    gate_copy.wait()
    mem_copy.wait()
    gate = jnp.broadcast_to(gate_ref[...].astype(F32)[None, :], (8, D))
    mem0 = mem_ref[...].astype(F32)
    for k in range(4):
        A.stf(GW + 8 * k, gate[:, 128 * k:128 * k + 128])
        B.stf(HS + 40 * k, mem0[:, 128 * k:128 * k + 128])
    A.stf(GW + 32, jnp.concatenate([gate[:, 512:]] * 2, 1))
    B.stf(HS + 160, jnp.concatenate([mem0[:, 512:]] * 2, 1))
    for i in range(2):
        b_start(i)

    def first_two(*parts):
        return _chain(*[_a_qkv(A, AX + 288 * j, proj(j), no_tick, parts) for j in range(2)])

    w_copy[0].wait()
    _a_transpose_w(A, wqkv, range(4, 9))
    x_copy[0].wait()
    w_copy[1].wait()
    x_stage(0, 0)
    x_stage(1, 1)
    _interleave(first_two(3, 1))
    _a_transpose_w(A, wqkv, range(0, 4))
    w_copy[2].wait()
    _interleave(first_two(0))
    _a_transpose_w(A, wqkv, range(9, 14))
    wo_copy.wait()
    _interleave(first_two(2), _a_transpose_wo(A, wo))
    qkv_all[AK:AG, :] = jnp.broadcast_to(qkv_all[SLOT + AK:SLOT + AG, :1], (AG - AK, 128))

    def tick_raw(r):
        raw[RAW_TICK:RAW_TICK + 16, :] = r[:16].astype(BF16)

    def tick_attend(r):
        qkv_all[TICK:TICK + 8, :] = pltpu.bitcast(r[:8], I32)

    def tick_both(r):
        tick_raw(r)
        tick_attend(r)

    def a_trip(j, project_out, prepare):
        mxu = [_a_qkv(A, AX, proj(j + 2), tick_raw if prepare else no_tick)]
        side = [_a_attend(j, proj(j), proj(j - 1), o_all.at[j], omg)]
        if prepare:
            i = j - 6
            b_wait(i, PART - 16)
            src = raw.at[pl.ds(pl.multiple_of(offs[4 + i], 16), PART)]
            dst = b_ref.at[pl.ds(pl.multiple_of(i * 32, 32), HS), :]
            side.append(_chain(*[
                _b_split_heads(src.at[pl.ds(2048 * m, 2048)], dst, to)
                for m, to in enumerate(((QA, QA + 288), (KA, KA + 256), (VA, VA + 256)))]))
            side.append(_b_transpose_wo(src.at[pl.ds(6144, 4 * D)], dst))
        if project_out:
            A.stb(AO, o_all[j - 4])
            mxu.append(_a_out(A, AO, ga_all.at[j - 4], tick_both if prepare else tick_attend))
        _interleave(_chain(*mxu), *side)
        x_stage(jnp.minimum(j + 3, NB - 1), 0)

    x_copy[1].wait()
    x_stage(2, 0)
    for i in range(2, 5):
        b_start(i)
    lax.fori_loop(0, 4, lambda j, c: a_trip(j, False, False), None)
    x_copy[2].wait()
    for i in range(5, 9):
        b_start(i)
    lax.fori_loop(4, 6, lambda j, c: a_trip(j, True, False), None)
    lax.fori_loop(6, NB - 2, lambda j, c: a_trip(j, True, True), None)

    def k2_transpose():
        for j in range(NP):
            B.stb(PSTRIDE * j + K2, B.ldb(PSTRIDE * j + K2, 64).T)
            yield

    def last_trip(i, carry):
        j = NB - 2 + i
        for b in range(2):
            A.stb(AO + 288 * b, o_all[NB - 6 + 2 * i + b])
        _interleave(_chain(*[_a_out(A, AO + 288 * b, ga_all.at[NB - 6 + 2 * i + b], tick_attend) for b in range(2)]),
                    _a_attend(j, proj(j), proj(j - 1), o_all.at[j], omg), span=(-0.3, 0.7))

    lax.fori_loop(0, 2, last_trip, None)
    b_wait(8, 6144)
    src = [raw.at[pl.ds(8 * PART + 2048 * m, 2048)] for m in range(3)]
    for b in range(2):
        A.stb(AO + 288 * b, o_all[NB - 2 + b])
    _interleave(
        _chain(*[_a_out(A, AO + 288 * b, ga_all.at[NB - 2 + b], no_tick) for b in range(2)]),
        _chain(_b_split_heads(src[1], b_ref, (K2 + 32, K2)),
               _b_split_heads(src[0], b_ref, (QA + 256, QA + 544)),
               (NP, k2_transpose()),
               _b_split_heads(src[2], b_ref, (PV + 32, PV + 64))))

    def x_transpose(j, n):
        cols = pl.ds(pl.multiple_of(j * 128, 128), 128)
        if n < 4:
            t = xt[128 * n:128 * n + 128, cols]
        else:
            t = jnp.concatenate([xt[512:576, cols]] * 2, 0)
        B.stb(XN + 64 * n, t.T)

    def x_place(u):
        for n in range(5):
            B.stf(HS + 200 * u + 40 * n + M, B.ldb(XN + 64 * n + 16 * u, 16).astype(F32))

    def mix(j, n):
        rows = min(128, D - 128 * n)
        bt = B.ldf(BO + 128 * n, 128).T[:rows]
        w = jnp.concatenate([omg[j]] * (rows // 8), 0)
        out_buf[j, 128 * n:128 * n + rows, :] = (
            ga_all[j, 128 * n:128 * n + rows, :] + w * bt).astype(BF16)

    def out_copy(j):
        return pltpu.make_async_copy(
            out_buf.at[j], out_hbm.at[:, pl.ds(pl.multiple_of(j * 128, 128), 128)], sem_out)

    for n in range(5):
        x_transpose(0, n)
    for u in range(U):
        x_place(u)

    def b_body(g, carry):
        jn, jp = jnp.minimum(g + 1, NB - 1), jnp.maximum(g - 1, 0)
        for u in range(U):
            extra = {("o", 3, 0): functools.partial(x_place, u)}
            if u == 0:
                for n in range(5):
                    extra["v", 20 + 2 * n] = functools.partial(mix, jp, n)
                    extra["o", 0, 6 * n] = functools.partial(x_transpose, jn, n)
            _b_step(B, u, extra)

        @pl.when(g > 0)
        def _():
            out_copy(jp).start()

        return carry

    lax.fori_loop(0, NB, b_body, 0)
    for n in range(5):
        mix(NB - 1, n)
    out_copy(NB - 1).start()
    for j in range(NB):
        out_copy(j).wait()


@functools.partial(jax.jit, static_argnames=("B_seg_len",))
def pallas_gated_mix__sliding_local_dilated__memory_aug_recurrent_mem_tr__prompt_kernel(
    A_x: jax.Array,
    A_wqkv: jax.Array,
    A_wo: jax.Array,
    B_x: jax.Array,
    B_mem0: jax.Array,
    B_Wq: jax.Array,
    B_Wk: jax.Array,
    B_Wv: jax.Array,
    B_Wo: jax.Array,
    B_seg_len: int,
    gate_w: jax.Array,
):
    del B_x
    assert A_x.shape == (1, S, D) and B_mem0.shape == (1, M, D) and B_Wq.shape == (D, H, DH)
    assert B_seg_len == SEG
    hbm = pl.BlockSpec(memory_space=pl.ANY)
    out_t = pl.pallas_call(
        _kernel,
        out_shape=jax.ShapeDtypeStruct((D, S), BF16),
        in_specs=[hbm] * 9,
        out_specs=hbm,
        scratch_shapes=[
            pltpu.VMEM((D, S), BF16),
            pltpu.VMEM((D, 3 * D), BF16),
            pltpu.VMEM((D, D), BF16),
            pltpu.VMEM((M, D), BF16),
            pltpu.VMEM((D,), BF16),
            pltpu.VMEM((9 * PART, DH), BF16),
            pltpu.VMEM((A_ROWS, 128), I32),
            pltpu.VMEM((B_ROWS, 128), I32),
            pltpu.VMEM((4 * SLOT, 128), I32),
            pltpu.VMEM((NB, D, 128), F32),
            pltpu.VMEM((NB, D, 128), F32),
            pltpu.VMEM((NB, 8, 128), F32),
            pltpu.VMEM((NB, D, 128), BF16),
            pltpu.SMEM((12,), I32),
            pltpu.SemaphoreType.DMA((9,)),
            pltpu.SemaphoreType.DMA((9,)),
            pltpu.SemaphoreType.DMA,
        ],
        compiler_params=pltpu.CompilerParams(vmem_limit_bytes=100 * 1024 * 1024),
    )(
        A_x.reshape(S, D).T, A_wqkv, A_wo, B_mem0.reshape(M, D), gate_w,
        B_Wq.reshape(D * H, DH), B_Wk.reshape(D * H, DH), B_Wv.reshape(D * H, DH),
        B_Wo.transpose(0, 2, 1).reshape(H * D, DH),
    )
    return out_t.T.reshape(1, S, D)
```

```python
import functools

import jax
import jax.numpy as jnp
from jax import lax
import jax.experimental.pallas as pl
import jax.experimental.pallas.tpu as pltpu

F32, BF16, I32 = jnp.float32, jnp.bfloat16, jnp.int32

S, D = 2048, 576
NB = S // 128
HA, DA, WIN, DIL = 32, 18, 8, 2
H, DH, M, SEG = 32, 128, 8, 32
L = M + SEG
NP = H // 2
U = 128 // SEG
NEG = -1000000000.0

QA = 0
KA = QA + 576
K2 = KA + 512
VA = K2 + 64
PV = VA + 512
PSTRIDE = PV + 128 + 4
OA = NP * PSTRIDE
HS = OA + H * 320
GS = HS + U * 200
GT = GS + 64
QS = GT + 64
KS = QS + H * 40
RE = KS + NP * 64
PS = RE + H * 40
RS = PS + NP * 40
OS = RS + NP * 40
XN = OS + H * 40
BO = XN + 320
B2 = BO + 512
OT = B2 + 128
B_ROWS = OT + H * 64

PART = 3 * 2048 + 4 * D + 16
RAW_TICK = 4 * PART - 16

WT = 0
GW = WT + 5 * 1728
WOT = GW + 40
AX = WOT + 5 * 288
AO = AX + 2 * 288
A_ROWS = AO + 2 * 288
AQ, AK, AV, AG, TICK, SLOT = 0, 576, 864, 1152, 1160, 1168


def _dot(a, b):
    return lax.dot_general(a, b, (((1,), (0,)), ((), ())), preferred_element_type=F32)


class _Arena:
    def __init__(self, ref):
        self.r = ref

    def ldi(self, o, n):
        return self.r[o:o + n, :]

    def ldf(self, o, n):
        return pltpu.bitcast(self.r[o:o + n, :], F32)

    def ldb(self, o, n):
        return pltpu.bitcast(self.r[o:o + n, :], BF16)

    def stf(self, o, v):
        self.r[o:o + v.shape[0], :] = pltpu.bitcast(v, I32)

    def stb(self, o, v):
        self.r[o:o + v.shape[0] // 2, :] = pltpu.bitcast(v.astype(BF16), I32)


def _pad2(t, rows, cols):
    r, c = t.shape
    if c < cols:
        t = jnp.concatenate([t, jnp.zeros((r, cols - c), t.dtype)], 1)
    if r < rows:
        t = jnp.concatenate([t, jnp.zeros((rows - r, cols), t.dtype)], 0)
    return t


def _interleave(main, *side, span=(0.0, 0.9)):
    jobs = (main,) + side
    order = [((i + 1) / main[0], 0) for i in range(main[0])]
    order += [(span[0] + (span[1] - span[0]) * i / n, k + 1) for k, (n, _) in enumerate(side) for i in range(n)]
    for _, k in sorted(order):
        next(jobs[k][1])
    for _, gen in jobs:
        assert next(gen, "end") == "end"


def _chain(*jobs):
    def gen():
        for _, g in jobs:
            yield from g
    return sum(n for n, _ in jobs), gen()


def _a_transpose_w(A, w_ref, cblocks):
    for c in cblocks:
        nc = min(128, 3 * D - 128 * c)
        for k in range(5):
            nk = min(128, D - 128 * k)
            t = _pad2(w_ref[128 * k:128 * k + nk, 128 * c:128 * c + nc], 128, 128).T
            A.stf(WT + 1728 * k + 128 * c, t[:nc].astype(F32))


def _a_transpose_wo(A, w_ref):
    def gen():
        for c in range(5):
            nc = min(128, D - 128 * c)
            for k in range(5):
                nk = min(128, D - 128 * k)
                t = _pad2(w_ref[128 * k:128 * k + nk, 128 * c:128 * c + nc], 128, 128).T
                A.stb(WOT + 288 * k + 64 * c, t[:nc])
                yield
    return 25, gen()


def _a_qkv(A, x_off, dst, tick, parts=(3, 1, 0, 2)):
    def proj(rows_of_k):
        ch = [rows_of_k(k) for k in range(5)]
        return _dot(jnp.concatenate(ch[:4] + [ch[4][:, :64]], 1), A.ldb(x_off, 288))

    def gen():
        for part in parts:
            if part == 3:
                dst.stf(AG, jax.nn.sigmoid(proj(lambda k: A.ldf(GW + 8 * k, 8))))
                continue
            for d0 in range(0, DA, 2):
                r = proj(lambda k: jnp.concatenate([
                    pltpu.bitcast(A.r[pl.ds(WT + 1728 * k + D * part + 8 * DA * hg + d, 8, stride=DA), :], F32)
                    for hg in range(4) for d in (d0, d0 + 1)], 0))
                tick(r)
                if part == 0:
                    dst.stf(AQ + 32 * d0, r)
                else:
                    dst.stb((AK if part == 1 else AV) + 16 * d0, r)
                yield
    return sum(DA // 2 for p in parts if p < 3), gen()


def _a_attend(j, cur, old, o_ref, omg_ref):
    def window(o):
        lane = lax.broadcasted_iota(I32, (8, 128), 1)
        c, p = cur.ldi(o, 8), old.ldi(o, 8)
        out = []
        for w in range(WIN):
            sh = DIL * w
            t = c if w == 0 else pltpu.roll(jnp.where(lane >= 128 - sh, p, c), sh, 1)
            out.append(pltpu.bitcast(t, BF16).astype(F32))
        return out

    def gen():
        pos = j * 128 + lax.broadcasted_iota(I32, (8, 128), 1)
        for hg in range(4):
            lg = None
            for d in range(0, DA, 2):
                q = cur.ldf(AQ + 32 * d + 16 * hg, 16)
                pr = [q * kw for kw in window(AK + 16 * d + 8 * hg)]
                pr = [t[:8] + t[8:] for t in pr]
                lg = pr if d == 0 else [a + b for a, b in zip(lg, pr)]
                yield
            lg = [jnp.where(pos >= DIL * w, t * DA ** -0.5, NEG) for w, t in enumerate(lg)]
            mx = functools.reduce(jnp.maximum, lg)
            e = [jnp.exp(t - mx) for t in lg]
            g = cur.ldf(AG, 8)
            if hg == 0:
                omg_ref[j] = 1.0 - g
            r = g / functools.reduce(jnp.add, e)
            p = [jnp.concatenate([t * r] * 2, 0) for t in e]
            yield
            for d in range(0, DA, 2):
                o = functools.reduce(jnp.add, [a * b for a, b in zip(p, window(AV + 16 * d + 8 * hg))])
                o_ref[pl.ds(8 * DA * hg + d, 8, stride=DA), :] = o[:8]
                o_ref[pl.ds(8 * DA * hg + d + 1, 8, stride=DA), :] = o[8:]
                yield
    return 4 * DA + 4, gen()


def _a_out(A, o_off, ga_ref, tick):
    def gen():
        for r0 in range(0, D, 64):
            ch = [A.ldb(WOT + 288 * k + r0 // 2, 32) for k in range(5)]
            r = _dot(jnp.concatenate(ch[:4] + [ch[4][:, :64]], 1), A.ldb(o_off, 288))
            tick(r)
            ga_ref[r0:r0 + 64, :] = r
            yield
    return D // 64, gen()


def _b_split_heads(raw, dst, offs):
    def gen():
        for r in range(32):
            e = pltpu.bitcast(raw[64 * r:64 * r + 32, :], I32)
            o = pltpu.bitcast(raw[64 * r + 32:64 * r + 64, :], I32)
            dst[pl.ds(offs[0] + r, NP, stride=PSTRIDE), :] = (e & 0xFFFF) | (o << 16)
            dst[pl.ds(offs[1] + r, NP, stride=PSTRIDE), :] = lax.shift_right_logical(e, 16) | (o & -65536)
            yield
    return 32, gen()


def _wo_piece(h, k):
    return OA + 256 * (10 * (h % 4) + k) + 32 * (h // 4)


def _b_transpose_wo(wot, dst):
    def put(t, o0, o1):
        t = pltpu.bitcast(t, I32)
        dst[o0:o0 + 32, :] = t[:32]
        dst[o1:o1 + 32, :] = t[32:]

    def gen():
        for h in range(4):
            for n in range(4):
                put(wot[D * h + 128 * n:D * h + 128 * n + 128, :].T, _wo_piece(h, 2 * n), _wo_piece(h, 2 * n + 1))
                yield
            if h % 2:
                t = jnp.concatenate([wot[D * i + 512:D * i + D, :] for i in (h - 1, h)], 0)
                put(t, _wo_piece(h - 1, 9), _wo_piece(h, 9))
                put(t.T, _wo_piece(h - 1, 8), _wo_piece(h, 8))
                yield
    return 18, gen()


def _b_out_tail(B, u):
    return functools.reduce(jnp.add, [
        lax.dot_general(B.ldb(_wo_piece(h, 9), 32), B.ldb(OT + 64 * h, 64), (((1,), (1,)), ((), ())),
                        preferred_element_type=F32)
        for h in range(8 * u, 8 * u + 8)])


def _b_step(B, u, extra):
    hs, hs_next = HS + 200 * u, HS + 200 * ((u + 1) % U)
    row = lax.broadcasted_iota(I32, (L, 128), 0)
    lane = lax.broadcasted_iota(I32, (L, 128), 1)
    lo = lane < 64
    lo64 = lax.broadcasted_iota(I32, (64, 128), 1) < 64
    col = lane & 63
    mask = (col < L) & ((row < M) | (row >= col))
    fill = jnp.where(col < L, NEG, -jnp.inf).astype(F32)
    z24 = jnp.zeros((24, 128), F32)
    z8 = jnp.zeros((8, 128), F32)

    def w(base, size, h):
        return PSTRIDE * (h // 2) + base + size * (h % 2)

    def tile(o0, o1):
        return pltpu.bitcast(jnp.concatenate([B.ldi(o0, 32), B.ldi(o1, 32)], 0), BF16)

    def h1():
        return jnp.concatenate([B.ldf(hs + 40 * n, 40) for n in range(4)], 1)

    def t_g():
        c4 = B.ldf(hs + 160, 40)
        g = jnp.concatenate([jnp.where(lo, 0.0, c4), z24, jnp.where(lo, c4, 0.0), z24], 0)
        B.stb(GS, g)
        B.stb(GT, g.T)

    k1 = {}

    def t_k(h):
        k1[h] = _dot(h1(), B.ldb(w(KA, 256, h), 256))
        if h % 2:
            B.stb(KS + 64 * (h // 2), jnp.concatenate([k1[h - 1], z24, k1[h], z24], 0).astype(BF16).T)

    def t_q(h):
        o = w(QA, 288, h)
        B.stf(QS + 40 * h, _dot(h1(), B.ldb(o, 256)) + _dot(B.ldf(hs + 160, 40)[:, :64], B.ldb(o + 256, 32)))

    def t_s(h):
        kt, w2 = B.ldi(KS + 64 * (h // 2), 64), B.ldi(w(K2, 0, h), 64)
        rhs = jnp.where(lo64, w2, kt) if h % 2 else jnp.where(lo64, kt, w2)
        B.stf(RE + 40 * h, _dot(B.ldf(QS + 40 * h, 40), pltpu.bitcast(rhs, BF16)))

    def t_s2(j):
        a, b = B.ldf(RE + 80 * j, 40), B.ldf(RE + 80 * j + 40, 40)
        s = jnp.where(lo, a, b) + _dot(jnp.where(lo, b, a), B.ldb(GT, 64))
        s = jnp.where(mask, s * DH ** -0.5, fill)
        ma = jnp.max(jnp.where(lo, s, -jnp.inf), axis=1, keepdims=True)
        mb = jnp.max(jnp.where(lo, -jnp.inf, s), axis=1, keepdims=True)
        e = jnp.exp(s - jnp.where(lo, ma, mb))
        la = jnp.sum(jnp.where(lo, e, 0.0), axis=1, keepdims=True)
        lb = jnp.sum(jnp.where(lo, 0.0, e), axis=1, keepdims=True)
        B.stf(PS + 40 * j, e / jnp.where(lo, la, lb))

    def t_r(j):
        B.stf(RS + 40 * j, _dot(B.ldf(PS + 40 * j, 40), B.ldb(GS, 64)))

    def t_v(h):
        v = _dot(h1(), B.ldb(w(VA, 256, h), 256))
        B.stb(w(PV, 96, h), jnp.concatenate([v, z8], 0))

    def t_pv(h):
        p, r = B.ldf(PS + 40 * (h // 2), 40), B.ldf(RS + 40 * (h // 2), 40)
        lhs = jnp.where(lo, r, p) if h % 2 else jnp.where(lo, p, r)
        o = _dot(lhs, B.ldb(w(PV, 64, h), 64))
        B.stf(OS + 40 * h, o)
        B.stb(OT + 64 * h + 16 * u, o[M:])

    d_s, d_s2, d_r, d_pv, ahead = 20, 18, 64, 22, 7
    big = [("k", h) for h in range(ahead)] + [("g",)]
    for h in range(H):
        if h + ahead < H:
            big.append(("k", h + ahead))
        big.append(("q", h))
    big += [("v", h) for h in range(H)]
    for i in range(4 * H):
        big.append(("o", i // H, i % H))
        if i % 8 == 7:
            big.append(("m", i // 8))
    small = {"pv": t_pv, "r": t_r, "s2": t_s2, "s": t_s}
    nxt = dict.fromkeys(small, 0)
    done = {}
    now = 0

    def old(key, dist):
        return key in done and now - done[key] >= dist

    def ready(kind, i):
        if kind == "s":
            return old(("q", i), d_s)
        if kind == "s2":
            return old(("s", 2 * i + 1), d_s2)
        if kind == "r":
            return old(("s2", i), d_r)
        return old(("r", i // 2), d_s2) and old(("v", i), d_pv)

    acc = mem2 = None
    for t in big:
        for kind, fn in small.items():
            if ready(kind, nxt[kind]):
                fn(nxt[kind])
                now += 1
                done[kind, nxt[kind]] = now
                nxt[kind] += 1
        if t in extra:
            extra[t]()
        if t[0] == "k":
            t_k(t[1])
            now += 4
        elif t[0] == "g":
            t_g()
        elif t[0] == "q":
            t_q(t[1])
            now += 5
        elif t[0] == "v":
            t_v(t[1])
            now += 4
        elif t[0] == "m":
            a, b = 2 * t[1], 2 * t[1] + 1
            y = _dot(jnp.concatenate([B.ldf(OS + 40 * a, M), B.ldf(OS + 40 * b, M)], 0),
                     tile(_wo_piece(a, 8), _wo_piece(b, 8)))
            mem2 = y if a == 0 else mem2 + y
        else:
            _, n, h = t
            assert ("pv", h) in done
            y = _dot(B.ldf(OS + 40 * h, 40), tile(_wo_piece(h, 2 * n), _wo_piece(h, 2 * n + 1)))
            acc = y if h == 0 else acc + y
            if h == H - 1:
                B.stf(hs_next + 40 * n, acc[:M])
                B.stf(BO + 128 * n + SEG * u, acc[M:])
            now += 1
        done[t] = now
    mem2 = jnp.where(lo[:M], mem2[:M], mem2[M:])
    B.stf(hs_next + 160, mem2 + pltpu.roll(mem2, 64, 1))
    y = _b_out_tail(B, u)
    if u == U - 1:
        B.stf(B2 + 64, B.ldf(B2, 64) + y)
    else:
        new = lax.broadcasted_iota(I32, (64, 128), 1) < SEG * (u + 1)
        B.stf(B2, jnp.where(new, y, 0.0) + (B.ldf(B2, 64) if u else 0.0))
        B.stf(B2 + 64, jnp.where(new, 0.0, y) + B.ldf(B2 + 64, 64))


def _kernel(xt_hbm, wqkv_hbm, wo_hbm, mem_hbm, gate_hbm, wq_hbm, wk_hbm, wv_hbm, wot_hbm,
            out_hbm,
            xt, wqkv, wo, mem_ref, gate_ref, raw, a_ref, b_ref, qkv_all, o_all, ga_all, omg, out_buf,
            offs, sem_in, sem_w, sem_out):
    A, B = _Arena(a_ref), _Arena(b_ref)

    def cols(src, dst, c0, c1, sem):
        return pltpu.make_async_copy(src.at[:, pl.ds(c0, c1 - c0)], dst.at[:, pl.ds(c0, c1 - c0)], sem_in.at[sem])

    x_copy = [cols(xt_hbm, xt, 0, 256, 0), cols(xt_hbm, xt, 256, 896, 1), cols(xt_hbm, xt, 896, S, 2)]
    w_copy = [cols(wqkv_hbm, wqkv, 512, 1152, 4), cols(wqkv_hbm, wqkv, 0, 512, 5),
              cols(wqkv_hbm, wqkv, 1152, 3 * D, 6)]
    wo_copy = pltpu.make_async_copy(wo_hbm, wo, sem_in.at[3])
    mem_copy = pltpu.make_async_copy(mem_hbm, mem_ref, sem_in.at[7])
    gate_copy = pltpu.make_async_copy(gate_hbm, gate_ref, sem_in.at[8])

    def b_start(i):
        srcs = [w.at[pl.ds(2048 * i, 2048)] for w in (wq_hbm, wk_hbm, wv_hbm)]
        if i < 8:
            srcs.append(wot_hbm.at[pl.ds(4 * D * i, 4 * D)])
        for m, src in enumerate(srcs):
            pltpu.make_async_copy(src, raw.at[pl.ds(i * PART + 2048 * m, src.shape[0])], sem_w.at[i]).start()

    def b_wait(i, rows):
        part = raw.at[pl.ds(pl.multiple_of(i * PART, 16), rows)]
        pltpu.make_async_copy(part, part, sem_w.at[i]).wait()

    def x_stage(j, slot):
        A.stb(AX + 288 * slot, xt[:, pl.ds(pl.multiple_of(j * 128, 128), 128)])

    def proj(j):
        if isinstance(j, int):
            return _Arena(qkv_all.at[pl.ds(((j + 1) & 3) * SLOT, SLOT)])
        return _Arena(qkv_all.at[pl.ds(pl.multiple_of(offs[(j + 1) & 3], 8), SLOT)])

    def no_tick(r):
        pass

    for c in (gate_copy, mem_copy, w_copy[0], x_copy[0], w_copy[1], w_copy[2], wo_copy, x_copy[1], x_copy[2]):
        c.start()

    for i in range(4):
        offs[i] = i * SLOT
    for i in range(8):
        offs[4 + i] = i * PART
    for j in range(NP):
        B.stf(PSTRIDE * j + PV + 24, jnp.zeros((8, 128), F32))
        B.stf(PSTRIDE * j + PV + 120, jnp.zeros((8, 128), F32))
    B.stf(BO, jnp.zeros((B_ROWS - BO, 128), F32))
    gate_copy.wait()
    mem_copy.wait()
    gate = jnp.broadcast_to(gate_ref[...].astype(F32)[None, :], (8, D))
    mem0 = mem_ref[...].astype(F32)
    for k in range(4):
        A.stf(GW + 8 * k, gate[:, 128 * k:128 * k + 128])
        B.stf(HS + 40 * k, mem0[:, 128 * k:128 * k + 128])
    A.stf(GW + 32, jnp.concatenate([gate[:, 512:]] * 2, 1))
    B.stf(HS + 160, jnp.concatenate([mem0[:, 512:]] * 2, 1))
    for i in range(2):
        b_start(i)

    def first_two(*parts):
        return _chain(*[_a_qkv(A, AX + 288 * j, proj(j), no_tick, parts) for j in range(2)])

    w_copy[0].wait()
    _a_transpose_w(A, wqkv, range(4, 9))
    x_copy[0].wait()
    w_copy[1].wait()
    x_stage(0, 0)
    x_stage(1, 1)
    _interleave(first_two(3, 1))
    _a_transpose_w(A, wqkv, range(0, 4))
    w_copy[2].wait()
    _interleave(first_two(0))
    _a_transpose_w(A, wqkv, range(9, 14))
    wo_copy.wait()
    _interleave(first_two(2), _a_transpose_wo(A, wo))
    qkv_all[AK:AG, :] = jnp.broadcast_to(qkv_all[SLOT + AK:SLOT + AG, :1], (AG - AK, 128))

    def tick_raw(r):
        raw[RAW_TICK:RAW_TICK + 16, :] = r[:16].astype(BF16)

    def tick_attend(r):
        qkv_all[TICK:TICK + 8, :] = pltpu.bitcast(r[:8], I32)

    def tick_both(r):
        tick_raw(r)
        tick_attend(r)

    def a_trip(j, project_out, prepare):
        mxu = [_a_qkv(A, AX, proj(j + 2), tick_raw if prepare else no_tick)]
        side = [_a_attend(j, proj(j), proj(j - 1), o_all.at[j], omg)]
        if prepare:
            i = j - 6
            b_wait(i, PART - 16)
            src = raw.at[pl.ds(pl.multiple_of(offs[4 + i], 16), PART)]
            dst = b_ref.at[pl.ds(pl.multiple_of(i * 32, 32), HS), :]
            side.append(_chain(*[
                _b_split_heads(src.at[pl.ds(2048 * m, 2048)], dst, to)
                for m, to in enumerate(((QA, QA + 288), (KA, KA + 256), (VA, VA + 256)))]))
            side.append(_b_transpose_wo(src.at[pl.ds(6144, 4 * D)], dst))
        if project_out:
            A.stb(AO, o_all[j - 4])
            mxu.append(_a_out(A, AO, ga_all.at[j - 4], tick_both if prepare else tick_attend))
        _interleave(_chain(*mxu), *side)
        x_stage(jnp.minimum(j + 3, NB - 1), 0)

    x_copy[1].wait()
    x_stage(2, 0)
    for i in range(2, 5):
        b_start(i)
    lax.fori_loop(0, 4, lambda j, c: a_trip(j, False, False), None)
    x_copy[2].wait()
    for i in range(5, 9):
        b_start(i)
    lax.fori_loop(4, 6, lambda j, c: a_trip(j, True, False), None)
    lax.fori_loop(6, NB - 2, lambda j, c: a_trip(j, True, True), None)

    def k2_transpose():
        for j in range(NP):
            B.stb(PSTRIDE * j + K2, B.ldb(PSTRIDE * j + K2, 64).T)
            yield

    def last_trip(i, carry):
        j = NB - 2 + i
        for b in range(2):
            A.stb(AO + 288 * b, o_all[NB - 6 + 2 * i + b])
        _interleave(_chain(*[_a_out(A, AO + 288 * b, ga_all.at[NB - 6 + 2 * i + b], tick_attend) for b in range(2)]),
                    _a_attend(j, proj(j), proj(j - 1), o_all.at[j], omg), span=(-0.3, 0.7))

    lax.fori_loop(0, 2, last_trip, None)
    b_wait(8, 6144)
    src = [raw.at[pl.ds(8 * PART + 2048 * m, 2048)] for m in range(3)]
    for b in range(2):
        A.stb(AO + 288 * b, o_all[NB - 2 + b])
    _interleave(
        _chain(*[_a_out(A, AO + 288 * b, ga_all.at[NB - 2 + b], no_tick) for b in range(2)]),
        _chain(_b_split_heads(src[1], b_ref, (K2 + 32, K2)),
               _b_split_heads(src[0], b_ref, (QA + 256, QA + 544)),
               (NP, k2_transpose()),
               _b_split_heads(src[2], b_ref, (PV + 32, PV + 64))))

    def x_transpose(j, n):
        cols = pl.ds(pl.multiple_of(j * 128, 128), 128)
        if n < 4:
            t = xt[128 * n:128 * n + 128, cols]
        else:
            t = jnp.concatenate([xt[512:576, cols]] * 2, 0)
        B.stb(XN + 64 * n, t.T)

    def x_place(u):
        for n in range(5):
            B.stf(HS + 200 * u + 40 * n + M, B.ldb(XN + 64 * n + 16 * u, 16).astype(F32))

    def mix(j, n):
        rows = min(128, D - 128 * n)
        bt = B.ldf(BO + 128 * n, 128).T if n < 4 else B.ldf(B2 + 64, 64)
        w = jnp.concatenate([omg[j]] * (rows // 8), 0)
        out_buf[j, 128 * n:128 * n + rows, :] = (
            ga_all[j, 128 * n:128 * n + rows, :] + w * bt).astype(BF16)

    def out_copy(j):
        return pltpu.make_async_copy(
            out_buf.at[j], out_hbm.at[:, pl.ds(pl.multiple_of(j * 128, 128), 128)], sem_out)

    for n in range(5):
        x_transpose(0, n)
    for u in range(U):
        x_place(u)

    def b_body(g, carry):
        jn, jp = jnp.minimum(g + 1, NB - 1), jnp.maximum(g - 1, 0)
        for u in range(U):
            extra = {("o", 3, 0): functools.partial(x_place, u)}
            if u == 0:
                for n in range(4):
                    extra["v", 20 + 2 * n] = functools.partial(mix, jp, n)
                for n in range(5):
                    extra["o", 0, 6 * n] = functools.partial(x_transpose, jn, n)
            if u == U - 1:
                extra["v", 20] = functools.partial(mix, jp, 4)
            _b_step(B, u, extra)

        @pl.when(g > 0)
        def _():
            out_copy(jp).start()

        return carry

    lax.fori_loop(0, NB, b_body, 0)
    lane = lax.broadcasted_iota(I32, (64, 128), 1)
    B.stf(B2 + 64, functools.reduce(jnp.add, [B.ldf(B2 + 64, 64)] + [
        jnp.where(lane < SEG * (u + 1), 0.0, _b_out_tail(B, u)) for u in range(U - 1)]))
    for n in range(5):
        mix(NB - 1, n)
    out_copy(NB - 1).start()
    for j in range(NB):
        out_copy(j).wait()


@functools.partial(jax.jit, static_argnames=("B_seg_len",))
def pallas_gated_mix__sliding_local_dilated__memory_aug_recurrent_mem_tr__prompt_kernel(
    A_x: jax.Array,
    A_wqkv: jax.Array,
    A_wo: jax.Array,
    B_x: jax.Array,
    B_mem0: jax.Array,
    B_Wq: jax.Array,
    B_Wk: jax.Array,
    B_Wv: jax.Array,
    B_Wo: jax.Array,
    B_seg_len: int,
    gate_w: jax.Array,
):
    del B_x
    assert A_x.shape == (1, S, D) and B_mem0.shape == (1, M, D) and B_Wq.shape == (D, H, DH)
    assert B_seg_len == SEG
    hbm = pl.BlockSpec(memory_space=pl.ANY)
    out_t = pl.pallas_call(
        _kernel,
        out_shape=jax.ShapeDtypeStruct((D, S), BF16),
        in_specs=[hbm] * 9,
        out_specs=hbm,
        scratch_shapes=[
            pltpu.VMEM((D, S), BF16),
            pltpu.VMEM((D, 3 * D), BF16),
            pltpu.VMEM((D, D), BF16),
            pltpu.VMEM((M, D), BF16),
            pltpu.VMEM((D,), BF16),
            pltpu.VMEM((9 * PART, DH), BF16),
            pltpu.VMEM((A_ROWS, 128), I32),
            pltpu.VMEM((B_ROWS, 128), I32),
            pltpu.VMEM((4 * SLOT, 128), I32),
            pltpu.VMEM((NB, D, 128), F32),
            pltpu.VMEM((NB, D, 128), F32),
            pltpu.VMEM((NB, 8, 128), F32),
            pltpu.VMEM((NB, D, 128), BF16),
            pltpu.SMEM((12,), I32),
            pltpu.SemaphoreType.DMA((9,)),
            pltpu.SemaphoreType.DMA((9,)),
            pltpu.SemaphoreType.DMA,
        ],
        compiler_params=pltpu.CompilerParams(vmem_limit_bytes=100 * 1024 * 1024),
    )(
        A_x.reshape(S, D).T, A_wqkv, A_wo, B_mem0.reshape(M, D), gate_w,
        B_Wq.reshape(D * H, DH), B_Wk.reshape(D * H, DH), B_Wv.reshape(D * H, DH),
        B_Wo.transpose(0, 2, 1).reshape(H * D, DH),
    )
    return out_t.T.reshape(1, S, D)
```

```python
import functools

import jax
import jax.numpy as jnp
from jax import lax
import jax.experimental.pallas as pl
import jax.experimental.pallas.tpu as pltpu

F32, BF16, I32 = jnp.float32, jnp.bfloat16, jnp.int32

S, D = 2048, 576
NB = S // 128
HA, DA, WIN, DIL = 32, 18, 8, 2
H, DH, M, SEG = 32, 128, 8, 32
L = M + SEG
NP = H // 2
U = 128 // SEG
NEG = -1000000000.0

QA = 0
KA = QA + 576
K2 = KA + 512
VA = K2 + 64
PV = VA + 512
PSTRIDE = PV + 128 + 4
OA = NP * PSTRIDE
HS = OA + H * 320
GS = HS + U * 200
GT = GS + 64
QS = GT + 64
KS = QS + H * 40
RE = KS + NP * 64
PS = RE + H * 40
RS = PS + NP * 40
OS = RS + NP * 40
XN = OS + H * 40
BO = XN + 320
B2 = BO + 512
OT = B2 + 128
B_ROWS = OT + H * 64

PART = 3 * 2048 + 4 * D + 16
RAW_TICK = 4 * PART - 16

WT = 0
GW = WT + 5 * 1728
WOT = GW + 40
AX = WOT + 5 * 288
AO = AX + 2 * 288
A_ROWS = AO + 2 * 288
AQ, AK, AV, AG, TICK, SLOT = 0, 576, 864, 1152, 1160, 1168


def _dot(a, b):
    return lax.dot_general(a, b, (((1,), (0,)), ((), ())), preferred_element_type=F32)


class _Arena:
    def __init__(self, ref):
        self.r = ref

    def ldi(self, o, n):
        return self.r[o:o + n, :]

    def ldf(self, o, n):
        return pltpu.bitcast(self.r[o:o + n, :], F32)

    def ldb(self, o, n):
        return pltpu.bitcast(self.r[o:o + n, :], BF16)

    def stf(self, o, v):
        self.r[o:o + v.shape[0], :] = pltpu.bitcast(v, I32)

    def stb(self, o, v):
        self.r[o:o + v.shape[0] // 2, :] = pltpu.bitcast(v.astype(BF16), I32)


def _pad2(t, rows, cols):
    r, c = t.shape
    if c < cols:
        t = jnp.concatenate([t, jnp.zeros((r, cols - c), t.dtype)], 1)
    if r < rows:
        t = jnp.concatenate([t, jnp.zeros((rows - r, cols), t.dtype)], 0)
    return t


def _interleave(main, *side, span=(0.0, 0.9)):
    jobs = (main,) + side
    order = [((i + 1) / main[0], 0) for i in range(main[0])]
    order += [(span[0] + (span[1] - span[0]) * i / n, k + 1) for k, (n, _) in enumerate(side) for i in range(n)]
    for _, k in sorted(order):
        next(jobs[k][1])
    for _, gen in jobs:
        assert next(gen, "end") == "end"


def _chain(*jobs):
    def gen():
        for _, g in jobs:
            yield from g
    return sum(n for n, _ in jobs), gen()


def _a_transpose_w(A, w_ref, cblocks):
    for c in cblocks:
        nc = min(128, 3 * D - 128 * c)
        for k in range(5):
            nk = min(128, D - 128 * k)
            t = _pad2(w_ref[128 * k:128 * k + nk, 128 * c:128 * c + nc], 128, 128).T
            A.stf(WT + 1728 * k + 128 * c, t[:nc].astype(F32))


def _a_transpose_wo(A, w_ref):
    def gen():
        for c in range(5):
            nc = min(128, D - 128 * c)
            for k in range(5):
                nk = min(128, D - 128 * k)
                t = _pad2(w_ref[128 * k:128 * k + nk, 128 * c:128 * c + nc], 128, 128).T
                A.stb(WOT + 288 * k + 64 * c, t[:nc])
                yield
    return 25, gen()


def _a_qkv(A, x_off, dst, tick, parts=(3, 1, 0, 2)):
    def proj(rows_of_k):
        ch = [rows_of_k(k) for k in range(5)]
        return _dot(jnp.concatenate(ch[:4] + [ch[4][:, :64]], 1), A.ldb(x_off, 288))

    def gen():
        for part in parts:
            if part == 3:
                dst.stf(AG, jax.nn.sigmoid(proj(lambda k: A.ldf(GW + 8 * k, 8))))
                continue
            for d0 in range(0, DA, 2):
                r = proj(lambda k: jnp.concatenate([
                    pltpu.bitcast(A.r[pl.ds(WT + 1728 * k + D * part + 8 * DA * hg + d, 8, stride=DA), :], F32)
                    for hg in range(4) for d in (d0, d0 + 1)], 0))
                tick(r)
                if part == 0:
                    dst.stf(AQ + 32 * d0, r)
                else:
                    dst.stb((AK if part == 1 else AV) + 16 * d0, r)
                yield
    return sum(DA // 2 for p in parts if p < 3), gen()


def _a_attend(j, cur, old, o_ref, omg_ref):
    def window(o):
        lane = lax.broadcasted_iota(I32, (8, 128), 1)
        c, p = cur.ldi(o, 8), old.ldi(o, 8)
        out = []
        for w in range(WIN):
            sh = DIL * w
            t = c if w == 0 else pltpu.roll(jnp.where(lane >= 128 - sh, p, c), sh, 1)
            out.append(pltpu.bitcast(t, BF16).astype(F32))
        return out

    def gen():
        pos = j * 128 + lax.broadcasted_iota(I32, (8, 128), 1)
        for hg in range(4):
            lg = None
            for d in range(0, DA, 2):
                q = cur.ldf(AQ + 32 * d + 16 * hg, 16)
                pr = [q * kw for kw in window(AK + 16 * d + 8 * hg)]
                pr = [t[:8] + t[8:] for t in pr]
                lg = pr if d == 0 else [a + b for a, b in zip(lg, pr)]
                yield
            lg = [jnp.where(pos >= DIL * w, t * DA ** -0.5, NEG) for w, t in enumerate(lg)]
            mx = functools.reduce(jnp.maximum, lg)
            e = [jnp.exp(t - mx) for t in lg]
            g = cur.ldf(AG, 8)
            if hg == 0:
                omg_ref[j] = 1.0 - g
            r = g / functools.reduce(jnp.add, e)
            p = [jnp.concatenate([t * r] * 2, 0) for t in e]
            yield
            for d in range(0, DA, 2):
                o = functools.reduce(jnp.add, [a * b for a, b in zip(p, window(AV + 16 * d + 8 * hg))])
                o_ref[pl.ds(8 * DA * hg + d, 8, stride=DA), :] = o[:8]
                o_ref[pl.ds(8 * DA * hg + d + 1, 8, stride=DA), :] = o[8:]
                yield
    return 4 * DA + 4, gen()


def _a_out(A, o_off, ga_ref, tick):
    def gen():
        for r0 in range(0, D, 64):
            ch = [A.ldb(WOT + 288 * k + r0 // 2, 32) for k in range(5)]
            r = _dot(jnp.concatenate(ch[:4] + [ch[4][:, :64]], 1), A.ldb(o_off, 288))
            tick(r)
            ga_ref[r0:r0 + 64, :] = r
            yield
    return D // 64, gen()


def _b_split_heads(raw, dst, offs):
    def gen():
        for r in range(32):
            e = pltpu.bitcast(raw[64 * r:64 * r + 32, :], I32)
            o = pltpu.bitcast(raw[64 * r + 32:64 * r + 64, :], I32)
            dst[pl.ds(offs[0] + r, NP, stride=PSTRIDE), :] = (e & 0xFFFF) | (o << 16)
            dst[pl.ds(offs[1] + r, NP, stride=PSTRIDE), :] = lax.shift_right_logical(e, 16) | (o & -65536)
            yield
    return 32, gen()


def _wo_piece(h, k):
    return OA + 256 * (10 * (h % 4) + k) + 32 * (h // 4)


def _b_transpose_wo(wot, dst):
    def put(t, o0, o1):
        t = pltpu.bitcast(t, I32)
        dst[o0:o0 + 32, :] = t[:32]
        dst[o1:o1 + 32, :] = t[32:]

    def gen():
        for h in range(4):
            for n in range(4):
                put(wot[D * h + 128 * n:D * h + 128 * n + 128, :].T, _wo_piece(h, 2 * n), _wo_piece(h, 2 * n + 1))
                yield
            if h % 2:
                t = jnp.concatenate([wot[D * i + 512:D * i + D, :] for i in (h - 1, h)], 0)
                put(t, _wo_piece(h - 1, 9), _wo_piece(h, 9))
                put(t.T, _wo_piece(h - 1, 8), _wo_piece(h, 8))
                yield
    return 18, gen()


def _b_out_tail(B, u):
    return functools.reduce(jnp.add, [
        lax.dot_general(B.ldb(_wo_piece(h, 9), 32), B.ldb(OT + 64 * h, 64), (((1,), (1,)), ((), ())),
                        preferred_element_type=F32)
        for h in range(8 * u, 8 * u + 8)])


def _b_step(B, u, extra):
    hs, hs_next = HS + 200 * u, HS + 200 * ((u + 1) % U)
    row = lax.broadcasted_iota(I32, (L, 128), 0)
    lane = lax.broadcasted_iota(I32, (L, 128), 1)
    lo = lane < 64
    lo64 = lax.broadcasted_iota(I32, (64, 128), 1) < 64
    col = lane & 63
    mask = (row < M) | (row >= col)
    in_a, in_b = lane < L, (lane >= 64) & (lane < 64 + L)
    z24 = jnp.zeros((24, 128), F32)
    z8 = jnp.zeros((8, 128), F32)

    def w(base, size, h):
        return PSTRIDE * (h // 2) + base + size * (h % 2)

    def tile(o0, o1):
        return pltpu.bitcast(jnp.concatenate([B.ldi(o0, 32), B.ldi(o1, 32)], 0), BF16)

    def h1():
        return jnp.concatenate([B.ldf(hs + 40 * n, 40) for n in range(4)], 1)

    def t_g():
        c4 = B.ldf(hs + 160, 40)
        g = jnp.concatenate([jnp.where(lo, 0.0, c4), z24, jnp.where(lo, c4, 0.0), z24], 0)
        B.stb(GS, g)
        B.stb(GT, g.T)

    def t_k(h):
        B.stf(RE + 40 * h, _dot(h1(), B.ldb(w(KA, 256, h), 256)))
        if h % 2:
            k = jnp.concatenate([B.ldf(RE + 40 * (h - 1), 40), z24, B.ldf(RE + 40 * h, 40), z24], 0)
            B.stb(KS + 64 * (h // 2), k.astype(BF16).T)

    def t_q(h):
        o = w(QA, 288, h)
        B.stf(QS + 40 * h, _dot(h1(), B.ldb(o, 256)) + _dot(B.ldf(hs + 160, 40)[:, :64], B.ldb(o + 256, 32)))

    def t_s(h):
        kt, w2 = B.ldi(KS + 64 * (h // 2), 64), B.ldi(w(K2, 0, h), 64)
        rhs = jnp.where(lo64, w2, kt) if h % 2 else jnp.where(lo64, kt, w2)
        B.stf(RE + 40 * h, _dot(B.ldf(QS + 40 * h, 40), pltpu.bitcast(rhs, BF16)))

    def t_s2(j):
        a, b = B.ldf(RE + 80 * j, 40), B.ldf(RE + 80 * j + 40, 40)
        s = jnp.where(lo, a, b) + _dot(jnp.where(lo, b, a), B.ldb(GT, 64))
        s = jnp.where(mask, s * DH ** -0.5, NEG)
        B.stf(RS + 40 * j, s)
        ma = jnp.max(jnp.where(in_a, s, -jnp.inf), axis=1, keepdims=True)
        mb = jnp.max(jnp.where(in_b, s, -jnp.inf), axis=1, keepdims=True)
        e = jnp.exp(B.ldf(RS + 40 * j, 40) - jnp.where(lo, ma, mb))
        ea, eb = jnp.where(in_a, e, 0.0), jnp.where(in_b, e, 0.0)
        B.stf(PS + 40 * j, ea + eb)
        la = jnp.sum(ea, axis=1, keepdims=True)
        lb = jnp.sum(eb, axis=1, keepdims=True)
        B.stf(PS + 40 * j, B.ldf(PS + 40 * j, 40) / jnp.where(lo, la, lb))

    def t_r(j):
        B.stf(RS + 40 * j, _dot(B.ldf(PS + 40 * j, 40), B.ldb(GS, 64)))

    def t_v(h):
        v = _dot(h1(), B.ldb(w(VA, 256, h), 256))
        B.stb(w(PV, 96, h), jnp.concatenate([v, z8], 0))

    def t_pv(h):
        p, r = B.ldf(PS + 40 * (h // 2), 40), B.ldf(RS + 40 * (h // 2), 40)
        lhs = jnp.where(lo, r, p) if h % 2 else jnp.where(lo, p, r)
        o = _dot(lhs, B.ldb(w(PV, 64, h), 64))
        B.stf(OS + 40 * h, o)
        B.stb(OT + 64 * h + 16 * u, o[M:])

    d_s, d_s2, d_pv = 20, 18, 22
    big = [("k", h) for h in range(H)] + [("g",)] + [(p, h) for p in "qv" for h in range(H)]
    for i in range(4 * H):
        big.append(("o", i // H, i % H))
        if i % 8 == 7:
            big.append(("m", i // 8))
    small = {"pv": t_pv, "r": t_r, "s2": t_s2, "s": t_s}
    nxt = dict.fromkeys(small, 0)
    done = {}
    now = 0

    def old(key, dist):
        return key in done and now - done[key] >= dist

    def ready(kind, i):
        if kind == "s":
            return old(("q", i), d_s)
        if kind == "s2":
            return old(("s", 2 * i + 1), d_s2)
        if kind == "r":
            return old(("s2", i), 64) and old(("v", 2 * i), 0)
        return old(("r", i // 2), d_s2) and old(("v", i), d_pv)

    acc = mem2 = None
    for t in big:
        for kind, fn in small.items():
            if ready(kind, nxt[kind]):
                fn(nxt[kind])
                now += 1
                done[kind, nxt[kind]] = now
                nxt[kind] += 1
        if t in extra:
            extra[t]()
        if t[0] == "k":
            t_k(t[1])
            now += 4
        elif t[0] == "g":
            t_g()
        elif t[0] == "q":
            t_q(t[1])
            now += 5
        elif t[0] == "v":
            t_v(t[1])
            now += 4
        elif t[0] == "m":
            a, b = 2 * t[1], 2 * t[1] + 1
            y = _dot(jnp.concatenate([B.ldf(OS + 40 * a, M), B.ldf(OS + 40 * b, M)], 0),
                     tile(_wo_piece(a, 8), _wo_piece(b, 8)))
            mem2 = y if a == 0 else mem2 + y
        else:
            _, n, h = t
            assert ("pv", h) in done
            y = _dot(B.ldf(OS + 40 * h, 40), tile(_wo_piece(h, 2 * n), _wo_piece(h, 2 * n + 1)))
            acc = y if h == 0 else acc + y
            if h == H - 1:
                B.stf(hs_next + 40 * n, acc[:M])
                B.stf(BO + 128 * n + SEG * u, acc[M:])
            now += 1
        done[t] = now
    mem2 = jnp.where(lo[:M], mem2[:M], mem2[M:])
    B.stf(hs_next + 160, mem2 + pltpu.roll(mem2, 64, 1))
    y = _b_out_tail(B, u)
    if u == U - 1:
        B.stf(B2 + 64, B.ldf(B2, 64) + y)
    else:
        new = lax.broadcasted_iota(I32, (64, 128), 1) < SEG * (u + 1)
        B.stf(B2, jnp.where(new, y, 0.0) + (B.ldf(B2, 64) if u else 0.0))
        B.stf(B2 + 64, jnp.where(new, 0.0, y) + B.ldf(B2 + 64, 64))


def _kernel(xt_hbm, wqkv_hbm, wo_hbm, mem_hbm, gate_hbm, wq_hbm, wk_hbm, wv_hbm, wot_hbm,
            out_hbm,
            xt, wqkv, wo, mem_ref, gate_ref, raw, a_ref, b_ref, qkv_all, o_all, ga_all, omg, out_buf,
            offs, sem_in, sem_w, sem_out):
    A, B = _Arena(a_ref), _Arena(b_ref)

    def cols(src, dst, c0, c1, sem):
        return pltpu.make_async_copy(src.at[:, pl.ds(c0, c1 - c0)], dst.at[:, pl.ds(c0, c1 - c0)], sem_in.at[sem])

    x_copy = [cols(xt_hbm, xt, 0, 256, 0), cols(xt_hbm, xt, 256, 896, 1), cols(xt_hbm, xt, 896, S, 2)]
    w_copy = [cols(wqkv_hbm, wqkv, 512, 1152, 4), cols(wqkv_hbm, wqkv, 0, 512, 5),
              cols(wqkv_hbm, wqkv, 1152, 3 * D, 6)]
    wo_copy = pltpu.make_async_copy(wo_hbm, wo, sem_in.at[3])
    mem_copy = pltpu.make_async_copy(mem_hbm, mem_ref, sem_in.at[7])
    gate_copy = pltpu.make_async_copy(gate_hbm, gate_ref, sem_in.at[8])

    def b_start(i):
        srcs = [w.at[pl.ds(2048 * i, 2048)] for w in (wq_hbm, wk_hbm, wv_hbm)]
        if i < 8:
            srcs.append(wot_hbm.at[pl.ds(4 * D * i, 4 * D)])
        for m, src in enumerate(srcs):
            pltpu.make_async_copy(src, raw.at[pl.ds(i * PART + 2048 * m, src.shape[0])], sem_w.at[i]).start()

    def b_wait(i, rows):
        part = raw.at[pl.ds(pl.multiple_of(i * PART, 16), rows)]
        pltpu.make_async_copy(part, part, sem_w.at[i]).wait()

    def x_stage(j, slot):
        A.stb(AX + 288 * slot, xt[:, pl.ds(pl.multiple_of(j * 128, 128), 128)])

    def proj(j):
        if isinstance(j, int):
            return _Arena(qkv_all.at[pl.ds(((j + 1) & 3) * SLOT, SLOT)])
        return _Arena(qkv_all.at[pl.ds(pl.multiple_of(offs[(j + 1) & 3], 8), SLOT)])

    def no_tick(r):
        pass

    for c in (gate_copy, mem_copy, w_copy[0], x_copy[0], w_copy[1], w_copy[2], wo_copy, x_copy[1], x_copy[2]):
        c.start()

    for i in range(4):
        offs[i] = i * SLOT
    for i in range(8):
        offs[4 + i] = i * PART
    for j in range(NP):
        B.stf(PSTRIDE * j + PV + 24, jnp.zeros((8, 128), F32))
        B.stf(PSTRIDE * j + PV + 120, jnp.zeros((8, 128), F32))
    B.stf(BO, jnp.zeros((B_ROWS - BO, 128), F32))
    gate_copy.wait()
    mem_copy.wait()
    gate = jnp.broadcast_to(gate_ref[...].astype(F32)[None, :], (8, D))
    mem0 = mem_ref[...].astype(F32)
    for k in range(4):
        A.stf(GW + 8 * k, gate[:, 128 * k:128 * k + 128])
        B.stf(HS + 40 * k, mem0[:, 128 * k:128 * k + 128])
    A.stf(GW + 32, jnp.concatenate([gate[:, 512:]] * 2, 1))
    B.stf(HS + 160, jnp.concatenate([mem0[:, 512:]] * 2, 1))
    for i in range(2):
        b_start(i)

    def first_two(*parts):
        return _chain(*[_a_qkv(A, AX + 288 * j, proj(j), no_tick, parts) for j in range(2)])

    w_copy[0].wait()
    _a_transpose_w(A, wqkv, range(4, 9))
    x_copy[0].wait()
    w_copy[1].wait()
    x_stage(0, 0)
    x_stage(1, 1)
    _interleave(first_two(3, 1))
    _a_transpose_w(A, wqkv, range(0, 4))
    w_copy[2].wait()
    _interleave(first_two(0))
    _a_transpose_w(A, wqkv, range(9, 14))
    wo_copy.wait()
    _interleave(first_two(2), _a_transpose_wo(A, wo))
    qkv_all[AK:AG, :] = jnp.broadcast_to(qkv_all[SLOT + AK:SLOT + AG, :1], (AG - AK, 128))

    def tick_raw(r):
        raw[RAW_TICK:RAW_TICK + 16, :] = r[:16].astype(BF16)

    def tick_attend(r):
        qkv_all[TICK:TICK + 8, :] = pltpu.bitcast(r[:8], I32)

    def tick_both(r):
        tick_raw(r)
        tick_attend(r)

    def a_trip(j, project_out, prepare):
        mxu = [_a_qkv(A, AX, proj(j + 2), tick_raw if prepare else no_tick)]
        side = [_a_attend(j, proj(j), proj(j - 1), o_all.at[j], omg)]
        if prepare:
            i = j - 6
            b_wait(i, PART - 16)
            src = raw.at[pl.ds(pl.multiple_of(offs[4 + i], 16), PART)]
            dst = b_ref.at[pl.ds(pl.multiple_of(i * 32, 32), HS), :]
            side.append(_chain(*[
                _b_split_heads(src.at[pl.ds(2048 * m, 2048)], dst, to)
                for m, to in enumerate(((QA, QA + 288), (KA, KA + 256), (VA, VA + 256)))]))
            side.append(_b_transpose_wo(src.at[pl.ds(6144, 4 * D)], dst))
        if project_out:
            A.stb(AO, o_all[j - 4])
            mxu.append(_a_out(A, AO, ga_all.at[j - 4], tick_both if prepare else tick_attend))
        _interleave(_chain(*mxu), *side)
        x_stage(jnp.minimum(j + 3, NB - 1), 0)

    x_copy[1].wait()
    x_stage(2, 0)
    for i in range(2, 5):
        b_start(i)
    lax.fori_loop(0, 4, lambda j, c: a_trip(j, False, False), None)
    x_copy[2].wait()
    for i in range(5, 9):
        b_start(i)
    lax.fori_loop(4, 6, lambda j, c: a_trip(j, True, False), None)
    lax.fori_loop(6, NB - 2, lambda j, c: a_trip(j, True, True), None)

    def k2_transpose():
        for j in range(NP):
            B.stb(PSTRIDE * j + K2, B.ldb(PSTRIDE * j + K2, 64).T)
            yield

    def last_trip(i, carry):
        j = NB - 2 + i
        for b in range(2):
            A.stb(AO + 288 * b, o_all[NB - 6 + 2 * i + b])
        _interleave(_chain(*[_a_out(A, AO + 288 * b, ga_all.at[NB - 6 + 2 * i + b], tick_attend) for b in range(2)]),
                    _a_attend(j, proj(j), proj(j - 1), o_all.at[j], omg), span=(-0.3, 0.7))

    lax.fori_loop(0, 2, last_trip, None)
    b_wait(8, 6144)
    src = [raw.at[pl.ds(8 * PART + 2048 * m, 2048)] for m in range(3)]
    for b in range(2):
        A.stb(AO + 288 * b, o_all[NB - 2 + b])
    _interleave(
        _chain(*[_a_out(A, AO + 288 * b, ga_all.at[NB - 2 + b], no_tick) for b in range(2)]),
        _chain(_b_split_heads(src[1], b_ref, (K2 + 32, K2)),
               _b_split_heads(src[0], b_ref, (QA + 256, QA + 544)),
               (NP, k2_transpose()),
               _b_split_heads(src[2], b_ref, (PV + 32, PV + 64))))

    def x_transpose(j, n):
        cols = pl.ds(pl.multiple_of(j * 128, 128), 128)
        if n < 4:
            t = xt[128 * n:128 * n + 128, cols]
        else:
            t = jnp.concatenate([xt[512:576, cols]] * 2, 0)
        B.stb(XN + 64 * n, t.T)

    def x_place(u):
        for n in range(5):
            B.stf(HS + 200 * u + 40 * n + M, B.ldb(XN + 64 * n + 16 * u, 16).astype(F32))

    def mix(j, n):
        rows = min(128, D - 128 * n)
        bt = B.ldf(BO + 128 * n, 128).T if n < 4 else B.ldf(B2 + 64, 64)
        w = jnp.concatenate([omg[j]] * (rows // 8), 0)
        out_buf[j, 128 * n:128 * n + rows, :] = (
            ga_all[j, 128 * n:128 * n + rows, :] + w * bt).astype(BF16)

    def out_copy(j):
        return pltpu.make_async_copy(
            out_buf.at[j], out_hbm.at[:, pl.ds(pl.multiple_of(j * 128, 128), 128)], sem_out)

    for n in range(5):
        x_transpose(0, n)
    for u in range(U):
        x_place(u)

    def b_body(g, carry):
        jn, jp = jnp.minimum(g + 1, NB - 1), jnp.maximum(g - 1, 0)
        for u in range(U):
            extra = {("o", 3, 0): functools.partial(x_place, u)}
            if u == 0:
                for n in range(4):
                    extra["o", n, 16] = functools.partial(mix, jp, n)
                for n in range(5):
                    extra["o", 1, 6 * n] = functools.partial(x_transpose, jn, n)
            if u == U - 1:
                extra["v", 20] = functools.partial(mix, jp, 4)
            _b_step(B, u, extra)

        @pl.when(g > 0)
        def _():
            out_copy(jp).start()

        return carry

    lax.fori_loop(0, NB, b_body, 0)
    lane = lax.broadcasted_iota(I32, (64, 128), 1)
    B.stf(B2 + 64, functools.reduce(jnp.add, [B.ldf(B2 + 64, 64)] + [
        jnp.where(lane < SEG * (u + 1), 0.0, _b_out_tail(B, u)) for u in range(U - 1)]))
    for n in range(5):
        mix(NB - 1, n)
    out_copy(NB - 1).start()
    for j in range(NB):
        out_copy(j).wait()


@functools.partial(jax.jit, static_argnames=("B_seg_len",))
def pallas_gated_mix__sliding_local_dilated__memory_aug_recurrent_mem_tr__prompt_kernel(
    A_x: jax.Array,
    A_wqkv: jax.Array,
    A_wo: jax.Array,
    B_x: jax.Array,
    B_mem0: jax.Array,
    B_Wq: jax.Array,
    B_Wk: jax.Array,
    B_Wv: jax.Array,
    B_Wo: jax.Array,
    B_seg_len: int,
    gate_w: jax.Array,
):
    del B_x
    assert A_x.shape == (1, S, D) and B_mem0.shape == (1, M, D) and B_Wq.shape == (D, H, DH)
    assert B_seg_len == SEG
    hbm = pl.BlockSpec(memory_space=pl.ANY)
    out_t = pl.pallas_call(
        _kernel,
        out_shape=jax.ShapeDtypeStruct((D, S), BF16),
        in_specs=[hbm] * 9,
        out_specs=hbm,
        scratch_shapes=[
            pltpu.VMEM((D, S), BF16),
            pltpu.VMEM((D, 3 * D), BF16),
            pltpu.VMEM((D, D), BF16),
            pltpu.VMEM((M, D), BF16),
            pltpu.VMEM((D,), BF16),
            pltpu.VMEM((9 * PART, DH), BF16),
            pltpu.VMEM((A_ROWS, 128), I32),
            pltpu.VMEM((B_ROWS, 128), I32),
            pltpu.VMEM((4 * SLOT, 128), I32),
            pltpu.VMEM((NB, D, 128), F32),
            pltpu.VMEM((NB, D, 128), F32),
            pltpu.VMEM((NB, 8, 128), F32),
            pltpu.VMEM((NB, D, 128), BF16),
            pltpu.SMEM((12,), I32),
            pltpu.SemaphoreType.DMA((9,)),
            pltpu.SemaphoreType.DMA((9,)),
            pltpu.SemaphoreType.DMA,
        ],
        compiler_params=pltpu.CompilerParams(vmem_limit_bytes=100 * 1024 * 1024),
    )(
        A_x.reshape(S, D).T, A_wqkv, A_wo, B_mem0.reshape(M, D), gate_w,
        B_Wq.reshape(D * H, DH), B_Wk.reshape(D * H, DH), B_Wv.reshape(D * H, DH),
        B_Wo.transpose(0, 2, 1).reshape(H * D, DH),
    )
    return out_t.T.reshape(1, S, D)
```

```python
import functools

import jax
import jax.numpy as jnp
from jax import lax
import jax.experimental.pallas as pl
import jax.experimental.pallas.tpu as pltpu

F32, BF16, I32 = jnp.float32, jnp.bfloat16, jnp.int32

S, D = 2048, 576
NB = S // 128
HA, DA, WIN, DIL = 32, 18, 8, 2
H, DH, M, SEG = 32, 128, 8, 32
L = M + SEG
NP = H // 2
U = 128 // SEG
NEG = -1000000000.0

QA = 0
KA = QA + 576
KR = KA + 512
VA = KR + 64
PV = VA + 512
PSTRIDE = PV + 128 + 4
OA = NP * PSTRIDE
K2 = OA + H * 320
HS = K2 + 2048
GS = HS + U * 200
GT = GS + 64
QS = GT + 64
KS = QS + H * 40
RE = KS + NP * 64
PS = RE + H * 40
RS = PS + NP * 40
OS = RS + NP * 40
XN = OS + H * 40
BO = XN + 320
B2 = BO + 512
OT = B2 + 128
B_ROWS = OT + H * 64

PART = 3 * 2048 + 16
RAW_TICK = 4 * PART - 16

WT = 0
GW = WT + 5 * 1728
WP = GW + 40
WOT = WP + 27 * 160
AX = WOT + 5 * 288
A_ROWS = AX + 2 * 288
AQ, AK, AV, AG, TICK, SLOT = 0, 576, 864, 1152, 1160, 1168


def _dot(a, b):
    return lax.dot_general(a, b, (((1,), (0,)), ((), ())), preferred_element_type=F32)


class _Arena:
    def __init__(self, ref):
        self.r = ref

    def ldi(self, o, n):
        return self.r[o:o + n, :]

    def ldf(self, o, n):
        return pltpu.bitcast(self.r[o:o + n, :], F32)

    def ldb(self, o, n):
        return pltpu.bitcast(self.r[o:o + n, :], BF16)

    def stf(self, o, v):
        self.r[o:o + v.shape[0], :] = pltpu.bitcast(v, I32)

    def stb(self, o, v):
        self.r[o:o + v.shape[0] // 2, :] = pltpu.bitcast(v.astype(BF16), I32)


def _pad2(t, rows, cols):
    r, c = t.shape
    if c < cols:
        t = jnp.concatenate([t, jnp.zeros((r, cols - c), t.dtype)], 1)
    if r < rows:
        t = jnp.concatenate([t, jnp.zeros((rows - r, cols), t.dtype)], 0)
    return t


def _interleave(main, *side, span=(0.0, 0.9)):
    jobs = (main,) + side
    order = [((i + 1) / main[0], 0) for i in range(main[0])]
    order += [(span[0] + (span[1] - span[0]) * i / n, k + 1) for k, (n, _) in enumerate(side) for i in range(n)]
    for _, k in sorted(order):
        next(jobs[k][1])
    for _, gen in jobs:
        assert next(gen, "end") == "end"


def _once(fn, *args):
    def gen():
        fn(*args)
        yield
    return 1, gen()


def _chain(*jobs):
    def gen():
        for _, g in jobs:
            yield from g
    return sum(n for n, _ in jobs), gen()


def _a_transpose_w(A, w_ref, cblocks):
    for c in cblocks:
        nc = min(128, 3 * D - 128 * c)
        for k in range(5):
            nk = min(128, D - 128 * k)
            t = _pad2(w_ref[128 * k:128 * k + nk, 128 * c:128 * c + nc], 128, 128).T
            A.stf(WT + 1728 * k + 128 * c, t[:nc].astype(F32))


def _a_transpose_wo(A, w_ref):
    def gen():
        for c in range(5):
            nc = min(128, D - 128 * c)
            for k in range(5):
                nk = min(128, D - 128 * k)
                t = _pad2(w_ref[128 * k:128 * k + nk, 128 * c:128 * c + nc], 128, 128).T
                A.stb(WOT + 288 * k + 64 * c, t[:nc])
                yield
    return 25, gen()


def _a_qkv(A, x_off, dst, parts=(3, 1, 0, 2), first=False):
    def proj(rows_of_k):
        ch = [rows_of_k(k) for k in range(5)]
        return _dot(jnp.concatenate(ch[:4] + [ch[4][:, :64]], 1), A.ldb(x_off, 288))

    def gen():
        for part in parts:
            if part == 3:
                dst.stf(AG, jax.nn.sigmoid(proj(lambda k: A.ldf(GW + 8 * k, 8))))
                continue
            for d0 in range(0, DA, 2):
                def weights(k):
                    packed = WP + 160 * (9 * part + d0 // 2) + 32 * k
                    if not first:
                        return A.ldb(packed, 32)
                    w = jnp.concatenate([
                        pltpu.bitcast(A.r[pl.ds(WT + 1728 * k + D * part + 8 * DA * hg + d, 8, stride=DA), :], F32)
                        for hg in range(4) for d in (d0, d0 + 1)], 0)
                    A.stb(packed, w)
                    return w

                r = proj(weights)
                for i in range(0, 64, 16):
                    if part == 0:
                        dst.stf(AQ + 32 * d0 + i, r[i:i + 16])
                    else:
                        dst.stb((AK if part == 1 else AV) + 16 * d0 + i // 2, r[i:i + 16])
                    yield
    return sum(2 * DA for p in parts if p < 3), gen()


def _a_attend(j, cur, old, o_ref, omg_ref):
    def window(o):
        lane = lax.broadcasted_iota(I32, (8, 128), 1)
        c, p = cur.ldi(o, 8), old.ldi(o, 8)
        out = []
        for w in range(WIN):
            sh = DIL * w
            t = c if w == 0 else pltpu.roll(jnp.where(lane >= 128 - sh, p, c), sh, 1)
            out.append(pltpu.bitcast(t, BF16).astype(F32))
        return out

    def gen():
        pos = j * 128 + lax.broadcasted_iota(I32, (8, 128), 1)
        for hg in range(4):
            lg = None
            for d in range(0, DA, 2):
                q = cur.ldf(AQ + 32 * d + 16 * hg, 16)
                pr = [q * kw for kw in window(AK + 16 * d + 8 * hg)]
                pr = [t[:8] + t[8:] for t in pr]
                lg = pr if d == 0 else [a + b for a, b in zip(lg, pr)]
                yield
            lg = [jnp.where(pos >= DIL * w, t * DA ** -0.5, NEG) for w, t in enumerate(lg)]
            mx = functools.reduce(jnp.maximum, lg)
            e = [jnp.exp(t - mx) for t in lg]
            g = cur.ldf(AG, 8)
            if hg == 0:
                omg_ref[j] = 1.0 - g
            r = g / functools.reduce(jnp.add, e)
            p = [jnp.concatenate([t * r] * 2, 0) for t in e]
            yield
            for d in range(0, DA, 2):
                o = functools.reduce(jnp.add, [a * b for a, b in zip(p, window(AV + 16 * d + 8 * hg))])
                o = pltpu.bitcast(o.astype(BF16).astype(F32), I32)
                o_ref[pl.ds(4 * DA * hg + d // 2, 8, stride=DA // 2), :] = (
                    lax.shift_right_logical(o[:8], 16) | o[8:])
                yield
    return 4 * DA + 4, gen()


def _a_out(A, o_ref, ga_ref, tick):
    def gen():
        for r0 in range(0, D, 96):
            ch = [A.ldb(WOT + 288 * k + r0 // 2, 48) for k in range(5)]
            r = _dot(jnp.concatenate(ch[:4] + [ch[4][:, :64]], 1), pltpu.bitcast(o_ref[...], BF16))
            for i in range(0, 96, 32):
                tick(r[i:i + 32])
                ga_ref[r0 + i:r0 + i + 32, :] = r[i:i + 32]
                yield
    return D // 32, gen()


def _b_split_heads(raw, dst, even, odd):
    def gen():
        for r in range(raw.shape[0] // 64):
            e = pltpu.bitcast(raw[64 * r:64 * r + 32, :], I32)
            o = pltpu.bitcast(raw[64 * r + 32:64 * r + 64, :], I32)
            dst[pl.ds(even + r, NP, stride=PSTRIDE), :] = (e & 0xFFFF) | (o << 16)
            dst[pl.ds(odd + r, NP, stride=PSTRIDE), :] = lax.shift_right_logical(e, 16) | (o & -65536)
            yield
    return raw.shape[0] // 64, gen()


def _wo_piece(h, k):
    return OA + 256 * (10 * (h % 4) + k) + 32 * (h // 4)


def _b_transpose_wo(wot, dst, h0):
    def put(t, o0, o1):
        t = pltpu.bitcast(t, I32)
        dst[o0:o0 + 32, :] = t[:32]
        dst[o1:o1 + 32, :] = t[32:]

    def gen():
        for h in range(4):
            for n in range(4):
                put(wot[D * h + 128 * n:D * h + 128 * n + 128, :].T, _wo_piece(h0 + h, 2 * n), _wo_piece(h0 + h, 2 * n + 1))
                yield
            if h % 2:
                t = jnp.concatenate([wot[D * i + 512:D * i + D, :] for i in (h - 1, h)], 0)
                put(t, _wo_piece(h0 + h - 1, 9), _wo_piece(h0 + h, 9))
                put(t.T, _wo_piece(h0 + h - 1, 8), _wo_piece(h0 + h, 8))
                yield
    return 18, gen()


def _b_out_tail(B, u):
    return functools.reduce(jnp.add, [
        lax.dot_general(B.ldb(_wo_piece(h, 9), 32), B.ldb(OT + 64 * h, 64), (((1,), (1,)), ((), ())),
                        preferred_element_type=F32)
        for h in range(8 * u, 8 * u + 8)])


def _b_step(B, u, extra):
    hs, hs_next = HS + 200 * u, HS + 200 * ((u + 1) % U)
    row = lax.broadcasted_iota(I32, (L, 128), 0)
    lane = lax.broadcasted_iota(I32, (L, 128), 1)
    lo = lane < 64
    lo64 = lax.broadcasted_iota(I32, (64, 128), 1) < 64
    col = lane & 63
    mask = (row < M) | (row >= col)
    in_a, in_b = lane < L, (lane >= 64) & (lane < 64 + L)
    z24 = jnp.zeros((24, 128), F32)
    z8 = jnp.zeros((8, 128), F32)

    def w(base, size, h):
        return PSTRIDE * (h // 2) + base + size * (h % 2)

    def tile(o0, o1):
        return pltpu.bitcast(jnp.concatenate([B.ldi(o0, 32), B.ldi(o1, 32)], 0), BF16)

    def h1():
        return jnp.concatenate([B.ldf(hs + 40 * n, 40) for n in range(4)], 1)

    def t_g():
        c4 = B.ldf(hs + 160, 40)
        g = jnp.concatenate([jnp.where(lo, 0.0, c4), z24, jnp.where(lo, c4, 0.0), z24], 0)
        B.stb(GS, g)
        B.stb(GT, g.T)

    def t_k(h):
        B.stf(RE + 40 * h, _dot(h1(), B.ldb(w(KA, 256, h), 256)))
        if h % 2:
            k = jnp.concatenate([B.ldf(RE + 40 * (h - 1), 40), z24, B.ldf(RE + 40 * h, 40), z24], 0)
            B.stb(KS + 64 * (h // 2), k.astype(BF16).T)

    def t_q(h):
        o = w(QA, 288, h)
        B.stf(QS + 40 * h, _dot(h1(), B.ldb(o, 256)) + _dot(B.ldf(hs + 160, 40)[:, :64], B.ldb(o + 256, 32)))

    def t_s(h):
        kt, w2 = B.ldi(KS + 64 * (h // 2), 64), B.ldi(K2 + 256 * (h // 2 % 8) + 128 * (h // 16), 64)
        rhs = jnp.where(lo64, w2, kt) if h % 2 else jnp.where(lo64, kt, w2)
        B.stf(RE + 40 * h, _dot(B.ldf(QS + 40 * h, 40), pltpu.bitcast(rhs, BF16)))

    def t_s2(j):
        a, b = B.ldf(RE + 80 * j, 40), B.ldf(RE + 80 * j + 40, 40)
        s = jnp.where(lo, a, b) + _dot(jnp.where(lo, b, a), B.ldb(GT, 64))
        s = jnp.where(mask, s * DH ** -0.5, NEG)
        B.stf(RS + 40 * j, s)
        ma = jnp.max(jnp.where(in_a, s, -jnp.inf), axis=1, keepdims=True)
        mb = jnp.max(jnp.where(in_b, s, -jnp.inf), axis=1, keepdims=True)
        e = jnp.exp(B.ldf(RS + 40 * j, 40) - jnp.where(lo, ma, mb))
        ea, eb = jnp.where(in_a, e, 0.0), jnp.where(in_b, e, 0.0)
        B.stf(PS + 40 * j, ea + eb)
        la = jnp.sum(ea, axis=1, keepdims=True)
        lb = jnp.sum(eb, axis=1, keepdims=True)
        B.stf(PS + 40 * j, B.ldf(PS + 40 * j, 40) / jnp.where(lo, la, lb))

    def t_r(j):
        B.stf(RS + 40 * j, _dot(B.ldf(PS + 40 * j, 40), B.ldb(GS, 64)))

    def t_v(h):
        v = _dot(h1(), B.ldb(w(VA, 256, h), 256))
        B.stb(w(PV, 96, h), jnp.concatenate([v, z8], 0))

    def t_pv(h):
        p, r = B.ldf(PS + 40 * (h // 2), 40), B.ldf(RS + 40 * (h // 2), 40)
        lhs = jnp.where(lo, r, p) if h % 2 else jnp.where(lo, p, r)
        o = _dot(lhs, B.ldb(w(PV, 64, h), 64))
        B.stf(OS + 40 * h, o)
        B.stb(OT + 64 * h + 16 * u, o[M:])

    d_s, d_s2, d_pv = 20, 18, 22
    big = [("k", h) for h in range(H)] + [("g",)] + [(p, h) for p in "qv" for h in range(H)]
    for i in range(4 * H):
        big.append(("o", i // H, i % H))
        if i % 8 == 7:
            big.append(("m", i // 8))
    small = {"pv": t_pv, "r": t_r, "s2": t_s2, "s": t_s}
    nxt = dict.fromkeys(small, 0)
    done = {}
    now = 0

    def old(key, dist):
        return key in done and now - done[key] >= dist

    def ready(kind, i):
        if kind == "s":
            return old(("q", i), d_s)
        if kind == "s2":
            return old(("s", 2 * i + 1), d_s2)
        if kind == "r":
            return old(("s2", i), 64) and old(("v", 2 * i), 0)
        return old(("r", i // 2), d_s2) and old(("v", i), d_pv)

    acc = mem2 = None
    for t in big:
        for kind, fn in small.items():
            if ready(kind, nxt[kind]):
                fn(nxt[kind])
                now += 1
                done[kind, nxt[kind]] = now
                nxt[kind] += 1
        if t in extra:
            extra[t]()
        if t[0] == "k":
            t_k(t[1])
            now += 4
        elif t[0] == "g":
            t_g()
        elif t[0] == "q":
            t_q(t[1])
            now += 5
        elif t[0] == "v":
            t_v(t[1])
            now += 4
        elif t[0] == "m":
            a, b = 2 * t[1], 2 * t[1] + 1
            y = _dot(jnp.concatenate([B.ldf(OS + 40 * a, M), B.ldf(OS + 40 * b, M)], 0),
                     tile(_wo_piece(a, 8), _wo_piece(b, 8)))
            mem2 = y if a == 0 else mem2 + y
        else:
            _, n, h = t
            assert ("pv", h) in done
            y = _dot(B.ldf(OS + 40 * h, 40), tile(_wo_piece(h, 2 * n), _wo_piece(h, 2 * n + 1)))
            acc = y if h == 0 else acc + y
            if h == H - 1:
                B.stf(hs_next + 40 * n, acc[:M])
                B.stf(BO + 128 * n + SEG * u, acc[M:])
            now += 1
        done[t] = now
    mem2 = jnp.where(lo[:M], mem2[:M], mem2[M:])
    B.stf(hs_next + 160, mem2 + pltpu.roll(mem2, 64, 1))
    y = _b_out_tail(B, u)
    if u == U - 1:
        B.stf(B2 + 64, B.ldf(B2, 64) + y)
    else:
        new = lax.broadcasted_iota(I32, (64, 128), 1) < SEG * (u + 1)
        B.stf(B2, jnp.where(new, y, 0.0) + (B.ldf(B2, 64) if u else 0.0))
        B.stf(B2 + 64, jnp.where(new, 0.0, y) + B.ldf(B2 + 64, 64))


def _kernel(xt_hbm, wqkv_hbm, wo_hbm, mem_hbm, gate_hbm, wq_hbm, wk_hbm, wv_hbm, wot_hbm,
            out_hbm,
            xt, wqkv, wo, mem_ref, gate_ref, raw, wot, a_ref, b_ref, qkv_all, o_all, o_last, ga_all, omg, out_buf,
            offs, sem_in, sem_w, sem_out):
    A, B = _Arena(a_ref), _Arena(b_ref)

    def cols(src, dst, c0, c1, sem):
        return pltpu.make_async_copy(src.at[:, pl.ds(c0, c1 - c0)], dst.at[:, pl.ds(c0, c1 - c0)], sem_in.at[sem])

    x_copy = [cols(xt_hbm, xt, c0, c1, i) for i, (c0, c1) in
              enumerate(((0, 256), (256, 768), (768, S)))]
    w_copy = [cols(wqkv_hbm, wqkv, c0, c1, 3 + i) for i, (c0, c1) in
              enumerate(((512, 896), (896, 1152), (0, 512), (1152, 3 * D)))]
    wo_copy = pltpu.make_async_copy(wo_hbm, wo, sem_in.at[8])
    mem_copy = pltpu.make_async_copy(mem_hbm, mem_ref, sem_in.at[9])
    gate_copy = pltpu.make_async_copy(gate_hbm, gate_ref, sem_in.at[10])

    def b_start(i):
        for m, w in enumerate((wq_hbm, wk_hbm, wv_hbm)):
            pltpu.make_async_copy(w.at[pl.ds(pl.multiple_of(2048 * i, 16), 2048)],
                                  raw.at[pl.ds(pl.multiple_of(i * PART + 2048 * m, 16), 2048)], sem_w.at[i]).start()

    def b_wait(i):
        part = raw.at[pl.ds(pl.multiple_of(i * PART, 16), 3 * 2048)]
        pltpu.make_async_copy(part, part, sem_w.at[i]).wait()

    def wot_copy(i):
        rows = pl.ds(pl.multiple_of(8 * D * i, 16), 8 * D)
        return pltpu.make_async_copy(wot_hbm.at[rows], wot.at[rows], sem_w.at[9 + i])

    def x_stage(j, slot):
        A.stb(AX + 288 * slot, xt[:, pl.ds(pl.multiple_of(j * 128, 128), 128)])

    def proj(j):
        if isinstance(j, int):
            return _Arena(qkv_all.at[pl.ds((j + 1) % 5 * SLOT, SLOT)])
        return _Arena(qkv_all.at[pl.ds(pl.multiple_of(offs[lax.rem(j + 1, 5)], 8), SLOT)])

    for c in (w_copy[0], gate_copy, mem_copy, w_copy[1], x_copy[0], w_copy[2], w_copy[3],
              wo_copy):
        c.start()

    for i in range(5):
        offs[i] = i * SLOT
    for i in range(2):
        offs[5 + i] = 4 * i * PART
        offs[7 + i] = 8 * PART + 1024 * i
    for j in range(NP):
        B.stf(PSTRIDE * j + PV + 24, jnp.zeros((8, 128), F32))
        B.stf(PSTRIDE * j + PV + 120, jnp.zeros((8, 128), F32))
    B.stf(BO, jnp.zeros((B_ROWS - BO, 128), F32))
    w_copy[0].wait()
    gate_copy.wait()
    mem_copy.wait()
    gate = jnp.broadcast_to(gate_ref[...].astype(F32)[None, :], (8, D))
    mem0 = mem_ref[...].astype(F32)
    for k in range(4):
        A.stf(GW + 8 * k, gate[:, 128 * k:128 * k + 128])
        B.stf(HS + 40 * k, mem0[:, 128 * k:128 * k + 128])
    A.stf(GW + 32, jnp.concatenate([gate[:, 512:]] * 2, 1))
    B.stf(HS + 160, jnp.concatenate([mem0[:, 512:]] * 2, 1))

    def project(j, *parts):
        return _a_qkv(A, AX + 288 * j, proj(j), parts, first=j == 0)

    _a_transpose_w(A, wqkv, range(4, 7))
    w_copy[1].wait()
    _a_transpose_w(A, wqkv, range(7, 9))
    x_copy[0].wait()
    x_stage(0, 0)
    x_stage(1, 1)
    _interleave(_chain(project(0, 3, 1), project(1, 3, 1)))
    w_copy[2].wait()
    x_copy[1].start()
    _a_transpose_w(A, wqkv, range(0, 4))
    _interleave(project(0, 0))
    w_copy[3].wait()
    x_copy[2].start()
    _a_transpose_w(A, wqkv, range(9, 14))
    _interleave(_chain(project(1, 0), project(0, 2)))
    wo_copy.wait()
    b_start(8)
    _interleave(project(1, 2), _a_transpose_wo(A, wo))
    qkv_all[AK:AG, :] = jnp.broadcast_to(qkv_all[SLOT + AK:SLOT + AG, :1], (AG - AK, 128))

    def tick_raw(r):
        raw[RAW_TICK:RAW_TICK + 16, :] = r[:16].astype(BF16)

    def tick_attend(r):
        qkv_all[TICK:TICK + 8, :] = pltpu.bitcast(r[:8], I32)

    def attend(j):
        return _a_attend(j, proj(j), proj(j - 1), o_all.at[j], omg)

    def project_out(j0, n, tick):
        return _chain(*[_a_out(A, o_all.at[j0 + b], ga_all.at[j0 + b], tick) for b in range(n)])

    def attend_trip(t, carry):
        pl.when(t == 1)(x_copy[2].wait)

        @pl.when(t < 4)
        def _():
            b_start(2 * t)
            b_start(2 * t + 1)
            wot_copy(t).start()

        def project(i):
            return _chain(_a_qkv(A, AX + 288 * i, proj(2 * t + 2 + i)),
                          _once(x_stage, jnp.minimum(2 * t + 4 + i, NB - 1), i))

        _interleave(_chain(project(0), project(1)), _chain(attend(2 * t), attend(2 * t + 1)), span=(-0.04, 0.87))

    x_copy[1].wait()
    x_stage(2, 0)
    x_stage(3, 1)
    lax.fori_loop(0, NB // 2 - 1, attend_trip, None)

    def last_trip(t, carry):
        src = raw.at[pl.ds(pl.multiple_of(offs[7 + t], 16), 5120)]
        dst = b_ref.at[pl.ds(pl.multiple_of(t * 16, 16), OA), :]
        _interleave(
            project_out(3 * t, 3, lambda r: (tick_attend(r), tick_raw(r))), _a_attend(NB - 2 + t, proj(NB - 2 + t), proj(NB - 3 + t), o_last.at[t], omg),
            _chain(*[_b_split_heads(src.at[pl.ds(2048 * m, 1024)], dst, even, odd) for m, (even, odd) in
                     enumerate(((QA + 256, QA + 544), (KR + 32, KR), (PV + 32, PV + 64)))]),
            span=(-0.08, 0.82))

    b_wait(8)
    lax.fori_loop(0, 2, last_trip, None)
    o_all[NB - 2:] = o_last[...]

    def prepare_trip(t, carry):
        for c in range(4):
            b_wait(4 * t + c)
        for c in range(2):
            wot_copy(2 * t + c).wait()
        src = raw.at[pl.ds(pl.multiple_of(offs[5 + t], 16), 4 * PART)]
        dst = b_ref.at[pl.ds(pl.multiple_of(t * 128, 128), HS), :]
        pairs = _Arena(b_ref.at[pl.ds(pl.multiple_of(t * 8 * PSTRIDE, 8), 8 * PSTRIDE), :])
        k2 = [pairs.ldb(PSTRIDE * j + KR, 64).T for j in range(8)]
        for j in range(8):
            _Arena(dst).stb(K2 + 256 * j, k2[j])
        split = [_b_split_heads(src.at[pl.ds(PART * c + 2048 * m, 2048)], dst, o + 32 * c, o + 32 * c + n)
                 for c in range(4) for m, (o, n) in enumerate(((QA, 288), (KA, 256), (VA, 256)))]
        wo_t = [_b_transpose_wo(wot.at[pl.ds(pl.multiple_of(4 * D * (4 * t + c), 16), 4 * D)], dst, 4 * c) for c in range(4)]
        _interleave(project_out(6 + 5 * t, 5, tick_raw), _chain(*split), _chain(*wo_t), span=(-0.04, 0.93))

    lax.fori_loop(0, 2, prepare_trip, None)

    def x_transpose(j, n):
        cols = pl.ds(pl.multiple_of(j * 128, 128), 128)
        if n < 4:
            t = xt[128 * n:128 * n + 128, cols]
        else:
            t = jnp.concatenate([xt[512:576, cols]] * 2, 0)
        B.stb(XN + 64 * n, t.T)

    def x_place(u):
        for n in range(5):
            B.stf(HS + 200 * u + 40 * n + M, B.ldb(XN + 64 * n + 16 * u, 16).astype(F32))

    def mix(j, n):
        rows = min(128, D - 128 * n)
        bt = B.ldf(BO + 128 * n, 128).T if n < 4 else B.ldf(B2 + 64, 64)
        w = jnp.concatenate([omg[j]] * (rows // 8), 0)
        out_buf[j, 128 * n:128 * n + rows, :] = (
            ga_all[j, 128 * n:128 * n + rows, :] + w * bt).astype(BF16)

    def out_copy(j):
        return pltpu.make_async_copy(
            out_buf.at[j], out_hbm.at[:, pl.ds(pl.multiple_of(j * 128, 128), 128)], sem_out)

    for n in range(5):
        x_transpose(0, n)
    for u in range(U):
        x_place(u)

    def b_body(g, carry):
        jn, jp = jnp.minimum(g + 1, NB - 1), jnp.maximum(g - 1, 0)
        for u in range(U):
            extra = {("o", 3, 0): functools.partial(x_place, u)}
            if u == 0:
                for n in range(4):
                    extra["o", n, 16] = functools.partial(mix, jp, n)
                for n in range(5):
                    extra["o", 1, 6 * n] = functools.partial(x_transpose, jn, n)
            if u == U - 1:
                extra["v", 20] = functools.partial(mix, jp, 4)
            _b_step(B, u, extra)

        @pl.when(g > 0)
        def _():
            out_copy(jp).start()

        return carry

    lax.fori_loop(0, NB, b_body, 0)
    lane = lax.broadcasted_iota(I32, (64, 128), 1)
    B.stf(B2 + 64, functools.reduce(jnp.add, [B.ldf(B2 + 64, 64)] + [
        jnp.where(lane < SEG * (u + 1), 0.0, _b_out_tail(B, u)) for u in range(U - 1)]))
    for n in range(5):
        mix(NB - 1, n)
    out_copy(NB - 1).start()
    for j in range(NB):
        out_copy(j).wait()


@functools.partial(jax.jit, static_argnames=("B_seg_len",))
def pallas_gated_mix__sliding_local_dilated__memory_aug_recurrent_mem_tr__prompt_kernel(
    A_x: jax.Array,
    A_wqkv: jax.Array,
    A_wo: jax.Array,
    B_x: jax.Array,
    B_mem0: jax.Array,
    B_Wq: jax.Array,
    B_Wk: jax.Array,
    B_Wv: jax.Array,
    B_Wo: jax.Array,
    B_seg_len: int,
    gate_w: jax.Array,
):
    del B_x
    assert A_x.shape == (1, S, D) and B_mem0.shape == (1, M, D) and B_Wq.shape == (D, H, DH)
    assert B_seg_len == SEG
    hbm = pl.BlockSpec(memory_space=pl.ANY)
    out_t = pl.pallas_call(
        _kernel,
        out_shape=jax.ShapeDtypeStruct((D, S), BF16),
        in_specs=[hbm] * 9,
        out_specs=hbm,
        scratch_shapes=[
            pltpu.VMEM((D, S), BF16),
            pltpu.VMEM((D, 3 * D), BF16),
            pltpu.VMEM((D, D), BF16),
            pltpu.VMEM((M, D), BF16),
            pltpu.VMEM((D,), BF16),
            pltpu.VMEM((9 * PART, DH), BF16),
            pltpu.VMEM((H * D, DH), BF16),
            pltpu.VMEM((A_ROWS, 128), I32),
            pltpu.VMEM((B_ROWS, 128), I32),
            pltpu.VMEM((5 * SLOT, 128), I32),
            pltpu.VMEM((NB, D // 2, 128), I32),
            pltpu.VMEM((2, D // 2, 128), I32),
            pltpu.VMEM((NB, D, 128), F32),
            pltpu.VMEM((NB, 8, 128), F32),
            pltpu.VMEM((NB, D, 128), BF16),
            pltpu.SMEM((9,), I32),
            pltpu.SemaphoreType.DMA((11,)),
            pltpu.SemaphoreType.DMA((13,)),
            pltpu.SemaphoreType.DMA,
        ],
        compiler_params=pltpu.CompilerParams(vmem_limit_bytes=100 * 1024 * 1024),
    )(
        A_x.reshape(S, D).T, A_wqkv, A_wo, B_mem0.reshape(M, D), gate_w,
        B_Wq.reshape(D * H, DH), B_Wk.reshape(D * H, DH), B_Wv.reshape(D * H, DH),
        B_Wo.transpose(0, 2, 1).reshape(H * D, DH),
    )
    return out_t.T.reshape(1, S, D)
```

```python
import functools

import jax
import jax.numpy as jnp
from jax import lax
import jax.experimental.pallas as pl
import jax.experimental.pallas.tpu as pltpu

F32, BF16, I32 = jnp.float32, jnp.bfloat16, jnp.int32

S, D = 2048, 576
NB = S // 128
HA, DA, WIN, DIL = 32, 18, 8, 2
H, DH, M, SEG = 32, 128, 8, 32
L = M + SEG
NP = H // 2
U = 128 // SEG
NEG = -1000000000.0

QA = 0
KA = QA + 576
KR = KA + 512
VA = KR + 64
PV = VA + 512
PSTRIDE = PV + 128 + 4
OA = NP * PSTRIDE
K2 = OA + H * 320
HS = K2 + 2048
GS = HS + U * 200
GT = GS + 64
QS = GT + 64
KS = QS + H * 40
RE = KS + NP * 64
PS = RE + H * 40
RS = PS + NP * 40
OS = RS + NP * 40
XN = OS + H * 40
BO = XN + 320
B2 = BO + 512
OT = B2 + 128
B_ROWS = OT + H * 64

RAW = D * H + 16

WT = 0
GW = WT + 5 * 1728
WP = GW + 40
WOT = WP + 27 * 160
AX = WOT + 5 * 288
A_ROWS = AX + 2 * 288
AQ, AK, AV, AG, TICK, SLOT = 0, 576, 864, 1152, 1160, 1168


def _dot(a, b):
    return lax.dot_general(a, b, (((1,), (0,)), ((), ())), preferred_element_type=F32)


class _Arena:
    def __init__(self, ref):
        self.r = ref

    def ldi(self, o, n):
        return self.r[o:o + n, :]

    def ldf(self, o, n):
        return pltpu.bitcast(self.r[o:o + n, :], F32)

    def ldb(self, o, n):
        return pltpu.bitcast(self.r[o:o + n, :], BF16)

    def stf(self, o, v):
        self.r[o:o + v.shape[0], :] = pltpu.bitcast(v, I32)

    def stb(self, o, v):
        self.r[o:o + v.shape[0] // 2, :] = pltpu.bitcast(v.astype(BF16), I32)


def _pad2(t, rows, cols):
    r, c = t.shape
    if c < cols:
        t = jnp.concatenate([t, jnp.zeros((r, cols - c), t.dtype)], 1)
    if r < rows:
        t = jnp.concatenate([t, jnp.zeros((rows - r, cols), t.dtype)], 0)
    return t


def _interleave(main, *side, span=(0.0, 0.9)):
    jobs = (main,) + side
    order = [((i + 1) / main[0], 0) for i in range(main[0])]
    order += [(span[0] + (span[1] - span[0]) * i / n, k + 1) for k, (n, _) in enumerate(side) for i in range(n)]
    for _, k in sorted(order):
        next(jobs[k][1])
    for _, gen in jobs:
        assert next(gen, "end") == "end"


def _once(fn, *args):
    def gen():
        fn(*args)
        yield
    return 1, gen()


def _chain(*jobs):
    def gen():
        for _, g in jobs:
            yield from g
    return sum(n for n, _ in jobs), gen()


def _a_transpose_w(A, w_ref, cblocks):
    for c in cblocks:
        nc = min(128, 3 * D - 128 * c)
        for k in range(5):
            nk = min(128, D - 128 * k)
            t = _pad2(w_ref[128 * k:128 * k + nk, 128 * c:128 * c + nc], 128, 128).T
            A.stf(WT + 1728 * k + 128 * c, t[:nc].astype(F32))


def _a_transpose_wo(A, w_ref):
    def gen():
        for c in range(5):
            nc = min(128, D - 128 * c)
            for k in range(5):
                nk = min(128, D - 128 * k)
                t = _pad2(w_ref[128 * k:128 * k + nk, 128 * c:128 * c + nc], 128, 128).T
                A.stb(WOT + 288 * k + 64 * c, t[:nc])
                yield
    return 25, gen()


def _a_qkv(A, x_off, dst, parts=(3, 1, 0, 2), first=False):
    def proj(rows_of_k):
        ch = [rows_of_k(k) for k in range(5)]
        return _dot(jnp.concatenate(ch[:4] + [ch[4][:, :64]], 1), A.ldb(x_off, 288))

    def gen():
        for part in parts:
            if part == 3:
                dst.stf(AG, jax.nn.sigmoid(proj(lambda k: A.ldf(GW + 8 * k, 8))))
                continue
            for d0 in range(0, DA, 2):
                def weights(k):
                    packed = WP + 160 * (9 * part + d0 // 2) + 32 * k
                    if not first:
                        return A.ldb(packed, 32)
                    w = jnp.concatenate([
                        pltpu.bitcast(A.r[pl.ds(WT + 1728 * k + D * part + 8 * DA * hg + d, 8, stride=DA), :], F32)
                        for hg in range(4) for d in (d0, d0 + 1)], 0)
                    A.stb(packed, w)
                    return w

                r = proj(weights)
                for i in range(0, 64, 16):
                    if part == 0:
                        dst.stf(AQ + 32 * d0 + i, r[i:i + 16])
                    else:
                        dst.stb((AK if part == 1 else AV) + 16 * d0 + i // 2, r[i:i + 16])
                    yield
    return sum(2 * DA for p in parts if p < 3), gen()


def _a_attend(j, cur, old, o_ref, omg_ref):
    def window(o):
        lane = lax.broadcasted_iota(I32, (8, 128), 1)
        c, p = cur.ldi(o, 8), old.ldi(o, 8)
        out = []
        for w in range(WIN):
            sh = DIL * w
            t = c if w == 0 else pltpu.roll(jnp.where(lane >= 128 - sh, p, c), sh, 1)
            out.append(pltpu.bitcast(t, BF16).astype(F32))
        return out

    def gen():
        pos = j * 128 + lax.broadcasted_iota(I32, (8, 128), 1)
        for hg in range(4):
            lg = None
            for d in range(0, DA, 2):
                q = cur.ldf(AQ + 32 * d + 16 * hg, 16)
                pr = [q * kw for kw in window(AK + 16 * d + 8 * hg)]
                pr = [t[:8] + t[8:] for t in pr]
                lg = pr if d == 0 else [a + b for a, b in zip(lg, pr)]
                yield
            lg = [jnp.where(pos >= DIL * w, t * DA ** -0.5, NEG) for w, t in enumerate(lg)]
            mx = functools.reduce(jnp.maximum, lg)
            e = [jnp.exp(t - mx) for t in lg]
            g = cur.ldf(AG, 8)
            if hg == 0:
                omg_ref[j] = 1.0 - g
            r = g / functools.reduce(jnp.add, e)
            p = [jnp.concatenate([t * r] * 2, 0) for t in e]
            yield
            for d in range(0, DA, 2):
                o = functools.reduce(jnp.add, [a * b for a, b in zip(p, window(AV + 16 * d + 8 * hg))])
                o = pltpu.bitcast(o.astype(BF16).astype(F32), I32)
                o_ref[pl.ds(4 * DA * hg + d // 2, 8, stride=DA // 2), :] = (
                    lax.shift_right_logical(o[:8], 16) | o[8:])
                yield
    return 4 * DA + 4, gen()


def _a_out(A, o_ref, ga_ref, tick):
    def gen():
        for r0 in range(0, D, 96):
            ch = [A.ldb(WOT + 288 * k + r0 // 2, 48) for k in range(5)]
            r = _dot(jnp.concatenate(ch[:4] + [ch[4][:, :64]], 1), pltpu.bitcast(o_ref[...], BF16))
            for i in range(0, 96, 32):
                tick(r[i:i + 32])
                ga_ref[r0 + i:r0 + i + 32, :] = r[i:i + 32]
                yield
    return D // 32, gen()


def _b_split_heads(raw, dst, even, odd):
    def gen():
        for r in range(raw.shape[0] // 64):
            e = pltpu.bitcast(raw[64 * r:64 * r + 32, :], I32)
            o = pltpu.bitcast(raw[64 * r + 32:64 * r + 64, :], I32)
            dst[pl.ds(even + r, NP, stride=PSTRIDE), :] = (e & 0xFFFF) | (o << 16)
            dst[pl.ds(odd + r, NP, stride=PSTRIDE), :] = lax.shift_right_logical(e, 16) | (o & -65536)
            yield
    return raw.shape[0] // 64, gen()


def _wo_piece(h, k):
    return OA + 256 * (10 * (h % 4) + k) + 32 * (h // 4)


def _b_transpose_wo(wot, dst, h0):
    def put(t, o0, o1):
        t = pltpu.bitcast(t, I32)
        dst[o0:o0 + 32, :] = t[:32]
        dst[o1:o1 + 32, :] = t[32:]

    def gen():
        for h in range(4):
            for n in range(4):
                put(wot[D * h + 128 * n:D * h + 128 * n + 128, :].T, _wo_piece(h0 + h, 2 * n), _wo_piece(h0 + h, 2 * n + 1))
                yield
            if h % 2:
                t = jnp.concatenate([wot[D * i + 512:D * i + D, :] for i in (h - 1, h)], 0)
                put(t, _wo_piece(h0 + h - 1, 9), _wo_piece(h0 + h, 9))
                put(t.T, _wo_piece(h0 + h - 1, 8), _wo_piece(h0 + h, 8))
                yield
    return 18, gen()


def _b_out_tail(B, u):
    return functools.reduce(jnp.add, [
        lax.dot_general(B.ldb(_wo_piece(h, 9), 32), B.ldb(OT + 64 * h, 64), (((1,), (1,)), ((), ())),
                        preferred_element_type=F32)
        for h in range(8 * u, 8 * u + 8)])


def _b_step(B, u, extra):
    hs, hs_next = HS + 200 * u, HS + 200 * ((u + 1) % U)
    row = lax.broadcasted_iota(I32, (L, 128), 0)
    lane = lax.broadcasted_iota(I32, (L, 128), 1)
    lo = lane < 64
    lo64 = lax.broadcasted_iota(I32, (64, 128), 1) < 64
    col = lane & 63
    mask = (row < M) | (row >= col)
    in_a, in_b = lane < L, (lane >= 64) & (lane < 64 + L)
    z24 = jnp.zeros((24, 128), F32)
    z8 = jnp.zeros((8, 128), F32)

    def w(base, size, h):
        return PSTRIDE * (h // 2) + base + size * (h % 2)

    def tile(o0, o1):
        return pltpu.bitcast(jnp.concatenate([B.ldi(o0, 32), B.ldi(o1, 32)], 0), BF16)

    def h1():
        return jnp.concatenate([B.ldf(hs + 40 * n, 40) for n in range(4)], 1)

    def t_g():
        c4 = B.ldf(hs + 160, 40)
        g = jnp.concatenate([jnp.where(lo, 0.0, c4), z24, jnp.where(lo, c4, 0.0), z24], 0)
        B.stb(GS, g)
        B.stb(GT, g.T)

    def t_k(h):
        B.stf(RE + 40 * h, _dot(h1(), B.ldb(w(KA, 256, h), 256)))
        if h % 2:
            k = jnp.concatenate([B.ldf(RE + 40 * (h - 1), 40), z24, B.ldf(RE + 40 * h, 40), z24], 0)
            B.stb(KS + 64 * (h // 2), k.astype(BF16).T)

    def t_q(h):
        o = w(QA, 288, h)
        B.stf(QS + 40 * h, _dot(h1(), B.ldb(o, 256)) + _dot(B.ldf(hs + 160, 40)[:, :64], B.ldb(o + 256, 32)))

    def t_s(h):
        kt, w2 = B.ldi(KS + 64 * (h // 2), 64), B.ldi(K2 + 256 * (h // 2 % 8) + 128 * (h // 16), 64)
        rhs = jnp.where(lo64, w2, kt) if h % 2 else jnp.where(lo64, kt, w2)
        B.stf(RE + 40 * h, _dot(B.ldf(QS + 40 * h, 40), pltpu.bitcast(rhs, BF16)))

    def t_s2(j):
        a, b = B.ldf(RE + 80 * j, 40), B.ldf(RE + 80 * j + 40, 40)
        s = jnp.where(lo, a, b) + _dot(jnp.where(lo, b, a), B.ldb(GT, 64))
        s = jnp.where(mask, s * DH ** -0.5, NEG)
        B.stf(RS + 40 * j, s)
        ma = jnp.max(jnp.where(in_a, s, -jnp.inf), axis=1, keepdims=True)
        mb = jnp.max(jnp.where(in_b, s, -jnp.inf), axis=1, keepdims=True)
        e = jnp.exp(B.ldf(RS + 40 * j, 40) - jnp.where(lo, ma, mb))
        ea, eb = jnp.where(in_a, e, 0.0), jnp.where(in_b, e, 0.0)
        B.stf(PS + 40 * j, ea + eb)
        la = jnp.sum(ea, axis=1, keepdims=True)
        lb = jnp.sum(eb, axis=1, keepdims=True)
        B.stf(PS + 40 * j, B.ldf(PS + 40 * j, 40) / jnp.where(lo, la, lb))

    def t_r(j):
        B.stf(RS + 40 * j, _dot(B.ldf(PS + 40 * j, 40), B.ldb(GS, 64)))

    def t_v(h):
        v = _dot(h1(), B.ldb(w(VA, 256, h), 256))
        B.stb(w(PV, 96, h), jnp.concatenate([v, z8], 0))

    def t_pv(h):
        p, r = B.ldf(PS + 40 * (h // 2), 40), B.ldf(RS + 40 * (h // 2), 40)
        lhs = jnp.where(lo, r, p) if h % 2 else jnp.where(lo, p, r)
        o = _dot(lhs, B.ldb(w(PV, 64, h), 64))
        B.stf(OS + 40 * h, o)
        B.stb(OT + 64 * h + 16 * u, o[M:])

    d_s, d_s2, d_pv = 18, 16, 18
    big = [("k", h) for h in range(H)] + [("g",)] + [(p, h) for p in "qv" for h in range(H)]
    for i, (n, h) in enumerate((n, h) for ns in ((0, 1), (2, 3)) for h in range(H) for n in ns):
        big.append(("o", n, h))
        if i % 8 == 7:
            big.append(("m", i // 8))
    small = {"pv": t_pv, "r": t_r, "s2": t_s2, "s": t_s}
    nxt = dict.fromkeys(small, 0)
    done = {}
    now = 0

    def old(key, dist):
        return key in done and now - done[key] >= dist

    def ready(kind, i):
        if kind == "s":
            return old(("q", i), d_s)
        if kind == "s2":
            return old(("s", 2 * i + 1), d_s2)
        if kind == "r":
            return old(("s2", i), 64) and old(("v", 2 * i), 0)
        return old(("r", i // 2), d_s2) and old(("v", i), d_pv)

    acc, mem2 = {}, None
    for t in big:
        for kind, fn in small.items():
            if ready(kind, nxt[kind]):
                fn(nxt[kind])
                now += 1
                done[kind, nxt[kind]] = now
                nxt[kind] += 1
        if t in extra:
            extra[t]()
        if t[0] == "k":
            t_k(t[1])
            now += 4
        elif t[0] == "g":
            t_g()
        elif t[0] == "q":
            t_q(t[1])
            now += 5
        elif t[0] == "v":
            t_v(t[1])
            now += 4
        elif t[0] == "m":
            a, b = 2 * t[1], 2 * t[1] + 1
            y = _dot(jnp.concatenate([B.ldf(OS + 40 * a, M), B.ldf(OS + 40 * b, M)], 0),
                     tile(_wo_piece(a, 8), _wo_piece(b, 8)))
            mem2 = y if a == 0 else mem2 + y
        else:
            _, n, h = t
            assert ("pv", h) in done
            y = _dot(B.ldf(OS + 40 * h, 40), tile(_wo_piece(h, 2 * n), _wo_piece(h, 2 * n + 1)))
            acc[n] = y if h == 0 else acc[n] + y
            if h == H - 1:
                B.stf(hs_next + 40 * n, acc[n][:M])
                B.stf(BO + 128 * n + SEG * u, acc[n][M:])
            now += 1
        done[t] = now
    mem2 = jnp.where(lo[:M], mem2[:M], mem2[M:])
    B.stf(hs_next + 160, mem2 + pltpu.roll(mem2, 64, 1))
    y = _b_out_tail(B, u)
    if u == U - 1:
        B.stf(B2 + 64, B.ldf(B2, 64) + y)
    else:
        new = lax.broadcasted_iota(I32, (64, 128), 1) < SEG * (u + 1)
        B.stf(B2, jnp.where(new, y, 0.0) + (B.ldf(B2, 64) if u else 0.0))
        B.stf(B2 + 64, jnp.where(new, 0.0, y) + B.ldf(B2 + 64, 64))


def _kernel(xt_hbm, wqkv_hbm, wo_hbm, mem_hbm, gate_hbm, wq_hbm, wk_hbm, wv_hbm, wot_hbm,
            out_hbm,
            xt, wqkv, wo, mem_ref, gate_ref, raw, wot, a_ref, b_ref, qkv_all, o_all, o_last, ga_all, omg, out_buf,
            offs, sem_in, sem_w, sem_out):
    A, B = _Arena(a_ref), _Arena(b_ref)

    def cols(src, dst, c0, c1, sem):
        return pltpu.make_async_copy(src.at[:, pl.ds(c0, c1 - c0)], dst.at[:, pl.ds(c0, c1 - c0)], sem_in.at[sem])

    x_copy = [cols(xt_hbm, xt, c0, c1, i) for i, (c0, c1) in
              enumerate(((0, 256), (256, 768), (768, S)))]
    w_copy = [cols(wqkv_hbm, wqkv, c0, c1, 3 + i) for i, (c0, c1) in
              enumerate(((512, 896), (896, 1152), (0, 512), (1152, 3 * D)))]
    wo_copy = pltpu.make_async_copy(wo_hbm, wo, sem_in.at[8])
    mem_copy = pltpu.make_async_copy(mem_hbm, mem_ref, sem_in.at[9])
    gate_copy = pltpu.make_async_copy(gate_hbm, gate_ref, sem_in.at[10])

    def b_copies(i):
        r0, n = pl.multiple_of(i * 256 * H, 256 * H), 64 * H if isinstance(i, int) and i == 2 else 256 * H
        cps = [pltpu.make_async_copy(w.at[pl.ds(r0, n)], raw.at[pl.ds(RAW * m + r0, n)], sem_w.at[i])
               for m, w in enumerate((wq_hbm, wk_hbm, wv_hbm))]
        if n == 256 * H:
            rows = pl.ds(pl.multiple_of(i * 16 * D, 16 * D), 16 * D)
            cps.append(pltpu.make_async_copy(wot_hbm.at[rows], wot.at[rows], sem_w.at[i]))
        return cps

    def x_stage(j, slot):
        A.stb(AX + 288 * slot, xt[:, pl.ds(pl.multiple_of(j * 128, 128), 128)])

    def x_transpose(j, n):
        cols = pl.ds(pl.multiple_of(j * 128, 128), 128)
        if n < 4:
            t = xt[128 * n:128 * n + 128, cols]
        else:
            t = jnp.concatenate([xt[512:576, cols]] * 2, 0)
        B.stb(XN + 64 * n, t.T)

    def x_place(u):
        for n in range(5):
            B.stf(HS + 200 * u + 40 * n + M, B.ldb(XN + 64 * n + 16 * u, 16).astype(F32))

    def proj(j):
        if isinstance(j, int):
            return _Arena(qkv_all.at[pl.ds((j + 1) % 5 * SLOT, SLOT)])
        return _Arena(qkv_all.at[pl.ds(pl.multiple_of(offs[lax.rem(j + 1, 5)], 8), SLOT)])

    for c in (w_copy[0], gate_copy, mem_copy, w_copy[1], x_copy[0], w_copy[2], w_copy[3],
              wo_copy):
        c.start()

    for i in range(5):
        offs[i] = i * SLOT
    for i in range(2):
        offs[5 + i] = 256 * H * i
        offs[7 + i] = 512 * H + 32 * H * i
    for j in range(NP):
        B.stf(PSTRIDE * j + PV + 24, jnp.zeros((8, 128), F32))
        B.stf(PSTRIDE * j + PV + 120, jnp.zeros((8, 128), F32))
    B.stf(BO, jnp.zeros((B_ROWS - BO, 128), F32))
    w_copy[0].wait()
    gate_copy.wait()
    mem_copy.wait()
    gate = jnp.broadcast_to(gate_ref[...].astype(F32)[None, :], (8, D))
    mem0 = mem_ref[...].astype(F32)
    for k in range(4):
        A.stf(GW + 8 * k, gate[:, 128 * k:128 * k + 128])
        B.stf(HS + 40 * k, mem0[:, 128 * k:128 * k + 128])
    A.stf(GW + 32, jnp.concatenate([gate[:, 512:]] * 2, 1))
    B.stf(HS + 160, jnp.concatenate([mem0[:, 512:]] * 2, 1))

    def project(j, *parts):
        return _a_qkv(A, AX + 288 * j, proj(j), parts, first=j == 0)

    _a_transpose_w(A, wqkv, range(4, 7))
    w_copy[1].wait()
    _a_transpose_w(A, wqkv, range(7, 9))
    x_copy[0].wait()
    x_stage(0, 0)
    x_stage(1, 1)
    _interleave(project(0, 3, 1))
    for n in range(5):
        x_transpose(0, n)
    for u in range(U):
        x_place(u)
    w_copy[2].wait()
    x_copy[1].start()
    _a_transpose_w(A, wqkv, range(0, 4))
    _interleave(_chain(project(1, 3, 1), project(0, 0)))
    w_copy[3].wait()
    x_copy[2].start()
    _a_transpose_w(A, wqkv, range(9, 14))
    _interleave(_chain(project(1, 0), project(0, 2)))
    wo_copy.wait()
    for c in b_copies(2):
        c.start()
    _interleave(project(1, 2), _a_transpose_wo(A, wo))
    qkv_all[AK:AG, :] = jnp.broadcast_to(qkv_all[SLOT + AK:SLOT + AG, :1], (AG - AK, 128))

    def tick_raw(r):
        raw[D * H:RAW, :] = r[:16].astype(BF16)

    def tick_attend(r):
        qkv_all[TICK:TICK + 8, :] = pltpu.bitcast(r[:8], I32)

    def attend(j):
        return _a_attend(j, proj(j), proj(j - 1), o_all.at[j], omg)

    def project_out(j0, n, tick):
        return _chain(*[_a_out(A, o_all.at[j0 + b], ga_all.at[j0 + b], tick) for b in range(n)])

    def attend_trip(t, carry):
        @pl.when(t == 1)
        def _():
            x_copy[2].wait()
            for c in b_copies(1):
                c.start()

        def project(i):
            return _chain(_a_qkv(A, AX + 288 * i, proj(2 * t + 2 + i)),
                          _once(x_stage, jnp.minimum(2 * t + 4 + i, NB - 1), i))

        _interleave(_chain(project(0), project(1)), _chain(attend(2 * t), attend(2 * t + 1)), span=(-0.04, 0.87))

    x_copy[1].wait()
    for c in b_copies(0):
        c.start()
    x_stage(2, 0)
    x_stage(3, 1)
    lax.fori_loop(0, NB // 2 - 1, attend_trip, None)

    def last_trip(t, carry):
        src = raw.at[pl.ds(pl.multiple_of(offs[7 + t], 16), 2 * RAW + 32 * H)]
        dst = b_ref.at[pl.ds(pl.multiple_of(t * 16, 16), OA), :]
        _interleave(
            project_out(3 * t, 3, lambda r: (tick_attend(r), tick_raw(r))), _a_attend(NB - 2 + t, proj(NB - 2 + t), proj(NB - 3 + t), o_last.at[t], omg),
            _chain(*[_b_split_heads(src.at[pl.ds(RAW * m, 32 * H)], dst, even, odd) for m, (even, odd) in
                     enumerate(((QA + 256, QA + 544), (KR + 32, KR), (PV + 32, PV + 64)))]),
            span=(-0.08, 0.82))

    for c in b_copies(2):
        c.wait()
    lax.fori_loop(0, 2, last_trip, None)
    o_all[NB - 2:] = o_last[...]

    def prepare_trip(t, carry):
        for c in b_copies(t):
            c.wait()
        src = raw.at[pl.ds(pl.multiple_of(offs[5 + t], 16), 2 * RAW + 256 * H)]
        dst = b_ref.at[pl.ds(pl.multiple_of(t * 128, 128), HS), :]
        pairs = _Arena(b_ref.at[pl.ds(pl.multiple_of(t * 8 * PSTRIDE, 8), 8 * PSTRIDE), :])
        k2 = [pairs.ldb(PSTRIDE * j + KR, 64).T for j in range(8)]
        for j in range(8):
            _Arena(dst).stb(K2 + 256 * j, k2[j])
        split = [_b_split_heads(src.at[pl.ds(RAW * m, 256 * H)], dst, o, o + n)
                 for m, (o, n) in enumerate(((QA, 288), (KA, 256), (VA, 256)))]
        wo_t = [_b_transpose_wo(wot.at[pl.ds(pl.multiple_of(4 * D * (4 * t + c), 16), 4 * D)], dst, 4 * c) for c in range(4)]
        _interleave(project_out(6 + 5 * t, 5, tick_raw), _chain(*split), _chain(*wo_t), span=(-0.04, 0.93))

    lax.fori_loop(0, 2, prepare_trip, None)

    def mix(j, n):
        rows = min(128, D - 128 * n)
        bt = B.ldf(BO + 128 * n, 128).T if n < 4 else B.ldf(B2 + 64, 64)
        w = jnp.concatenate([omg[j]] * (rows // 8), 0)
        out_buf[j, 128 * n:128 * n + rows, :] = (
            ga_all[j, 128 * n:128 * n + rows, :] + w * bt).astype(BF16)

    def out_copy(j):
        return pltpu.make_async_copy(
            out_buf.at[j], out_hbm.at[:, pl.ds(pl.multiple_of(j * 128, 128), 128)], sem_out)

    def b_body(g, carry):
        jn, jp = jnp.minimum(g + 1, NB - 1), jnp.maximum(g - 1, 0)
        for u in range(U):
            extra = {("o", 3, 0): functools.partial(x_place, u)}
            if u == 0:
                for n in range(4):
                    extra["o", n, 16] = functools.partial(mix, jp, n)
                for n in range(5):
                    extra["o", 1, 6 * n] = functools.partial(x_transpose, jn, n)
            if u == U - 1:
                extra["v", 20] = functools.partial(mix, jp, 4)
            _b_step(B, u, extra)

        @pl.when(g > 0)
        def _():
            out_copy(jp).start()

        return carry

    lax.fori_loop(0, NB, b_body, 0)
    lane = lax.broadcasted_iota(I32, (64, 128), 1)
    B.stf(B2 + 64, functools.reduce(jnp.add, [B.ldf(B2 + 64, 64)] + [
        jnp.where(lane < SEG * (u + 1), 0.0, _b_out_tail(B, u)) for u in range(U - 1)]))
    for n in range(5):
        mix(NB - 1, n)
    out_copy(NB - 1).start()
    for j in range(NB):
        out_copy(j).wait()


@functools.partial(jax.jit, static_argnames=("B_seg_len",))
def pallas_gated_mix__sliding_local_dilated__memory_aug_recurrent_mem_tr__prompt_kernel(
    A_x: jax.Array,
    A_wqkv: jax.Array,
    A_wo: jax.Array,
    B_x: jax.Array,
    B_mem0: jax.Array,
    B_Wq: jax.Array,
    B_Wk: jax.Array,
    B_Wv: jax.Array,
    B_Wo: jax.Array,
    B_seg_len: int,
    gate_w: jax.Array,
):
    del B_x
    assert A_x.shape == (1, S, D) and B_mem0.shape == (1, M, D) and B_Wq.shape == (D, H, DH)
    assert B_seg_len == SEG
    hbm = pl.BlockSpec(memory_space=pl.ANY)
    out_t = pl.pallas_call(
        _kernel,
        out_shape=jax.ShapeDtypeStruct((D, S), BF16),
        in_specs=[hbm] * 9,
        out_specs=hbm,
        scratch_shapes=[
            pltpu.VMEM((D, S), BF16),
            pltpu.VMEM((D, 3 * D), BF16),
            pltpu.VMEM((D, D), BF16),
            pltpu.VMEM((M, D), BF16),
            pltpu.VMEM((D,), BF16),
            pltpu.VMEM((3 * RAW, DH), BF16),
            pltpu.VMEM((H * D, DH), BF16),
            pltpu.VMEM((A_ROWS, 128), I32),
            pltpu.VMEM((B_ROWS, 128), I32),
            pltpu.VMEM((5 * SLOT, 128), I32),
            pltpu.VMEM((NB, D // 2, 128), I32),
            pltpu.VMEM((2, D // 2, 128), I32),
            pltpu.VMEM((NB, D, 128), F32),
            pltpu.VMEM((NB, 8, 128), F32),
            pltpu.VMEM((NB, D, 128), BF16),
            pltpu.SMEM((9,), I32),
            pltpu.SemaphoreType.DMA((11,)),
            pltpu.SemaphoreType.DMA((3,)),
            pltpu.SemaphoreType.DMA,
        ],
        compiler_params=pltpu.CompilerParams(vmem_limit_bytes=100 * 1024 * 1024),
    )(
        A_x.reshape(S, D).T, A_wqkv, A_wo, B_mem0.reshape(M, D), gate_w,
        B_Wq.reshape(D * H, DH), B_Wk.reshape(D * H, DH), B_Wv.reshape(D * H, DH),
        B_Wo.transpose(0, 2, 1).reshape(H * D, DH),
    )
    return out_t.T.reshape(1, S, D)
```

```python
import functools

import jax
import jax.numpy as jnp
from jax import lax
import jax.experimental.pallas as pl
import jax.experimental.pallas.tpu as pltpu

F32, BF16, I32 = jnp.float32, jnp.bfloat16, jnp.int32

S, D = 2048, 576
NB = S // 128
HA, DA, WIN, DIL = 32, 18, 8, 2
H, DH, M, SEG = 32, 128, 8, 32
L = M + SEG
NP = H // 2
U = 128 // SEG
NEG = -1000000000.0

QA = 0
KA = QA + 576
KR = KA + 512
VA = KR + 64
PV = VA + 512
PSTRIDE = PV + 128 + 4
OA = NP * PSTRIDE
K2 = OA + H * 320
HS = K2 + 2048
GS = HS + U * 200
QS = GS + 64
KS = QS + H * 40
RE = KS + NP * 64
PS = RE + H * 40
RS = PS + NP * 40
OS = RS + NP * 40
XN = OS + H * 40
BO = XN + 320
B2 = BO + 512
OT = B2 + 128
B_ROWS = OT + H * 64

RAW = D * H + 16

WT = 0
GW = WT + 5 * 1728
WP = GW + 40
WOT = WP + 27 * 160
AX = WOT + 5 * 288
A_ROWS = AX + 2 * 288
AQ, AK, AV, AG, TICK, SLOT = 0, 576, 864, 1152, 1160, 1168


def _dot(a, b):
    return lax.dot_general(a, b, (((1,), (0,)), ((), ())), preferred_element_type=F32)


def _dot_nt(a, b):
    return lax.dot_general(a, b, (((1,), (1,)), ((), ())), preferred_element_type=F32)


class _Arena:
    def __init__(self, ref):
        self.r = ref

    def ldi(self, o, n):
        return self.r[o:o + n, :]

    def ldf(self, o, n):
        return pltpu.bitcast(self.r[o:o + n, :], F32)

    def ldb(self, o, n):
        return pltpu.bitcast(self.r[o:o + n, :], BF16)

    def stf(self, o, v):
        self.r[o:o + v.shape[0], :] = pltpu.bitcast(v, I32)

    def stb(self, o, v):
        self.r[o:o + v.shape[0] // 2, :] = pltpu.bitcast(v.astype(BF16), I32)


def _pad2(t, rows, cols):
    r, c = t.shape
    if c < cols:
        t = jnp.concatenate([t, jnp.zeros((r, cols - c), t.dtype)], 1)
    if r < rows:
        t = jnp.concatenate([t, jnp.zeros((rows - r, cols), t.dtype)], 0)
    return t


def _interleave(main, *side, span=(0.0, 0.9)):
    jobs = (main,) + side
    order = [((i + 1) / main[0], 0) for i in range(main[0])]
    order += [(span[0] + (span[1] - span[0]) * i / n, k + 1) for k, (n, _) in enumerate(side) for i in range(n)]
    for _, k in sorted(order):
        next(jobs[k][1])
    for _, gen in jobs:
        assert next(gen, "end") == "end"


def _once(fn, *args):
    def gen():
        fn(*args)
        yield
    return 1, gen()


def _chain(*jobs):
    def gen():
        for _, g in jobs:
            yield from g
    return sum(n for n, _ in jobs), gen()


def _a_transpose_w(A, w_ref, cblocks):
    for c in cblocks:
        nc = min(128, 3 * D - 128 * c)
        for k in range(5):
            nk = min(128, D - 128 * k)
            t = _pad2(w_ref[128 * k:128 * k + nk, 128 * c:128 * c + nc], 128, 128).T
            A.stf(WT + 1728 * k + 128 * c, t[:nc].astype(F32))


def _a_transpose_wo(A, w_ref):
    def gen():
        for c in range(5):
            nc = min(128, D - 128 * c)
            for k in range(5):
                nk = min(128, D - 128 * k)
                t = _pad2(w_ref[128 * k:128 * k + nk, 128 * c:128 * c + nc], 128, 128).T
                A.stb(WOT + 288 * k + 64 * c, t[:nc])
                yield
    return 25, gen()


def _a_qkv(A, x_off, dst, parts=(3, 1, 0, 2), first=False):
    def proj(rows_of_k):
        ch = [rows_of_k(k) for k in range(5)]
        return _dot(jnp.concatenate(ch[:4] + [ch[4][:, :64]], 1), A.ldb(x_off, 288))

    def gen():
        for part in parts:
            if part == 3:
                dst.stf(AG, jax.nn.sigmoid(proj(lambda k: A.ldf(GW + 8 * k, 8))))
                continue
            for d0 in range(0, DA, 2):
                def weights(k):
                    packed = WP + 160 * (9 * part + d0 // 2) + 32 * k
                    if not first:
                        return A.ldb(packed, 32)
                    w = jnp.concatenate([
                        pltpu.bitcast(A.r[pl.ds(WT + 1728 * k + D * part + 8 * DA * hg + d, 8, stride=DA), :], F32)
                        for hg in range(4) for d in (d0, d0 + 1)], 0)
                    A.stb(packed, w)
                    return w

                r = proj(weights)
                for i in range(0, 64, 16):
                    if part == 0:
                        dst.stf(AQ + 32 * d0 + i, r[i:i + 16])
                    else:
                        dst.stb((AK if part == 1 else AV) + 16 * d0 + i // 2, r[i:i + 16])
                    yield
    return sum(2 * DA for p in parts if p < 3), gen()


def _a_attend(j, cur, old, o_ref, omg_ref):
    def window(o):
        lane = lax.broadcasted_iota(I32, (8, 128), 1)
        c, p = cur.ldi(o, 8), old.ldi(o, 8)
        out = []
        for w in range(WIN):
            sh = DIL * w
            t = c if w == 0 else pltpu.roll(jnp.where(lane >= 128 - sh, p, c), sh, 1)
            out.append(pltpu.bitcast(t, BF16).astype(F32))
        return out

    def gen():
        pos = j * 128 + lax.broadcasted_iota(I32, (8, 128), 1)
        for hg in range(4):
            lg = None
            for d in range(0, DA, 2):
                q = cur.ldf(AQ + 32 * d + 16 * hg, 16)
                pr = [q * kw for kw in window(AK + 16 * d + 8 * hg)]
                pr = [t[:8] + t[8:] for t in pr]
                lg = pr if d == 0 else [a + b for a, b in zip(lg, pr)]
                yield
            lg = [jnp.where(pos >= DIL * w, t * DA ** -0.5, NEG) for w, t in enumerate(lg)]
            mx = functools.reduce(jnp.maximum, lg)
            e = [jnp.exp(t - mx) for t in lg]
            g = cur.ldf(AG, 8)
            if hg == 0:
                omg_ref[j] = 1.0 - g
            r = g / functools.reduce(jnp.add, e)
            p = [jnp.concatenate([t * r] * 2, 0) for t in e]
            yield
            for d in range(0, DA, 2):
                o = functools.reduce(jnp.add, [a * b for a, b in zip(p, window(AV + 16 * d + 8 * hg))])
                o = pltpu.bitcast(o.astype(BF16).astype(F32), I32)
                o_ref[pl.ds(4 * DA * hg + d // 2, 8, stride=DA // 2), :] = (
                    lax.shift_right_logical(o[:8], 16) | o[8:])
                yield
    return 4 * DA + 4, gen()


def _a_out(A, o_ref, ga_ref, tick):
    def gen():
        for r0 in range(0, D, 96):
            ch = [A.ldb(WOT + 288 * k + r0 // 2, 48) for k in range(5)]
            r = _dot(jnp.concatenate(ch[:4] + [ch[4][:, :64]], 1), pltpu.bitcast(o_ref[...], BF16))
            for i in range(0, 96, 32):
                tick(r[i:i + 32])
                ga_ref[r0 + i:r0 + i + 32, :] = r[i:i + 32]
                yield
    return D // 32, gen()


def _b_split_heads(raw, dst, even, odd):
    def gen():
        for r in range(raw.shape[0] // 64):
            e = pltpu.bitcast(raw[64 * r:64 * r + 32, :], I32)
            o = pltpu.bitcast(raw[64 * r + 32:64 * r + 64, :], I32)
            dst[pl.ds(even + r, NP, stride=PSTRIDE), :] = (e & 0xFFFF) | (o << 16)
            dst[pl.ds(odd + r, NP, stride=PSTRIDE), :] = lax.shift_right_logical(e, 16) | (o & -65536)
            yield
    return raw.shape[0] // 64, gen()


def _wo_piece(h, k):
    return OA + 256 * (10 * (h % 4) + k) + 32 * (h // 4)


def _b_transpose_wo(wot, dst, h0):
    def put(t, o0, o1):
        t = pltpu.bitcast(t, I32)
        dst[o0:o0 + 32, :] = t[:32]
        dst[o1:o1 + 32, :] = t[32:]

    def gen():
        for h in range(4):
            for n in range(4):
                put(wot[D * h + 128 * n:D * h + 128 * n + 128, :].T, _wo_piece(h0 + h, 2 * n), _wo_piece(h0 + h, 2 * n + 1))
                yield
            if h % 2:
                t = jnp.concatenate([wot[D * i + 512:D * i + D, :] for i in (h - 1, h)], 0)
                put(t, _wo_piece(h0 + h - 1, 9), _wo_piece(h0 + h, 9))
                put(t.T, _wo_piece(h0 + h - 1, 8), _wo_piece(h0 + h, 8))
                yield
    return 18, gen()


def _b_out_tail(B, u):
    return functools.reduce(jnp.add, [
        _dot_nt(B.ldb(_wo_piece(h, 9), 32), B.ldb(OT + 64 * h, 64)) for h in range(8 * u, 8 * u + 8)])


def _b_step(B, u, before_out, after_use):
    hs, hs_next = HS + 200 * u, HS + 200 * ((u + 1) % U)
    row = lax.broadcasted_iota(I32, (L, 128), 0)
    lane = lax.broadcasted_iota(I32, (L, 128), 1)
    lo = lane < 64
    lo64 = lax.broadcasted_iota(I32, (64, 128), 1) < 64
    col = lane & 63
    mask = (row < M) | (row >= col)
    in_a, in_b = lane < L, (lane >= 64) & (lane < 64 + L)
    z24 = jnp.zeros((24, 128), F32)
    z8 = jnp.zeros((8, 128), F32)

    def w(base, size, h):
        return PSTRIDE * (h // 2) + base + size * (h % 2)

    def tile(o0, o1):
        return pltpu.bitcast(jnp.concatenate([B.ldi(o0, 32), B.ldi(o1, 32)], 0), BF16)

    def h1():
        return jnp.concatenate([B.ldf(hs + 40 * n, 40) for n in range(4)], 1)

    def t_g():
        c4 = B.ldf(hs + 160, 40)
        g = jnp.concatenate([jnp.where(lo, 0.0, c4), z24, jnp.where(lo, c4, 0.0), z24], 0)
        B.stb(GS, g)

    def t_k(h):
        B.stf(OS + 40 * h, _dot(h1(), B.ldb(w(KA, 256, h), 256)))
        if h % 2:
            k = jnp.concatenate([B.ldf(OS + 40 * (h - 1), 40), z24, B.ldf(OS + 40 * h, 40), z24], 0)
            B.stb(KS + 64 * (h // 2), k.astype(BF16).T)

    def t_q(h):
        o = w(QA, 288, h)
        B.stf(QS + 40 * h, _dot(h1(), B.ldb(o, 256)) + _dot(B.ldf(hs + 160, 40)[:, :64], B.ldb(o + 256, 32)))

    def t_s(h):
        kt, w2 = B.ldi(KS + 64 * (h // 2), 64), B.ldi(K2 + 256 * (h // 2 % 8) + 128 * (h // 16), 64)
        rhs = jnp.where(lo64, w2, kt) if h % 2 else jnp.where(lo64, kt, w2)
        B.stf(RE + 40 * (NP * (h % 2) + h // 2), _dot(B.ldf(QS + 40 * h, 40), pltpu.bitcast(rhs, BF16)))

    def t_s2(i):
        c4 = B.ldf(hs + 160, 40)
        a, b = B.ldf(RE + 128 * i, 128), B.ldf(RE + 40 * NP + 128 * i, 128)
        t = jnp.where(lax.broadcasted_iota(I32, (128, 128), 1) < 64, b, a).astype(BF16)
        y = _dot_nt(jnp.concatenate([jnp.where(lo, 0.0, c4), jnp.where(lo, c4, 0.0)], 0), t)
        B.stf(RS + 128 * i, jnp.concatenate([y[:L], z24, y[L:], z24], 0).T)
        for j in range(128 * i // L, 128 * (i + 1) // L):
            softmax(j)

    def softmax(j):
        s = jnp.where(lo, B.ldf(RE + 40 * j, 40), B.ldf(RE + 40 * (NP + j), 40)) + B.ldf(RS + 40 * j, 40)
        s = jnp.where(mask, s * DH ** -0.5, NEG)
        B.stf(RS + 40 * j, s)
        ma = jnp.max(jnp.where(in_a, s, -jnp.inf), axis=1, keepdims=True)
        mb = jnp.max(jnp.where(in_b, s, -jnp.inf), axis=1, keepdims=True)
        e = jnp.exp(B.ldf(RS + 40 * j, 40) - jnp.where(lo, ma, mb))
        B.stf(PS + 40 * j, jnp.where(in_a | in_b, e, 0.0))

    def t_r(j):
        B.stf(RS + 40 * j, _dot(B.ldf(PS + 40 * j, 40), B.ldb(GS, 64)))

    def t_v(h):
        v = _dot(h1(), B.ldb(w(VA, 256, h), 256))
        B.stb(w(PV, 96, h), jnp.concatenate([v, z8], 0))

    def t_pv(h):
        p, r = B.ldf(PS + 40 * (h // 2), 40), B.ldf(RS + 40 * (h // 2), 40)
        lhs = jnp.where(lo, r, p) if h % 2 else jnp.where(lo, p, r)
        l = jnp.sum(jnp.where(in_b if h % 2 else in_a, lhs, 0.0), axis=1, keepdims=True)
        o = _dot(lhs, B.ldb(w(PV, 64, h), 64)) / l
        B.stf(OS + 40 * h, o)
        B.stb(OT + 64 * h + 16 * u, o[M:])

    acc = {}

    def t_o(n, h):
        y = _dot(B.ldf(OS + 40 * h, 40), tile(_wo_piece(h, 2 * n), _wo_piece(h, 2 * n + 1)))
        acc[n] = y if h == 0 else acc[n] + y
        if h == H - 1:
            B.stf(hs_next + 40 * n, acc[n][:M])
            B.stf(BO + 128 * n + SEG * u, acc[n][M:])

    def t_m(j):
        y = _dot(jnp.concatenate([B.ldf(OS + 80 * j, M), B.ldf(OS + 80 * j + 40, M)], 0),
                 tile(_wo_piece(2 * j, 8), _wo_piece(2 * j + 1, 8)))
        acc[4] = y if j == 0 else acc[4] + y

    lag_s, lag_s2, lag_o, v_late = 4, 6, 4, 4
    for h in range(H):
        t_k(h)
    t_g()
    s2_after = [(128 * i + 127) // L * 2 + 1 + lag_s + lag_s2 for i in range(5)]
    for i in range(2 * H - v_late):
        t_q(i) if i < H else t_v(i - H)
        if 0 <= i - lag_s < H:
            t_s(i - lag_s)
        if i in s2_after:
            t_s2(s2_after.index(i))
        if i >= 2 * H - v_late - NP:
            t_r(i - (2 * H - v_late - NP))
    before_out()
    for i in range(NP + lag_o):
        if i < NP:
            t_pv(2 * i)
            t_pv(2 * i + 1)
        if i < lag_o:
            for h in range(v_late * i // lag_o, v_late * (i + 1) // lag_o):
                t_v(H - v_late + h)
        else:
            j = i - lag_o
            for h in (2 * j, 2 * j + 1):
                t_o(0, h)
                t_o(1, h)
            if j % 2:
                t_m(j // 2)
    after_use()
    for h in range(H):
        t_o(2, h)
        t_o(3, h)
        if h % 4 == 3:
            t_m(8 + h // 4)
    mem2 = acc[4]
    mem2 = jnp.where(lo[:M], mem2[:M], mem2[M:])
    B.stf(hs_next + 160, mem2 + pltpu.roll(mem2, 64, 1))
    y = _b_out_tail(B, u)
    if u == U - 1:
        B.stf(B2 + 64, B.ldf(B2, 64) + y)
    else:
        new = lax.broadcasted_iota(I32, (64, 128), 1) < SEG * (u + 1)
        B.stf(B2, jnp.where(new, y, 0.0) + (B.ldf(B2, 64) if u else 0.0))
        B.stf(B2 + 64, jnp.where(new, 0.0, y) + B.ldf(B2 + 64, 64))


def _kernel(xt_hbm, wqkv_hbm, wo_hbm, mem_hbm, gate_hbm, wq_hbm, wk_hbm, wv_hbm, wot_hbm,
            out_hbm,
            xt, wqkv, wo, mem_ref, gate_ref, raw, wot, a_ref, b_ref, qkv_all, o_all, o_last, ga_all, omg, out_buf,
            offs, sem_in, sem_w, sem_out):
    A, B = _Arena(a_ref), _Arena(b_ref)

    def cols(src, dst, c0, c1, sem):
        return pltpu.make_async_copy(src.at[:, pl.ds(c0, c1 - c0)], dst.at[:, pl.ds(c0, c1 - c0)], sem_in.at[sem])

    x_copy = [cols(xt_hbm, xt, c0, c1, i) for i, (c0, c1) in
              enumerate(((0, 256), (256, 768), (768, S)))]
    w_copy = [cols(wqkv_hbm, wqkv, c0, c1, 3 + i) for i, (c0, c1) in
              enumerate(((512, 896), (896, 1152), (0, 512), (1152, 3 * D)))]
    wo_copy = pltpu.make_async_copy(wo_hbm, wo, sem_in.at[8])
    mem_copy = pltpu.make_async_copy(mem_hbm, mem_ref, sem_in.at[9])
    gate_copy = pltpu.make_async_copy(gate_hbm, gate_ref, sem_in.at[10])

    def b_copies(i):
        r0, n = pl.multiple_of(i * 256 * H, 256 * H), 64 * H if isinstance(i, int) and i == 2 else 256 * H
        cps = [pltpu.make_async_copy(w.at[pl.ds(r0, n)], raw.at[pl.ds(RAW * m + r0, n)], sem_w.at[i])
               for m, w in enumerate((wq_hbm, wk_hbm, wv_hbm))]
        if n == 256 * H:
            rows = pl.ds(pl.multiple_of(i * 16 * D, 16 * D), 16 * D)
            cps.append(pltpu.make_async_copy(wot_hbm.at[rows], wot.at[rows], sem_w.at[i]))
        return cps

    def x_stage(j, slot):
        A.stb(AX + 288 * slot, xt[:, pl.ds(pl.multiple_of(j * 128, 128), 128)])

    def x_transpose(j, n):
        cols = pl.ds(pl.multiple_of(j * 128, 128), 128)
        if n < 4:
            t = xt[128 * n:128 * n + 128, cols]
        else:
            t = jnp.concatenate([xt[512:576, cols]] * 2, 0)
        B.stb(XN + 64 * n, t.T)

    def x_place(u):
        for n in range(5):
            B.stf(HS + 200 * u + 40 * n + M, B.ldb(XN + 64 * n + 16 * u, 16).astype(F32))

    def proj(j):
        if isinstance(j, int):
            return _Arena(qkv_all.at[pl.ds((j + 1) % 5 * SLOT, SLOT)])
        return _Arena(qkv_all.at[pl.ds(pl.multiple_of(offs[lax.rem(j + 1, 5)], 8), SLOT)])

    for c in (w_copy[0], gate_copy, mem_copy, w_copy[1], x_copy[0], w_copy[2], w_copy[3],
              wo_copy):
        c.start()

    for i in range(5):
        offs[i] = i * SLOT
    for i in range(2):
        offs[5 + i] = 256 * H * i
        offs[7 + i] = 512 * H + 32 * H * i
    for j in range(NP):
        B.stf(PSTRIDE * j + PV + 24, jnp.zeros((8, 128), F32))
        B.stf(PSTRIDE * j + PV + 120, jnp.zeros((8, 128), F32))
    B.stf(BO, jnp.zeros((B_ROWS - BO, 128), F32))
    w_copy[0].wait()
    gate_copy.wait()
    mem_copy.wait()
    gate = jnp.broadcast_to(gate_ref[...].astype(F32)[None, :], (8, D))
    mem0 = mem_ref[...].astype(F32)
    for k in range(4):
        A.stf(GW + 8 * k, gate[:, 128 * k:128 * k + 128])
        B.stf(HS + 40 * k, mem0[:, 128 * k:128 * k + 128])
    A.stf(GW + 32, jnp.concatenate([gate[:, 512:]] * 2, 1))
    B.stf(HS + 160, jnp.concatenate([mem0[:, 512:]] * 2, 1))

    def project(j, *parts):
        return _a_qkv(A, AX + 288 * j, proj(j), parts, first=j == 0)

    _a_transpose_w(A, wqkv, range(4, 7))
    w_copy[1].wait()
    _a_transpose_w(A, wqkv, range(7, 9))
    x_copy[0].wait()
    x_stage(0, 0)
    x_stage(1, 1)
    _interleave(project(0, 3, 1))
    for n in range(5):
        x_transpose(0, n)
    for u in range(U):
        x_place(u)
    w_copy[2].wait()
    x_copy[1].start()
    _a_transpose_w(A, wqkv, range(0, 4))
    _interleave(_chain(project(1, 3, 1), project(0, 0)))
    w_copy[3].wait()
    x_copy[2].start()
    _a_transpose_w(A, wqkv, range(9, 14))
    _interleave(_chain(project(1, 0), project(0, 2)))
    wo_copy.wait()
    for c in b_copies(2):
        c.start()
    _interleave(project(1, 2), _a_transpose_wo(A, wo))
    qkv_all[AK:AG, :] = jnp.broadcast_to(qkv_all[SLOT + AK:SLOT + AG, :1], (AG - AK, 128))

    def tick_raw(r):
        raw[D * H:RAW, :] = r[:16].astype(BF16)

    def tick_attend(r):
        qkv_all[TICK:TICK + 8, :] = pltpu.bitcast(r[:8], I32)

    def attend(j):
        return _a_attend(j, proj(j), proj(j - 1), o_all.at[j], omg)

    def project_out(j0, n, tick):
        return _chain(*[_a_out(A, o_all.at[j0 + b], ga_all.at[j0 + b], tick) for b in range(n)])

    def attend_trip(t, carry):
        @pl.when(t == 1)
        def _():
            x_copy[2].wait()
            for c in b_copies(1):
                c.start()

        def project(i):
            return _chain(_a_qkv(A, AX + 288 * i, proj(2 * t + 2 + i)),
                          _once(x_stage, jnp.minimum(2 * t + 4 + i, NB - 1), i))

        _interleave(_chain(project(0), project(1)), _chain(attend(2 * t), attend(2 * t + 1)), span=(-0.04, 0.87))

    x_copy[1].wait()
    for c in b_copies(0):
        c.start()
    x_stage(2, 0)
    x_stage(3, 1)
    lax.fori_loop(0, NB // 2 - 1, attend_trip, None)

    def last_trip(t, carry):
        src = raw.at[pl.ds(pl.multiple_of(offs[7 + t], 16), 2 * RAW + 32 * H)]
        dst = b_ref.at[pl.ds(pl.multiple_of(t * 16, 16), OA), :]
        _interleave(
            project_out(3 * t, 3, lambda r: (tick_attend(r), tick_raw(r))), _a_attend(NB - 2 + t, proj(NB - 2 + t), proj(NB - 3 + t), o_last.at[t], omg),
            _chain(*[_b_split_heads(src.at[pl.ds(RAW * m, 32 * H)], dst, even, odd) for m, (even, odd) in
                     enumerate(((QA + 256, QA + 544), (KR + 32, KR), (PV + 32, PV + 64)))]),
            span=(-0.08, 0.82))

    for c in b_copies(2):
        c.wait()
    lax.fori_loop(0, 2, last_trip, None)
    o_all[NB - 2:] = o_last[...]

    def prepare_trip(t, carry):
        for c in b_copies(t):
            c.wait()
        src = raw.at[pl.ds(pl.multiple_of(offs[5 + t], 16), 2 * RAW + 256 * H)]
        dst = b_ref.at[pl.ds(pl.multiple_of(t * 128, 128), HS), :]
        pairs = _Arena(b_ref.at[pl.ds(pl.multiple_of(t * 8 * PSTRIDE, 8), 8 * PSTRIDE), :])
        k2 = [pairs.ldb(PSTRIDE * j + KR, 64).T for j in range(8)]
        for j in range(8):
            _Arena(dst).stb(K2 + 256 * j, k2[j])
        split = [_b_split_heads(src.at[pl.ds(RAW * m, 256 * H)], dst, o, o + n)
                 for m, (o, n) in enumerate(((QA, 288), (KA, 256), (VA, 256)))]
        wo_t = [_b_transpose_wo(wot.at[pl.ds(pl.multiple_of(4 * D * (4 * t + c), 16), 4 * D)], dst, 4 * c) for c in range(4)]
        _interleave(project_out(6 + 5 * t, 5, tick_raw), _chain(*split), _chain(*wo_t), span=(-0.04, 0.93))

    lax.fori_loop(0, 2, prepare_trip, None)

    def mix(j, n):
        rows = min(128, D - 128 * n)
        bt = B.ldf(BO + 128 * n, 128).T if n < 4 else B.ldf(B2 + 64, 64)
        w = jnp.concatenate([omg[j]] * (rows // 8), 0)
        out_buf[j, 128 * n:128 * n + rows, :] = (
            ga_all[j, 128 * n:128 * n + rows, :] + w * bt).astype(BF16)

    def out_copy(j):
        return pltpu.make_async_copy(
            out_buf.at[j], out_hbm.at[:, pl.ds(pl.multiple_of(j * 128, 128), 128)], sem_out)

    def b_body(g, carry):
        jn, jp = jnp.minimum(g + 1, NB - 1), jnp.maximum(g - 1, 0)
        for u in range(U):
            def before_out():
                for n in {0: range(4), U - 1: (4,)}.get(u, ()):
                    mix(jp, n)

            def after_use():
                if u == 0:
                    for n in range(5):
                        x_transpose(jn, n)
                x_place(u)

            _b_step(B, u, before_out, after_use)

        @pl.when(g > 0)
        def _():
            out_copy(jp).start()

        return carry

    lax.fori_loop(0, NB, b_body, 0)
    lane = lax.broadcasted_iota(I32, (64, 128), 1)
    B.stf(B2 + 64, functools.reduce(jnp.add, [B.ldf(B2 + 64, 64)] + [
        jnp.where(lane < SEG * (u + 1), 0.0, _b_out_tail(B, u)) for u in range(U - 1)]))
    for n in range(5):
        mix(NB - 1, n)
    out_copy(NB - 1).start()
    for j in range(NB):
        out_copy(j).wait()


@functools.partial(jax.jit, static_argnames=("B_seg_len",))
def pallas_gated_mix__sliding_local_dilated__memory_aug_recurrent_mem_tr__prompt_kernel(
    A_x: jax.Array,
    A_wqkv: jax.Array,
    A_wo: jax.Array,
    B_x: jax.Array,
    B_mem0: jax.Array,
    B_Wq: jax.Array,
    B_Wk: jax.Array,
    B_Wv: jax.Array,
    B_Wo: jax.Array,
    B_seg_len: int,
    gate_w: jax.Array,
):
    del B_x
    assert A_x.shape == (1, S, D) and B_mem0.shape == (1, M, D) and B_Wq.shape == (D, H, DH)
    assert B_seg_len == SEG
    hbm = pl.BlockSpec(memory_space=pl.ANY)
    out_t = pl.pallas_call(
        _kernel,
        out_shape=jax.ShapeDtypeStruct((D, S), BF16),
        in_specs=[hbm] * 9,
        out_specs=hbm,
        scratch_shapes=[
            pltpu.VMEM((D, S), BF16),
            pltpu.VMEM((D, 3 * D), BF16),
            pltpu.VMEM((D, D), BF16),
            pltpu.VMEM((M, D), BF16),
            pltpu.VMEM((D,), BF16),
            pltpu.VMEM((3 * RAW, DH), BF16),
            pltpu.VMEM((H * D, DH), BF16),
            pltpu.VMEM((A_ROWS, 128), I32),
            pltpu.VMEM((B_ROWS, 128), I32),
            pltpu.VMEM((5 * SLOT, 128), I32),
            pltpu.VMEM((NB, D // 2, 128), I32),
            pltpu.VMEM((2, D // 2, 128), I32),
            pltpu.VMEM((NB, D, 128), F32),
            pltpu.VMEM((NB, 8, 128), F32),
            pltpu.VMEM((NB, D, 128), BF16),
            pltpu.SMEM((9,), I32),
            pltpu.SemaphoreType.DMA((11,)),
            pltpu.SemaphoreType.DMA((3,)),
            pltpu.SemaphoreType.DMA,
        ],
        compiler_params=pltpu.CompilerParams(vmem_limit_bytes=100 * 1024 * 1024),
    )(
        A_x.reshape(S, D).T, A_wqkv, A_wo, B_mem0.reshape(M, D), gate_w,
        B_Wq.reshape(D * H, DH), B_Wk.reshape(D * H, DH), B_Wv.reshape(D * H, DH),
        B_Wo.transpose(0, 2, 1).reshape(H * D, DH),
    )
    return out_t.T.reshape(1, S, D)
```

```python
import functools

import jax
import jax.numpy as jnp
from jax import lax
import jax.experimental.pallas as pl
import jax.experimental.pallas.tpu as pltpu

F32, BF16, I32 = jnp.float32, jnp.bfloat16, jnp.int32

S, D = 2048, 576
NB = S // 128
HA, DA, WIN, DIL = 32, 18, 8, 2
H, DH, M, SEG = 32, 128, 8, 32
L = M + SEG
NP = H // 2
U = 128 // SEG
NEG = -1000000000.0

NG = 2
PRODUCTS = (
    ({(0, 0): 1}, {(0, 1): 1, (1, 1): -1}, {(0, 1): 1, (1, 1): 1}),
    ({(1, 1): 1}, {(1, 0): 1, (0, 0): -1}, {(0, 0): 1, (1, 0): 1}),
    ({(0, 0): 1, (0, 1): 1}, {(1, 1): 1}, {(0, 0): -1, (0, 1): 1}),
    ({(1, 0): 1, (1, 1): 1}, {(0, 0): 1}, {(1, 0): 1, (1, 1): -1}),
    ({(0, 0): 1, (1, 1): 1}, {(0, 0): 1, (1, 1): 1}, {(0, 0): 1, (1, 1): 1}),
    ({(0, 1): 1, (1, 1): -1}, {(1, 0): 1, (1, 1): 1}, {(0, 0): 1}),
    ({(1, 0): 1, (0, 0): -1}, {(0, 0): 1, (0, 1): 1}, {(1, 1): 1}),
)
NPR = len(PRODUCTS)
NC = 4 // NG
TURN = tuple(tuple(p for p, (a, _, c) in enumerate(PRODUCTS)
                   if any(k[0] == r for k in a) and any(k[0] == r for k in c)) for r in range(2))

GSTRIDE = 3 * NPR * NC * 64 + 4
TAIL = H // NG * GSTRIDE
Q2 = TAIL
K2 = Q2 + 64
PV = K2 + 64
PSTRIDE = 256 + 4
OA = TAIL + NP * PSTRIDE
O2 = OA + H // NG * NPR * NC * 64
O2T = O2 + NP * 64
LH = O2T + H * 32
GS = LH + U * (NG * NG * NC + 2) * 40
TK = GS + 64
MK = TK + 3 * H * 128
KS = MK + 3 * H * M
RE = KS + NP * 64
PS = RE + H * 40
RS = PS + NP * 40
XN = RS + NP * 40
OM = XN + 320
OF = OM + H * M
BO = OF + U * H * SEG
B2 = BO + 512
OT = B2 + 128
B_ROWS = OT + H * 64

RAW = D * H + 16

WT = 0
GW = WT + 5 * 1728
WP = GW + 40
WOT = WP + 27 * 160
AX = WOT + 5 * 288
A_ROWS = AX + 2 * 288
AQ, AK, AV, AG, TICK, SLOT = 0, 576, 864, 1152, 1160, 1168


def _dot(a, b):
    return lax.dot_general(a, b, (((1,), (0,)), ((), ())), preferred_element_type=F32)


def _dot_nt(a, b):
    return lax.dot_general(a, b, (((1,), (1,)), ((), ())), preferred_element_type=F32)


class _Arena:
    def __init__(self, ref):
        self.r = ref

    def ldi(self, o, n):
        return self.r[o:o + n, :]

    def ldf(self, o, n):
        return pltpu.bitcast(self.r[o:o + n, :], F32)

    def ldb(self, o, n):
        return pltpu.bitcast(self.r[o:o + n, :], BF16)

    def stf(self, o, v):
        self.r[o:o + v.shape[0], :] = pltpu.bitcast(v, I32)

    def stb(self, o, v):
        self.r[o:o + v.shape[0] // 2, :] = pltpu.bitcast(v.astype(BF16), I32)


def _pad2(t, rows, cols):
    r, c = t.shape
    if c < cols:
        t = jnp.concatenate([t, jnp.zeros((r, cols - c), t.dtype)], 1)
    if r < rows:
        t = jnp.concatenate([t, jnp.zeros((rows - r, cols), t.dtype)], 0)
    return t


def _interleave(main, *side, span=(0.0, 0.9)):
    jobs = (main,) + side
    order = [((i + 1) / main[0], 0) for i in range(main[0])]
    order += [(span[0] + (span[1] - span[0]) * i / n, k + 1) for k, (n, _) in enumerate(side) for i in range(n)]
    for _, k in sorted(order):
        next(jobs[k][1])
    for _, gen in jobs:
        assert next(gen, "end") == "end"


def _once(fn, *args):
    def gen():
        fn(*args)
        yield
    return 1, gen()


def _chain(*jobs):
    def gen():
        for _, g in jobs:
            yield from g
    return sum(n for n, _ in jobs), gen()


def _a_transpose_w(A, w_ref, cblocks):
    for c in cblocks:
        nc = min(128, 3 * D - 128 * c)
        for k in range(5):
            nk = min(128, D - 128 * k)
            t = _pad2(w_ref[128 * k:128 * k + nk, 128 * c:128 * c + nc], 128, 128).T
            A.stf(WT + 1728 * k + 128 * c, t[:nc].astype(F32))


def _a_transpose_wo(A, w_ref):
    def gen():
        for c in range(5):
            nc = min(128, D - 128 * c)
            for k in range(5):
                nk = min(128, D - 128 * k)
                t = _pad2(w_ref[128 * k:128 * k + nk, 128 * c:128 * c + nc], 128, 128).T
                A.stb(WOT + 288 * k + 64 * c, t[:nc])
                yield
    return 25, gen()


def _a_qkv(A, x_off, dst, parts=(3, 1, 0, 2), first=False):
    def proj(rows_of_k):
        ch = [rows_of_k(k) for k in range(5)]
        return _dot(jnp.concatenate(ch[:4] + [ch[4][:, :64]], 1), A.ldb(x_off, 288))

    def gen():
        for part in parts:
            if part == 3:
                dst.stf(AG, jax.nn.sigmoid(proj(lambda k: A.ldf(GW + 8 * k, 8))))
                continue
            for d0 in range(0, DA, 2):
                def weights(k):
                    packed = WP + 160 * (9 * part + d0 // 2) + 32 * k
                    if not first:
                        return A.ldb(packed, 32)
                    w = jnp.concatenate([
                        pltpu.bitcast(A.r[pl.ds(WT + 1728 * k + D * part + 8 * DA * hg + d, 8, stride=DA), :], F32)
                        for hg in range(4) for d in (d0, d0 + 1)], 0)
                    A.stb(packed, w)
                    return w

                r = proj(weights)
                for i in range(0, 64, 16):
                    if part == 0:
                        dst.stf(AQ + 32 * d0 + i, r[i:i + 16])
                    else:
                        dst.stb((AK if part == 1 else AV) + 16 * d0 + i // 2, r[i:i + 16])
                    yield
    return sum(2 * DA for p in parts if p < 3), gen()


def _a_attend(j, cur, old, o_ref, omg_ref):
    def window(o):
        lane = lax.broadcasted_iota(I32, (8, 128), 1)
        c, p = cur.ldi(o, 8), old.ldi(o, 8)
        out = []
        for w in range(WIN):
            sh = DIL * w
            t = c if w == 0 else pltpu.roll(jnp.where(lane >= 128 - sh, p, c), sh, 1)
            out.append(pltpu.bitcast(t, BF16).astype(F32))
        return out

    def gen():
        pos = j * 128 + lax.broadcasted_iota(I32, (8, 128), 1)
        for hg in range(4):
            lg = None
            for d in range(0, DA, 2):
                q = cur.ldf(AQ + 32 * d + 16 * hg, 16)
                pr = [q * kw for kw in window(AK + 16 * d + 8 * hg)]
                pr = [t[:8] + t[8:] for t in pr]
                lg = pr if d == 0 else [a + b for a, b in zip(lg, pr)]
                yield
            lg = [jnp.where(pos >= DIL * w, t * DA ** -0.5, NEG) for w, t in enumerate(lg)]
            mx = functools.reduce(jnp.maximum, lg)
            e = [jnp.exp(t - mx) for t in lg]
            g = cur.ldf(AG, 8)
            if hg == 0:
                omg_ref[j] = 1.0 - g
            r = g / functools.reduce(jnp.add, e)
            p = [jnp.concatenate([t * r] * 2, 0) for t in e]
            yield
            for d in range(0, DA, 2):
                o = functools.reduce(jnp.add, [a * b for a, b in zip(p, window(AV + 16 * d + 8 * hg))])
                o = pltpu.bitcast(o.astype(BF16).astype(F32), I32)
                o_ref[pl.ds(4 * DA * hg + d // 2, 8, stride=DA // 2), :] = (
                    lax.shift_right_logical(o[:8], 16) | o[8:])
                yield
    return 4 * DA + 4, gen()


def _a_out(A, o_ref, ga_ref, tick):
    def gen():
        for r0 in range(0, D, 96):
            ch = [A.ldb(WOT + 288 * k + r0 // 2, 48) for k in range(5)]
            r = _dot(jnp.concatenate(ch[:4] + [ch[4][:, :64]], 1), pltpu.bitcast(o_ref[...], BF16))
            for i in range(0, 96, 32):
                tick(r[i:i + 32])
                ga_ref[r0 + i:r0 + i + 32, :] = r[i:i + 32]
                yield
    return D // 32, gen()


def _b_split_heads(raw, dst, even, odd):
    def gen():
        for r in range(raw.shape[0] // 64):
            e = pltpu.bitcast(raw[64 * r:64 * r + 32, :], I32)
            o = pltpu.bitcast(raw[64 * r + 32:64 * r + 64, :], I32)
            dst[pl.ds(even + r, NP, stride=PSTRIDE), :] = (e & 0xFFFF) | (o << 16)
            dst[pl.ds(odd + r, NP, stride=PSTRIDE), :] = lax.shift_right_logical(e, 16) | (o & -65536)
            yield
    return raw.shape[0] // 64, gen()


def _signed_sum(terms):
    terms = sorted(terms, key=lambda t: -t[0])
    acc = terms[0][1] if terms[0][0] > 0 else -terms[0][1]
    for c, t in terms[1:]:
        acc = acc + t if c > 0 else acc - t
    return acc


def _pairs(g):
    return [g + 8 * i for i in range(NG // 2)]


def _heads(g):
    return [2 * j + i for j in _pairs(g) for i in range(2)]


def _b_product_tiles(raw, dst, off, rows):
    def gen():
        for r in range(rows):
            word = [[pltpu.bitcast(raw[o:o + 32, :], I32) for o in (o0, o0 + 32)]
                    for o0 in range(64 * r, 512 * H, 512 * H // NG)]

            def block(k, n, i):
                t = word[k][i][8 * (n // 2):8 * (n // 2) + H // NG]
                return pltpu.bitcast(t & -65536 if n % 2 else t << 16, F32)

            for p, (_, w, _) in enumerate(PRODUCTS):
                e, o = [pltpu.bitcast(_signed_sum([(c, block(k, n, i)) for (k, n), c in w.items()]), I32)
                        for i in range(2)]
                if len(w) > 1:
                    e, o = e + 0x8000, (o + 0x7FFF) & -65536
                dst[pl.ds(off + p * NC * 64 + r, H // NG, stride=GSTRIDE), :] = lax.shift_right_logical(e, 16) | o
            yield
    return rows, gen()


def _b_transpose_wo(B, wot):
    def gen():
        for g in range(H // NG):
            for p, (_, w, _) in enumerate(PRODUCTS):
                for i in range(NC):
                    t = [(c, wot[pl.ds(D * _heads(g)[k] + 128 * (NC * n + i), 128), :]) for (k, n), c in w.items()]
                    if len(t) > 1 or t[0][0] < 0:
                        t = [(1, _signed_sum([(c, v.astype(F32)) for c, v in t]).astype(BF16))]
                    B.stb(OA + ((g * NPR + p) * NC + i) * 64, t[0][1].T)
                    yield
            for j in _pairs(g):
                t = jnp.concatenate([wot[D * h + 512:D * h + D, :] for h in (2 * j, 2 * j + 1)], 0)
                B.stb(O2T + 64 * j, t)
                B.stb(O2 + 64 * j, t.T)
                B.stb(K2 + PSTRIDE * j, B.ldb(K2 + PSTRIDE * j, 64).T)
    return H // NG * NPR * NC, gen()


def _turn(u):
    return 1 - u % 2


def _halves(p, r):
    return (r,) if p in TURN[1 - r] else (0, 1)


def _lh(u, i):
    return LH + 40 * ((NG * NG * NC + 2) * (u % U) + i)


def _b_place_memory(B, u, mem):
    r = _turn(u)
    for i, p in enumerate(TURN[r]):
        for c in range(NC):
            B.stf(_lh(u, 2 + NC * i + c), _signed_sum(
                [(s, mem[NC * k + c]) for (rr, k), s in PRODUCTS[p][0].items() if rr == r]))


def _b_place_tokens(B, u):
    r = _turn(u)
    top = (u + 1 - r) % U

    def x(seg, n, half):
        return B.ldb(XN + 64 * n + 16 * seg + 8 * half, 8).astype(F32)

    for i, p in enumerate(TURN[r]):
        for c in range(NC):
            for at, half in enumerate(_halves(p, r)):
                B.stf(_lh(u, 2 + NC * i + c) + M + 16 * at, _signed_sum(
                    [(s, x(top + rr, NC * k + c, half)) for (rr, k), s in PRODUCTS[p][0].items()]))
    for half in range(2):
        B.stf(_lh(u, 1) + M + 16 * half, x((u + 1) % U, 4, half))


def _b_collect(B, r, ys, m, at, plain=None):
    mem, tok = {}, {}
    items = [(PRODUCTS[p][2], _halves(p, r), y) for p, y in zip(TURN[r], ys)]
    if plain:
        items += [({(r, n): 1}, (0, 1), y) for n, y in enumerate(plain)]
    for c, halves, y in items:
        for (rr, n), s in c.items():
            if m and rr == r:
                mem.setdefault(n, []).append((s, y[:m]))
            for i, half in enumerate(halves):
                tok.setdefault((rr, n, half), []).append((s, y[m + 16 * i:m + 16 * i + 16]))
    for (rr, n, half), terms in sorted(tok.items()):
        o = at(rr, n) + 16 * half
        if r == 1 and any((rr, n) in PRODUCTS[p][2] and half in _halves(p, 0) for p in TURN[0]):
            terms.append((1, B.ldf(o, 16)))
        B.stf(o, _signed_sum(terms))
    return [_signed_sum(mem[n]) for n in sorted(mem)]


def _b_project(B, u, mat, g, m=M):
    r = _turn(u)
    top = (u + 1 - r) % U
    ys = [_dot(jnp.concatenate([B.ldf(_lh(u, 2 + NC * i + c) + M - m, m + 16 * len(_halves(p, r)))
                                for c in range(NC)], 1),
               B.ldb(GSTRIDE * g + (mat * NPR + p) * NC * 64, NC * 64)) for i, p in enumerate(TURN[r])]
    plain = None
    if mat == 0:
        plain = [_dot(B.ldf(_lh(u, 1) + M - m, m + SEG)[:, :64], B.ldb(Q2 + PSTRIDE * (h // 2) + 32 * (h % 2), 32))
                 for h in _heads(g)]
    mem = _b_collect(B, r, ys, m, lambda rr, n: TK + 128 * (H * mat + _heads(g)[n]) + SEG * (top + rr), plain)
    for h, t in zip(_heads(g), mem):
        B.stf(MK + M * (H * mat + h), t)


def _b_out_product(B, u, p, g, acc, m=M):
    r = _turn(u)
    top = (u - 1 - r) % U
    a = PRODUCTS[p][0].items()
    lhs = [_signed_sum([(s, B.ldf(OM + M * _heads(g)[k], M)) for (rr, k), s in a if rr == r])] if m else []
    lhs += [_signed_sum([(s, B.ldf(OF + SEG * (H * (top + rr) + _heads(g)[k]) + 16 * half, 16)) for (rr, k), s in a])
            for half in _halves(p, r)]
    for c in range(NC):
        y = _dot(jnp.concatenate(lhs, 0), B.ldb(OA + ((g * NPR + p) * NC + c) * 64, 64))
        acc[p, c] = acc[p, c] + y if g else y


def _b_out_collect(B, u, acc, m=M):
    r = _turn(u)
    top = (u - 1 - r) % U
    mem = [_b_collect(B, r, [acc[p, c] for p in TURN[r]], m,
                      lambda rr, n: BO + 128 * (NC * n + c) + SEG * (top + rr)) for c in range(NC)]
    return [mem[c][n] for n in range(NG) for c in range(NC)] if m else None


def _b_out_tail(B, u):
    return functools.reduce(jnp.add, [
        _dot_nt(B.ldb(O2T + 32 * h, 32), B.ldb(OT + 64 * h, 64)) for h in range(8 * u, 8 * u + 8)])


def _b_step(B, u, before_out, after_use):
    row = lax.broadcasted_iota(I32, (L, 128), 0)
    lane = lax.broadcasted_iota(I32, (L, 128), 1)
    lo = lane < 64
    lo64 = lax.broadcasted_iota(I32, (64, 128), 1) < 64
    mask = (row < M) | (row >= (lane & 63))
    in_a, in_b = lane < L, (lane >= 64) & (lane < 64 + L)
    z24 = jnp.zeros((24, 128), F32)
    z8 = jnp.zeros((8, 128), F32)
    pair = [j for g in range(H // NG) for j in _pairs(g)]

    def rows(mat, h):
        return [B.ldf(MK + M * (H * mat + h), M), B.ldf(TK + 128 * (H * mat + h) + SEG * u, SEG)]

    def t_g():
        c4 = B.ldf(_lh(u, 0), L)
        B.stb(GS, jnp.concatenate([jnp.where(lo, 0.0, c4), z24, jnp.where(lo, c4, 0.0), z24], 0))

    def t_k(g):
        _b_project(B, u, 1, g)
        for j in _pairs(g):
            k = jnp.concatenate(rows(1, 2 * j) + [z24] + rows(1, 2 * j + 1) + [z24], 0)
            B.stb(KS + 64 * j, k.astype(BF16).T)

    def t_s(i):
        j = pair[i]
        kt, w2 = B.ldi(KS + 64 * j, 64), B.ldi(K2 + PSTRIDE * j, 64)
        for b, rhs in enumerate((jnp.where(lo64, kt, w2), jnp.where(lo64, w2, kt))):
            B.stf(RE + 40 * (NP * b + i), _dot(jnp.concatenate(rows(0, 2 * j + b), 0), pltpu.bitcast(rhs, BF16)))

    def t_s2(n):
        c4 = B.ldf(_lh(u, 0), L)
        a, b = B.ldf(RE + 128 * n, 128), B.ldf(RE + 40 * NP + 128 * n, 128)
        t = jnp.where(lax.broadcasted_iota(I32, (128, 128), 1) < 64, b, a).astype(BF16)
        y = _dot_nt(jnp.concatenate([jnp.where(lo, 0.0, c4), jnp.where(lo, c4, 0.0)], 0), t)
        B.stf(RS + 128 * n, jnp.concatenate([y[:L], z24, y[L:], z24], 0).T)
        for i in range(128 * n // L, 128 * (n + 1) // L):
            softmax(i)

    def softmax(i):
        s = jnp.where(lo, B.ldf(RE + 40 * i, 40), B.ldf(RE + 40 * (NP + i), 40)) + B.ldf(RS + 40 * i, 40)
        s = jnp.where(mask, s * DH ** -0.5, NEG)
        B.stf(RS + 40 * i, s)
        ma = jnp.max(jnp.where(in_a, s, -jnp.inf), axis=1, keepdims=True)
        mb = jnp.max(jnp.where(in_b, s, -jnp.inf), axis=1, keepdims=True)
        e = jnp.exp(B.ldf(RS + 40 * i, 40) - jnp.where(lo, ma, mb))
        B.stf(PS + 40 * i, jnp.where(in_a | in_b, e, 0.0))

    def t_r(i):
        B.stf(RS + 40 * i, _dot(B.ldf(PS + 40 * i, 40), B.ldb(GS, 64)))

    def t_v(g):
        _b_project(B, u, 2, g)
        for h in _heads(g):
            B.stb(PV + PSTRIDE * (h // 2) + 96 * (h % 2), jnp.concatenate(rows(2, h) + [z8], 0))

    def t_pv(i):
        p, r = B.ldf(PS + 40 * i, 40), B.ldf(RS + 40 * i, 40)
        for b, (lhs, keys) in enumerate(((jnp.where(lo, p, r), in_a), (jnp.where(lo, r, p), in_b))):
            h = 2 * pair[i] + b
            l = jnp.sum(jnp.where(keys, p, 0.0), axis=1, keepdims=True)
            l = jnp.broadcast_to(l, (L, 128))
            rc = pltpu.reciprocal(l, approx=True)
            o = _dot(lhs, B.ldb(PV + PSTRIDE * pair[i] + 64 * b, 64)) * (rc * (2.0 - l * rc))
            B.stf(OM + M * h, o[:M])
            B.stf(OF + SEG * (H * u + h), o[M:])
            B.stb(OT + 64 * h + 16 * u, o[M:])

    acc = {}

    def t_m(i):
        y = _dot(B.ldf(OM + 2 * M * pair[i], 2 * M), B.ldb(O2 + 64 * pair[i], 64))
        acc["tail"] = acc["tail"] + y if i else y

    lag_s, lag_s2, lag_o, v_late = 3, 4, 4, 2
    prods = TURN[_turn(u)]
    for g in range(NP):
        t_k(g)
    t_g()
    s2_after = [(128 * n + 127) // L + lag_s + lag_s2 for n in range(5)]
    for i in range(2 * NP - v_late):
        _b_project(B, u, 0, i) if i < NP else t_v(i - NP)
        if 0 <= i - lag_s < NP:
            t_s(i - lag_s)
        if i in s2_after:
            t_s2(s2_after.index(i))
        if i >= 2 * NP - v_late - 8:
            for b in range(2):
                t_r(2 * (i - (2 * NP - v_late - 8)) + b)
    before_out()
    for i in range(NP + lag_o):
        if i < NP:
            t_pv(i)
        if i < lag_o:
            for g in range(v_late * i // lag_o, v_late * (i + 1) // lag_o):
                t_v(NP - v_late + g)
        else:
            _b_out_product(B, u, prods[2], i - lag_o, acc)
            _b_out_product(B, u, prods[0], i - lag_o, acc)
    after_use()
    for g in range(NP):
        _b_out_product(B, u, prods[3], g, acc)
        t_m(g)
        _b_out_product(B, u, prods[1], g, acc)
    _b_place_memory(B, u + 1, _b_out_collect(B, u, acc))
    mem2 = jnp.where(lo[:M], acc["tail"][:M], acc["tail"][M:])
    mem2 = mem2 + pltpu.roll(mem2, 64, 1)
    for i in range(2):
        B.stf(_lh(u + 1, i), mem2)
    y = _b_out_tail(B, u)
    if u == U - 1:
        B.stf(B2 + 64, B.ldf(B2, 64) + y)
    else:
        new = lax.broadcasted_iota(I32, (64, 128), 1) < SEG * (u + 1)
        B.stf(B2, jnp.where(new, y, 0.0) + (B.ldf(B2, 64) if u else 0.0))
        B.stf(B2 + 64, jnp.where(new, 0.0, y) + B.ldf(B2 + 64, 64))


def _kernel(xt_hbm, wqkv_hbm, wo_hbm, mem_hbm, gate_hbm, wq_hbm, wk_hbm, wv_hbm, wot_hbm,
            out_hbm,
            xt, wqkv, wo, mem_ref, gate_ref, raw, wot, a_ref, b_ref, qkv_all, o_all, o_last, ga_all, omg, out_buf,
            offs, sem_in, sem_w, sem_out):
    A, B = _Arena(a_ref), _Arena(b_ref)

    def cols(src, dst, c0, c1, sem):
        return pltpu.make_async_copy(src.at[:, pl.ds(c0, c1 - c0)], dst.at[:, pl.ds(c0, c1 - c0)], sem_in.at[sem])

    x_copy = [cols(xt_hbm, xt, c0, c1, i) for i, (c0, c1) in
              enumerate(((0, 256), (256, 768), (768, S)))]
    w_copy = [cols(wqkv_hbm, wqkv, c0, c1, 3 + i) for i, (c0, c1) in
              enumerate(((512, 896), (896, 1152), (0, 512), (1152, 3 * D)))]
    wo_copy = pltpu.make_async_copy(wo_hbm, wo, sem_in.at[8])
    mem_copy = pltpu.make_async_copy(mem_hbm, mem_ref, sem_in.at[9])
    gate_copy = pltpu.make_async_copy(gate_hbm, gate_ref, sem_in.at[10])

    def rows(r0, r1, sem):
        return [pltpu.make_async_copy(w.at[pl.ds(r0 * H, (r1 - r0) * H)],
                                      raw.at[pl.ds(RAW * m + r0 * H, (r1 - r0) * H)], sem_w.at[sem])
                for m, w in enumerate((wq_hbm, wk_hbm, wv_hbm))]

    tail_copies, main_copies = rows(512, D, 0), rows(0, 512, 1)
    wot_copy = pltpu.make_async_copy(wot_hbm, wot, sem_w.at[2])

    def x_stage(j, slot):
        A.stb(AX + 288 * slot, xt[:, pl.ds(pl.multiple_of(j * 128, 128), 128)])

    def x_transpose(j, n):
        cols = pl.ds(pl.multiple_of(j * 128, 128), 128)
        if n < 4:
            t = xt[128 * n:128 * n + 128, cols]
        else:
            t = jnp.concatenate([xt[512:576, cols]] * 2, 0)
        B.stb(XN + 64 * n, t.T)

    def x_tail(u):
        B.stf(_lh(u, 0) + M, B.ldb(XN + 256 + 16 * u, 16).astype(F32))

    def proj(j):
        if isinstance(j, int):
            return _Arena(qkv_all.at[pl.ds((j + 1) % 5 * SLOT, SLOT)])
        return _Arena(qkv_all.at[pl.ds(pl.multiple_of(offs[lax.rem(j + 1, 5)], 8), SLOT)])

    for c in (w_copy[0], gate_copy, mem_copy, w_copy[1], x_copy[0], w_copy[2], w_copy[3],
              wo_copy):
        c.start()

    for i in range(5):
        offs[i] = i * SLOT
    for i in range(2):
        offs[5 + i] = 512 * H + 32 * H * i
    for i in range(4):
        offs[7 + i] = 128 // NG * H * i
    for j in range(NP):
        B.stf(PSTRIDE * j + PV + 24, jnp.zeros((8, 128), F32))
        B.stf(PSTRIDE * j + PV + 120, jnp.zeros((8, 128), F32))
    B.stf(OF + 2 * H * SEG, jnp.zeros((B_ROWS - OF - 2 * H * SEG, 128), F32))
    w_copy[0].wait()
    gate_copy.wait()
    mem_copy.wait()
    gate = jnp.broadcast_to(gate_ref[...].astype(F32)[None, :], (8, D))
    mem0 = mem_ref[...].astype(F32)
    for k in range(4):
        A.stf(GW + 8 * k, gate[:, 128 * k:128 * k + 128])
    A.stf(GW + 32, jnp.concatenate([gate[:, 512:]] * 2, 1))
    _b_place_memory(B, 0, [mem0[:, 128 * k:128 * k + 128] for k in range(4)])
    for i in range(2):
        B.stf(_lh(0, i), jnp.concatenate([mem0[:, 512:]] * 2, 1))

    def project(j, *parts):
        return _a_qkv(A, AX + 288 * j, proj(j), parts, first=j == 0)

    _a_transpose_w(A, wqkv, range(4, 7))
    w_copy[1].wait()
    _a_transpose_w(A, wqkv, range(7, 9))
    x_copy[0].wait()
    x_stage(0, 0)
    x_stage(1, 1)
    _interleave(project(0, 3, 1))
    for n in range(5):
        x_transpose(0, n)
    for u in range(U):
        x_tail(u)
        _b_place_tokens(B, u)
    w_copy[2].wait()
    x_copy[1].start()
    _a_transpose_w(A, wqkv, range(0, 4))
    _interleave(_chain(project(1, 3, 1), project(0, 0)))
    w_copy[3].wait()
    x_copy[2].start()
    _a_transpose_w(A, wqkv, range(9, 14))
    _interleave(_chain(project(1, 0), project(0, 2)))
    wo_copy.wait()
    for c in tail_copies:
        c.start()
    _interleave(project(1, 2), _a_transpose_wo(A, wo))
    qkv_all[AK:AG, :] = jnp.broadcast_to(qkv_all[SLOT + AK:SLOT + AG, :1], (AG - AK, 128))

    def tick_raw(r):
        raw[D * H:RAW, :] = r[:16].astype(BF16)

    def tick_attend(r):
        qkv_all[TICK:TICK + 8, :] = pltpu.bitcast(r[:8], I32)

    def attend(j):
        return _a_attend(j, proj(j), proj(j - 1), o_all.at[j], omg)

    def project_out(j0, n, tick):
        return _chain(*[_a_out(A, o_all.at[j0 + b], ga_all.at[j0 + b], tick) for b in range(n)])

    def attend_trip(t, carry):
        @pl.when(t == 1)
        def _():
            x_copy[2].wait()
            wot_copy.start()

        def project(i):
            return _chain(_a_qkv(A, AX + 288 * i, proj(2 * t + 2 + i)),
                          _once(x_stage, jnp.minimum(2 * t + 4 + i, NB - 1), i))

        _interleave(_chain(project(0), project(1)), _chain(attend(2 * t), attend(2 * t + 1)), span=(-0.04, 0.87))

    x_copy[1].wait()
    for c in main_copies:
        c.start()
    x_stage(2, 0)
    x_stage(3, 1)
    lax.fori_loop(0, NB // 2 - 1, attend_trip, None)

    def last_trip(t, carry):
        src = raw.at[pl.ds(pl.multiple_of(offs[5 + t], 16), 2 * RAW + 32 * H)]
        dst = b_ref.at[pl.ds(pl.multiple_of(t * 16, 16), O2), :]
        _interleave(
            project_out(3 * t, 3, lambda r: (tick_attend(r), tick_raw(r))), _a_attend(NB - 2 + t, proj(NB - 2 + t), proj(NB - 3 + t), o_last.at[t], omg),
            _chain(*[_b_split_heads(src.at[pl.ds(RAW * m, 32 * H)], dst, even, odd) for m, (even, odd) in
                     enumerate(((Q2, Q2 + 32), (K2 + 32, K2), (PV + 32, PV + 64)))]),
            span=(-0.08, 0.82))

    for c in tail_copies:
        c.wait()
    lax.fori_loop(0, 2, last_trip, None)
    o_all[NB - 2:] = o_last[...]

    def prepare_trip(t, carry):
        n = 64 // NG
        src = raw.at[pl.ds(pl.multiple_of(offs[7 + t], 16), 2 * RAW + (512 - 6 * n) * H)]
        dst = b_ref.at[pl.ds(pl.multiple_of(t * n, n), O2), :]
        _interleave(project_out(6 + 2 * t, 2, tick_raw), _chain(*[
            _b_product_tiles(src.at[pl.ds(RAW * m, (512 - 6 * n) * H)], dst, m * NPR * NC * 64, n)
            for m in range(3)]), span=(-0.04, 0.93))

    for c in main_copies:
        c.wait()
    lax.fori_loop(0, 4, prepare_trip, None)
    wot_copy.wait()
    _interleave(
        _chain(project_out(NB - 2, 2, lambda r: None),
               *[_once(_b_project, B, U - 1, mat, g, 0) for mat in range(3) for g in range(H // NG)]),
        _b_transpose_wo(B, wot))

    def mix(j, n):
        rows = min(128, D - 128 * n)
        bt = B.ldf(BO + 128 * n, 128).T if n < 4 else B.ldf(B2 + 64, 64)
        w = jnp.concatenate([omg[j]] * (rows // 8), 0)
        out_buf[j, 128 * n:128 * n + rows, :] = (
            ga_all[j, 128 * n:128 * n + rows, :] + w * bt).astype(BF16)

    def out_copy(j):
        return pltpu.make_async_copy(
            out_buf.at[j], out_hbm.at[:, pl.ds(pl.multiple_of(j * 128, 128), 128)], sem_out)

    def b_body(g, carry):
        jn, jp = jnp.minimum(g + 1, NB - 1), jnp.maximum(g - 1, 0)
        for u in range(U):
            def before_out():
                for n in {1: range(4), U - 1: (4,)}.get(u, ()):
                    mix(jp, n)

            def after_use():
                if u == 0:
                    for n in range(5):
                        x_transpose(jn, n)
                    _b_place_tokens(B, U - 1)
                if u < U - 1:
                    _b_place_tokens(B, u)
                x_tail(u)

            _b_step(B, u, before_out, after_use)

        @pl.when(g > 0)
        def _():
            out_copy(jp).start()

        return carry

    lax.fori_loop(0, NB, b_body, 0)
    acc = {}
    for g in range(H // NG):
        for p in TURN[1]:
            _b_out_product(B, 0, p, g, acc, 0)
    _b_out_collect(B, 0, acc, 0)
    lane = lax.broadcasted_iota(I32, (64, 128), 1)
    B.stf(B2 + 64, functools.reduce(jnp.add, [B.ldf(B2 + 64, 64)] + [
        jnp.where(lane < SEG * (u + 1), 0.0, _b_out_tail(B, u)) for u in range(U - 1)]))
    for n in range(5):
        mix(NB - 1, n)
    out_copy(NB - 1).start()
    for j in range(NB):
        out_copy(j).wait()


@functools.partial(jax.jit, static_argnames=("B_seg_len",))
def pallas_gated_mix__sliding_local_dilated__memory_aug_recurrent_mem_tr__prompt_kernel(
    A_x: jax.Array,
    A_wqkv: jax.Array,
    A_wo: jax.Array,
    B_x: jax.Array,
    B_mem0: jax.Array,
    B_Wq: jax.Array,
    B_Wk: jax.Array,
    B_Wv: jax.Array,
    B_Wo: jax.Array,
    B_seg_len: int,
    gate_w: jax.Array,
):
    del B_x
    assert A_x.shape == (1, S, D) and B_mem0.shape == (1, M, D) and B_Wq.shape == (D, H, DH)
    assert B_seg_len == SEG
    hbm = pl.BlockSpec(memory_space=pl.ANY)
    out_t = pl.pallas_call(
        _kernel,
        out_shape=jax.ShapeDtypeStruct((D, S), BF16),
        in_specs=[hbm] * 9,
        out_specs=hbm,
        scratch_shapes=[
            pltpu.VMEM((D, S), BF16),
            pltpu.VMEM((D, 3 * D), BF16),
            pltpu.VMEM((D, D), BF16),
            pltpu.VMEM((M, D), BF16),
            pltpu.VMEM((D,), BF16),
            pltpu.VMEM((3 * RAW, DH), BF16),
            pltpu.VMEM((H * D, DH), BF16),
            pltpu.VMEM((A_ROWS, 128), I32),
            pltpu.VMEM((B_ROWS, 128), I32),
            pltpu.VMEM((5 * SLOT, 128), I32),
            pltpu.VMEM((NB, D // 2, 128), I32),
            pltpu.VMEM((2, D // 2, 128), I32),
            pltpu.VMEM((NB, D, 128), F32),
            pltpu.VMEM((NB, 8, 128), F32),
            pltpu.VMEM((NB, D, 128), BF16),
            pltpu.SMEM((11,), I32),
            pltpu.SemaphoreType.DMA((11,)),
            pltpu.SemaphoreType.DMA((3,)),
            pltpu.SemaphoreType.DMA,
        ],
        compiler_params=pltpu.CompilerParams(vmem_limit_bytes=110 * 1024 * 1024),
    )(
        A_x.reshape(S, D).T, A_wqkv, A_wo, B_mem0.reshape(M, D), gate_w,
        B_Wq.reshape(D * H, DH), B_Wk.reshape(D * H, DH), B_Wv.reshape(D * H, DH),
        B_Wo.transpose(0, 2, 1).reshape(H * D, DH),
    )
    return out_t.T.reshape(1, S, D)
```

```python
import functools

import jax
import jax.numpy as jnp
from jax import lax
import jax.experimental.pallas as pl
import jax.experimental.pallas.tpu as pltpu

F32, BF16, I32 = jnp.float32, jnp.bfloat16, jnp.int32

S, D = 2048, 576
NB = S // 128
HA, DA, WIN, DIL = 32, 18, 8, 2
H, DH, M, SEG = 32, 128, 8, 32
L = M + SEG
NP = H // 2
U = 128 // SEG
NEG = -1000000000.0

NG = 2
PRODUCTS = (
    ({(0, 0): 1}, {(0, 1): 1, (1, 1): -1}, {(0, 1): 1, (1, 1): 1}),
    ({(1, 1): 1}, {(1, 0): 1, (0, 0): -1}, {(0, 0): 1, (1, 0): 1}),
    ({(0, 0): 1, (0, 1): 1}, {(1, 1): 1}, {(0, 0): -1, (0, 1): 1}),
    ({(1, 0): 1, (1, 1): 1}, {(0, 0): 1}, {(1, 0): 1, (1, 1): -1}),
    ({(0, 0): 1, (1, 1): 1}, {(0, 0): 1, (1, 1): 1}, {(0, 0): 1, (1, 1): 1}),
    ({(0, 1): 1, (1, 1): -1}, {(1, 0): 1, (1, 1): 1}, {(0, 0): 1}),
    ({(1, 0): 1, (0, 0): -1}, {(0, 0): 1, (0, 1): 1}, {(1, 1): 1}),
)
NPR = len(PRODUCTS)
NC = 4 // NG
TURN = tuple(tuple(p for p, (a, _, c) in enumerate(PRODUCTS)
                   if any(k[0] == r for k in a) and any(k[0] == r for k in c)) for r in range(2))

GSTRIDE = 3 * NPR * NC * 64 + 4
TAIL = H // NG * GSTRIDE
Q2 = TAIL
K2 = Q2 + 64
V2 = K2 + 64
PSTRIDE = 192 + 4
OA = TAIL + NP * PSTRIDE
O2 = OA + H // NG * NPR * NC * 64
O2T = O2 + NP * 64
LH = O2T + H * 32
GS = LH + U * (NG * NG * NC + 2) * 40
TK = GS + 64
MK = TK + 3 * H * 128
VS = MK + H * M
KS = VS + H * 40
RE = KS + NP * 64
PS = RE + H * 40
RS = PS + NP * 40
XN = RS + NP * 40
OM = XN + 320
OF = OM + H * M
BO = OF + U * H * SEG
B2 = BO + 512
OT = B2 + 128
B_ROWS = OT + H * 64

RAW = D * H + 16

WT = 0
GW = WT + 5 * 1728
WP = GW + 40
WOT = WP + 27 * 160
AX = WOT + 5 * 288
A_ROWS = AX + 2 * 288
AQ, AK, AV, AG, TICK, SLOT = 0, 576, 864, 1152, 1160, 1168


def _dot(a, b):
    return lax.dot_general(a, b, (((1,), (0,)), ((), ())), preferred_element_type=F32)


def _dot_nt(a, b):
    return lax.dot_general(a, b, (((1,), (1,)), ((), ())), preferred_element_type=F32)


class _Arena:
    def __init__(self, ref):
        self.r = ref

    def ldi(self, o, n):
        return self.r[o:o + n, :]

    def ldf(self, o, n):
        return pltpu.bitcast(self.r[o:o + n, :], F32)

    def ldb(self, o, n):
        return pltpu.bitcast(self.r[o:o + n, :], BF16)

    def stf(self, o, v):
        self.r[o:o + v.shape[0], :] = pltpu.bitcast(v, I32)

    def stb(self, o, v):
        self.r[o:o + v.shape[0] // 2, :] = pltpu.bitcast(v.astype(BF16), I32)


def _pad2(t, rows, cols):
    r, c = t.shape
    if c < cols:
        t = jnp.concatenate([t, jnp.zeros((r, cols - c), t.dtype)], 1)
    if r < rows:
        t = jnp.concatenate([t, jnp.zeros((rows - r, cols), t.dtype)], 0)
    return t


def _interleave(main, *side, span=(0.0, 0.9)):
    jobs = (main,) + side
    order = [((i + 1) / main[0], 0) for i in range(main[0])]
    order += [(span[0] + (span[1] - span[0]) * i / n, k + 1) for k, (n, _) in enumerate(side) for i in range(n)]
    for _, k in sorted(order):
        next(jobs[k][1])
    for _, gen in jobs:
        assert next(gen, "end") == "end"


def _once(fn, *args):
    def gen():
        fn(*args)
        yield
    return 1, gen()


def _chain(*jobs):
    def gen():
        for _, g in jobs:
            yield from g
    return sum(n for n, _ in jobs), gen()


def _a_transpose_w(A, w_ref, cblocks):
    for c in cblocks:
        nc = min(128, 3 * D - 128 * c)
        for k in range(5):
            nk = min(128, D - 128 * k)
            t = _pad2(w_ref[128 * k:128 * k + nk, 128 * c:128 * c + nc], 128, 128).T
            A.stf(WT + 1728 * k + 128 * c, t[:nc].astype(F32))


def _a_transpose_wo(A, w_ref):
    def gen():
        for c in range(5):
            nc = min(128, D - 128 * c)
            for k in range(5):
                nk = min(128, D - 128 * k)
                t = _pad2(w_ref[128 * k:128 * k + nk, 128 * c:128 * c + nc], 128, 128).T
                A.stb(WOT + 288 * k + 64 * c, t[:nc])
                yield
    return 25, gen()


def _a_qkv(A, x_off, dst, parts=(3, 1, 0, 2), first=False):
    def proj(rows_of_k):
        ch = [rows_of_k(k) for k in range(5)]
        return _dot(jnp.concatenate(ch[:4] + [ch[4][:, :64]], 1), A.ldb(x_off, 288))

    def gen():
        for part in parts:
            if part == 3:
                dst.stf(AG, jax.nn.sigmoid(proj(lambda k: A.ldf(GW + 8 * k, 8))))
                continue
            for d0 in range(0, DA, 2):
                def weights(k):
                    packed = WP + 160 * (9 * part + d0 // 2) + 32 * k
                    if not first:
                        return A.ldb(packed, 32)
                    w = jnp.concatenate([
                        pltpu.bitcast(A.r[pl.ds(WT + 1728 * k + D * part + 8 * DA * hg + d, 8, stride=DA), :], F32)
                        for hg in range(4) for d in (d0, d0 + 1)], 0)
                    A.stb(packed, w)
                    return w

                r = proj(weights)
                for i in range(0, 64, 16):
                    if part == 0:
                        dst.stf(AQ + 32 * d0 + i, r[i:i + 16])
                    else:
                        dst.stb((AK if part == 1 else AV) + 16 * d0 + i // 2, r[i:i + 16])
                    yield
    return sum(2 * DA for p in parts if p < 3), gen()


def _a_attend(j, cur, old, o_ref, omg_ref):
    def window(o):
        lane = lax.broadcasted_iota(I32, (8, 128), 1)
        c, p = cur.ldi(o, 8), old.ldi(o, 8)
        out = []
        for w in range(WIN):
            sh = DIL * w
            t = c if w == 0 else pltpu.roll(jnp.where(lane >= 128 - sh, p, c), sh, 1)
            out.append(pltpu.bitcast(t, BF16).astype(F32))
        return out

    def gen():
        pos = j * 128 + lax.broadcasted_iota(I32, (8, 128), 1)
        for hg in range(4):
            lg = None
            for d in range(0, DA, 2):
                q = cur.ldf(AQ + 32 * d + 16 * hg, 16)
                pr = [q * kw for kw in window(AK + 16 * d + 8 * hg)]
                pr = [t[:8] + t[8:] for t in pr]
                lg = pr if d == 0 else [a + b for a, b in zip(lg, pr)]
                yield
            lg = [jnp.where(pos >= DIL * w, t * DA ** -0.5, NEG) for w, t in enumerate(lg)]
            mx = functools.reduce(jnp.maximum, lg)
            e = [jnp.exp(t - mx) for t in lg]
            g = cur.ldf(AG, 8)
            if hg == 0:
                omg_ref[j] = 1.0 - g
            r = g / functools.reduce(jnp.add, e)
            p = [jnp.concatenate([t * r] * 2, 0) for t in e]
            yield
            for d in range(0, DA, 2):
                o = functools.reduce(jnp.add, [a * b for a, b in zip(p, window(AV + 16 * d + 8 * hg))])
                o = pltpu.bitcast(o.astype(BF16).astype(F32), I32)
                o_ref[pl.ds(4 * DA * hg + d // 2, 8, stride=DA // 2), :] = (
                    lax.shift_right_logical(o[:8], 16) | o[8:])
                yield
    return 4 * DA + 4, gen()


def _a_out(A, o_ref, ga_ref, tick):
    def gen():
        for r0 in range(0, D, 96):
            ch = [A.ldb(WOT + 288 * k + r0 // 2, 48) for k in range(5)]
            r = _dot(jnp.concatenate(ch[:4] + [ch[4][:, :64]], 1), pltpu.bitcast(o_ref[...], BF16))
            for i in range(0, 96, 32):
                tick(r[i:i + 32])
                ga_ref[r0 + i:r0 + i + 32, :] = r[i:i + 32]
                yield
    return D // 32, gen()


def _b_split_heads(raw, dst, even, odd):
    def gen():
        for r in range(raw.shape[0] // 64):
            e = pltpu.bitcast(raw[64 * r:64 * r + 32, :], I32)
            o = pltpu.bitcast(raw[64 * r + 32:64 * r + 64, :], I32)
            dst[pl.ds(even + r, NP, stride=PSTRIDE), :] = (e & 0xFFFF) | (o << 16)
            dst[pl.ds(odd + r, NP, stride=PSTRIDE), :] = lax.shift_right_logical(e, 16) | (o & -65536)
            yield
    return raw.shape[0] // 64, gen()


def _signed_sum(terms):
    terms = sorted(terms, key=lambda t: -t[0])
    acc = terms[0][1] if terms[0][0] > 0 else -terms[0][1]
    for c, t in terms[1:]:
        acc = acc + t if c > 0 else acc - t
    return acc


def _pairs(g):
    return [g + 8 * i for i in range(NG // 2)]


def _heads(g):
    return [2 * j + i for j in _pairs(g) for i in range(2)]


def _b_product_tiles(raw, dst, off, rows):
    def gen():
        for r in range(rows):
            word = [[pltpu.bitcast(raw[o:o + 32, :], I32) for o in (o0, o0 + 32)]
                    for o0 in range(64 * r, 512 * H, 512 * H // NG)]

            def block(k, n, i):
                t = word[k][i][8 * (n // 2):8 * (n // 2) + H // NG]
                return pltpu.bitcast(t & -65536 if n % 2 else t << 16, F32)

            for p, (_, w, _) in enumerate(PRODUCTS):
                e, o = [pltpu.bitcast(_signed_sum([(c, block(k, n, i)) for (k, n), c in w.items()]), I32)
                        for i in range(2)]
                if len(w) > 1:
                    e, o = e + 0x8000, (o + 0x7FFF) & -65536
                dst[pl.ds(off + p * NC * 64 + r, H // NG, stride=GSTRIDE), :] = lax.shift_right_logical(e, 16) | o
            yield
    return rows, gen()


def _b_transpose_wo(B, wot):
    def gen():
        for g in range(H // NG):
            for p, (_, w, _) in enumerate(PRODUCTS):
                for i in range(NC):
                    t = [(c, wot[pl.ds(D * _heads(g)[k] + 128 * (NC * n + i), 128), :]) for (k, n), c in w.items()]
                    if len(t) > 1 or t[0][0] < 0:
                        t = [(1, _signed_sum([(c, v.astype(F32)) for c, v in t]).astype(BF16))]
                    B.stb(OA + ((g * NPR + p) * NC + i) * 64, t[0][1].T)
                    yield
            for j in _pairs(g):
                t = jnp.concatenate([wot[D * h + 512:D * h + D, :] for h in (2 * j, 2 * j + 1)], 0)
                B.stb(O2T + 64 * j, t)
                B.stb(O2 + 64 * j, t.T)
                B.stb(K2 + PSTRIDE * j, B.ldb(K2 + PSTRIDE * j, 64).T)
    return H // NG * NPR * NC, gen()


def _turn(u):
    return 1 - u % 2


def _halves(p, r):
    return (r,) if p in TURN[1 - r] else (0, 1)


def _lh(u, i):
    return LH + 40 * ((NG * NG * NC + 2) * (u % U) + i)


def _b_place_memory(B, u, mem):
    r = _turn(u)
    for i, p in enumerate(TURN[r]):
        for c in range(NC):
            B.stf(_lh(u, 2 + NC * i + c), _signed_sum(
                [(s, mem[NC * k + c]) for (rr, k), s in PRODUCTS[p][0].items() if rr == r]))


def _b_place_tokens(B, u):
    r = _turn(u)
    top = (u + 1 - r) % U

    def x(seg, n, half):
        return B.ldb(XN + 64 * n + 16 * seg + 8 * half, 8).astype(F32)

    for i, p in enumerate(TURN[r]):
        for c in range(NC):
            for at, half in enumerate(_halves(p, r)):
                B.stf(_lh(u, 2 + NC * i + c) + M + 16 * at, _signed_sum(
                    [(s, x(top + rr, NC * k + c, half)) for (rr, k), s in PRODUCTS[p][0].items()]))
    for half in range(2):
        B.stf(_lh(u, 1) + M + 16 * half, x((u + 1) % U, 4, half))


def _b_collect(B, r, ys, m, at, plain=None, keep=()):
    mem, tok, kept = {}, {}, {}
    items = [(PRODUCTS[p][2], _halves(p, r), y) for p, y in zip(TURN[r], ys)]
    if plain:
        items += [({(r, n): 1}, (0, 1), y) for n, y in enumerate(plain)]
    for c, halves, y in items:
        for (rr, n), s in c.items():
            if m and rr == r:
                mem.setdefault(n, []).append((s, y[:m]))
            for i, half in enumerate(halves):
                tok.setdefault((rr, n, half), []).append((s, y[m + 16 * i:m + 16 * i + 16]))
    for (rr, n, half), terms in sorted(tok.items()):
        o = at(rr, n) + 16 * half
        if r == 1 and any((rr, n) in PRODUCTS[p][2] and half in _halves(p, 0) for p in TURN[0]):
            terms.append((1, B.ldf(o, 16)))
        if r == 1 and rr in keep:
            kept[rr, n, half] = _signed_sum(terms)
        else:
            B.stf(o, _signed_sum(terms))
    return [_signed_sum(mem[n]) for n in sorted(mem)], kept


def _b_project(B, u, mat, g, m=M, keep=()):
    r = _turn(u)
    top = (u + 1 - r) % U
    ys = [_dot(jnp.concatenate([B.ldf(_lh(u, 2 + NC * i + c) + M - m, m + 16 * len(_halves(p, r)))
                                for c in range(NC)], 1),
               B.ldb(GSTRIDE * g + (mat * NPR + p) * NC * 64, NC * 64)) for i, p in enumerate(TURN[r])]
    plain = None
    if mat == 0:
        plain = [_dot(B.ldf(_lh(u, 1) + M - m, m + SEG)[:, :64], B.ldb(Q2 + PSTRIDE * (h // 2) + 32 * (h % 2), 32))
                 for h in _heads(g)]
    mem, kept = _b_collect(B, r, ys, m, lambda rr, n: TK + 128 * (H * mat + _heads(g)[n]) + SEG * (top + rr),
                           plain, keep)

    def tokens(n, seg):
        return [kept[seg - top, n, i] if (seg - top, n, i) in kept else
                B.ldf(TK + 128 * (H * mat + _heads(g)[n]) + SEG * seg + 16 * i, 16) for i in range(2)]

    return mem, tokens


def _b_out_product(B, u, p, g, acc, m=M):
    r = _turn(u)
    top = (u - 1 - r) % U
    a = PRODUCTS[p][0].items()
    lhs = [_signed_sum([(s, B.ldf(OM + M * _heads(g)[k], M)) for (rr, k), s in a if rr == r])] if m else []
    lhs += [_signed_sum([(s, B.ldf(OF + SEG * (H * (top + rr) + _heads(g)[k]) + 16 * half, 16)) for (rr, k), s in a])
            for half in _halves(p, r)]
    for c in range(NC):
        y = _dot(jnp.concatenate(lhs, 0), B.ldb(OA + ((g * NPR + p) * NC + c) * 64, 64))
        acc[p, c] = acc[p, c] + y if g else y


def _b_out_collect(B, u, acc, m=M):
    r = _turn(u)
    top = (u - 1 - r) % U
    mem = [_b_collect(B, r, [acc[p, c] for p in TURN[r]], m,
                      lambda rr, n: BO + 128 * (NC * n + c) + SEG * (top + rr))[0] for c in range(NC)]
    return [mem[c][n] for n in range(NG) for c in range(NC)] if m else None


def _b_out_tail(B, u):
    return functools.reduce(jnp.add, [
        _dot_nt(B.ldb(O2T + 32 * h, 32), B.ldb(OT + 64 * h, 64)) for h in range(8 * u, 8 * u + 8)])


def _b_step(B, u, before_out, after_use):
    row = lax.broadcasted_iota(I32, (L, 128), 0)
    lane = lax.broadcasted_iota(I32, (L, 128), 1)
    lo = lane < 64
    lo64 = lax.broadcasted_iota(I32, (64, 128), 1) < 64
    mask = (row < M) | ((lane & 63) >= SEG) | (row - M >= (lane & 63))
    in_a, in_b = lane < L, (lane >= 64) & (lane < 64 + L)
    z24 = jnp.zeros((24, 128), F32)
    z8 = jnp.zeros((8, 128), F32)
    pair = [j for g in range(H // NG) for j in _pairs(g)]

    def h2():
        return jnp.concatenate([B.ldf(_lh(u, 0) + M, SEG), B.ldf(_lh(u, 0), M)], 0)

    def t_q(g):
        for h, t in zip(_heads(g), _b_project(B, u, 0, g)[0]):
            B.stf(MK + M * h, t)

    def t_g():
        c4 = h2()
        B.stb(GS, jnp.concatenate([jnp.where(lo, 0.0, c4), z24, jnp.where(lo, c4, 0.0), z24], 0))

    def t_k(g):
        mem, tokens = _b_project(B, u, 1, g, keep=(0,))
        for i, j in enumerate(_pairs(g)):
            k = jnp.concatenate([t for n in (2 * i, 2 * i + 1) for t in tokens(n, u) + [mem[n], z24]], 0)
            B.stb(KS + 64 * j, k.astype(BF16).T)

    def t_s(i):
        j = pair[i]
        kt, w2 = B.ldi(KS + 64 * j, 64), B.ldi(K2 + PSTRIDE * j, 64)
        for b, rhs in enumerate((jnp.where(lo64, kt, w2), jnp.where(lo64, w2, kt))):
            q = jnp.concatenate([B.ldf(MK + M * (2 * j + b), M), B.ldf(TK + 128 * (2 * j + b) + SEG * u, SEG)], 0)
            B.stf(RE + 40 * (NP * b + i), _dot(q, pltpu.bitcast(rhs, BF16)))

    def t_s2(n):
        c4 = h2()
        a, b = B.ldf(RE + 128 * n, 128), B.ldf(RE + 40 * NP + 128 * n, 128)
        t = jnp.where(lax.broadcasted_iota(I32, (128, 128), 1) < 64, b, a).astype(BF16)
        y = _dot_nt(jnp.concatenate([jnp.where(lo, 0.0, c4), jnp.where(lo, c4, 0.0)], 0), t)
        B.stf(RS + 128 * n, jnp.concatenate([y[:L], z24, y[L:], z24], 0).T)
        for i in range(128 * n // L, 128 * (n + 1) // L):
            softmax(i)

    def softmax(i):
        s = jnp.where(lo, B.ldf(RE + 40 * i, 40), B.ldf(RE + 40 * (NP + i), 40)) + B.ldf(RS + 40 * i, 40)
        s = jnp.where(mask, s * DH ** -0.5, NEG)
        B.stf(RS + 40 * i, s)
        ma = jnp.max(jnp.where(in_a, s, -jnp.inf), axis=1, keepdims=True)
        mb = jnp.max(jnp.where(in_b, s, -jnp.inf), axis=1, keepdims=True)
        e = jnp.exp(B.ldf(RS + 40 * i, 40) - jnp.where(lo, ma, mb))
        B.stf(PS + 40 * i, jnp.where(in_a | in_b, e, 0.0))

    def t_r(i):
        B.stf(RS + 40 * i, _dot(B.ldf(PS + 40 * i, 40), B.ldb(GS, 64)))

    def t_v(g):
        mem, tokens = _b_project(B, u, 2, g, keep=(0, 1))
        for n, h in enumerate(_heads(g)):
            B.stb(VS + 40 * h + 32, jnp.concatenate([mem[n], z8], 0))
            if _turn(u):
                B.stb(VS + 40 * h, jnp.concatenate(tokens(n, u) + tokens(n, u + 1), 0))

    def t_pv(i):
        p, r = B.ldf(PS + 40 * i, 40), B.ldf(RS + 40 * i, 40)
        for b, (lhs, keys) in enumerate(((jnp.where(lo, p, r), in_a), (jnp.where(lo, r, p), in_b))):
            h = 2 * pair[i] + b
            l = jnp.sum(jnp.where(keys, p, 0.0), axis=1, keepdims=True)
            l = jnp.broadcast_to(l, (L, 128))
            rc = pltpu.reciprocal(l, approx=True)
            v = [B.ldi(VS + 40 * h + 16 * (u % 2), 16), B.ldi(VS + 40 * h + 32, 8), jnp.zeros((8, 128), I32)]
            w2 = [B.ldi(V2 + PSTRIDE * pair[i] + 32 * b, 32)]
            o = _dot(lhs, pltpu.bitcast(jnp.concatenate(w2 + v if b else v + w2, 0), BF16)) * (rc * (2.0 - l * rc))
            B.stf(OM + M * h, o[:M])
            B.stf(OF + SEG * (H * u + h), o[M:])
            B.stb(OT + 64 * h + 16 * u, o[M:])

    acc = {}

    def t_m(i):
        y = _dot(B.ldf(OM + 2 * M * pair[i], 2 * M), B.ldb(O2 + 64 * pair[i], 64))
        acc["tail"] = acc["tail"] + y if i else y

    lag_s, lag_s2, lag_o, v_late = 3, 4, 3, 2
    prods = TURN[_turn(u)]
    for g in range(NP):
        t_k(g)
    t_g()
    s2_after = [(128 * n + 127) // L + lag_s + lag_s2 for n in range(5)]
    for i in range(2 * NP - v_late):
        t_q(i) if i < NP else t_v(i - NP)
        if 0 <= i - lag_s < NP:
            t_s(i - lag_s)
        if i in s2_after:
            t_s2(s2_after.index(i))
        if i >= 2 * NP - v_late - 8:
            for b in range(2):
                t_r(2 * (i - (2 * NP - v_late - 8)) + b)
    before_out()
    for i in range(NP + lag_o):
        if i < NP:
            t_pv(i)
        if i < lag_o:
            for g in range(v_late * i // lag_o, v_late * (i + 1) // lag_o):
                t_v(NP - v_late + g)
        else:
            _b_out_product(B, u, prods[2], i - lag_o, acc)
            _b_out_product(B, u, prods[0], i - lag_o, acc)
    after_use()
    for g in range(NP):
        _b_out_product(B, u, prods[3], g, acc)
        t_m(g)
        _b_out_product(B, u, prods[1], g, acc)
    _b_place_memory(B, u + 1, _b_out_collect(B, u, acc))
    mem2 = jnp.where(lo[:M], acc["tail"][:M], acc["tail"][M:])
    mem2 = mem2 + pltpu.roll(mem2, 64, 1)
    for i in range(2):
        B.stf(_lh(u + 1, i), mem2)
    y = _b_out_tail(B, u)
    if u == U - 1:
        B.stf(B2 + 64, B.ldf(B2, 64) + y)
    else:
        new = lax.broadcasted_iota(I32, (64, 128), 1) < SEG * (u + 1)
        B.stf(B2, jnp.where(new, y, 0.0) + (B.ldf(B2, 64) if u else 0.0))
        B.stf(B2 + 64, jnp.where(new, 0.0, y) + B.ldf(B2 + 64, 64))


def _kernel(xt_hbm, wqkv_hbm, wo_hbm, mem_hbm, gate_hbm, wq_hbm, wk_hbm, wv_hbm, wot_hbm,
            out_hbm,
            xt, wqkv, wo, mem_ref, gate_ref, raw, wot, a_ref, b_ref, qkv_all, o_all, o_last, ga_all, omg, out_buf,
            offs, sem_in, sem_w, sem_out):
    A, B = _Arena(a_ref), _Arena(b_ref)

    def cols(src, dst, c0, c1, sem):
        return pltpu.make_async_copy(src.at[:, pl.ds(c0, c1 - c0)], dst.at[:, pl.ds(c0, c1 - c0)], sem_in.at[sem])

    x_copy = [cols(xt_hbm, xt, c0, c1, i) for i, (c0, c1) in
              enumerate(((0, 256), (256, 768), (768, S)))]
    w_copy = [cols(wqkv_hbm, wqkv, c0, c1, 3 + i) for i, (c0, c1) in
              enumerate(((512, 896), (896, 1152), (0, 512), (1152, 3 * D)))]
    wo_copy = pltpu.make_async_copy(wo_hbm, wo, sem_in.at[8])
    mem_copy = pltpu.make_async_copy(mem_hbm, mem_ref, sem_in.at[9])
    gate_copy = pltpu.make_async_copy(gate_hbm, gate_ref, sem_in.at[10])

    def rows(r0, r1, sem):
        return [pltpu.make_async_copy(w.at[pl.ds(r0 * H, (r1 - r0) * H)],
                                      raw.at[pl.ds(RAW * m + r0 * H, (r1 - r0) * H)], sem_w.at[sem])
                for m, w in enumerate((wq_hbm, wk_hbm, wv_hbm))]

    tail_copies, main_copies = rows(512, D, 0), rows(0, 512, 1)
    wot_copy = pltpu.make_async_copy(wot_hbm, wot, sem_w.at[2])

    def x_stage(j, slot):
        A.stb(AX + 288 * slot, xt[:, pl.ds(pl.multiple_of(j * 128, 128), 128)])

    def x_transpose(j, n):
        cols = pl.ds(pl.multiple_of(j * 128, 128), 128)
        if n < 4:
            t = xt[128 * n:128 * n + 128, cols]
        else:
            t = jnp.concatenate([xt[512:576, cols]] * 2, 0)
        B.stb(XN + 64 * n, t.T)

    def x_tail(u):
        B.stf(_lh(u, 0) + M, B.ldb(XN + 256 + 16 * u, 16).astype(F32))

    def proj(j):
        if isinstance(j, int):
            return _Arena(qkv_all.at[pl.ds((j + 1) % 5 * SLOT, SLOT)])
        return _Arena(qkv_all.at[pl.ds(pl.multiple_of(offs[lax.rem(j + 1, 5)], 8), SLOT)])

    for c in (w_copy[0], gate_copy, mem_copy, w_copy[1], x_copy[0], w_copy[2], w_copy[3],
              wo_copy):
        c.start()

    for i in range(5):
        offs[i] = i * SLOT
    for i in range(2):
        offs[5 + i] = 512 * H + 32 * H * i
    for i in range(4):
        offs[7 + i] = 128 // NG * H * i
    B.stf(OF + 2 * H * SEG, jnp.zeros((B_ROWS - OF - 2 * H * SEG, 128), F32))
    w_copy[0].wait()
    gate_copy.wait()
    mem_copy.wait()
    gate = jnp.broadcast_to(gate_ref[...].astype(F32)[None, :], (8, D))
    mem0 = mem_ref[...].astype(F32)
    for k in range(4):
        A.stf(GW + 8 * k, gate[:, 128 * k:128 * k + 128])
    A.stf(GW + 32, jnp.concatenate([gate[:, 512:]] * 2, 1))
    _b_place_memory(B, 0, [mem0[:, 128 * k:128 * k + 128] for k in range(4)])
    for i in range(2):
        B.stf(_lh(0, i), jnp.concatenate([mem0[:, 512:]] * 2, 1))

    def project(j, *parts):
        return _a_qkv(A, AX + 288 * j, proj(j), parts, first=j == 0)

    _a_transpose_w(A, wqkv, range(4, 7))
    w_copy[1].wait()
    _a_transpose_w(A, wqkv, range(7, 9))
    x_copy[0].wait()
    x_stage(0, 0)
    x_stage(1, 1)
    _interleave(project(0, 3, 1))
    for n in range(5):
        x_transpose(0, n)
    for u in range(U):
        x_tail(u)
        _b_place_tokens(B, u)
    w_copy[2].wait()
    x_copy[1].start()
    _a_transpose_w(A, wqkv, range(0, 4))
    _interleave(_chain(project(1, 3, 1), project(0, 0)))
    w_copy[3].wait()
    x_copy[2].start()
    _a_transpose_w(A, wqkv, range(9, 14))
    _interleave(_chain(project(1, 0), project(0, 2)))
    wo_copy.wait()
    for c in tail_copies:
        c.start()
    _interleave(project(1, 2), _a_transpose_wo(A, wo))
    qkv_all[AK:AG, :] = jnp.broadcast_to(qkv_all[SLOT + AK:SLOT + AG, :1], (AG - AK, 128))

    def tick_raw(r):
        raw[D * H:RAW, :] = r[:16].astype(BF16)

    def tick_attend(r):
        qkv_all[TICK:TICK + 8, :] = pltpu.bitcast(r[:8], I32)

    def attend(j):
        return _a_attend(j, proj(j), proj(j - 1), o_all.at[j], omg)

    def project_out(j0, n, tick):
        return _chain(*[_a_out(A, o_all.at[j0 + b], ga_all.at[j0 + b], tick) for b in range(n)])

    def attend_trip(t, carry):
        @pl.when(t == 1)
        def _():
            x_copy[2].wait()
            wot_copy.start()

        def project(i):
            return _chain(_a_qkv(A, AX + 288 * i, proj(2 * t + 2 + i)),
                          _once(x_stage, jnp.minimum(2 * t + 4 + i, NB - 1), i))

        _interleave(_chain(project(0), project(1)), _chain(attend(2 * t), attend(2 * t + 1)), span=(-0.04, 0.87))

    x_copy[1].wait()
    for c in main_copies:
        c.start()
    x_stage(2, 0)
    x_stage(3, 1)
    lax.fori_loop(0, NB // 2 - 1, attend_trip, None)

    def last_trip(t, carry):
        src = raw.at[pl.ds(pl.multiple_of(offs[5 + t], 16), 2 * RAW + 32 * H)]
        dst = b_ref.at[pl.ds(pl.multiple_of(t * 16, 16), O2), :]
        _interleave(
            project_out(3 * t, 3, lambda r: (tick_attend(r), tick_raw(r))), _a_attend(NB - 2 + t, proj(NB - 2 + t), proj(NB - 3 + t), o_last.at[t], omg),
            _chain(*[_b_split_heads(src.at[pl.ds(RAW * m, 32 * H)], dst, even, odd) for m, (even, odd) in
                     enumerate(((Q2, Q2 + 32), (K2 + 32, K2), (V2, V2 + 32)))]),
            span=(-0.08, 0.82))

    for c in tail_copies:
        c.wait()
    lax.fori_loop(0, 2, last_trip, None)
    o_all[NB - 2:] = o_last[...]

    def prepare_trip(t, carry):
        n = 64 // NG
        src = raw.at[pl.ds(pl.multiple_of(offs[7 + t], 16), 2 * RAW + (512 - 6 * n) * H)]
        dst = b_ref.at[pl.ds(pl.multiple_of(t * n, n), O2), :]
        _interleave(project_out(6 + 2 * t, 2, tick_raw), _chain(*[
            _b_product_tiles(src.at[pl.ds(RAW * m, (512 - 6 * n) * H)], dst, m * NPR * NC * 64, n)
            for m in range(3)]), span=(-0.04, 0.93))

    for c in main_copies:
        c.wait()
    lax.fori_loop(0, 4, prepare_trip, None)
    wot_copy.wait()
    _interleave(
        _chain(project_out(NB - 2, 2, lambda r: None),
               *[_once(_b_project, B, U - 1, mat, g, 0) for mat in range(3) for g in range(H // NG)]),
        _b_transpose_wo(B, wot))

    def mix(j, n):
        rows = min(128, D - 128 * n)
        bt = B.ldf(BO + 128 * n, 128).T if n < 4 else B.ldf(B2 + 64, 64)
        w = jnp.concatenate([omg[j]] * (rows // 8), 0)
        out_buf[j, 128 * n:128 * n + rows, :] = (
            ga_all[j, 128 * n:128 * n + rows, :] + w * bt).astype(BF16)

    def out_copy(j):
        return pltpu.make_async_copy(
            out_buf.at[j], out_hbm.at[:, pl.ds(pl.multiple_of(j * 128, 128), 128)], sem_out)

    def b_body(g, carry):
        jn, jp = jnp.minimum(g + 1, NB - 1), jnp.maximum(g - 1, 0)
        for u in range(U):
            def before_out():
                for n in {1: range(4), U - 1: (4,)}.get(u, ()):
                    mix(jp, n)

            def after_use():
                if u == 0:
                    for n in range(5):
                        x_transpose(jn, n)
                    _b_place_tokens(B, U - 1)
                if u < U - 1:
                    _b_place_tokens(B, u)
                x_tail(u)

            _b_step(B, u, before_out, after_use)

        @pl.when(g > 0)
        def _():
            out_copy(jp).start()

        return carry

    lax.fori_loop(0, NB, b_body, 0)
    acc = {}
    for g in range(H // NG):
        for p in TURN[1]:
            _b_out_product(B, 0, p, g, acc, 0)
    _b_out_collect(B, 0, acc, 0)
    lane = lax.broadcasted_iota(I32, (64, 128), 1)
    B.stf(B2 + 64, functools.reduce(jnp.add, [B.ldf(B2 + 64, 64)] + [
        jnp.where(lane < SEG * (u + 1), 0.0, _b_out_tail(B, u)) for u in range(U - 1)]))
    for n in range(5):
        mix(NB - 1, n)
    out_copy(NB - 1).start()
    for j in range(NB):
        out_copy(j).wait()


@functools.partial(jax.jit, static_argnames=("B_seg_len",))
def pallas_gated_mix__sliding_local_dilated__memory_aug_recurrent_mem_tr__prompt_kernel(
    A_x: jax.Array,
    A_wqkv: jax.Array,
    A_wo: jax.Array,
    B_x: jax.Array,
    B_mem0: jax.Array,
    B_Wq: jax.Array,
    B_Wk: jax.Array,
    B_Wv: jax.Array,
    B_Wo: jax.Array,
    B_seg_len: int,
    gate_w: jax.Array,
):
    del B_x
    assert A_x.shape == (1, S, D) and B_mem0.shape == (1, M, D) and B_Wq.shape == (D, H, DH)
    assert B_seg_len == SEG
    hbm = pl.BlockSpec(memory_space=pl.ANY)
    out_t = pl.pallas_call(
        _kernel,
        out_shape=jax.ShapeDtypeStruct((D, S), BF16),
        in_specs=[hbm] * 9,
        out_specs=hbm,
        scratch_shapes=[
            pltpu.VMEM((D, S), BF16),
            pltpu.VMEM((D, 3 * D), BF16),
            pltpu.VMEM((D, D), BF16),
            pltpu.VMEM((M, D), BF16),
            pltpu.VMEM((D,), BF16),
            pltpu.VMEM((3 * RAW, DH), BF16),
            pltpu.VMEM((H * D, DH), BF16),
            pltpu.VMEM((A_ROWS, 128), I32),
            pltpu.VMEM((B_ROWS, 128), I32),
            pltpu.VMEM((5 * SLOT, 128), I32),
            pltpu.VMEM((NB, D // 2, 128), I32),
            pltpu.VMEM((2, D // 2, 128), I32),
            pltpu.VMEM((NB, D, 128), F32),
            pltpu.VMEM((NB, 8, 128), F32),
            pltpu.VMEM((NB, D, 128), BF16),
            pltpu.SMEM((11,), I32),
            pltpu.SemaphoreType.DMA((11,)),
            pltpu.SemaphoreType.DMA((3,)),
            pltpu.SemaphoreType.DMA,
        ],
        compiler_params=pltpu.CompilerParams(vmem_limit_bytes=110 * 1024 * 1024),
    )(
        A_x.reshape(S, D).T, A_wqkv, A_wo, B_mem0.reshape(M, D), gate_w,
        B_Wq.reshape(D * H, DH), B_Wk.reshape(D * H, DH), B_Wv.reshape(D * H, DH),
        B_Wo.transpose(0, 2, 1).reshape(H * D, DH),
    )
    return out_t.T.reshape(1, S, D)
```

```python
import functools

import jax
import jax.numpy as jnp
from jax import lax
import jax.experimental.pallas as pl
import jax.experimental.pallas.tpu as pltpu

F32, BF16, I32 = jnp.float32, jnp.bfloat16, jnp.int32

S, D = 2048, 576
NB = S // 128
HA, DA, WIN, DIL = 32, 18, 8, 2
H, DH, M, SEG = 32, 128, 8, 32
L = M + SEG
NP = H // 2
U = 128 // SEG
NEG = -1000000000.0

NG = 4
PRODUCTS = tuple(tuple({(int(t[1]), int(t[2])): int(t[0] + "1") for t in form.split()} for form in p) for p in (
    ("+00 -10", "-03 +30 -10 +00 -02", "+00"),
    ("+10", "+03 -30 +00 -01 -20", "+00 +10"),
    ("+03 -13", "-13 -32 +33", "+03"),
    ("+13", "-23 -31 +33", "+03 +13"),
    ("+02 +10", "-02 +20", "+00 -12"),
    ("+02", "-02 -21 +22 -32", "+02 +12"),
    ("+02 -12", "-12 -20 +22 -23", "-12"),
    ("+00 +02", "+02", "+00 +02"),
    ("+10 +12", "+20", "+10 +12"),
    ("+02 +13", "+23 -32", "+03 -12"),
    ("+02 +03", "+32", "+02 +03"),
    ("+12 +13", "+23", "+12 +13"),
    ("+00 +01 -10", "+03 -30 +10 -01", "+00 +10 +11"),
    ("+01", "+03 -01 +11 -12 -31", "+01"),
    ("+11", "+10 -30 -11 +13 +21", "-11"),
    ("+00 +01", "-03 +01", "+00 +01 +10 +11"),
    ("+11 +12", "+21", "+01 +02 +11 +12"),
    ("-02 +11 +12", "+12 -21", "+01 +02 +12"),
    ("+01 +03", "-03 +31", "+01 +03 +11 +13"),
    ("+10 +11 +13", "+30", "+10 +11 +13"),
    ("+01 +03 -13", "-13 +31", "-03 -11 -13"),
    ("+00 +01 +03", "+03", "+00 +01 +03"),
    ("+00 +01 -10 -11", "+10 -30", "-10 -11"),
    ("+01 +02 -11 -12", "+12", "+01 +02"),
    ("+01 +03 -11 -13", "-30 +13", "-11 -13"),
    ("+01 +03 +10", "-03 +30", "+00 -11 -13"),
))
NPR = len(PRODUCTS)
NC = 4 // NG
TURN = tuple(tuple(p for p, (a, _, c) in enumerate(PRODUCTS)
                   if any(k[0] == r for k in a) and any(k[0] == r for k in c)) for r in range(2))
LONG = tuple(p for p in range(NPR) if len(PRODUCTS[p][1]) == 5)

GSTRIDE = 3 * NPR * NC * 64 + 4
TAIL = H // NG * GSTRIDE
Q2 = TAIL
K2 = Q2 + 64
V2 = K2 + 64
PSTRIDE = 192 + 4
OA = TAIL + NP * PSTRIDE
O2 = OA + H // NG * NPR * NC * 64
O2T = O2 + NP * 64
LH = O2T + H * 32
GS = LH + U * (NG * NG * NC + 2) * 40
TK = GS + 64
MK = TK + 3 * H * 128
VS = MK + H * M
KS = VS + H * 40
RE = KS + NP * 64
PS = RE + H * 40
RS = PS + NP * 40
XN = RS + NP * 40
OM = XN + 320
OF = OM + H * M
BO = OF + (U + 1) * H * SEG
B2 = BO + 512
B_ROWS = B2 + 128

RAW = D * H + 16

WT = 0
GW = WT + 5 * 1728
WP = GW + 40
WOT = WP + 27 * 160
AX = WOT + 5 * 288
SUMS = AX + 2 * 288
A_ROWS = SUMS + 4 * len(LONG)
AQ, AK, AV, AG, TICK, SLOT = 0, 576, 864, 1152, 1160, 1168


def _dot(a, b):
    return lax.dot_general(a, b, (((1,), (0,)), ((), ())), preferred_element_type=F32)


def _dot_nt(a, b):
    return lax.dot_general(a, b, (((1,), (1,)), ((), ())), preferred_element_type=F32)


class _Arena:
    def __init__(self, ref):
        self.r = ref

    def ldi(self, o, n):
        return self.r[o:o + n, :]

    def ldf(self, o, n):
        return pltpu.bitcast(self.r[o:o + n, :], F32)

    def ldb(self, o, n):
        return pltpu.bitcast(self.r[o:o + n, :], BF16)

    def stf(self, o, v):
        self.r[o:o + v.shape[0], :] = pltpu.bitcast(v, I32)

    def stb(self, o, v):
        self.r[o:o + v.shape[0] // 2, :] = pltpu.bitcast(v.astype(BF16), I32)


def _pad2(t, rows, cols):
    r, c = t.shape
    if c < cols:
        t = jnp.concatenate([t, jnp.zeros((r, cols - c), t.dtype)], 1)
    if r < rows:
        t = jnp.concatenate([t, jnp.zeros((rows - r, cols), t.dtype)], 0)
    return t


def _interleave(main, *side, span=(0.0, 0.9)):
    jobs = (main,) + side
    order = [((i + 1) / main[0], 0) for i in range(main[0])]
    order += [(span[0] + (span[1] - span[0]) * i / n, k + 1) for k, (n, _) in enumerate(side) for i in range(n)]
    for _, k in sorted(order):
        next(jobs[k][1])
    for _, gen in jobs:
        assert next(gen, "end") == "end"


def _once(fn, *args):
    def gen():
        fn(*args)
        yield
    return 1, gen()


def _chain(*jobs):
    def gen():
        for _, g in jobs:
            yield from g
    return sum(n for n, _ in jobs), gen()


def _a_transpose_w(A, w_ref, cblocks):
    for c in cblocks:
        nc = min(128, 3 * D - 128 * c)
        for k in range(5):
            nk = min(128, D - 128 * k)
            t = _pad2(w_ref[128 * k:128 * k + nk, 128 * c:128 * c + nc], 128, 128).T
            A.stf(WT + 1728 * k + 128 * c, t[:nc].astype(F32))


def _a_transpose_wo(A, w_ref):
    def gen():
        for c in range(5):
            nc = min(128, D - 128 * c)
            for k in range(5):
                nk = min(128, D - 128 * k)
                t = _pad2(w_ref[128 * k:128 * k + nk, 128 * c:128 * c + nc], 128, 128).T
                A.stb(WOT + 288 * k + 64 * c, t[:nc])
                yield
    return 25, gen()


def _a_qkv(A, x_off, dst, parts=(3, 1, 0, 2), first=False):
    def proj(rows_of_k):
        ch = [rows_of_k(k) for k in range(5)]
        return _dot(jnp.concatenate(ch[:4] + [ch[4][:, :64]], 1), A.ldb(x_off, 288))

    def gen():
        for part in parts:
            if part == 3:
                dst.stf(AG, jax.nn.sigmoid(proj(lambda k: A.ldf(GW + 8 * k, 8))))
                continue
            for d0 in range(0, DA, 2):
                def weights(k):
                    packed = WP + 160 * (9 * part + d0 // 2) + 32 * k
                    if not first:
                        return A.ldb(packed, 32)
                    w = jnp.concatenate([
                        pltpu.bitcast(A.r[pl.ds(WT + 1728 * k + D * part + 8 * DA * hg + d, 8, stride=DA), :], F32)
                        for hg in range(4) for d in (d0, d0 + 1)], 0)
                    A.stb(packed, w)
                    return w

                r = proj(weights)
                for i in range(0, 64, 16):
                    if part == 0:
                        dst.stf(AQ + 32 * d0 + i, r[i:i + 16])
                    else:
                        dst.stb((AK if part == 1 else AV) + 16 * d0 + i // 2, r[i:i + 16])
                    yield
    return sum(2 * DA for p in parts if p < 3), gen()


def _a_attend(j, cur, old, o_ref, omg_ref):
    def window(o):
        lane = lax.broadcasted_iota(I32, (8, 128), 1)
        c, p = cur.ldi(o, 8), old.ldi(o, 8)
        out = []
        for w in range(WIN):
            sh = DIL * w
            t = c if w == 0 else pltpu.roll(jnp.where(lane >= 128 - sh, p, c), sh, 1)
            out.append(pltpu.bitcast(t, BF16).astype(F32))
        return out

    def gen():
        pos = j * 128 + lax.broadcasted_iota(I32, (8, 128), 1)
        for hg in range(4):
            lg = None
            for d in range(0, DA, 2):
                q = cur.ldf(AQ + 32 * d + 16 * hg, 16)
                pr = [q * kw for kw in window(AK + 16 * d + 8 * hg)]
                pr = [t[:8] + t[8:] for t in pr]
                lg = pr if d == 0 else [a + b for a, b in zip(lg, pr)]
                yield
            lg = [jnp.where(pos >= DIL * w, t * DA ** -0.5, NEG) for w, t in enumerate(lg)]
            mx = functools.reduce(jnp.maximum, lg)
            e = [jnp.exp(t - mx) for t in lg]
            g = cur.ldf(AG, 8)
            if hg == 0:
                omg_ref[j] = 1.0 - g
            r = g / functools.reduce(jnp.add, e)
            p = [jnp.concatenate([t * r] * 2, 0) for t in e]
            yield
            for d in range(0, DA, 2):
                o = functools.reduce(jnp.add, [a * b for a, b in zip(p, window(AV + 16 * d + 8 * hg))])
                o = pltpu.bitcast(o.astype(BF16).astype(F32), I32)
                o_ref[pl.ds(4 * DA * hg + d // 2, 8, stride=DA // 2), :] = (
                    lax.shift_right_logical(o[:8], 16) | o[8:])
                yield
    return 4 * DA + 4, gen()


def _a_out(A, o_ref, ga_ref, tick):
    def gen():
        for r0 in range(0, D, 96):
            ch = [A.ldb(WOT + 288 * k + r0 // 2, 48) for k in range(5)]
            r = _dot(jnp.concatenate(ch[:4] + [ch[4][:, :64]], 1), pltpu.bitcast(o_ref[...], BF16))
            for i in range(0, 96, 32):
                tick(r[i:i + 32])
                ga_ref[r0 + i:r0 + i + 32, :] = r[i:i + 32]
                yield
    return D // 32, gen()


def _b_split_heads(raw, dst, even, odd):
    def gen():
        for r in range(raw.shape[0] // 64):
            e = pltpu.bitcast(raw[64 * r:64 * r + 32, :], I32)
            o = pltpu.bitcast(raw[64 * r + 32:64 * r + 64, :], I32)
            dst[pl.ds(even + r, NP, stride=PSTRIDE), :] = (e & 0xFFFF) | (o << 16)
            dst[pl.ds(odd + r, NP, stride=PSTRIDE), :] = lax.shift_right_logical(e, 16) | (o & -65536)
            yield
    return raw.shape[0] // 64, gen()


def _signed_sum(terms):
    sign, acc = terms[0]
    for c, t in terms[1:]:
        if c == sign:
            acc = acc + t
        else:
            sign, acc = 1, acc - t if sign > 0 else t - acc
    return acc if sign > 0 else -acc


def _pairs(g):
    return [g + 8 * i for i in range(NG // 2)]


def _heads(g):
    return [2 * j + i for j in _pairs(g) for i in range(2)]


def _b_sum_matrix():
    g = lax.broadcasted_iota(I32, (8, 128), 0)
    lane = lax.broadcasted_iota(I32, (8, 128), 1)
    return jnp.concatenate([functools.reduce(jnp.add, [
        jnp.where(lane == H * k + _heads(0)[n] + 2 * g, float(c), 0.0) for (k, n), c in PRODUCTS[p][1].items()])
        for p in LONG], 0)


def _b_product_tiles(A, raw, dst, off, rows):
    def gen():
        for r in range(rows):
            t = [jnp.concatenate([raw[o:o + H, :] for o in range(64 * r + H * i, 512 * H, 128 * H)], 0)
                 for i in range(2)]
            long = [_dot(A.ldb(SUMS, 4 * len(LONG)), v) for v in t]
            word = [pltpu.bitcast(v, I32) for v in t]

            def block(k, n, i):
                v = word[i][16 * k + 8 * (n // 2):16 * k + 8 * (n // 2) + 8]
                return pltpu.bitcast(v & -65536 if n % 2 else v << 16, F32)

            for p, (_, w, _) in enumerate(PRODUCTS):
                e, o = [pltpu.bitcast(
                    long[i][8 * LONG.index(p):8 * LONG.index(p) + 8] if p in LONG else
                    _signed_sum([(c, block(k, n, i)) for (k, n), c in w.items()]), I32) for i in range(2)]
                if len(w) > 1:
                    e, o = e + 0x8000, (o + 0x7FFF) & -65536
                dst[pl.ds(off + p * 64 + r, H // NG, stride=GSTRIDE), :] = lax.shift_right_logical(e, 16) | o
            yield
    return rows, gen()


def _b_transpose_wo(B, wot):
    def gen():
        for g in range(H // NG):
            for p, (_, w, _) in enumerate(PRODUCTS):
                for i in range(NC):
                    t = [(c, wot[pl.ds(D * _heads(g)[k] + 128 * (NC * n + i), 128), :]) for (k, n), c in w.items()]
                    if len(t) > 1 or t[0][0] < 0:
                        t = [(1, _signed_sum([(c, v.astype(F32)) for c, v in t]).astype(BF16))]
                    B.stb(OA + ((g * NPR + p) * NC + i) * 64, t[0][1].T)
                    yield
            for j in _pairs(g):
                t = jnp.concatenate([wot[D * h + 512:D * h + D, :] for h in (2 * j, 2 * j + 1)], 0)
                B.stb(O2T + 64 * j, t)
                B.stb(O2 + 64 * j, t.T)
                B.stb(K2 + PSTRIDE * j, B.ldb(K2 + PSTRIDE * j, 64).T)
    return H // NG * NPR * NC, gen()


def _turn(u):
    return 1 - u % 2


def _halves(p, r):
    return (r,) if p in TURN[1 - r] else (0, 1)


def _lh(u, i):
    return LH + 40 * ((NG * NG * NC + 2) * (u % U) + i)


def _b_place_memory(B, u, mem):
    r = _turn(u)
    for i, p in enumerate(TURN[r]):
        for c in range(NC):
            B.stf(_lh(u, 2 + NC * i + c), _signed_sum(
                [(s, mem[NC * k + c]) for (rr, k), s in PRODUCTS[p][0].items() if rr == r]))


def _b_place_tokens(B, u):
    r = _turn(u)
    top = (u + 1 - r) % U

    def x(seg, n, half):
        return B.ldb(XN + 64 * n + 16 * seg + 8 * half, 8).astype(F32)

    for i, p in enumerate(TURN[r]):
        for c in range(NC):
            for at, half in enumerate(_halves(p, r)):
                B.stf(_lh(u, 2 + NC * i + c) + M + 16 * at, _signed_sum(
                    [(s, x(top + rr, NC * k + c, half)) for (rr, k), s in PRODUCTS[p][0].items()]))
    for half in range(2):
        B.stf(_lh(u, 1) + M + 16 * half, x((u + 1) % U, 4, half))


def _b_collect(B, r, ys, m, at, plain=None, keep=()):
    mem, tok, kept = {}, {}, {}
    items = [(PRODUCTS[p][2], _halves(p, r), y) for p, y in zip(TURN[r], ys)]
    if plain:
        items += [({(r, n): 1}, (0, 1), y) for n, y in enumerate(plain)]
    for c, halves, y in items:
        for (rr, n), s in c.items():
            if m and rr == r:
                mem.setdefault(n, []).append((s, y[:m]))
            for i, half in enumerate(halves):
                tok.setdefault((rr, n, half), []).append((s, y[m + 16 * i:m + 16 * i + 16]))
    for (rr, n, half), terms in sorted(tok.items()):
        o = at(rr, n) + 16 * half
        if r == 1 and any((rr, n) in PRODUCTS[p][2] and half in _halves(p, 0) for p in TURN[0]):
            terms.append((1, B.ldf(o, 16)))
        if r == 1 and rr in keep:
            kept[rr, n, half] = _signed_sum(terms)
        else:
            B.stf(o, _signed_sum(terms))
    return [_signed_sum(mem[n]) for n in sorted(mem)], kept


def _b_project(B, u, mat, g, m=M, keep=()):
    r = _turn(u)
    top = (u + 1 - r) % U
    ys = [_dot(jnp.concatenate([B.ldf(_lh(u, 2 + NC * i + c) + M - m, m + 16 * len(_halves(p, r)))
                                for c in range(NC)], 1),
               B.ldb(GSTRIDE * g + (mat * NPR + p) * NC * 64, NC * 64)) for i, p in enumerate(TURN[r])]
    plain = None
    if mat == 0:
        plain = [_dot(B.ldf(_lh(u, 1) + M - m, m + SEG)[:, :64], B.ldb(Q2 + PSTRIDE * (h // 2) + 32 * (h % 2), 32))
                 for h in _heads(g)]
    mem, kept = _b_collect(B, r, ys, m, lambda rr, n: TK + 128 * (H * mat + _heads(g)[n]) + SEG * (top + rr),
                           plain, keep)

    def tokens(n, seg):
        return [kept[seg - top, n, i] if (seg - top, n, i) in kept else
                B.ldf(TK + 128 * (H * mat + _heads(g)[n]) + SEG * seg + 16 * i, 16) for i in range(2)]

    return mem, tokens


def _b_out_product(B, u, p, g, acc, m=M):
    r = _turn(u)
    top = (u - 1 - r) % U
    a = PRODUCTS[p][0].items()
    lhs = [_signed_sum([(s, B.ldf(OM + M * _heads(g)[k], M)) for (rr, k), s in a if rr == r])] if m else []
    both = [k for (rr, k), s in a if rr and PRODUCTS[p][0].get((0, k)) == -s]
    lhs += [_signed_sum([(s, B.ldf(OF + SEG * (H * (U if k in both else top + rr) + _heads(g)[k]) + 16 * half, 16))
                         for (rr, k), s in a if not (rr and k in both)]) for half in _halves(p, r)]
    for c in range(NC):
        y = _dot(jnp.concatenate(lhs, 0), B.ldb(OA + ((g * NPR + p) * NC + c) * 64, 64))
        acc[p, c] = acc[p, c] + y if g else y


def _b_out_collect(B, u, acc, m=M):
    r = _turn(u)
    top = (u - 1 - r) % U
    mem = [_b_collect(B, r, [acc[p, c] for p in TURN[r]], m,
                      lambda rr, n: BO + 128 * (NC * n + c) + SEG * (top + rr))[0] for c in range(NC)]
    return [mem[c][n] for n in range(NG) for c in range(NC)] if m else None


def _b_out_tail(B, u):
    return functools.reduce(jnp.add, [
        _dot_nt(B.ldb(O2T + 32 * h, 32),
                jnp.concatenate([B.ldf(OF + SEG * (H * i + h), SEG) for i in range(U)], 0).astype(BF16))
        for h in range(8 * u, 8 * u + 8)])


def _b_step(B, u, before_out, after_use):
    row = lax.broadcasted_iota(I32, (L, 128), 0)
    lane = lax.broadcasted_iota(I32, (L, 128), 1)
    lo = lane < 64
    lo64 = lax.broadcasted_iota(I32, (64, 128), 1) < 64
    mask = (row < M) | ((lane & 63) >= SEG) | (row - M >= (lane & 63))
    in_a, in_b = lane < L, (lane >= 64) & (lane < 64 + L)
    z24 = jnp.zeros((24, 128), F32)
    z8 = jnp.zeros((8, 128), F32)
    pair = [j for g in range(H // NG) for j in _pairs(g)]

    def h2():
        return jnp.concatenate([B.ldf(_lh(u, 0) + M, SEG), B.ldf(_lh(u, 0), M)], 0)

    def t_q(g):
        for h, t in zip(_heads(g), _b_project(B, u, 0, g)[0]):
            B.stf(MK + M * h, t)

    def t_g():
        c4 = h2()
        B.stb(GS, jnp.concatenate([jnp.where(lo, 0.0, c4), z24, jnp.where(lo, c4, 0.0), z24], 0))

    def t_k(g):
        mem, tokens = _b_project(B, u, 1, g, keep=(0,))
        for i, j in enumerate(_pairs(g)):
            k = jnp.concatenate([t for n in (2 * i, 2 * i + 1) for t in tokens(n, u) + [mem[n], z24]], 0)
            B.stb(KS + 64 * j, k.astype(BF16).T)

    def t_s(i):
        j = pair[i]
        kt, w2 = B.ldi(KS + 64 * j, 64), B.ldi(K2 + PSTRIDE * j, 64)
        for b, rhs in enumerate((jnp.where(lo64, kt, w2), jnp.where(lo64, w2, kt))):
            q = jnp.concatenate([B.ldf(MK + M * (2 * j + b), M), B.ldf(TK + 128 * (2 * j + b) + SEG * u, SEG)], 0)
            B.stf(RE + 40 * (NP * b + i), _dot(q, pltpu.bitcast(rhs, BF16)))

    def t_s2(n):
        c4 = h2()
        a, b = B.ldf(RE + 128 * n, 128), B.ldf(RE + 40 * NP + 128 * n, 128)
        t = jnp.where(lax.broadcasted_iota(I32, (128, 128), 1) < 64, b, a).astype(BF16)
        y = _dot_nt(jnp.concatenate([jnp.where(lo, 0.0, c4), jnp.where(lo, c4, 0.0)], 0), t)
        B.stf(RS + 128 * n, jnp.concatenate([y[:L], z24, y[L:], z24], 0).T)
        for i in range(128 * n // L, 128 * (n + 1) // L):
            softmax(i)

    def softmax(i):
        s = jnp.where(lo, B.ldf(RE + 40 * i, 40), B.ldf(RE + 40 * (NP + i), 40)) + B.ldf(RS + 40 * i, 40)
        s = jnp.where(mask, s * DH ** -0.5, NEG)
        B.stf(RS + 40 * i, s)
        ma = jnp.max(jnp.where(in_a, s, -jnp.inf), axis=1, keepdims=True)
        mb = jnp.max(jnp.where(in_b, s, -jnp.inf), axis=1, keepdims=True)
        e = jnp.exp(B.ldf(RS + 40 * i, 40) - jnp.where(lo, ma, mb))
        B.stf(PS + 40 * i, jnp.where(in_a | in_b, e, 0.0))

    def t_r(i):
        B.stf(RS + 40 * i, _dot(B.ldf(PS + 40 * i, 40), B.ldb(GS, 64)))

    def t_v(g):
        mem, tokens = _b_project(B, u, 2, g, keep=(0, 1))
        for n, h in enumerate(_heads(g)):
            B.stb(VS + 40 * h + 32, jnp.concatenate([mem[n], z8], 0))
            if _turn(u):
                B.stb(VS + 40 * h, jnp.concatenate(tokens(n, u) + tokens(n, u + 1), 0))

    def t_pv(i):
        p, r = B.ldf(PS + 40 * i, 40), B.ldf(RS + 40 * i, 40)
        for b, (lhs, keys) in enumerate(((jnp.where(lo, p, r), in_a), (jnp.where(lo, r, p), in_b))):
            h = 2 * pair[i] + b
            l = jnp.sum(jnp.where(keys, p, 0.0), axis=1, keepdims=True)
            l = jnp.broadcast_to(l, (L, 128))
            rc = pltpu.reciprocal(l, approx=True)
            v = [B.ldi(VS + 40 * h + 16 * (u % 2), 16), B.ldi(VS + 40 * h + 32, 8), jnp.zeros((8, 128), I32)]
            w2 = [B.ldi(V2 + PSTRIDE * pair[i] + 32 * b, 32)]
            o = _dot(lhs, pltpu.bitcast(jnp.concatenate(w2 + v if b else v + w2, 0), BF16)) * (rc * (2.0 - l * rc))
            B.stf(OM + M * h, o[:M])
            B.stf(OF + SEG * (H * u + h), o[M:])
            if u % 2:
                B.stf(OF + SEG * (H * U + h), B.ldf(OF + SEG * (H * (u - 1) + h), SEG) - o[M:])

    acc = {}

    def t_m(i):
        y = _dot(B.ldf(OM + 2 * M * pair[i], 2 * M), B.ldb(O2 + 64 * pair[i], 64))
        acc["tail"] = acc["tail"] + y if i else y

    lag_s, lag_s2 = 2, 4
    prods = TURN[_turn(u)]
    for g in range(8):
        t_k(g)
    t_g()
    s2_after = [(128 * n + 127) // L + lag_s + lag_s2 for n in range(5)]
    for i in range(2 * NP - 2):
        if i % 2 == 0:
            t_q(i // 2) if i < NP else t_v((i - NP) // 2)
        if 0 <= i - lag_s < NP:
            t_s(i - lag_s)
        if i in s2_after:
            t_s2(s2_after.index(i))
        if i >= 2 * NP - 6:
            for b in range(4):
                t_r(4 * (i - (2 * NP - 6)) + b)
    before_out()
    passes = ((0, 2, 5, 1, 7), (3, 4, 10, 6), (8, 9, 12, 11), (13, 15, 14))
    for g in range(10):
        if g < 8:
            t_pv(2 * g)
            t_pv(2 * g + 1)
        if g == 1:
            t_v(7)
        if g >= 2:
            for i in passes[0]:
                _b_out_product(B, u, prods[i], g - 2, acc)
            t_m(g - 2)
    after_use()
    for k in range(1, len(passes)):
        for g in range(8):
            for i in passes[k]:
                _b_out_product(B, u, prods[i], g, acc)
            if k == 1:
                t_m(8 + g)
    _b_place_memory(B, u + 1, _b_out_collect(B, u, acc))
    mem2 = jnp.where(lo[:M], acc["tail"][:M], acc["tail"][M:])
    mem2 = mem2 + pltpu.roll(mem2, 64, 1)
    for i in range(2):
        B.stf(_lh(u + 1, i), mem2)
    y = _b_out_tail(B, u)
    if u == U - 1:
        B.stf(B2 + 64, B.ldf(B2, 64) + y)
    else:
        new = lax.broadcasted_iota(I32, (64, 128), 1) < SEG * (u + 1)
        B.stf(B2, jnp.where(new, y, 0.0) + (B.ldf(B2, 64) if u else 0.0))
        B.stf(B2 + 64, jnp.where(new, 0.0, y) + B.ldf(B2 + 64, 64))


def _kernel(xt_hbm, wqkv_hbm, wo_hbm, mem_hbm, gate_hbm, wq_hbm, wk_hbm, wv_hbm, wot_hbm,
            out_hbm,
            xt, wqkv, wo, mem_ref, gate_ref, raw, wot, a_ref, b_ref, qkv_all, o_all, o_last, ga_all, omg, out_buf,
            offs, sem_in, sem_w, sem_out):
    A, B = _Arena(a_ref), _Arena(b_ref)

    def cols(src, dst, c0, c1, sem):
        return pltpu.make_async_copy(src.at[:, pl.ds(c0, c1 - c0)], dst.at[:, pl.ds(c0, c1 - c0)], sem_in.at[sem])

    x_copy = [cols(xt_hbm, xt, c0, c1, i) for i, (c0, c1) in
              enumerate(((0, 256), (256, 768), (768, S)))]
    w_copy = [cols(wqkv_hbm, wqkv, c0, c1, 3 + i) for i, (c0, c1) in
              enumerate(((512, 896), (896, 1152), (0, 512), (1152, 3 * D)))]
    wo_copy = pltpu.make_async_copy(wo_hbm, wo, sem_in.at[8])
    mem_copy = pltpu.make_async_copy(mem_hbm, mem_ref, sem_in.at[9])
    gate_copy = pltpu.make_async_copy(gate_hbm, gate_ref, sem_in.at[10])

    def rows(r0, r1, sem):
        return [pltpu.make_async_copy(w.at[pl.ds(r0 * H, (r1 - r0) * H)],
                                      raw.at[pl.ds(RAW * m + r0 * H, (r1 - r0) * H)], sem_w.at[sem])
                for m, w in enumerate((wq_hbm, wk_hbm, wv_hbm))]

    tail_copies, main_copies = rows(512, D, 0), rows(0, 512, 1)
    wot_copy = pltpu.make_async_copy(wot_hbm, wot, sem_w.at[2])

    def x_stage(j, slot):
        A.stb(AX + 288 * slot, xt[:, pl.ds(pl.multiple_of(j * 128, 128), 128)])

    def x_transpose(j, n):
        cols = pl.ds(pl.multiple_of(j * 128, 128), 128)
        if n < 4:
            t = xt[128 * n:128 * n + 128, cols]
        else:
            t = jnp.concatenate([xt[512:576, cols]] * 2, 0)
        B.stb(XN + 64 * n, t.T)

    def x_tail(u):
        B.stf(_lh(u, 0) + M, B.ldb(XN + 256 + 16 * u, 16).astype(F32))

    def proj(j):
        if isinstance(j, int):
            return _Arena(qkv_all.at[pl.ds((j + 1) % 5 * SLOT, SLOT)])
        return _Arena(qkv_all.at[pl.ds(pl.multiple_of(offs[lax.rem(j + 1, 5)], 8), SLOT)])

    for c in (w_copy[0], gate_copy, mem_copy, w_copy[1], x_copy[0], w_copy[2], w_copy[3],
              wo_copy):
        c.start()

    for i in range(5):
        offs[i] = i * SLOT
    for i in range(2):
        offs[5 + i] = 512 * H + 32 * H * i
    for i in range(4):
        offs[7 + i] = 128 // NG * H * i
    A.stb(SUMS, _b_sum_matrix())
    B.stf(OF + H * SEG, jnp.zeros((B_ROWS - OF - H * SEG, 128), F32))
    w_copy[0].wait()
    gate_copy.wait()
    mem_copy.wait()
    gate = jnp.broadcast_to(gate_ref[...].astype(F32)[None, :], (8, D))
    mem0 = mem_ref[...].astype(F32)
    for k in range(4):
        A.stf(GW + 8 * k, gate[:, 128 * k:128 * k + 128])
    A.stf(GW + 32, jnp.concatenate([gate[:, 512:]] * 2, 1))
    _b_place_memory(B, 0, [mem0[:, 128 * k:128 * k + 128] for k in range(4)])
    for i in range(2):
        B.stf(_lh(0, i), jnp.concatenate([mem0[:, 512:]] * 2, 1))

    def project(j, *parts):
        return _a_qkv(A, AX + 288 * j, proj(j), parts, first=j == 0)

    _a_transpose_w(A, wqkv, range(4, 7))
    w_copy[1].wait()
    _a_transpose_w(A, wqkv, range(7, 9))
    x_copy[0].wait()
    x_stage(0, 0)
    x_stage(1, 1)
    _interleave(project(0, 3, 1))
    for n in range(5):
        x_transpose(0, n)
    for u in range(U):
        x_tail(u)
        _b_place_tokens(B, u)
    w_copy[2].wait()
    x_copy[1].start()
    _a_transpose_w(A, wqkv, range(0, 4))
    _interleave(_chain(project(1, 3, 1), project(0, 0)))
    w_copy[3].wait()
    x_copy[2].start()
    _a_transpose_w(A, wqkv, range(9, 14))
    _interleave(_chain(project(1, 0), project(0, 2)))
    wo_copy.wait()
    for c in tail_copies:
        c.start()
    _interleave(project(1, 2), _a_transpose_wo(A, wo))
    qkv_all[AK:AG, :] = jnp.broadcast_to(qkv_all[SLOT + AK:SLOT + AG, :1], (AG - AK, 128))

    def tick_raw(r):
        raw[D * H:RAW, :] = r[:16].astype(BF16)

    def tick_attend(r):
        qkv_all[TICK:TICK + 8, :] = pltpu.bitcast(r[:8], I32)

    def attend(j):
        return _a_attend(j, proj(j), proj(j - 1), o_all.at[j], omg)

    def project_out(j0, n, tick):
        return _chain(*[_a_out(A, o_all.at[j0 + b], ga_all.at[j0 + b], tick) for b in range(n)])

    def attend_trip(t, carry):
        @pl.when(t == 1)
        def _():
            x_copy[2].wait()
            wot_copy.start()

        def project(i):
            return _chain(_a_qkv(A, AX + 288 * i, proj(2 * t + 2 + i)),
                          _once(x_stage, jnp.minimum(2 * t + 4 + i, NB - 1), i))

        _interleave(_chain(project(0), project(1)), _chain(attend(2 * t), attend(2 * t + 1)), span=(-0.04, 0.87))

    x_copy[1].wait()
    for c in main_copies:
        c.start()
    x_stage(2, 0)
    x_stage(3, 1)
    lax.fori_loop(0, NB // 2 - 1, attend_trip, None)

    def last_trip(t, carry):
        src = raw.at[pl.ds(pl.multiple_of(offs[5 + t], 16), 2 * RAW + 32 * H)]
        dst = b_ref.at[pl.ds(pl.multiple_of(t * 16, 16), O2), :]
        _interleave(
            project_out(3 * t, 3, lambda r: (tick_attend(r), tick_raw(r))), _a_attend(NB - 2 + t, proj(NB - 2 + t), proj(NB - 3 + t), o_last.at[t], omg),
            _chain(*[_b_split_heads(src.at[pl.ds(RAW * m, 32 * H)], dst, even, odd) for m, (even, odd) in
                     enumerate(((Q2, Q2 + 32), (K2 + 32, K2), (V2, V2 + 32)))]),
            span=(-0.08, 0.82))

    for c in tail_copies:
        c.wait()
    lax.fori_loop(0, 2, last_trip, None)
    o_all[NB - 2:] = o_last[...]

    def prepare_trip(t, carry):
        n = 64 // NG
        src = raw.at[pl.ds(pl.multiple_of(offs[7 + t], 16), 2 * RAW + (512 - 6 * n) * H)]
        dst = b_ref.at[pl.ds(pl.multiple_of(t * n, n), O2), :]
        _interleave(project_out(6 + 2 * t, 2, lambda r: None), _chain(*[
            _b_product_tiles(A, src.at[pl.ds(RAW * m, (512 - 6 * n) * H)], dst, m * NPR * NC * 64, n)
            for m in range(3)]), span=(-0.04, 0.93))

    for c in main_copies:
        c.wait()
    lax.fori_loop(0, 4, prepare_trip, None)
    wot_copy.wait()
    _interleave(
        _chain(project_out(NB - 2, 2, lambda r: None),
               *[_once(_b_project, B, U - 1, mat, g, 0) for mat in range(3) for g in range(H // NG)]),
        _b_transpose_wo(B, wot))

    def mix(j, n):
        rows = min(128, D - 128 * n)
        bt = B.ldf(BO + 128 * n, 128).T if n < 4 else B.ldf(B2 + 64, 64)
        w = jnp.concatenate([omg[j]] * (rows // 8), 0)
        out_buf[j, 128 * n:128 * n + rows, :] = (
            ga_all[j, 128 * n:128 * n + rows, :] + w * bt).astype(BF16)

    def out_copy(j):
        return pltpu.make_async_copy(
            out_buf.at[j], out_hbm.at[:, pl.ds(pl.multiple_of(j * 128, 128), 128)], sem_out)

    def b_body(g, carry):
        jn, jp = jnp.minimum(g + 1, NB - 1), jnp.maximum(g - 1, 0)
        for u in range(U):
            def before_out():
                for n in {1: range(4), U - 1: (4,)}.get(u, ()):
                    mix(jp, n)

            def after_use():
                if u == 0:
                    for n in range(5):
                        x_transpose(jn, n)
                    _b_place_tokens(B, U - 1)
                if u < U - 1:
                    _b_place_tokens(B, u)
                x_tail(u)

            _b_step(B, u, before_out, after_use)

        @pl.when(g > 0)
        def _():
            out_copy(jp).start()

        return carry

    lax.fori_loop(0, NB, b_body, 0)
    acc = {}
    for g in range(H // NG):
        for p in TURN[1]:
            _b_out_product(B, 0, p, g, acc, 0)
    _b_out_collect(B, 0, acc, 0)
    lane = lax.broadcasted_iota(I32, (64, 128), 1)
    B.stf(B2 + 64, functools.reduce(jnp.add, [B.ldf(B2 + 64, 64)] + [
        jnp.where(lane < SEG * (u + 1), 0.0, _b_out_tail(B, u)) for u in range(U - 1)]))
    for n in range(5):
        mix(NB - 1, n)
    out_copy(NB - 1).start()
    for j in range(NB):
        out_copy(j).wait()


@functools.partial(jax.jit, static_argnames=("B_seg_len",))
def pallas_gated_mix__sliding_local_dilated__memory_aug_recurrent_mem_tr__prompt_kernel(
    A_x: jax.Array,
    A_wqkv: jax.Array,
    A_wo: jax.Array,
    B_x: jax.Array,
    B_mem0: jax.Array,
    B_Wq: jax.Array,
    B_Wk: jax.Array,
    B_Wv: jax.Array,
    B_Wo: jax.Array,
    B_seg_len: int,
    gate_w: jax.Array,
):
    del B_x
    assert A_x.shape == (1, S, D) and B_mem0.shape == (1, M, D) and B_Wq.shape == (D, H, DH)
    assert B_seg_len == SEG
    hbm = pl.BlockSpec(memory_space=pl.ANY)
    out_t = pl.pallas_call(
        _kernel,
        out_shape=jax.ShapeDtypeStruct((D, S), BF16),
        in_specs=[hbm] * 9,
        out_specs=hbm,
        scratch_shapes=[
            pltpu.VMEM((D, S), BF16),
            pltpu.VMEM((D, 3 * D), BF16),
            pltpu.VMEM((D, D), BF16),
            pltpu.VMEM((M, D), BF16),
            pltpu.VMEM((D,), BF16),
            pltpu.VMEM((3 * RAW, DH), BF16),
            pltpu.VMEM((H * D, DH), BF16),
            pltpu.VMEM((A_ROWS, 128), I32),
            pltpu.VMEM((B_ROWS, 128), I32),
            pltpu.VMEM((5 * SLOT, 128), I32),
            pltpu.VMEM((NB, D // 2, 128), I32),
            pltpu.VMEM((2, D // 2, 128), I32),
            pltpu.VMEM((NB, D, 128), F32),
            pltpu.VMEM((NB, 8, 128), F32),
            pltpu.VMEM((NB, D, 128), BF16),
            pltpu.SMEM((11,), I32),
            pltpu.SemaphoreType.DMA((11,)),
            pltpu.SemaphoreType.DMA((3,)),
            pltpu.SemaphoreType.DMA,
        ],
        compiler_params=pltpu.CompilerParams(vmem_limit_bytes=110 * 1024 * 1024),
    )(
        A_x.reshape(S, D).T, A_wqkv, A_wo, B_mem0.reshape(M, D), gate_w,
        B_Wq.reshape(D * H, DH), B_Wk.reshape(D * H, DH), B_Wv.reshape(D * H, DH),
        B_Wo.transpose(0, 2, 1).reshape(H * D, DH),
    )
    return out_t.T.reshape(1, S, D)
```

```python
import functools

import jax
import jax.numpy as jnp
from jax import lax
import jax.experimental.pallas as pl
import jax.experimental.pallas.tpu as pltpu

F32, BF16, I32 = jnp.float32, jnp.bfloat16, jnp.int32

S, D = 2048, 576
NB = S // 128
HA, DA, WIN, DIL = 32, 18, 8, 2
H, DH, M, SEG = 32, 128, 8, 32
L = M + SEG
NP = H // 2
U = 128 // SEG
NEG = -1000000000.0

NG = 4
PRODUCTS = tuple(tuple({(int(t[1]), int(t[2])): int(t[0] + "1") for t in form.split()} for form in p) for p in (
    ("+00 -10", "-03 +30 -10 +00 -02", "+00"),
    ("+10", "+03 -30 +00 -01 -20", "+00 +10"),
    ("+03 -13", "-13 -32 +33", "+03"),
    ("+13", "-23 -31 +33", "+03 +13"),
    ("+02 +10", "-02 +20", "+00 -12"),
    ("+02", "-02 -21 +22 -32", "+02 +12"),
    ("+02 -12", "-12 -20 +22 -23", "-12"),
    ("+00 +02", "+02", "+00 +02"),
    ("+10 +12", "+20", "+10 +12"),
    ("+02 +13", "+23 -32", "+03 -12"),
    ("+02 +03", "+32", "+02 +03"),
    ("+12 +13", "+23", "+12 +13"),
    ("+00 +01 -10", "+03 -30 +10 -01", "+00 +10 +11"),
    ("+01", "+03 -01 +11 -12 -31", "+01"),
    ("+11", "+10 -30 -11 +13 +21", "-11"),
    ("+00 +01", "-03 +01", "+00 +01 +10 +11"),
    ("+11 +12", "+21", "+01 +02 +11 +12"),
    ("-02 +11 +12", "+12 -21", "+01 +02 +12"),
    ("+01 +03", "-03 +31", "+01 +03 +11 +13"),
    ("+10 +11 +13", "+30", "+10 +11 +13"),
    ("+01 +03 -13", "-13 +31", "-03 -11 -13"),
    ("+00 +01 +03", "+03", "+00 +01 +03"),
    ("+00 +01 -10 -11", "+10 -30", "-10 -11"),
    ("+01 +02 -11 -12", "+12", "+01 +02"),
    ("+01 +03 -11 -13", "-30 +13", "-11 -13"),
    ("+01 +03 +10", "-03 +30", "+00 -11 -13"),
))
NPR = len(PRODUCTS)
NC = 4 // NG
TURN = tuple(tuple(p for p, (a, _, c) in enumerate(PRODUCTS)
                   if any(k[0] == r for k in a) and any(k[0] == r for k in c)) for r in range(2))
LONG = tuple(p for p in range(NPR) if len(PRODUCTS[p][1]) == 5)

GSTRIDE = 3 * NPR * NC * 64 + 4
TAIL = H // NG * GSTRIDE
Q2 = TAIL
K2 = Q2 + 64
V2 = K2 + 64
PSTRIDE = 192 + 4
OA = TAIL + NP * PSTRIDE
O2 = OA + H // NG * NPR * NC * 64
O2T = O2 + NP * 64
LH = O2T + H * 32
GS = LH + U * (NG * NG * NC + 2) * 40
TK = GS + 64
MK = TK + 3 * H * 128
VS = MK + H * M
KS = VS + H * 40
RE = KS + NP * 64
PS = RE + H * 40
RS = PS + NP * 40
AC = RS + NP * 40
XN = AC + NPR * SEG
OM = XN + 320
OF = OM + H * M
BO = OF + (U + 1) * H * SEG
B2 = BO + 512
B_ROWS = B2 + 64 * (U + 1)

RAW = D * H + 16

WT = 0
GW = WT + 5 * 1728
WP = GW + 40
WOT = WP + 27 * 160
AX = WOT + 5 * 288
SUMS = AX + 2 * 288
A_ROWS = SUMS + 4 * len(LONG)
AQ, AK, AV, AG, TICK, SLOT = 0, 576, 864, 1152, 1160, 1168


def _dot(a, b):
    return lax.dot_general(a, b, (((1,), (0,)), ((), ())), preferred_element_type=F32)


def _dot_nt(a, b):
    return lax.dot_general(a, b, (((1,), (1,)), ((), ())), preferred_element_type=F32)


class _Arena:
    def __init__(self, ref):
        self.r = ref

    def ldi(self, o, n):
        return self.r[o:o + n, :]

    def ldf(self, o, n):
        return pltpu.bitcast(self.r[o:o + n, :], F32)

    def ldb(self, o, n):
        return pltpu.bitcast(self.r[o:o + n, :], BF16)

    def stf(self, o, v):
        self.r[o:o + v.shape[0], :] = pltpu.bitcast(v, I32)

    def stb(self, o, v):
        self.r[o:o + v.shape[0] // 2, :] = pltpu.bitcast(v.astype(BF16), I32)


def _pad2(t, rows, cols):
    r, c = t.shape
    if c < cols:
        t = jnp.concatenate([t, jnp.zeros((r, cols - c), t.dtype)], 1)
    if r < rows:
        t = jnp.concatenate([t, jnp.zeros((rows - r, cols), t.dtype)], 0)
    return t


def _interleave(main, *side, span=(0.0, 0.9)):
    jobs = (main,) + side
    order = [((i + 1) / main[0], 0) for i in range(main[0])]
    order += [(span[0] + (span[1] - span[0]) * i / n, k + 1) for k, (n, _) in enumerate(side) for i in range(n)]
    for _, k in sorted(order):
        next(jobs[k][1])
    for _, gen in jobs:
        assert next(gen, "end") == "end"


def _once(fn, *args):
    def gen():
        fn(*args)
        yield
    return 1, gen()


def _chain(*jobs):
    def gen():
        for _, g in jobs:
            yield from g
    return sum(n for n, _ in jobs), gen()


def _a_transpose_w(A, w_ref, cblocks):
    for c in cblocks:
        nc = min(128, 3 * D - 128 * c)
        for k in range(5):
            nk = min(128, D - 128 * k)
            t = _pad2(w_ref[128 * k:128 * k + nk, 128 * c:128 * c + nc], 128, 128).T
            A.stf(WT + 1728 * k + 128 * c, t[:nc].astype(F32))


def _a_transpose_wo(A, w_ref):
    def gen():
        for c in range(5):
            nc = min(128, D - 128 * c)
            for k in range(5):
                nk = min(128, D - 128 * k)
                t = _pad2(w_ref[128 * k:128 * k + nk, 128 * c:128 * c + nc], 128, 128).T
                A.stb(WOT + 288 * k + 64 * c, t[:nc])
                yield
    return 25, gen()


def _a_qkv(A, x_off, dst, parts=(3, 1, 0, 2), first=False):
    def proj(rows_of_k):
        ch = [rows_of_k(k) for k in range(5)]
        return _dot(jnp.concatenate(ch[:4] + [ch[4][:, :64]], 1), A.ldb(x_off, 288))

    def gen():
        for part in parts:
            if part == 3:
                dst.stf(AG, jax.nn.sigmoid(proj(lambda k: A.ldf(GW + 8 * k, 8))))
                continue
            for d0 in range(0, DA, 2):
                def weights(k):
                    packed = WP + 160 * (9 * part + d0 // 2) + 32 * k
                    if not first:
                        return A.ldb(packed, 32)
                    w = jnp.concatenate([
                        pltpu.bitcast(A.r[pl.ds(WT + 1728 * k + D * part + 8 * DA * hg + d, 8, stride=DA), :], F32)
                        for hg in range(4) for d in (d0, d0 + 1)], 0)
                    A.stb(packed, w)
                    return w

                r = proj(weights)
                for i in range(0, 64, 16):
                    if part == 0:
                        dst.stf(AQ + 32 * d0 + i, r[i:i + 16])
                    else:
                        dst.stb((AK if part == 1 else AV) + 16 * d0 + i // 2, r[i:i + 16])
                    yield
    return sum(2 * DA for p in parts if p < 3), gen()


def _a_attend(j, cur, old, o_ref, omg_ref):
    def window(o):
        lane = lax.broadcasted_iota(I32, (8, 128), 1)
        c, p = cur.ldi(o, 8), old.ldi(o, 8)
        out = []
        for w in range(WIN):
            sh = DIL * w
            t = c if w == 0 else pltpu.roll(jnp.where(lane >= 128 - sh, p, c), sh, 1)
            out.append(pltpu.bitcast(t, BF16).astype(F32))
        return out

    def gen():
        pos = j * 128 + lax.broadcasted_iota(I32, (8, 128), 1)
        for hg in range(4):
            lg = None
            for d in range(0, DA, 2):
                q = cur.ldf(AQ + 32 * d + 16 * hg, 16)
                pr = [q * kw for kw in window(AK + 16 * d + 8 * hg)]
                pr = [t[:8] + t[8:] for t in pr]
                lg = pr if d == 0 else [a + b for a, b in zip(lg, pr)]
                yield
            lg = [jnp.where(pos >= DIL * w, t * DA ** -0.5, NEG) for w, t in enumerate(lg)]
            mx = functools.reduce(jnp.maximum, lg)
            e = [jnp.exp(t - mx) for t in lg]
            g = cur.ldf(AG, 8)
            if hg == 0:
                omg_ref[j] = 1.0 - g
            r = g / functools.reduce(jnp.add, e)
            p = [jnp.concatenate([t * r] * 2, 0) for t in e]
            yield
            for d in range(0, DA, 2):
                o = functools.reduce(jnp.add, [a * b for a, b in zip(p, window(AV + 16 * d + 8 * hg))])
                o = pltpu.bitcast(o.astype(BF16).astype(F32), I32)
                o_ref[pl.ds(4 * DA * hg + d // 2, 8, stride=DA // 2), :] = (
                    lax.shift_right_logical(o[:8], 16) | o[8:])
                yield
    return 4 * DA + 4, gen()


def _a_out(A, o_ref, ga_ref, tick):
    def gen():
        for r0 in range(0, D, 96):
            ch = [A.ldb(WOT + 288 * k + r0 // 2, 48) for k in range(5)]
            r = _dot(jnp.concatenate(ch[:4] + [ch[4][:, :64]], 1), pltpu.bitcast(o_ref[...], BF16))
            for i in range(0, 96, 32):
                tick(r[i:i + 32])
                ga_ref[r0 + i:r0 + i + 32, :] = r[i:i + 32]
                yield
    return D // 32, gen()


def _b_split_heads(raw, dst, even, odd):
    def gen():
        for r in range(raw.shape[0] // 64):
            e = pltpu.bitcast(raw[64 * r:64 * r + 32, :], I32)
            o = pltpu.bitcast(raw[64 * r + 32:64 * r + 64, :], I32)
            dst[pl.ds(even + r, NP, stride=PSTRIDE), :] = (e & 0xFFFF) | (o << 16)
            dst[pl.ds(odd + r, NP, stride=PSTRIDE), :] = lax.shift_right_logical(e, 16) | (o & -65536)
            yield
    return raw.shape[0] // 64, gen()


def _signed_sum(terms):
    sign, acc = terms[0]
    for c, t in terms[1:]:
        if c == sign:
            acc = acc + t
        else:
            sign, acc = 1, acc - t if sign > 0 else t - acc
    return acc if sign > 0 else -acc


def _pairs(g):
    return [g + 8 * i for i in range(NG // 2)]


def _heads(g):
    return [2 * j + i for j in _pairs(g) for i in range(2)]


def _b_sum_matrix():
    g = lax.broadcasted_iota(I32, (8, 128), 0)
    lane = lax.broadcasted_iota(I32, (8, 128), 1)
    return jnp.concatenate([functools.reduce(jnp.add, [
        jnp.where(lane == H * k + _heads(0)[n] + 2 * g, float(c), 0.0) for (k, n), c in PRODUCTS[p][1].items()])
        for p in LONG], 0)


def _b_product_tiles(A, raw, dst, off, rows):
    def gen():
        for r in range(rows):
            t = [jnp.concatenate([raw[o:o + H, :] for o in range(64 * r + H * i, 512 * H, 128 * H)], 0)
                 for i in range(2)]
            long = [_dot(A.ldb(SUMS, 4 * len(LONG)), v) for v in t]
            word = [pltpu.bitcast(v, I32) for v in t]

            def block(k, n, i):
                v = word[i][16 * k + 8 * (n // 2):16 * k + 8 * (n // 2) + 8]
                return pltpu.bitcast(v & -65536 if n % 2 else v << 16, F32)

            for p, (_, w, _) in enumerate(PRODUCTS):
                e, o = [pltpu.bitcast(
                    long[i][8 * LONG.index(p):8 * LONG.index(p) + 8] if p in LONG else
                    _signed_sum([(c, block(k, n, i)) for (k, n), c in w.items()]), I32) for i in range(2)]
                if len(w) > 1:
                    e, o = e + 0x8000, (o + 0x7FFF) & -65536
                dst[pl.ds(off + p * 64 + r, H // NG, stride=GSTRIDE), :] = lax.shift_right_logical(e, 16) | o
            yield
    return rows, gen()


def _b_transpose_wo(B, wot):
    def gen():
        for g in range(H // NG):
            for p, (_, w, _) in enumerate(PRODUCTS):
                for i in range(NC):
                    t = [(c, wot[pl.ds(D * _heads(g)[k] + 128 * (NC * n + i), 128), :]) for (k, n), c in w.items()]
                    if len(t) > 1 or t[0][0] < 0:
                        t = [(1, _signed_sum([(c, v.astype(F32)) for c, v in t]).astype(BF16))]
                    B.stb(OA + ((g * NPR + p) * NC + i) * 64, t[0][1].T)
                    yield
            for j in _pairs(g):
                t = jnp.concatenate([wot[D * h + 512:D * h + D, :] for h in (2 * j, 2 * j + 1)], 0)
                B.stb(O2T + 64 * j, t)
                B.stb(O2 + 64 * j, t.T)
                B.stb(K2 + PSTRIDE * j, B.ldb(K2 + PSTRIDE * j, 64).T)
    return H // NG * NPR * NC, gen()


def _turn(u):
    return 1 - u % 2


def _halves(p, r):
    return (r,) if p in TURN[1 - r] else (0, 1)


def _lh(u, i):
    return LH + 40 * ((NG * NG * NC + 2) * (u % U) + i)


def _b_place_memory(B, u, mem):
    r = _turn(u)
    for i, p in enumerate(TURN[r]):
        for c in range(NC):
            B.stf(_lh(u, 2 + NC * i + c), _signed_sum(
                [(s, mem[NC * k + c]) for (rr, k), s in PRODUCTS[p][0].items() if rr == r]))


def _b_place_tokens(B, u):
    r = _turn(u)
    top = (u + 1 - r) % U

    def x(seg, n, half):
        return B.ldb(XN + 64 * n + 16 * seg + 8 * half, 8).astype(F32)

    for i, p in enumerate(TURN[r]):
        for c in range(NC):
            for at, half in enumerate(_halves(p, r)):
                B.stf(_lh(u, 2 + NC * i + c) + M + 16 * at, _signed_sum(
                    [(s, x(top + rr, NC * k + c, half)) for (rr, k), s in PRODUCTS[p][0].items()]))
    for half in range(2):
        B.stf(_lh(u, 1) + M + 16 * half, x((u + 1) % U, 4, half))


def _b_collect(B, r, ys, m, at, plain=None, keep=()):
    mem, tok, kept = {}, {}, {}
    items = [(PRODUCTS[p][2], _halves(p, r), y) for p, y in ys]
    if plain:
        items += [({(r, n): 1}, (0, 1), y) for n, y in enumerate(plain)]
    for c, halves, y in items:
        for (rr, n), s in c.items():
            if m and rr == r:
                mem.setdefault(n, []).append((s, y[:m]))
            for i, half in enumerate(halves):
                tok.setdefault((rr, n, half), []).append((s, y[m + 16 * i:m + 16 * i + 16]))
    for (rr, n, half), terms in sorted(tok.items()):
        o = at(rr, n) + 16 * half
        if r == 1 and any((rr, n) in PRODUCTS[p][2] and half in _halves(p, 0) for p in TURN[0]):
            terms.append((1, B.ldf(o, 16)))
        if r == 1 and rr in keep:
            kept[rr, n, half] = _signed_sum(terms)
        else:
            B.stf(o, _signed_sum(terms))
    return [_signed_sum(mem[n]) for n in sorted(mem)], kept


def _b_project(B, u, mat, g, m=M, keep=()):
    r = _turn(u)
    top = (u + 1 - r) % U
    order = ((2, 9, 5, 10, 17, 23, 7, 4, 21, 20, 18, 25, 15, 13, 12, 0), (17, 16, 14, 4, 1, 22, 12, 8, 19, 25, 24, 20, 11, 3, 9, 6))[r]
    ys = [_dot(jnp.concatenate([B.ldf(_lh(u, 2 + NC * i + c) + M - m, m + 16 * len(_halves(p, r)))
                                for c in range(NC)], 1),
               B.ldb(GSTRIDE * g + (mat * NPR + p) * NC * 64, NC * 64)) for i, p in ((TURN[r].index(p), p) for p in order)]
    plain = None
    if mat == 0:
        plain = [_dot(B.ldf(_lh(u, 1) + M - m, m + SEG)[:, :64], B.ldb(Q2 + PSTRIDE * (h // 2) + 32 * (h % 2), 32))
                 for h in _heads(g)]
    mem, kept = _b_collect(B, r, zip(order, ys), m, lambda rr, n: TK + 128 * (H * mat + _heads(g)[n]) + SEG * (top + rr),
                           plain, keep)

    def tokens(n, seg):
        return [kept[seg - top, n, i] if (seg - top, n, i) in kept else
                B.ldf(TK + 128 * (H * mat + _heads(g)[n]) + SEG * seg + 16 * i, 16) for i in range(2)]

    return mem, tokens


def _b_out_product(B, u, p, g, acc, m=M):
    r = _turn(u)
    top = (u - 1 - r) % U
    a = PRODUCTS[p][0].items()
    lhs = [_signed_sum([(s, B.ldf(OM + M * _heads(g)[k], M)) for (rr, k), s in a if rr == r])] if m else []
    both = [k for (rr, k), s in a if rr and PRODUCTS[p][0].get((0, k)) == -s]
    lhs += [_signed_sum([(s, B.ldf(OF + SEG * (H * (U if k in both else top + rr) + _heads(g)[k]) + 16 * half, 16))
                         for (rr, k), s in a if not (rr and k in both)]) for half in _halves(p, r)]
    y = _dot(jnp.concatenate(lhs, 0), B.ldb(OA + (g * NPR + p) * 64, 64))
    acc[p] = acc[p] + y if g else y
    if g == H // NG - 1:
        B.stf(AC + SEG * p + 16 * _halves(p, r)[0], acc[p][m:])
        for (rr, n), s in PRODUCTS[p][2].items():
            if m and rr == r:
                acc.setdefault(("mem", n), []).append((s, acc[p][:m]))


def _b_out_collect(B, u):
    for rr in range(2):
        for n in range(NG):
            B.stf(BO + 128 * n + SEG * ((u - 2 + rr) % U), _signed_sum(
                [(c[rr, n], B.ldf(AC + SEG * p, SEG)) for p, (_, _, c) in enumerate(PRODUCTS) if (rr, n) in c]))


def _b_out_tail(B, u):
    return functools.reduce(jnp.add, [
        _dot_nt(B.ldb(O2T + 32 * h, 32),
                jnp.concatenate([B.ldf(OF + SEG * (H * i + h), SEG) for i in range(U)], 0).astype(BF16))
        for h in range(8 * u, 8 * u + 8)])


def _b_step(B, u, emit, after_use):
    row = lax.broadcasted_iota(I32, (L, 128), 0)
    lane = lax.broadcasted_iota(I32, (L, 128), 1)
    lo = lane < 64
    lo64 = lax.broadcasted_iota(I32, (64, 128), 1) < 64
    mask = (row < M) | ((lane & 63) >= SEG) | (row - M >= (lane & 63))
    in_a, in_b = lane < L, (lane >= 64) & (lane < 64 + L)
    z24 = jnp.zeros((24, 128), F32)
    z8 = jnp.zeros((8, 128), F32)
    pair = [j for g in range(H // NG) for j in _pairs(g)]

    def h2():
        return jnp.concatenate([B.ldf(_lh(u, 0) + M, SEG), B.ldf(_lh(u, 0), M)], 0)

    def t_q(g):
        for h, t in zip(_heads(g), _b_project(B, u, 0, g)[0]):
            B.stf(MK + M * h, t)

    def t_g():
        c4 = h2()
        B.stb(GS, jnp.concatenate([jnp.where(lo, 0.0, c4), z24, jnp.where(lo, c4, 0.0), z24], 0))

    def t_k(g):
        mem, tokens = _b_project(B, u, 1, g, keep=(0,))
        for i, j in enumerate(_pairs(g)):
            k = jnp.concatenate([t for n in (2 * i, 2 * i + 1) for t in tokens(n, u) + [mem[n], z24]], 0)
            B.stb(KS + 64 * j, k.astype(BF16).T)

    def t_s(i):
        j = pair[i]
        kt, w2 = B.ldi(KS + 64 * j, 64), B.ldi(K2 + PSTRIDE * j, 64)
        ya, yb = [_dot(jnp.concatenate([B.ldf(MK + M * h, M), B.ldf(TK + 128 * h + SEG * u, SEG)], 0),
                       pltpu.bitcast(rhs, BF16))
                  for h, rhs in ((2 * j, jnp.where(lo64, kt, w2)), (2 * j + 1, jnp.where(lo64, w2, kt)))]
        B.stf(RE + L * i, jnp.where(lo, ya, yb))
        B.stf(RE + L * (NP + i), jnp.where(lo, yb, ya))

    def t_s2(n):
        c4 = h2()
        y = _dot_nt(jnp.concatenate([jnp.where(lo, 0.0, c4), jnp.where(lo, c4, 0.0)], 0),
                    B.ldf(RE + L * NP + 128 * n, 128).astype(BF16))
        B.stf(RS + 128 * n, jnp.concatenate([y[:L], z24, y[L:], z24], 0).T)
        for i in range(128 * n // L, 128 * (n + 1) // L):
            s = jnp.where(mask, (B.ldf(RE + L * i, L) + B.ldf(RS + L * i, L)) * DH ** -0.5, NEG)
            ma = jnp.max(jnp.where(in_a, s, -jnp.inf), axis=1, keepdims=True)
            mb = jnp.max(jnp.where(in_b, s, -jnp.inf), axis=1, keepdims=True)
            e = jnp.exp(s - jnp.where(lo, ma, mb))
            B.stf(PS + L * i, jnp.where(in_a | in_b, e, 0.0))

    def t_r(i):
        B.stf(RS + 40 * i, _dot(B.ldf(PS + 40 * i, 40), B.ldb(GS, 64)))

    def t_v(g):
        mem, tokens = _b_project(B, u, 2, g, keep=(0, 1))
        for n, h in enumerate(_heads(g)):
            B.stb(VS + 40 * h + 32, jnp.concatenate([mem[n], z8], 0))
            if _turn(u):
                B.stb(VS + 40 * h, jnp.concatenate(tokens(n, u) + tokens(n, u + 1), 0))

    def t_pv(i):
        p, r = B.ldf(PS + 40 * i, 40), B.ldf(RS + 40 * i, 40)
        for b, lhs in enumerate((jnp.where(lo, p, r), jnp.where(lo, r, p))):
            h = 2 * pair[i] + b
            v = [B.ldi(VS + 40 * h + 16 * (u % 2), 16), B.ldi(VS + 40 * h + 32, 8), jnp.zeros((8, 128), I32)]
            w2 = [B.ldi(V2 + PSTRIDE * pair[i] + 32 * b, 32)]
            o = _dot(lhs, pltpu.bitcast(jnp.concatenate(w2 + v if b else v + w2, 0), BF16))
            l = jnp.broadcast_to(jnp.sum(jnp.where(in_b if b else in_a, p, 0.0), axis=1, keepdims=True), (L, 128))
            rc = pltpu.reciprocal(l, approx=True)
            o = o * (rc * (2.0 - l * rc))
            B.stf(OM + M * h, o[:M])
            B.stf(OF + SEG * (H * u + h), o[M:])
            if u % 2:
                B.stf(OF + SEG * (H * U + h), B.ldf(OF + SEG * (H * (u - 1) + h), SEG) - o[M:])

    acc = {}

    def t_m(i):
        y = _dot(B.ldf(OM + 2 * M * pair[i], 2 * M), B.ldb(O2 + 64 * pair[i], 64))
        acc["tail"] = acc["tail"] + y if i else y

    lag_s, lag_s2 = 2, 4
    prods = TURN[_turn(u)]
    for g in range(8):
        t_k(g)
        if g == 1 and u % 2:
            _b_out_collect(B, u - 1)
    t_g()
    s2_after = [(128 * n + 127) // L + lag_s + lag_s2 for n in range(5)]
    for i in range(2 * NP - 2):
        if i % 2 == 0:
            t_q(i // 2) if i < NP else t_v((i - NP) // 2)
        if 0 <= i - lag_s < NP:
            t_s(i - lag_s)
        if i in (2, 6):
            emit(i // 4)
        if i in s2_after:
            t_s2(s2_after.index(i))
        if i >= 2 * NP - 6:
            for b in range(4):
                t_r(4 * (i - (2 * NP - 6)) + b)
    passes = ((2, 5, 0, 7, 10), (1, 3, 4, 6), (8, 9, 12, 11), (13, 15, 14))
    for g in range(10):
        if g < 8:
            t_pv(2 * g)
            t_pv(2 * g + 1)
        if g == 1:
            t_v(7)
        if g >= 2:
            for i in passes[0]:
                _b_out_product(B, u, prods[i], g - 2, acc)
            t_m(g - 2)
    after_use()
    for k in range(1, len(passes)):
        for g in range(8):
            for i in passes[k]:
                _b_out_product(B, u, prods[i], g, acc)
            if k == 1:
                t_m(8 + g)
    _b_place_memory(B, u + 1, [_signed_sum(acc["mem", n]) for n in range(NG)])
    mem2 = jnp.where(lo[:M], acc["tail"][:M], acc["tail"][M:])
    mem2 = mem2 + pltpu.roll(mem2, 64, 1)
    for i in range(2):
        B.stf(_lh(u + 1, i), mem2)
    B.stf(B2 + 64 * u, _b_out_tail(B, u))


def _kernel(xt_hbm, wqkv_hbm, wo_hbm, mem_hbm, gate_hbm, wq_hbm, wk_hbm, wv_hbm, wot_hbm,
            out_hbm,
            xt, wqkv, wo, mem_ref, gate_ref, raw, wot, a_ref, b_ref, qkv_all, o_all, o_last, ga_all, omg, out_buf,
            offs, sem_in, sem_w, sem_out):
    A, B = _Arena(a_ref), _Arena(b_ref)

    def cols(src, dst, c0, c1, sem):
        return pltpu.make_async_copy(src.at[:, pl.ds(c0, c1 - c0)], dst.at[:, pl.ds(c0, c1 - c0)], sem_in.at[sem])

    x_copy = [cols(xt_hbm, xt, c0, c1, i) for i, (c0, c1) in
              enumerate(((0, 256), (256, 768), (768, S)))]
    w_copy = [cols(wqkv_hbm, wqkv, c0, c1, 3 + i) for i, (c0, c1) in
              enumerate(((512, 896), (896, 1152), (0, 512), (1152, 3 * D)))]
    wo_copy = pltpu.make_async_copy(wo_hbm, wo, sem_in.at[8])
    mem_copy = pltpu.make_async_copy(mem_hbm, mem_ref, sem_in.at[9])
    gate_copy = pltpu.make_async_copy(gate_hbm, gate_ref, sem_in.at[10])

    def rows(r0, r1, sem):
        return [pltpu.make_async_copy(w.at[pl.ds(r0 * H, (r1 - r0) * H)],
                                      raw.at[pl.ds(RAW * m + r0 * H, (r1 - r0) * H)], sem_w.at[sem])
                for m, w in enumerate((wq_hbm, wk_hbm, wv_hbm))]

    tail_copies, main_copies = rows(512, D, 0), rows(0, 512, 1)
    wot_copy = pltpu.make_async_copy(wot_hbm, wot, sem_w.at[2])

    def x_stage(j, slot):
        A.stb(AX + 288 * slot, xt[:, pl.ds(pl.multiple_of(j * 128, 128), 128)])

    def x_transpose(j, n):
        cols = pl.ds(pl.multiple_of(j * 128, 128), 128)
        if n < 4:
            t = xt[128 * n:128 * n + 128, cols]
        else:
            t = jnp.concatenate([xt[512:576, cols]] * 2, 0)
        B.stb(XN + 64 * n, t.T)

    def x_tail(u):
        B.stf(_lh(u, 0) + M, B.ldb(XN + 256 + 16 * u, 16).astype(F32))

    def proj(j):
        if isinstance(j, int):
            return _Arena(qkv_all.at[pl.ds((j + 1) % 5 * SLOT, SLOT)])
        return _Arena(qkv_all.at[pl.ds(pl.multiple_of(offs[lax.rem(j + 1, 5)], 8), SLOT)])

    for c in (w_copy[0], gate_copy, mem_copy, w_copy[1], x_copy[0], w_copy[2], w_copy[3],
              wo_copy):
        c.start()

    for i in range(5):
        offs[i] = i * SLOT
    for i in range(2):
        offs[5 + i] = 512 * H + 32 * H * i
    for i in range(4):
        offs[7 + i] = 128 // NG * H * i
    A.stb(SUMS, _b_sum_matrix())
    B.stf(OF + H * SEG, jnp.zeros((B_ROWS - OF - H * SEG, 128), F32))
    B.stf(AC, jnp.zeros((NPR * SEG, 128), F32))
    w_copy[0].wait()
    gate_copy.wait()
    mem_copy.wait()
    gate = jnp.broadcast_to(gate_ref[...].astype(F32)[None, :], (8, D))
    mem0 = mem_ref[...].astype(F32)
    for k in range(4):
        A.stf(GW + 8 * k, gate[:, 128 * k:128 * k + 128])
    A.stf(GW + 32, jnp.concatenate([gate[:, 512:]] * 2, 1))
    _b_place_memory(B, 0, [mem0[:, 128 * k:128 * k + 128] for k in range(4)])
    for i in range(2):
        B.stf(_lh(0, i), jnp.concatenate([mem0[:, 512:]] * 2, 1))

    def project(j, *parts):
        return _a_qkv(A, AX + 288 * j, proj(j), parts, first=j == 0)

    _a_transpose_w(A, wqkv, range(4, 7))
    w_copy[1].wait()
    _a_transpose_w(A, wqkv, range(7, 9))
    x_copy[0].wait()
    x_stage(0, 0)
    x_stage(1, 1)
    _interleave(project(0, 3, 1))
    for n in range(5):
        x_transpose(0, n)
    for u in range(U):
        x_tail(u)
        _b_place_tokens(B, u)
    for n in range(5):
        x_transpose(1, n)
    w_copy[2].wait()
    x_copy[1].start()
    _a_transpose_w(A, wqkv, range(0, 4))
    _interleave(_chain(project(1, 3, 1), project(0, 0)))
    w_copy[3].wait()
    x_copy[2].start()
    _a_transpose_w(A, wqkv, range(9, 14))
    _interleave(_chain(project(1, 0), project(0, 2)))
    wo_copy.wait()
    for c in tail_copies:
        c.start()
    _interleave(project(1, 2), _a_transpose_wo(A, wo))
    qkv_all[AK:AG, :] = jnp.broadcast_to(qkv_all[SLOT + AK:SLOT + AG, :1], (AG - AK, 128))

    def tick_raw(r):
        raw[D * H:RAW, :] = r[:16].astype(BF16)

    def tick_attend(r):
        qkv_all[TICK:TICK + 8, :] = pltpu.bitcast(r[:8], I32)

    def attend(j):
        return _a_attend(j, proj(j), proj(j - 1), o_all.at[j], omg)

    def project_out(j0, n, tick):
        return _chain(*[_a_out(A, o_all.at[j0 + b], ga_all.at[j0 + b], tick) for b in range(n)])

    def attend_trip(t, carry):
        @pl.when(t == 1)
        def _():
            x_copy[2].wait()
            wot_copy.start()

        def project(i):
            return _chain(_a_qkv(A, AX + 288 * i, proj(2 * t + 2 + i)),
                          _once(x_stage, jnp.minimum(2 * t + 4 + i, NB - 1), i))

        _interleave(_chain(project(0), project(1)), _chain(attend(2 * t), attend(2 * t + 1)), span=(-0.04, 0.87))

    x_copy[1].wait()
    for c in main_copies:
        c.start()
    x_stage(2, 0)
    x_stage(3, 1)
    lax.fori_loop(0, NB // 2 - 1, attend_trip, None)

    def last_trip(t, carry):
        src = raw.at[pl.ds(pl.multiple_of(offs[5 + t], 16), 2 * RAW + 32 * H)]
        dst = b_ref.at[pl.ds(pl.multiple_of(t * 16, 16), O2), :]
        _interleave(
            project_out(3 * t, 3, lambda r: (tick_attend(r), tick_raw(r))), _a_attend(NB - 2 + t, proj(NB - 2 + t), proj(NB - 3 + t), o_last.at[t], omg),
            _chain(*[_b_split_heads(src.at[pl.ds(RAW * m, 32 * H)], dst, even, odd) for m, (even, odd) in
                     enumerate(((Q2, Q2 + 32), (K2 + 32, K2), (V2, V2 + 32)))]),
            span=(-0.08, 0.82))

    for c in tail_copies:
        c.wait()
    lax.fori_loop(0, 2, last_trip, None)
    o_all[NB - 2:] = o_last[...]

    def prepare_trip(t, carry):
        n = 64 // NG
        src = raw.at[pl.ds(pl.multiple_of(offs[7 + t], 16), 2 * RAW + (512 - 6 * n) * H)]
        dst = b_ref.at[pl.ds(pl.multiple_of(t * n, n), O2), :]
        _interleave(project_out(6 + 2 * t, 2, lambda r: None), _chain(*[
            _b_product_tiles(A, src.at[pl.ds(RAW * m, (512 - 6 * n) * H)], dst, m * NPR * NC * 64, n)
            for m in range(3)]), span=(-0.04, 0.93))

    for c in main_copies:
        c.wait()
    lax.fori_loop(0, 4, prepare_trip, None)
    wot_copy.wait()
    _interleave(
        _chain(project_out(NB - 2, 2, lambda r: None),
               *[_once(_b_project, B, U - 1, mat, g, 0) for mat in range(3) for g in range(H // NG)]),
        _b_transpose_wo(B, wot))

    def tail_sum(last, first_steps):
        lane = lax.broadcasted_iota(I32, (64, 128), 1)
        return functools.reduce(jnp.add, [B.ldf(B2 + 64 * last, 64)] + [
            jnp.where(lane < SEG * (u + 1) if first_steps else lane >= SEG * (u + 1), B.ldf(B2 + 64 * u, 64), 0.0)
            for u in range(U - 1)])

    def b_transpose(n):
        B.stf(PS + 128 * n, B.ldf(BO + 128 * n, 128).T)

    def mix(j, n):
        rows = min(128, D - 128 * n)
        bt = B.ldf(PS + 128 * n, 128) if n < 4 else tail_sum(U, False)
        w = jnp.concatenate([omg[j]] * (rows // 8), 0)
        out_buf[j, 128 * n:128 * n + rows, :] = (
            ga_all[j, 128 * n:128 * n + rows, :] + w * bt).astype(BF16)

    def out_copy(j):
        return pltpu.make_async_copy(
            out_buf.at[j], out_hbm.at[:, pl.ds(pl.multiple_of(j * 128, 128), 128)], sem_out)

    def b_body(g, carry):
        jn, jp = jnp.minimum(g + 2, NB - 1), jnp.maximum(g - 1, 0)
        B.stf(B2 + 64 * U, tail_sum(U - 1, True))
        for u in range(U):
            def emit(stage):
                for n in {1: range(4), U - 1: (4,)}.get(u, ()):
                    if stage:
                        mix(jp, n)
                    elif n < 4:
                        b_transpose(n)

            def after_use():
                x_tail(u)
                if u == 0:
                    _b_place_tokens(B, U - 1)
                if u < U - 1:
                    _b_place_tokens(B, u)
                else:
                    for n in range(5):
                        x_transpose(jn, n)

            _b_step(B, u, emit, after_use)

        @pl.when(g > 0)
        def _():
            out_copy(jp).start()

        return carry

    lax.fori_loop(0, NB, b_body, 0)
    acc = {}
    for g in range(H // NG):
        for p in TURN[1]:
            _b_out_product(B, 0, p, g, acc, 0)
    _b_out_collect(B, 0)
    B.stf(B2 + 64 * U, tail_sum(U - 1, True))
    for u in range(U - 1):
        B.stf(B2 + 64 * u, _b_out_tail(B, u))
    for n in range(5):
        if n < 4:
            b_transpose(n)
        mix(NB - 1, n)
    out_copy(NB - 1).start()
    for j in range(NB):
        out_copy(j).wait()


@functools.partial(jax.jit, static_argnames=("B_seg_len",))
def pallas_gated_mix__sliding_local_dilated__memory_aug_recurrent_mem_tr__prompt_kernel(
    A_x: jax.Array,
    A_wqkv: jax.Array,
    A_wo: jax.Array,
    B_x: jax.Array,
    B_mem0: jax.Array,
    B_Wq: jax.Array,
    B_Wk: jax.Array,
    B_Wv: jax.Array,
    B_Wo: jax.Array,
    B_seg_len: int,
    gate_w: jax.Array,
):
    del B_x
    assert A_x.shape == (1, S, D) and B_mem0.shape == (1, M, D) and B_Wq.shape == (D, H, DH)
    assert B_seg_len == SEG
    hbm = pl.BlockSpec(memory_space=pl.ANY)
    out_t = pl.pallas_call(
        _kernel,
        out_shape=jax.ShapeDtypeStruct((D, S), BF16),
        in_specs=[hbm] * 9,
        out_specs=hbm,
        scratch_shapes=[
            pltpu.VMEM((D, S), BF16),
            pltpu.VMEM((D, 3 * D), BF16),
            pltpu.VMEM((D, D), BF16),
            pltpu.VMEM((M, D), BF16),
            pltpu.VMEM((D,), BF16),
            pltpu.VMEM((3 * RAW, DH), BF16),
            pltpu.VMEM((H * D, DH), BF16),
            pltpu.VMEM((A_ROWS, 128), I32),
            pltpu.VMEM((B_ROWS, 128), I32),
            pltpu.VMEM((5 * SLOT, 128), I32),
            pltpu.VMEM((NB, D // 2, 128), I32),
            pltpu.VMEM((2, D // 2, 128), I32),
            pltpu.VMEM((NB, D, 128), F32),
            pltpu.VMEM((NB, 8, 128), F32),
            pltpu.VMEM((NB, D, 128), BF16),
            pltpu.SMEM((11,), I32),
            pltpu.SemaphoreType.DMA((11,)),
            pltpu.SemaphoreType.DMA((3,)),
            pltpu.SemaphoreType.DMA,
        ],
        compiler_params=pltpu.CompilerParams(vmem_limit_bytes=110 * 1024 * 1024),
    )(
        A_x.reshape(S, D).T, A_wqkv, A_wo, B_mem0.reshape(M, D), gate_w,
        B_Wq.reshape(D * H, DH), B_Wk.reshape(D * H, DH), B_Wv.reshape(D * H, DH),
        B_Wo.transpose(0, 2, 1).reshape(H * D, DH),
    )
    return out_t.T.reshape(1, S, D)
```

```python
import functools

import jax
import jax.numpy as jnp
import numpy as np
from jax import lax
import jax.experimental.pallas as pl
import jax.experimental.pallas.tpu as pltpu

F32, BF16, I32 = jnp.float32, jnp.bfloat16, jnp.int32

S, D = 2048, 576
NB = S // 128
DA, WIN, DIL = 18, 8, 2
H, DH, M, SEG = 32, 128, 8, 32
L = M + SEG
NP = H // 2
NG = H // 4
U = 128 // SEG
NEG = -1000000000.0

PRODUCTS = tuple(tuple({(int(t[1]), int(t[2])): int(t[0] + "1") for t in form.split()} for form in p) for p in (
    ("+00 -10", "-03 +30 -10 +00 -02", "+00"),
    ("+10", "+03 -30 +00 -01 -20", "+00 +10"),
    ("+03 -13", "-13 -32 +33", "+03"),
    ("+13", "-23 -31 +33", "+03 +13"),
    ("+02 +10", "-02 +20", "+00 -12"),
    ("+02", "-02 -21 +22 -32", "+02 +12"),
    ("+02 -12", "-12 -20 +22 -23", "-12"),
    ("+00 +02", "+02", "+00 +02"),
    ("+10 +12", "+20", "+10 +12"),
    ("+02 +13", "+23 -32", "+03 -12"),
    ("+02 +03", "+32", "+02 +03"),
    ("+12 +13", "+23", "+12 +13"),
    ("+00 +01 -10", "+03 -30 +10 -01", "+00 +10 +11"),
    ("+01", "+03 -01 +11 -12 -31", "+01"),
    ("+11", "+10 -30 -11 +13 +21", "-11"),
    ("+00 +01", "-03 +01", "+00 +01 +10 +11"),
    ("+11 +12", "+21", "+01 +02 +11 +12"),
    ("-02 +11 +12", "+12 -21", "+01 +02 +12"),
    ("+01 +03", "-03 +31", "+01 +03 +11 +13"),
    ("+10 +11 +13", "+30", "+10 +11 +13"),
    ("+01 +03 -13", "-13 +31", "-03 -11 -13"),
    ("+00 +01 +03", "+03", "+00 +01 +03"),
    ("+00 +01 -10 -11", "+10 -30", "-10 -11"),
    ("+01 +02 -11 -12", "+12", "+01 +02"),
    ("+01 +03 -11 -13", "-30 +13", "-11 -13"),
    ("+01 +03 +10", "-03 +30", "+00 -11 -13"),
))
NPR = len(PRODUCTS)
TURN = tuple(tuple(p for p, (a, _, c) in enumerate(PRODUCTS)
                   if any(k[0] == r for k in a) and any(k[0] == r for k in c)) for r in range(2))
ORDER = ((2, 9, 5, 10, 17, 23, 7, 4, 21, 20, 18, 25, 15, 13, 12, 0),
         (17, 16, 14, 4, 1, 22, 12, 8, 19, 25, 24, 20, 11, 3, 9, 6))
LONG = tuple(p for p in range(NPR) if len(PRODUCTS[p][1]) == 5)


def _is_matrix_product():
    t = np.zeros((2, 4, 4, 4, 2, 4), int)
    for a, w, c in PRODUCTS:
        for i in a:
            for j in w:
                for k in c:
                    t[i + j + k] += a[i] * w[j] * c[k]
    return (t == np.einsum("rs,kl,nm->rklnsm", np.eye(2), np.eye(4), np.eye(4))).all()


assert _is_matrix_product() and len(set(TURN[0] + TURN[1])) == NPR
assert all(sorted(ORDER[r]) == list(TURN[r]) for r in range(2))

GSTRIDE = 3 * NPR * 64 + 4
Q2 = NG * GSTRIDE
K2 = Q2 + 64
V2 = K2 + 64
PSTRIDE = 192 + 4
OA = Q2 + NP * PSTRIDE
O2 = OA + NG * NPR * 64
O2T = O2 + NP * 64
LH = O2T + H * 32
GS = LH + U * 18 * L
TK = GS + 64
MQ = TK + 3 * H * 128
VS = MQ + H * M
KS = VS + H * 40
RE = KS + NP * 64
PS = RE + H * L
RS = PS + NP * L
AC = RS + NP * L
XN = AC + NPR * SEG
OM = XN + 320
OF = OM + H * M
BO = OF + (U + 1) * H * SEG
B2 = BO + 512
B_ROWS = B2 + 64 * (U + 1)

RAW = D * H + 16

WT = 0
GW = WT + 5 * 1728
WP = GW + 40
WOT = WP + 27 * 160
AX = WOT + 5 * 288
SUMS = AX + 2 * 288
A_ROWS = SUMS + 4 * len(LONG)
AQ, AK, AV, AG, TICK, SLOT = 0, 576, 864, 1152, 1160, 1168


def _dot(a, b):
    return lax.dot_general(a, b, (((1,), (0,)), ((), ())), preferred_element_type=F32)


def _dot_nt(a, b):
    return lax.dot_general(a, b, (((1,), (1,)), ((), ())), preferred_element_type=F32)


class _Arena:
    def __init__(self, ref):
        self.r = ref

    def ldi(self, o, n):
        return self.r[o:o + n, :]

    def ldf(self, o, n):
        return pltpu.bitcast(self.r[o:o + n, :], F32)

    def ldb(self, o, n):
        return pltpu.bitcast(self.r[o:o + n, :], BF16)

    def stf(self, o, v):
        self.r[o:o + v.shape[0], :] = pltpu.bitcast(v, I32)

    def stb(self, o, v):
        self.r[o:o + v.shape[0] // 2, :] = pltpu.bitcast(v.astype(BF16), I32)


def _signed_sum(terms):
    sign, acc = terms[0]
    for c, t in terms[1:]:
        if c == sign:
            acc = acc + t
        else:
            sign, acc = 1, acc - t if sign > 0 else t - acc
    return acc if sign > 0 else -acc


def _interleave(main, *side, span=(0.0, 0.9)):
    jobs = (main,) + side
    order = [((i + 1) / main[0], 0) for i in range(main[0])]
    order += [(span[0] + (span[1] - span[0]) * i / n, k + 1) for k, (n, _) in enumerate(side) for i in range(n)]
    for _, k in sorted(order):
        next(jobs[k][1])
    for _, gen in jobs:
        assert next(gen, "end") == "end"


def _once(fn, *args):
    def gen():
        fn(*args)
        yield
    return 1, gen()


def _chain(*jobs):
    def gen():
        for _, g in jobs:
            yield from g
    return sum(n for n, _ in jobs), gen()


def _tile_t(w_ref, k, c):
    t = w_ref[128 * k:min(128 * k + 128, w_ref.shape[0]), 128 * c:min(128 * c + 128, w_ref.shape[1])]
    nk, nc = t.shape
    if nc < 128:
        t = jnp.concatenate([t, jnp.zeros((nk, 128 - nc), t.dtype)], 1)
    if nk < 128:
        t = jnp.concatenate([t, jnp.zeros((128 - nk, 128), t.dtype)], 0)
    return t.T[:nc]


def _a_transpose_w(A, w_ref, cblocks):
    for c in cblocks:
        for k in range(5):
            A.stf(WT + 1728 * k + 128 * c, _tile_t(w_ref, k, c).astype(F32))


def _a_transpose_wo(A, w_ref):
    for c in range(5):
        for k in range(5):
            A.stb(WOT + 288 * k + 64 * c, _tile_t(w_ref, k, c))


def _cat576(chunk):
    ch = [chunk(k) for k in range(5)]
    return jnp.concatenate(ch[:4] + [ch[4][:, :64]], 1)


def _a_qkv(A, x_off, dst, parts=(3, 1, 0, 2), first=False):
    def gen():
        for part in parts:
            if part == 3:
                dst.stf(AG, jax.nn.sigmoid(_dot(_cat576(lambda k: A.ldf(GW + 8 * k, 8)), A.ldb(x_off, 288))))
                continue
            for d0 in range(0, DA, 2):
                def weights(k):
                    packed = WP + 160 * (9 * part + d0 // 2) + 32 * k
                    if not first:
                        return A.ldb(packed, 32)
                    w = jnp.concatenate([
                        pltpu.bitcast(A.r[pl.ds(WT + 1728 * k + D * part + 8 * DA * hg + d, 8, stride=DA), :], F32)
                        for hg in range(4) for d in (d0, d0 + 1)], 0)
                    A.stb(packed, w)
                    return w

                r = _dot(_cat576(weights), A.ldb(x_off, 288))
                for i in range(0, 64, 16):
                    if part == 0:
                        dst.stf(AQ + 32 * d0 + i, r[i:i + 16])
                    else:
                        dst.stb((AK if part == 1 else AV) + 16 * d0 + i // 2, r[i:i + 16])
                    yield
    return sum(2 * DA for p in parts if p < 3), gen()


def _a_attend(j, cur, old, o_ref, omg_ref):
    def window(o):
        lane = lax.broadcasted_iota(I32, (8, 128), 1)
        c, p = cur.ldi(o, 8), old.ldi(o, 8)
        out = []
        for w in range(WIN):
            sh = DIL * w
            t = c if w == 0 else pltpu.roll(jnp.where(lane >= 128 - sh, p, c), sh, 1)
            out.append(pltpu.bitcast(t, BF16).astype(F32))
        return out

    def gen():
        pos = j * 128 + lax.broadcasted_iota(I32, (8, 128), 1)
        for hg in range(4):
            lg = None
            for d in range(0, DA, 2):
                q = cur.ldf(AQ + 32 * d + 16 * hg, 16)
                pr = [q * kw for kw in window(AK + 16 * d + 8 * hg)]
                pr = [t[:8] + t[8:] for t in pr]
                lg = pr if d == 0 else [a + b for a, b in zip(lg, pr)]
                yield
            lg = [jnp.where(pos >= DIL * w, t * DA ** -0.5, NEG) for w, t in enumerate(lg)]
            mx = functools.reduce(jnp.maximum, lg)
            e = [jnp.exp(t - mx) for t in lg]
            g = cur.ldf(AG, 8)
            if hg == 0:
                omg_ref[j] = 1.0 - g
            r = g / functools.reduce(jnp.add, e)
            p = [jnp.concatenate([t * r] * 2, 0) for t in e]
            yield
            for d in range(0, DA, 2):
                o = functools.reduce(jnp.add, [a * b for a, b in zip(p, window(AV + 16 * d + 8 * hg))])
                o = pltpu.bitcast(o.astype(BF16).astype(F32), I32)
                o_ref[pl.ds(4 * DA * hg + d // 2, 8, stride=DA // 2), :] = (
                    lax.shift_right_logical(o[:8], 16) | o[8:])
                yield
    return 4 * DA + 4, gen()


def _a_out(A, o_ref, ga_ref, tick):
    def gen():
        for r0 in range(0, D, 96):
            r = _dot(_cat576(lambda k: A.ldb(WOT + 288 * k + r0 // 2, 48)), pltpu.bitcast(o_ref[:288, :], BF16))
            for i in range(0, 96, 32):
                tick(r[i:i + 32])
                ga_ref[r0 + i:r0 + i + 32, :] = r[i:i + 32]
                yield
    return D // 32, gen()


def _pairs(g):
    return g, g + NG


def _heads(g):
    return [2 * j + i for j in _pairs(g) for i in range(2)]


def _b_split_heads(raw, dst, even, odd, stride=PSTRIDE):
    def gen():
        for r in range(raw.shape[0] // 64):
            e = pltpu.bitcast(raw[64 * r:64 * r + 32, :], I32)
            o = pltpu.bitcast(raw[64 * r + 32:64 * r + 64, :], I32)
            dst[pl.ds(even + r, NP, stride=stride), :] = (e & 0xFFFF) | (o << 16)
            dst[pl.ds(odd + r, NP, stride=stride), :] = lax.shift_right_logical(e, 16) | (o & -65536)
            yield
    return raw.shape[0] // 64, gen()


def _b_sum_matrix():
    g = lax.broadcasted_iota(I32, (8, 128), 0)
    lane = lax.broadcasted_iota(I32, (8, 128), 1)
    return jnp.concatenate([functools.reduce(jnp.add, [
        jnp.where(lane == H * k + _heads(0)[n] + 2 * g, float(c), 0.0) for (k, n), c in PRODUCTS[p][1].items()])
        for p in LONG], 0)


def _b_product_tiles(A, raw, dst, off):
    def gen():
        for r in range(16):
            t = [jnp.concatenate([raw[o:o + H, :] for o in range(64 * r + H * i, 512 * H, 128 * H)], 0)
                 for i in range(2)]
            long = [_dot(A.ldb(SUMS, 4 * len(LONG)), v) for v in t]
            word = [pltpu.bitcast(v, I32) for v in t]

            def block(k, n, i):
                v = word[i][16 * k + 8 * (n // 2):16 * k + 8 * (n // 2) + 8]
                return pltpu.bitcast(v & -65536 if n % 2 else v << 16, F32)

            for p, (_, w, _) in enumerate(PRODUCTS):
                e, o = [pltpu.bitcast(
                    long[i][8 * LONG.index(p):8 * LONG.index(p) + 8] if p in LONG else
                    _signed_sum([(c, block(k, n, i)) for (k, n), c in w.items()]), I32) for i in range(2)]
                if len(w) > 1:
                    e, o = e + 0x8000, (o + 0x7FFF) & -65536
                dst[pl.ds(off + p * 64 + r, NG, stride=GSTRIDE), :] = lax.shift_right_logical(e, 16) | o
            yield
    return 16, gen()


def _b_transpose_wo(B, wot):
    def gen():
        for g in range(NG):
            for p, (_, w, _) in enumerate(PRODUCTS):
                t = [(c, wot[pl.ds(D * _heads(g)[k] + 128 * n, 128), :]) for (k, n), c in w.items()]
                if len(t) > 1 or t[0][0] < 0:
                    t = [(1, _signed_sum([(c, v.astype(F32)) for c, v in t]).astype(BF16))]
                B.stb(OA + (g * NPR + p) * 64, t[0][1].T)
                yield
            for j in _pairs(g):
                t = jnp.concatenate([wot[D * h + 512:D * h + D, :] for h in (2 * j, 2 * j + 1)], 0)
                B.stb(O2T + 64 * j, t)
                B.stb(O2 + 64 * j, t.T)
                B.stb(K2 + PSTRIDE * j, B.ldb(K2 + PSTRIDE * j, 64).T)
    return NG * NPR, gen()


def _turn(u):
    return 1 - u % 2


def _halves(p, r):
    return (r,) if p in TURN[1 - r] else (0, 1)


def _lh(u, i):
    return LH + L * (18 * (u % U) + i)


def _b_place_memory(B, u, mem):
    r = _turn(u)
    for i, p in enumerate(TURN[r]):
        B.stf(_lh(u, 2 + i), _signed_sum([(s, mem[k]) for (rr, k), s in PRODUCTS[p][0].items() if rr == r]))
    for i in range(2):
        B.stf(_lh(u, i), mem[4])


def _b_place_tokens(B, u):
    r = _turn(u)
    top = (u + 1 - r) % U

    def x(seg, n, half):
        return B.ldb(XN + 64 * n + 16 * seg + 8 * half, 8).astype(F32)

    for i, p in enumerate(TURN[r]):
        for at, half in enumerate(_halves(p, r)):
            B.stf(_lh(u, 2 + i) + M + 16 * at,
                  _signed_sum([(s, x(top + rr, k, half)) for (rr, k), s in PRODUCTS[p][0].items()]))
    for half in range(2):
        B.stf(_lh(u, 1) + M + 16 * half, x((u + 1) % U, 4, half))


def _b_project(B, u, mat, g, m=M, keep=()):
    r = _turn(u)
    top = (u + 1 - r) % U
    items = [(PRODUCTS[p][2], _halves(p, r),
              _dot(B.ldf(_lh(u, 2 + TURN[r].index(p)) + M - m, m + 16 * len(_halves(p, r))),
                   B.ldb(GSTRIDE * g + (mat * NPR + p) * 64, 64))) for p in ORDER[r]]
    if mat == 0:
        items += [({(r, n): 1}, (0, 1),
                   _dot(B.ldf(_lh(u, 1) + M - m, m + SEG)[:, :64],
                        B.ldb(Q2 + PSTRIDE * (h // 2) + 32 * (h % 2), 32))) for n, h in enumerate(_heads(g))]

    def at(n, seg, half):
        return TK + 128 * (H * mat + _heads(g)[n]) + SEG * seg + 16 * half

    mem, tok, kept = {}, {}, {}
    for c, halves, y in items:
        for (rr, n), s in c.items():
            if m and rr == r:
                mem.setdefault(n, []).append((s, y[:m]))
            for i, half in enumerate(halves):
                tok.setdefault((rr, n, half), []).append((s, y[m + 16 * i:m + 16 * i + 16]))
    for (rr, n, half), terms in sorted(tok.items()):
        if r == 1:
            terms.append((1, B.ldf(at(n, top + rr, half), 16)))
        if r == 1 and rr in keep:
            kept[n, top + rr, half] = _signed_sum(terms)
        else:
            B.stf(at(n, top + rr, half), _signed_sum(terms))
    assert len(tok) == 16

    def tokens(n, seg):
        return [kept[n, seg, i] if (n, seg, i) in kept else B.ldf(at(n, seg, i), 16) for i in range(2)]

    return [_signed_sum(mem[n]) for n in sorted(mem)], tokens


def _b_out_product(B, u, p, g, acc, m=M):
    r = _turn(u)
    top = (u - 1 - r) % U
    a = PRODUCTS[p][0].items()
    lhs = [_signed_sum([(s, B.ldf(OM + M * _heads(g)[k], M)) for (rr, k), s in a if rr == r])] if m else []
    both = [k for (rr, k), s in a if rr and PRODUCTS[p][0].get((0, k)) == -s]
    lhs += [_signed_sum([(s, B.ldf(OF + SEG * (H * (U if k in both else top + rr) + _heads(g)[k]) + 16 * half, 16))
                         for (rr, k), s in a if not (rr and k in both)]) for half in _halves(p, r)]
    y = _dot(jnp.concatenate(lhs, 0), B.ldb(OA + (g * NPR + p) * 64, 64))
    acc[p] = acc[p] + y if g else y
    if g == NG - 1:
        B.stf(AC + SEG * p + 16 * _halves(p, r)[0], acc[p][m:])
        for (rr, n), s in PRODUCTS[p][2].items():
            if m and rr == r:
                acc.setdefault(("mem", n), []).append((s, acc[p][:m]))


def _b_out_collect(B, u):
    for rr in range(2):
        for n in range(4):
            B.stf(BO + 128 * n + SEG * ((u - 2 + rr) % U), _signed_sum(
                [(c[rr, n], B.ldf(AC + SEG * p, SEG)) for p, (_, _, c) in enumerate(PRODUCTS) if (rr, n) in c]))


def _b_out_tail(B, u):
    B.stf(B2 + 64 * u, functools.reduce(jnp.add, [
        _dot_nt(B.ldb(O2T + 32 * h, 32),
                jnp.concatenate([B.ldf(OF + SEG * (H * i + h), SEG) for i in range(U)], 0).astype(BF16))
        for h in range(8 * u, 8 * u + 8)]))


def _b_step(B, u, emit, after_use, spare):
    row = lax.broadcasted_iota(I32, (L, 128), 0)
    lane = lax.broadcasted_iota(I32, (L, 128), 1)
    lo = lane < 64
    lo64 = lax.broadcasted_iota(I32, (64, 128), 1) < 64
    mask = (row < M) | ((lane & 63) >= SEG) | (row - M >= (lane & 63))
    in_a, in_b = lane < L, (lane >= 64) & (lane < 64 + L)
    z24 = jnp.zeros((24, 128), F32)
    pair = [j for g in range(NG) for j in _pairs(g)]

    def h2():
        return jnp.concatenate([B.ldf(_lh(u, 0) + M, SEG), B.ldf(_lh(u, 0), M)], 0)

    def t_k(g):
        mem, tokens = _b_project(B, u, 1, g, keep=(0,))
        for i, j in enumerate(_pairs(g)):
            k = jnp.concatenate([t for n in (2 * i, 2 * i + 1) for t in tokens(n, u) + [mem[n], z24]], 0)
            B.stb(KS + 64 * j, k.astype(BF16).T)

    def t_q(g):
        mem = _b_project(B, u, 0, g)[0]
        for h, t in zip(_heads(g), mem):
            B.stf(MQ + M * h, t)
            spare(t)

    def t_v(g):
        mem, tokens = _b_project(B, u, 2, g, keep=(0, 1))
        for n, h in enumerate(_heads(g)):
            B.stb(VS + 40 * h + 32, jnp.concatenate([mem[n], z24[:8]], 0))
            if _turn(u):
                B.stb(VS + 40 * h, jnp.concatenate(tokens(n, u) + tokens(n, u + 1), 0))

    def t_s(i):
        j = pair[i]
        kt, w2 = B.ldi(KS + 64 * j, 64), B.ldi(K2 + PSTRIDE * j, 64)
        ya, yb = [_dot(jnp.concatenate([B.ldf(MQ + M * h, M), B.ldf(TK + 128 * h + SEG * u, SEG)], 0),
                       pltpu.bitcast(rhs, BF16))
                  for h, rhs in ((2 * j, jnp.where(lo64, kt, w2)), (2 * j + 1, jnp.where(lo64, w2, kt)))]
        B.stf(RE + L * i, jnp.where(lo, ya, yb))
        B.stf(RE + L * (NP + i), jnp.where(lo, yb, ya))

    def t_softmax(n):
        c4 = h2()
        y = _dot_nt(jnp.concatenate([jnp.where(lo, 0.0, c4), jnp.where(lo, c4, 0.0)], 0),
                    B.ldf(RE + L * NP + 128 * n, 128).astype(BF16))
        B.stf(RS + 128 * n, jnp.concatenate([y[:L], z24, y[L:], z24], 0).T)
        for i in range(128 * n // L, 128 * (n + 1) // L):
            s = jnp.where(mask, (B.ldf(RE + L * i, L) + B.ldf(RS + L * i, L)) * DH ** -0.5, NEG)
            ma = jnp.max(jnp.where(in_a, s, -jnp.inf), axis=1, keepdims=True)
            mb = jnp.max(jnp.where(in_b, s, -jnp.inf), axis=1, keepdims=True)
            e = jnp.exp(s - jnp.where(lo, ma, mb))
            B.stf(PS + L * i, jnp.where(in_a | in_b, e, 0.0))

    def t_pv(i):
        p, r = B.ldf(PS + L * i, L), B.ldf(RS + L * i, L)
        for b, lhs in enumerate((jnp.where(lo, p, r), jnp.where(lo, r, p))):
            h = 2 * pair[i] + b
            v = [B.ldi(VS + 40 * h + 16 * (u % 2), 16), B.ldi(VS + 40 * h + 32, 8), jnp.zeros((8, 128), I32)]
            w2 = [B.ldi(V2 + PSTRIDE * pair[i] + 32 * b, 32)]
            o = _dot(lhs, pltpu.bitcast(jnp.concatenate(w2 + v if b else v + w2, 0), BF16))
            l = jnp.broadcast_to(jnp.sum(jnp.where(in_b if b else in_a, p, 0.0), axis=1, keepdims=True), (L, 128))
            rc = pltpu.reciprocal(l, approx=True)
            o = o * (rc * (2.0 - l * rc))
            B.stf(OM + M * h, o[:M])
            B.stf(OF + SEG * (H * u + h), o[M:])
            if u % 2:
                B.stf(OF + SEG * (H * U + h), B.ldf(OF + SEG * (H * (u - 1) + h), SEG) - o[M:])

    acc = {}

    def t_mem_tail(i):
        y = _dot(B.ldf(OM + 2 * M * pair[i], 2 * M), B.ldb(O2 + 64 * pair[i], 64))
        acc["tail"] = acc["tail"] + y if i else y

    for g in range(NG):
        t_k(g)
        if g == 1 and u % 2:
            _b_out_collect(B, u - 1)
    c4 = h2()
    B.stb(GS, jnp.concatenate([jnp.where(lo, 0.0, c4), z24, jnp.where(lo, c4, 0.0), z24], 0))
    lag_s, lag_softmax = 2, 4
    softmax_at = [(128 * n + 127) // L + lag_s + lag_softmax for n in range(5)]
    for i in range(2 * NP - 2):
        if i % 2 == 0:
            t_q(i // 2) if i < NP else t_v((i - NP) // 2)
        if 0 <= i - lag_s < NP:
            t_s(i - lag_s)
        if i in (2, 6):
            emit(i // 4)
        if i in softmax_at:
            t_softmax(softmax_at.index(i))
        for j in range(4 * (i - 2 * NP + 6), 4 * (i - 2 * NP + 7)):
            if j >= 0:
                B.stf(RS + L * j, _dot(B.ldf(PS + L * j, L), B.ldb(GS, 64)))
    prods = TURN[_turn(u)]
    passes = ((2, 5, 0, 7, 10), (1, 3, 4, 6), (8, 9, 12, 11), (13, 15, 14))
    for g in range(NG + 2):
        if g < NG:
            t_pv(2 * g)
            t_pv(2 * g + 1)
        if g == 1:
            t_v(NG - 1)
        if g >= 2:
            for i in passes[0]:
                _b_out_product(B, u, prods[i], g - 2, acc)
            t_mem_tail(g - 2)
    after_use()
    for k in range(1, len(passes)):
        for g in range(NG):
            for i in passes[k]:
                _b_out_product(B, u, prods[i], g, acc)
            if k == 1:
                t_mem_tail(NG + g)
    tail = jnp.where(lo[:M], acc["tail"][:M], acc["tail"][M:])
    _b_place_memory(B, u + 1, [_signed_sum(acc["mem", n]) for n in range(4)] + [tail + pltpu.roll(tail, 64, 1)])
    _b_out_tail(B, u)


def _squares(t):
    t = pltpu.bitcast(t, I32)
    even, odd = pltpu.bitcast(t << 16, F32), pltpu.bitcast(t, F32)
    return even * even, odd * odd


def _b_norms(qkv, wot, out):
    for m in range(3):
        acc = None
        for d in range(32):
            sq = jnp.concatenate(_squares(qkv[RAW * m + H * d:RAW * m + H * d + H, :]), 0)
            acc = acc + sq if d else sq
            if d == 31:
                out[32 * m:32 * m + 32, :] = acc
            yield
    for i in range(8):
        for d in range(4):
            o = D * (i // 4) + 128 * (i % 4) + 32 * d
            sq = jnp.add(*_squares(wot[o:o + 32, :]))
            acc = acc + sq if d else sq
            if d == 3:
                out[96 + 8 * i:104 + 8 * i, :] = acc[:8] + acc[8:]
            yield


def _b_one_scale(norms, mem0):
    def close(ts):
        lo, hi = jnp.min(functools.reduce(jnp.minimum, ts)), jnp.max(functools.reduce(jnp.maximum, ts))
        return (hi <= 4.0 * lo) & (lo > 0.0) & (hi < jnp.inf), lo

    ok = [close([functools.reduce(jnp.add, [norms[4 * k + i, 32 * m:32 * m + 32, :] for i in range(4)])
                 for k in range(4)])[0] for m in range(3)]
    ok.append(close([jnp.sum(norms[g, o:o + 8, :], axis=0, keepdims=True)
                     for g in range(NB) for o in range(96, 160, 8)])[0])
    tokens, lo = close([jnp.sum(norms[g, 160:168, :], axis=0, keepdims=True) for g in range(NB)])
    top = jnp.max(functools.reduce(jnp.maximum, [norms[g, 168:176, :] for g in range(NB)]))
    sq = mem0[:, :512] * mem0[:, :512]
    over = jnp.max(jnp.max(sq, axis=1, keepdims=True) - jnp.sum(sq, axis=1, keepdims=True) / 8.0)
    return functools.reduce(jnp.logical_and, ok + [tokens, top <= lo / 8.0, over <= 0.0])


def _b_direct(b_ref, raw, mem0, x_rows, emit):
    def split(i, carry):
        for m in range(3):
            _interleave(_b_split_heads(raw.at[pl.ds(pl.multiple_of(RAW * m + i * 16 * H, 16), 16 * H)],
                                       b_ref.at[pl.ds(pl.multiple_of(i * 8, 8), O2), :],
                                       288 * m, 288 * (3 + m), 6 * 288))

    lax.fori_loop(0, D // 16, split, None)
    row = lax.broadcasted_iota(I32, (L, L + 8), 0)
    col = lax.broadcasted_iota(I32, (L, L + 8), 1)

    def segment(u, mem):
        x = pltpu.bitcast(_cat576(lambda n: b_ref[pl.ds(pl.multiple_of(TK + 128 * n + SEG * u, SEG), SEG), :]), F32)
        h = jnp.concatenate([mem, x, jnp.zeros((8, D), F32)], 0).astype(BF16)

        def head(i, acc):
            q, k, v = [_dot(h, pltpu.bitcast(b_ref[pl.ds(pl.multiple_of(288 * (3 * i + m), 8), 288), :], BF16))
                       for m in range(3)]
            s = jnp.where((row < M) | (row >= col), _dot_nt(q[:L], k.astype(BF16)) * DH ** -0.5, NEG)
            s = jnp.where(col < L, s, -jnp.inf)
            e = jnp.exp(s - jnp.max(s, axis=1, keepdims=True))
            o = _dot(e / jnp.sum(e, axis=1, keepdims=True), v.astype(BF16))
            return acc + _dot_nt(o, raw[pl.ds(pl.multiple_of(3 * RAW + D * i, 16), D), :])

        out = lax.fori_loop(0, H, head, jnp.zeros((L, D), F32))
        for n in range(5):
            c = min(128 * n, D - 128)
            b_ref[pl.ds(pl.multiple_of(RE + 128 * n + SEG * u, 8), SEG), :] = pltpu.bitcast(out[M:, c:c + 128], I32)
        return out[:M]

    def block(j, mem):
        for n in range(5):
            _Arena(b_ref).stf(TK + 128 * n, x_rows(j, n).astype(F32))
        mem = lax.fori_loop(0, U, segment, mem)
        for n in range(5):
            emit(j, n, _Arena(b_ref).ldf(RE + 128 * n, 128).T[64 * (n // 4):])
        return mem

    lax.fori_loop(0, NB, block, mem0)


def _kernel(xt_hbm, wqkv_hbm, wo_hbm, mem_hbm, gate_hbm, wq_hbm, wk_hbm, wv_hbm, wot_hbm,
            out_hbm,
            xt, wqkv, wo, mem_ref, gate_ref, raw, a_ref, b_ref, qkv_all, o_all, o_last, ga_all, omg, out_buf,
            norms, offs, sem_in, sem_w, sem_out):
    A, B = _Arena(a_ref), _Arena(b_ref)
    wot = raw.at[pl.ds(3 * RAW, H * D)]

    def cols(src, dst, c0, c1, sem):
        return pltpu.make_async_copy(src.at[:, pl.ds(c0, c1 - c0)], dst.at[:, pl.ds(c0, c1 - c0)], sem_in.at[sem])

    def rows(r0, r1, sem):
        return [pltpu.make_async_copy(w.at[pl.ds(r0 * H, (r1 - r0) * H)],
                                      raw.at[pl.ds(RAW * m + r0 * H, (r1 - r0) * H)], sem_w.at[sem])
                for m, w in enumerate((wq_hbm, wk_hbm, wv_hbm))]

    def x_stage(j, slot):
        A.stb(AX + 288 * slot, xt[:, pl.ds(pl.multiple_of(j * 128, 128), 128)])

    def x_rows(j, n):
        block = pl.ds(pl.multiple_of(j * 128, 128), 128)
        return (xt[128 * n:128 * n + 128, block] if n < 4 else jnp.concatenate([xt[512:D, block]] * 2, 0)).T

    def x_transpose(j):
        for n in range(5):
            B.stb(XN + 64 * n, x_rows(j, n))

    def x_tail(u):
        B.stf(_lh(u, 0) + M, B.ldb(XN + 256 + 16 * u, 16).astype(F32))

    def tick_raw(r):
        raw[D * H:D * H + 8, :] = r[:8].astype(BF16)

    def proj(j):
        if isinstance(j, int):
            return _Arena(qkv_all.at[pl.ds((j + 1) % 5 * SLOT, SLOT)])
        return _Arena(qkv_all.at[pl.ds(pl.multiple_of(offs[lax.rem(j + 1, 5)], 8), SLOT)])

    def raw_from(i, n):
        return raw.at[pl.ds(pl.multiple_of(offs[5 + i], 16), 2 * RAW + n * H)]

    x_copy = [cols(xt_hbm, xt, c0, c1, i) for i, (c0, c1) in enumerate(((0, 256), (256, 768), (768, S)))]
    w_copy = [cols(wqkv_hbm, wqkv, c0, c1, 3 + i) for i, (c0, c1) in
              enumerate(((512, 896), (896, 1152), (0, 512), (1152, 3 * D)))]
    wo_copy = pltpu.make_async_copy(wo_hbm, wo, sem_in.at[7])
    mem_copy = pltpu.make_async_copy(mem_hbm, mem_ref, sem_in.at[8])
    gate_copy = pltpu.make_async_copy(gate_hbm, gate_ref, sem_in.at[9])
    tail_copies, main_copies = rows(512, D, 0), rows(0, 512, 1)
    wot_copy = pltpu.make_async_copy(wot_hbm, wot, sem_w.at[2])
    for c in (w_copy[0], gate_copy, mem_copy, w_copy[1], x_copy[0], w_copy[2], w_copy[3], wo_copy):
        c.start()

    for i in range(5):
        offs[i] = i * SLOT
    for i in range(18):
        offs[5 + i] = 32 * H * i
    for i in range(NB):
        offs[23 + i] = 3 * RAW + 2 * D * i
    A.stb(SUMS, _b_sum_matrix())
    B.stf(OF + H * SEG, jnp.zeros((B_ROWS - OF - H * SEG, 128), F32))
    B.stf(AC, jnp.zeros((NPR * SEG, 128), F32))
    w_copy[0].wait()
    gate_copy.wait()
    mem_copy.wait()
    gate = jnp.broadcast_to(gate_ref[...].astype(F32)[None, :], (8, D))
    mem0 = mem_ref[...].astype(F32)
    for k in range(4):
        A.stf(GW + 8 * k, gate[:, 128 * k:128 * k + 128])
    A.stf(GW + 32, jnp.concatenate([gate[:, 512:]] * 2, 1))
    _b_place_memory(B, 0, [mem0[:, 128 * k:128 * k + 128] for k in range(4)]
                    + [jnp.concatenate([mem0[:, 512:]] * 2, 1)])

    def project(j, *parts):
        return _a_qkv(A, AX + 288 * j, proj(j), parts, first=j == 0)

    _a_transpose_w(A, wqkv, range(4, 7))
    w_copy[1].wait()
    _a_transpose_w(A, wqkv, range(7, 9))
    x_copy[0].wait()
    x_stage(0, 0)
    x_stage(1, 1)
    _interleave(project(0, 3, 1))
    x_transpose(0)
    for u in range(U):
        x_tail(u)
        _b_place_tokens(B, u)
    x_transpose(1)
    w_copy[2].wait()
    x_copy[1].start()
    _a_transpose_w(A, wqkv, range(0, 4))
    _interleave(_chain(project(1, 3, 1), project(0, 0)))
    w_copy[3].wait()
    x_copy[2].start()
    _a_transpose_w(A, wqkv, range(9, 14))
    _interleave(_chain(project(1, 0), project(0, 2)))
    wo_copy.wait()
    for c in tail_copies:
        c.start()
    _interleave(project(1, 2))
    _a_transpose_wo(A, wo)
    qkv_all[AK:AG, :] = jnp.broadcast_to(qkv_all[SLOT + AK:SLOT + AG, :1], (AG - AK, 128))

    def project_out(j0, n, tick=lambda r: None):
        return _chain(*[_a_out(A, o_all.at[j0 + b], ga_all.at[j0 + b], tick) for b in range(n)])

    def attend_trip(t, carry):
        @pl.when(t == 1)
        def _():
            x_copy[2].wait()
            wot_copy.start()

        _interleave(
            _chain(*[_chain(_a_qkv(A, AX + 288 * i, proj(2 * t + 2 + i)),
                            _once(x_stage, jnp.minimum(2 * t + 4 + i, NB - 1), i)) for i in range(2)]),
            _chain(*[_a_attend(j, proj(j), proj(j - 1), o_all.at[j], omg) for j in (2 * t, 2 * t + 1)]),
            span=(-0.04, 0.87))

    x_copy[1].wait()
    for c in main_copies:
        c.start()
    x_stage(2, 0)
    x_stage(3, 1)
    lax.fori_loop(0, NB // 2 - 1, attend_trip, None)

    def last_trip(t, carry):
        def tick(r):
            qkv_all[TICK:TICK + 8, :] = pltpu.bitcast(r[:8], I32)
            tick_raw(r)

        j = NB - 2 + t
        src, dst = raw_from(16 + t, 32), b_ref.at[pl.ds(pl.multiple_of(t * 16, 16), O2), :]
        _interleave(
            project_out(3 * t, 3, tick), _a_attend(j, proj(j), proj(j - 1), o_last.at[t], omg),
            _chain(*[_b_split_heads(src.at[pl.ds(RAW * m, 32 * H)], dst, even, odd) for m, (even, odd) in
                     enumerate(((Q2, Q2 + 32), (K2 + 32, K2), (V2, V2 + 32)))]),
            span=(-0.08, 0.82))

    for c in tail_copies:
        c.wait()
    lax.fori_loop(0, 2, last_trip, None)
    o_all[NB - 2:, :288, :] = o_last[:, :288, :]

    def prepare_trip(t, carry):
        src, dst = raw_from(t, 416), b_ref.at[pl.ds(pl.multiple_of(t * 16, 16), O2), :]
        _interleave(project_out(6 + 2 * t, 2), _chain(*[
            _b_product_tiles(A, src.at[pl.ds(RAW * m, 416 * H)], dst, m * NPR * 64) for m in range(3)]),
            span=(-0.04, 0.93))

    for c in main_copies:
        c.wait()
    lax.fori_loop(0, 4, prepare_trip, None)
    wot_copy.wait()
    _interleave(
        _chain(project_out(NB - 2, 2),
               *[_once(_b_project, B, U - 1, mat, g, 0) for mat in range(3) for g in range(NG)]),
        _b_transpose_wo(B, wot))

    def tail_sum(last, first_steps):
        lane = lax.broadcasted_iota(I32, (64, 128), 1)
        return functools.reduce(jnp.add, [B.ldf(B2 + 64 * last, 64)] + [
            jnp.where(lane < SEG * (u + 1) if first_steps else lane >= SEG * (u + 1), B.ldf(B2 + 64 * u, 64), 0.0)
            for u in range(U - 1)])

    def mix(j, n, bt):
        part = slice(128 * n, 128 * n + bt.shape[0])
        w = jnp.concatenate([omg[j]] * (bt.shape[0] // 8), 0)
        out_buf[j, part, :] = (ga_all[j, part, :] + w * bt).astype(BF16)

    def out_copy(j):
        return pltpu.make_async_copy(
            out_buf.at[j], out_hbm.at[:, pl.ds(pl.multiple_of(j * 128, 128), 128)], sem_out)

    def b_body(g, carry):
        done = jnp.maximum(g - 1, 0)
        B.stf(B2 + 64 * U, tail_sum(U - 1, True))
        sq = [t[i:i + 8] for t in _squares(xt[:512, pl.ds(pl.multiple_of(g * 128, 128), 128)])
              for i in range(0, 256, 8)]
        norms[g, 160:168, :] = functools.reduce(jnp.add, sq)
        norms[g, 168:176, :] = functools.reduce(jnp.maximum, sq)
        weights = _b_norms(raw_from(g, 32), raw.at[pl.ds(pl.multiple_of(offs[23 + g], 16), 2 * D)], norms.at[g])

        def spare(r):
            tick_raw(r)
            next(weights)

        for u in range(U):
            def emit(stage):
                if u == 1:
                    for n in range(4):
                        if stage:
                            mix(done, n, B.ldf(PS + 128 * n, 128))
                        else:
                            B.stf(PS + 128 * n, B.ldf(BO + 128 * n, 128).T)
                if u == U - 1 and stage:
                    mix(done, 4, tail_sum(U, False))

            def after_use():
                x_tail(u)
                if u == 0:
                    _b_place_tokens(B, U - 1)
                if u < U - 1:
                    _b_place_tokens(B, u)
                else:
                    x_transpose(jnp.minimum(g + 2, NB - 1))

            _b_step(B, u, emit, after_use, spare)
        assert next(weights, "end") == "end"

        @pl.when(g > 0)
        def _():
            out_copy(done).start()

        return carry

    lax.fori_loop(0, NB, b_body, 0)
    acc = {}
    for g in range(NG):
        for p in TURN[1]:
            _b_out_product(B, 0, p, g, acc, 0)
    _b_out_collect(B, 0)
    B.stf(B2 + 64 * U, tail_sum(U - 1, True))
    for u in range(U - 1):
        _b_out_tail(B, u)
    for n in range(4):
        mix(NB - 1, n, B.ldf(BO + 128 * n, 128).T)
    mix(NB - 1, 4, tail_sum(U, False))
    out_copy(NB - 1).start()
    one_scale = _b_one_scale(norms, mem_ref[...].astype(F32))
    for j in range(NB):
        out_copy(j).wait()

    @pl.when(jnp.logical_not(one_scale))
    def _():
        _b_direct(b_ref, raw, mem_ref[...].astype(F32), x_rows, mix)
        copies = [out_copy(j) for j in range(NB)]
        for c in copies:
            c.start()
        for c in copies:
            c.wait()


@functools.partial(jax.jit, static_argnames=("B_seg_len",))
def pallas_gated_mix__sliding_local_dilated__memory_aug_recurrent_mem_tr__prompt_kernel(
    A_x: jax.Array,
    A_wqkv: jax.Array,
    A_wo: jax.Array,
    B_x: jax.Array,
    B_mem0: jax.Array,
    B_Wq: jax.Array,
    B_Wk: jax.Array,
    B_Wv: jax.Array,
    B_Wo: jax.Array,
    B_seg_len: int,
    gate_w: jax.Array,
):
    del B_x
    assert A_x.shape == (1, S, D) and B_mem0.shape == (1, M, D) and B_Wq.shape == (D, H, DH)
    assert B_seg_len == SEG
    hbm = pl.BlockSpec(memory_space=pl.ANY)
    out_t = pl.pallas_call(
        _kernel,
        out_shape=jax.ShapeDtypeStruct((D, S), BF16),
        in_specs=[hbm] * 9,
        out_specs=hbm,
        scratch_shapes=[
            pltpu.VMEM((D, S), BF16),
            pltpu.VMEM((D, 3 * D), BF16),
            pltpu.VMEM((D, D), BF16),
            pltpu.VMEM((M, D), BF16),
            pltpu.VMEM((D,), BF16),
            pltpu.VMEM((4 * RAW, DH), BF16),
            pltpu.VMEM((A_ROWS, 128), I32),
            pltpu.VMEM((B_ROWS, 128), I32),
            pltpu.VMEM((5 * SLOT, 128), I32),
            pltpu.VMEM((NB, 296, 128), I32),
            pltpu.VMEM((2, 296, 128), I32),
            pltpu.VMEM((NB, D, 128), F32),
            pltpu.VMEM((NB, 8, 128), F32),
            pltpu.VMEM((NB, D, 128), BF16),
            pltpu.VMEM((NB, 176, 128), F32),
            pltpu.SMEM((39,), I32),
            pltpu.SemaphoreType.DMA((10,)),
            pltpu.SemaphoreType.DMA((3,)),
            pltpu.SemaphoreType.DMA,
        ],
        compiler_params=pltpu.CompilerParams(vmem_limit_bytes=110 * 1024 * 1024),
    )(
        A_x.reshape(S, D).T, A_wqkv, A_wo, B_mem0.reshape(M, D), gate_w,
        B_Wq.reshape(D * H, DH), B_Wk.reshape(D * H, DH), B_Wv.reshape(D * H, DH),
        B_Wo.transpose(0, 2, 1).reshape(H * D, DH),
    )
    return out_t.T.reshape(1, S, D)
```

```python
import functools

import jax
import jax.numpy as jnp
import numpy as np
from jax import lax
import jax.experimental.pallas as pl
import jax.experimental.pallas.tpu as pltpu

F32, BF16, I32 = jnp.float32, jnp.bfloat16, jnp.int32

S, D = 2048, 576
NB = S // 128
DA, WIN, DIL = 18, 8, 2
H, DH, M, SEG = 32, 128, 8, 32
L = M + SEG
NP = H // 2
NG = H // 4
U = 128 // SEG
NEG = -1000000000.0

PRODUCTS = tuple(tuple({(int(t[1]), int(t[2])): int(t[0] + "1") for t in form.split()} for form in p) for p in (
    ("+00 -10", "-03 +30 -10 +00 -02", "+00"),
    ("+10", "+03 -30 +00 -01 -20", "+00 +10"),
    ("+03 -13", "-13 -32 +33", "+03"),
    ("+13", "-23 -31 +33", "+03 +13"),
    ("+02 +10", "-02 +20", "+00 -12"),
    ("+02", "-02 -21 +22 -32", "+02 +12"),
    ("+02 -12", "-12 -20 +22 -23", "-12"),
    ("+00 +02", "+02", "+00 +02"),
    ("+10 +12", "+20", "+10 +12"),
    ("+02 +13", "+23 -32", "+03 -12"),
    ("+02 +03", "+32", "+02 +03"),
    ("+12 +13", "+23", "+12 +13"),
    ("+00 +01 -10", "+03 -30 +10 -01", "+00 +10 +11"),
    ("+01", "+03 -01 +11 -12 -31", "+01"),
    ("+11", "+10 -30 -11 +13 +21", "-11"),
    ("+00 +01", "-03 +01", "+00 +01 +10 +11"),
    ("+11 +12", "+21", "+01 +02 +11 +12"),
    ("-02 +11 +12", "+12 -21", "+01 +02 +12"),
    ("+01 +03", "-03 +31", "+01 +03 +11 +13"),
    ("+10 +11 +13", "+30", "+10 +11 +13"),
    ("+01 +03 -13", "-13 +31", "-03 -11 -13"),
    ("+00 +01 +03", "+03", "+00 +01 +03"),
    ("+00 +01 -10 -11", "+10 -30", "-10 -11"),
    ("+01 +02 -11 -12", "+12", "+01 +02"),
    ("+01 +03 -11 -13", "-30 +13", "-11 -13"),
    ("+01 +03 +10", "-03 +30", "+00 -11 -13"),
))
NPR = len(PRODUCTS)
TURN = tuple(tuple(p for p, (a, _, c) in enumerate(PRODUCTS)
                   if any(k[0] == r for k in a) and any(k[0] == r for k in c)) for r in range(2))
ORDER = ((2, 9, 5, 10, 17, 23, 7, 4, 21, 20, 18, 25, 15, 0, 13, 12),
         (17, 16, 14, 4, 1, 22, 12, 8, 19, 25, 24, 20, 11, 3, 9, 6))
LONG = tuple(p for p in range(NPR) if len(PRODUCTS[p][1]) == 5)


def _is_matrix_product():
    t = np.zeros((2, 4, 4, 4, 2, 4), int)
    for a, w, c in PRODUCTS:
        for i in a:
            for j in w:
                for k in c:
                    t[i + j + k] += a[i] * w[j] * c[k]
    return (t == np.einsum("rs,kl,nm->rklnsm", np.eye(2), np.eye(4), np.eye(4))).all()


assert _is_matrix_product() and len(set(TURN[0] + TURN[1])) == NPR
assert all(sorted(ORDER[r]) == list(TURN[r]) for r in range(2))

GSTRIDE = 3 * NPR * 64 + 4
Q2 = NG * GSTRIDE
K2 = Q2 + 64
V2 = K2 + 64
PSTRIDE = 192 + 4
OA = Q2 + NP * PSTRIDE
O2 = OA + NG * NPR * 64
O2T = O2 + NP * 64
LH = O2T + H * 32
GS = LH + U * 18 * L
TK = GS + 64
MQ = TK + 3 * H * 128
VS = MQ + H * M
KS = VS + H * 40
RE = KS + NP * 64
PS = RE + H * L
RS = PS + NP * L
AC = RS + NP * L
XN = AC + NPR * SEG
OM = XN + 320
OF = OM + H * M
BO = OF + (U + 1) * H * SEG
B2 = BO + 512
B_ROWS = B2 + 64 * (U + 1)

RAW = D * H + 16

WT = 0
GW = WT + 5 * 1728
WP = GW + 40
WOT = WP + 27 * 160
AX = WOT + 5 * 288
SUMS = AX + 2 * 288
A_ROWS = SUMS + 4 * len(LONG)
AQ, AK, AV, AG, TICK, SLOT = 0, 576, 864, 1152, 1160, 1168


def _dot(a, b):
    return lax.dot_general(a, b, (((1,), (0,)), ((), ())), preferred_element_type=F32)


def _dot_nt(a, b):
    return lax.dot_general(a, b, (((1,), (1,)), ((), ())), preferred_element_type=F32)


class _Arena:
    def __init__(self, ref):
        self.r = ref

    def ldi(self, o, n):
        return self.r[o:o + n, :]

    def ldf(self, o, n):
        return pltpu.bitcast(self.r[o:o + n, :], F32)

    def ldb(self, o, n):
        return pltpu.bitcast(self.r[o:o + n, :], BF16)

    def stf(self, o, v):
        self.r[o:o + v.shape[0], :] = pltpu.bitcast(v, I32)

    def stb(self, o, v):
        self.r[o:o + v.shape[0] // 2, :] = pltpu.bitcast(v.astype(BF16), I32)


def _signed_sum(terms):
    sign, acc = terms[0]
    for c, t in terms[1:]:
        if c == sign:
            acc = acc + t
        else:
            sign, acc = 1, acc - t if sign > 0 else t - acc
    return acc if sign > 0 else -acc


def _interleave(main, *side, span=(0.0, 0.9)):
    jobs = (main,) + side
    order = [((i + 1) / main[0], 0) for i in range(main[0])]
    order += [(span[0] + (span[1] - span[0]) * i / n, k + 1) for k, (n, _) in enumerate(side) for i in range(n)]
    for _, k in sorted(order):
        next(jobs[k][1])
    for _, gen in jobs:
        assert next(gen, "end") == "end"


def _once(fn, *args):
    def gen():
        fn(*args)
        yield
    return 1, gen()


def _chain(*jobs):
    def gen():
        for _, g in jobs:
            yield from g
    return sum(n for n, _ in jobs), gen()


def _tile_t(w_ref, k, c):
    t = w_ref[128 * k:min(128 * k + 128, w_ref.shape[0]), 128 * c:min(128 * c + 128, w_ref.shape[1])]
    nk, nc = t.shape
    if nc < 128:
        t = jnp.concatenate([t, jnp.zeros((nk, 128 - nc), t.dtype)], 1)
    if nk < 128:
        t = jnp.concatenate([t, jnp.zeros((128 - nk, 128), t.dtype)], 0)
    return t.T[:nc]


def _a_transpose_w(A, w_ref, cblocks):
    for c in cblocks:
        for k in range(5):
            A.stf(WT + 1728 * k + 128 * c, _tile_t(w_ref, k, c).astype(F32))


def _a_transpose_wo(A, w_ref):
    for c in range(5):
        for k in range(5):
            A.stb(WOT + 288 * k + 64 * c, _tile_t(w_ref, k, c))


def _cat576(chunk):
    ch = [chunk(k) for k in range(5)]
    return jnp.concatenate(ch[:4] + [ch[4][:, :64]], 1)


def _a_qkv(A, x_off, dst, parts=(3, 1, 0, 2), first=False):
    def gen():
        for part in parts:
            if part == 3:
                dst.stf(AG, jax.nn.sigmoid(_dot(_cat576(lambda k: A.ldf(GW + 8 * k, 8)), A.ldb(x_off, 288))))
                continue
            for d0 in range(0, DA, 2):
                def weights(k):
                    packed = WP + 160 * (9 * part + d0 // 2) + 32 * k
                    if not first:
                        return A.ldb(packed, 32)
                    w = jnp.concatenate([
                        pltpu.bitcast(A.r[pl.ds(WT + 1728 * k + D * part + 8 * DA * hg + d, 8, stride=DA), :], F32)
                        for hg in range(4) for d in (d0, d0 + 1)], 0)
                    A.stb(packed, w)
                    return w

                r = _dot(_cat576(weights), A.ldb(x_off, 288))
                for i in range(0, 64, 16):
                    if part == 0:
                        dst.stf(AQ + 32 * d0 + i, r[i:i + 16])
                    else:
                        dst.stb((AK if part == 1 else AV) + 16 * d0 + i // 2, r[i:i + 16])
                    yield
    return sum(2 * DA for p in parts if p < 3), gen()


def _a_attend(j, cur, old, o_ref, omg_ref):
    lane = lax.broadcasted_iota(I32, (8, 128), 1)
    wraps = {w: lane >= 128 - DIL * w for w in range(1, WIN)}

    def window(o):
        c, p = cur.ldi(o, 8), old.ldi(o, 8)
        out = []
        for w in range(WIN):
            t = pltpu.roll(lax.select(wraps[w], p, c), DIL * w, 1) if w else c
            out.append(pltpu.bitcast(t, BF16).astype(F32))
        return out

    def gen():
        pos = j * 128 + lane
        for hg in range(4):
            lg = None
            for d in range(0, DA, 2):
                q = cur.ldf(AQ + 32 * d + 16 * hg, 16)
                pr = [q * kw for kw in window(AK + 16 * d + 8 * hg)]
                pr = [t[:8] + t[8:] for t in pr]
                lg = pr if d == 0 else [a + b for a, b in zip(lg, pr)]
                yield
            lg = [jnp.where(pos >= DIL * w, t * DA ** -0.5, NEG) for w, t in enumerate(lg)]
            mx = functools.reduce(jnp.maximum, lg)
            e = [jnp.exp(t - mx) for t in lg]
            g = cur.ldf(AG, 8)
            if hg == 0:
                omg_ref[j] = 1.0 - g
            r = g / functools.reduce(jnp.add, e)
            p = [jnp.concatenate([t * r] * 2, 0) for t in e]
            yield
            for d in range(0, DA, 2):
                o = functools.reduce(jnp.add, [a * b for a, b in zip(p, window(AV + 16 * d + 8 * hg))])
                o = pltpu.bitcast(o.astype(BF16).astype(F32), I32)
                o_ref[pl.ds(4 * DA * hg + d // 2, 8, stride=DA // 2), :] = (
                    lax.shift_right_logical(o[:8], 16) | o[8:])
                yield
    return 4 * DA + 4, gen()


def _a_out(A, o_ref, ga_ref, tick):
    def gen():
        for r0 in range(0, D, 96):
            r = _dot(_cat576(lambda k: A.ldb(WOT + 288 * k + r0 // 2, 48)), pltpu.bitcast(o_ref[:288, :], BF16))
            for i in range(0, 96, 32):
                tick(r[i:i + 32])
                ga_ref[r0 + i:r0 + i + 32, :] = r[i:i + 32]
                yield
    return D // 32, gen()


def _pairs(g):
    return g, g + NG


def _heads(g):
    return [2 * j + i for j in _pairs(g) for i in range(2)]


def _b_split_heads(raw, dst, even, odd, stride=PSTRIDE):
    def gen():
        for r in range(raw.shape[0] // 64):
            e = pltpu.bitcast(raw[64 * r:64 * r + 32, :], I32)
            o = pltpu.bitcast(raw[64 * r + 32:64 * r + 64, :], I32)
            dst[pl.ds(even + r, NP, stride=stride), :] = (e & 0xFFFF) | (o << 16)
            dst[pl.ds(odd + r, NP, stride=stride), :] = lax.shift_right_logical(e, 16) | (o & -65536)
            yield
    return raw.shape[0] // 64, gen()


def _b_sum_matrix():
    g = lax.broadcasted_iota(I32, (8, 128), 0)
    lane = lax.broadcasted_iota(I32, (8, 128), 1)
    return jnp.concatenate([functools.reduce(jnp.add, [
        jnp.where(lane == H * k + _heads(0)[n] + 2 * g, float(c), 0.0) for (k, n), c in PRODUCTS[p][1].items()])
        for p in LONG], 0)


def _b_product_tiles(A, raw, dst, off):
    def gen():
        for r in range(16):
            t = [jnp.concatenate([raw[o:o + H, :] for o in range(64 * r + H * i, 512 * H, 128 * H)], 0)
                 for i in range(2)]
            long = [_dot(A.ldb(SUMS, 4 * len(LONG)), v) for v in t]
            word = [pltpu.bitcast(v, I32) for v in t]

            @functools.cache
            def block(k, n, i):
                v = word[i][16 * k + 8 * (n // 2):16 * k + 8 * (n // 2) + 8]
                return pltpu.bitcast(v & -65536 if n % 2 else v << 16, F32)

            for p, (_, w, _) in enumerate(PRODUCTS):
                e, o = [pltpu.bitcast(
                    long[i][8 * LONG.index(p):8 * LONG.index(p) + 8] if p in LONG else
                    _signed_sum([(c, block(k, n, i)) for (k, n), c in w.items()]), I32) for i in range(2)]
                if len(w) > 1:
                    e, o = e + 0x8000, (o + 0x7FFF) & -65536
                dst[pl.ds(off + p * 64 + r, NG, stride=GSTRIDE), :] = lax.shift_right_logical(e, 16) | o
            yield
    return 16, gen()


def _b_transpose_wo(B, wot):
    def gen():
        for g in range(NG):
            for p, (_, w, _) in enumerate(PRODUCTS):
                t = [(c, wot[pl.ds(D * _heads(g)[k] + 128 * n, 128), :]) for (k, n), c in w.items()]
                if len(t) > 1 or t[0][0] < 0:
                    t = [(1, _signed_sum([(c, v.astype(F32)) for c, v in t]).astype(BF16))]
                B.stb(OA + (g * NPR + p) * 64, t[0][1].T)
                yield
            for j in _pairs(g):
                t = jnp.concatenate([wot[D * h + 512:D * h + D, :] for h in (2 * j, 2 * j + 1)], 0)
                B.stb(O2T + 64 * j, t)
                B.stb(O2 + 64 * j, t.T)
                B.stb(K2 + PSTRIDE * j, B.ldb(K2 + PSTRIDE * j, 64).T)
    return NG * NPR, gen()


def _turn(u):
    return 1 - u % 2


def _halves(p, r):
    return (r,) if p in TURN[1 - r] else (0, 1)


def _lh(u, i):
    return LH + L * (18 * (u % U) + i)


def _b_place_memory(B, u, mem):
    r = _turn(u)
    for i, p in enumerate(TURN[r]):
        B.stf(_lh(u, 2 + i), _signed_sum([(s, mem[k]) for (rr, k), s in PRODUCTS[p][0].items() if rr == r]))
    for i in range(2):
        B.stf(_lh(u, i), mem[4])


def _b_place_tokens(B, u):
    r = _turn(u)
    top = (u + 1 - r) % U

    def x(seg, n, half):
        return B.ldb(XN + 64 * n + 16 * seg + 8 * half, 8).astype(F32)

    for i, p in enumerate(TURN[r]):
        for at, half in enumerate(_halves(p, r)):
            B.stf(_lh(u, 2 + i) + M + 16 * at,
                  _signed_sum([(s, x(top + rr, k, half)) for (rr, k), s in PRODUCTS[p][0].items()]))
    for half in range(2):
        B.stf(_lh(u, 1) + M + 16 * half, x((u + 1) % U, 4, half))


def _b_project(B, u, mat, g, m=M, keep=()):
    r = _turn(u)
    top = (u + 1 - r) % U
    items = [(PRODUCTS[p][2], _halves(p, r),
              _dot(B.ldf(_lh(u, 2 + TURN[r].index(p)) + M - m, m + 16 * len(_halves(p, r))),
                   B.ldb(GSTRIDE * g + (mat * NPR + p) * 64, 64))) for p in ORDER[r]]
    if mat == 0:
        items += [({(r, n): 1}, (0, 1),
                   _dot(B.ldf(_lh(u, 1) + M - m, m + SEG)[:, :64],
                        B.ldb(Q2 + PSTRIDE * (h // 2) + 32 * (h % 2), 32))) for n, h in enumerate(_heads(g))]

    def at(n, seg, half):
        return TK + 128 * (H * mat + _heads(g)[n]) + SEG * seg + 16 * half

    mem, tok, kept = {}, {}, {}
    for c, halves, y in items:
        y_mem, y_tok = y[:m] if m else None, [y[o:o + 16] for o in range(m, y.shape[0], 16)]
        for (rr, n), s in c.items():
            if m and rr == r:
                mem.setdefault(n, []).append((s, y_mem))
            for half, t in zip(halves, y_tok):
                tok.setdefault((rr, n, half), []).append((s, t))
    for (rr, n, half), terms in sorted(tok.items()):
        if r == 1:
            terms.append((1, B.ldf(at(n, top + rr, half), 16)))
        if r == 1 and rr in keep:
            kept[n, top + rr, half] = _signed_sum(terms)
        else:
            B.stf(at(n, top + rr, half), _signed_sum(terms))
    assert len(tok) == 16

    def tokens(n, seg):
        return [kept[n, seg, i] if (n, seg, i) in kept else B.ldf(at(n, seg, i), 16) for i in range(2)]

    return [_signed_sum(mem[n]) for n in sorted(mem)], tokens


def _b_out_product(B, u, p, g, acc, m=M):
    r = _turn(u)
    top = (u - 1 - r) % U
    a = PRODUCTS[p][0].items()
    lhs = [_signed_sum([(s, B.ldf(OM + M * _heads(g)[k], M)) for (rr, k), s in a if rr == r])] if m else []
    both = [k for (rr, k), s in a if rr and PRODUCTS[p][0].get((0, k)) == -s]
    first, rows = 16 * _halves(p, r)[0], 16 * len(_halves(p, r))
    lhs.append(_signed_sum([(s, B.ldf(OF + SEG * (H * (U if k in both else top + rr) + _heads(g)[k]) + first, rows))
                            for (rr, k), s in a if not (rr and k in both)]))
    y = _dot(jnp.concatenate(lhs, 0), B.ldb(OA + (g * NPR + p) * 64, 64))
    acc[p] = acc[p] + y if g else y
    if g == NG - 1:
        B.stf(AC + SEG * p + first, acc[p][m:])
        for (rr, n), s in PRODUCTS[p][2].items():
            if m and rr == r:
                acc.setdefault(("mem", n), []).append((s, acc[p][:m]))


def _b_out_collect(B, u):
    for rr in range(2):
        for n in range(4):
            B.stf(BO + 128 * n + SEG * ((u - 2 + rr) % U), _signed_sum(
                [(c[rr, n], B.ldf(AC + SEG * p, SEG)) for p, (_, _, c) in enumerate(PRODUCTS) if (rr, n) in c]))


def _b_out_tail(B, u):
    B.stf(B2 + 64 * u, functools.reduce(jnp.add, [
        _dot_nt(B.ldb(O2T + 32 * h, 32),
                jnp.concatenate([B.ldf(OF + SEG * (H * i + h), SEG) for i in range(U)], 0).astype(BF16))
        for h in range(8 * u, 8 * u + 8)]))


def _b_step(B, u, emit, after_use, spare):
    row = lax.broadcasted_iota(I32, (L, 128), 0)
    lane = lax.broadcasted_iota(I32, (L, 128), 1)
    lo = lane < 64
    lo64 = lax.broadcasted_iota(I32, (64, 128), 1) < 64
    mask = (row < M) | ((lane & 63) >= SEG) | (row - M >= (lane & 63))
    in_a, in_b = lane < L, (lane >= 64) & (lane < 64 + L)
    z24 = jnp.zeros((24, 128), F32)
    pair = [j for g in range(NG) for j in _pairs(g)]

    def h2():
        return jnp.concatenate([B.ldf(_lh(u, 0) + M, SEG), B.ldf(_lh(u, 0), M)], 0)

    def t_k(g):
        mem, tokens = _b_project(B, u, 1, g, keep=(0,))
        for t in mem:
            spare(t)
        for i, j in enumerate(_pairs(g)):
            k = jnp.concatenate([t for n in (2 * i, 2 * i + 1) for t in tokens(n, u) + [mem[n], z24]], 0)
            B.stb(KS + 64 * j, k.astype(BF16).T)

    def t_q(g):
        mem = _b_project(B, u, 0, g)[0]
        for h, t in zip(_heads(g), mem):
            B.stf(MQ + M * h, t)

    def t_v(g):
        mem, tokens = _b_project(B, u, 2, g, keep=(0, 1))
        for n, h in enumerate(_heads(g)):
            B.stb(VS + 40 * h + 32, jnp.concatenate([mem[n], z24[:8]], 0))
            if _turn(u):
                B.stb(VS + 40 * h, jnp.concatenate(tokens(n, u) + tokens(n, u + 1), 0))

    def t_s(i):
        j = pair[i]
        kt, w2 = B.ldi(KS + 64 * j, 64), B.ldi(K2 + PSTRIDE * j, 64)
        ya, yb = [_dot(jnp.concatenate([B.ldf(MQ + M * h, M), B.ldf(TK + 128 * h + SEG * u, SEG)], 0),
                       pltpu.bitcast(rhs, BF16))
                  for h, rhs in ((2 * j, jnp.where(lo64, kt, w2)), (2 * j + 1, jnp.where(lo64, w2, kt)))]
        B.stf(RE + L * i, jnp.where(lo, ya, yb))
        B.stf(RE + L * (NP + i), jnp.where(lo, yb, ya))

    def t_softmax(n):
        c4 = h2()
        y = _dot_nt(jnp.concatenate([jnp.where(lo, 0.0, c4), jnp.where(lo, c4, 0.0)], 0),
                    B.ldf(RE + L * NP + 128 * n, 128).astype(BF16))
        B.stf(RS + 128 * n, jnp.concatenate([y[:L], z24, y[L:], z24], 0).T)
        for i in range(128 * n // L, 128 * (n + 1) // L):
            s = jnp.where(mask, (B.ldf(RE + L * i, L) + B.ldf(RS + L * i, L)) * DH ** -0.5, NEG)
            ma = jnp.max(jnp.where(in_a, s, -jnp.inf), axis=1, keepdims=True)
            mb = jnp.max(jnp.where(in_b, s, -jnp.inf), axis=1, keepdims=True)
            e = jnp.exp(s - jnp.where(lo, ma, mb))
            B.stf(PS + L * i, jnp.where(in_a | in_b, e, 0.0))

    def t_pv(i):
        p, r = B.ldf(PS + L * i, L), B.ldf(RS + L * i, L)
        for b, lhs in enumerate((jnp.where(lo, p, r), jnp.where(lo, r, p))):
            h = 2 * pair[i] + b
            v = [B.ldi(VS + 40 * h + 16 * (u % 2), 16), B.ldi(VS + 40 * h + 32, 8), jnp.zeros((8, 128), I32)]
            w2 = [B.ldi(V2 + PSTRIDE * pair[i] + 32 * b, 32)]
            o = _dot(lhs, pltpu.bitcast(jnp.concatenate(w2 + v if b else v + w2, 0), BF16))
            l = jnp.broadcast_to(jnp.sum(jnp.where(in_b if b else in_a, p, 0.0), axis=1, keepdims=True), (L, 128))
            rc = pltpu.reciprocal(l, approx=True)
            o = o * (rc * (2.0 - l * rc))
            B.stf(OM + M * h, o[:M])
            B.stf(OF + SEG * (H * u + h), o[M:])
            if u % 2:
                B.stf(OF + SEG * (H * U + h), B.ldf(OF + SEG * (H * (u - 1) + h), SEG) - o[M:])

    acc = {}

    def t_mem_tail(i):
        y = _dot(B.ldf(OM + 2 * M * pair[i], 2 * M), B.ldb(O2 + 64 * pair[i], 64))
        acc["tail"] = acc["tail"] + y if i else y

    for g in range(NG):
        t_k(g)
        if g == 1 and u % 2:
            _b_out_collect(B, u - 1)
    c4 = h2()
    B.stb(GS, jnp.concatenate([jnp.where(lo, 0.0, c4), z24, jnp.where(lo, c4, 0.0), z24], 0))
    lag_s, lag_softmax = 2, 4
    softmax_at = [(128 * n + 127) // L + lag_s + lag_softmax for n in range(5)]
    for i in range(2 * NP - 2):
        if i % 2 == 0:
            t_q(i // 2) if i < NP else t_v((i - NP) // 2)
        if 0 <= i - lag_s < NP:
            t_s(i - lag_s)
        if i in (2, 6):
            emit(i // 4)
        if i in softmax_at:
            t_softmax(softmax_at.index(i))
        for j in range(4 * (i - 2 * NP + 6), 4 * (i - 2 * NP + 7)):
            if j >= 0:
                B.stf(RS + L * j, _dot(B.ldf(PS + L * j, L), B.ldb(GS, 64)))
    prods = TURN[_turn(u)]
    passes = (((2, 5, 0, 7, 10), (1, 3, 4, 6), (8, 9, 15, 11), (13, 12, 14)),
              ((15, 5, 0, 12, 10), (1, 3, 4, 6), (8, 9, 7, 11), (13, 2, 14)))[_turn(u)]
    for g in range(NG + 2):
        if g < NG:
            t_pv(2 * g)
            t_pv(2 * g + 1)
        if g == 2:
            t_v(NG - 1)
        if g >= 2:
            for i in passes[0]:
                _b_out_product(B, u, prods[i], g - 2, acc)
            t_mem_tail(g - 2)
    after_use()
    for k in range(1, len(passes)):
        for g in range(NG):
            for i in passes[k]:
                _b_out_product(B, u, prods[i], g, acc)
            if k == 1:
                t_mem_tail(NG + g)
    tail = jnp.where(lo[:M], acc["tail"][:M], acc["tail"][M:])
    _b_place_memory(B, u + 1, [_signed_sum(acc["mem", n]) for n in range(4)] + [tail + pltpu.roll(tail, 64, 1)])
    _b_out_tail(B, u)


def _squares(t):
    t = pltpu.bitcast(t, I32)
    even, odd = pltpu.bitcast(t << 16, F32), pltpu.bitcast(t, F32)
    return even * even, odd * odd


def _b_norms(qkv, wot, out):
    for m in range(3):
        acc = None
        for d in range(32):
            sq = jnp.concatenate(_squares(qkv[RAW * m + H * d:RAW * m + H * d + H, :]), 0)
            acc = acc + sq if d else sq
            if d == 31:
                out[32 * m:32 * m + 32, :] = acc
            yield
    for i in range(8):
        for d in range(4):
            o = D * (i // 4) + 128 * (i % 4) + 32 * d
            sq = jnp.add(*_squares(wot[o:o + 32, :]))
            acc = acc + sq if d else sq
            if d == 3:
                out[96 + 8 * i:104 + 8 * i, :] = acc[:8] + acc[8:]
            yield


def _b_one_scale(norms, mem0):
    def close(ts):
        lo, hi = jnp.min(functools.reduce(jnp.minimum, ts)), jnp.max(functools.reduce(jnp.maximum, ts))
        return (hi <= 4.0 * lo) & (lo > 0.0) & (hi < jnp.inf), lo

    ok = [close([functools.reduce(jnp.add, [norms[4 * k + i, 32 * m:32 * m + 32, :] for i in range(4)])
                 for k in range(4)])[0] for m in range(3)]
    ok.append(close([jnp.sum(norms[g, o:o + 8, :], axis=0, keepdims=True)
                     for g in range(NB) for o in range(96, 160, 8)])[0])
    tokens, lo = close([jnp.sum(norms[g, 160:168, :], axis=0, keepdims=True) for g in range(NB)])
    top = jnp.max(functools.reduce(jnp.maximum, [norms[g, 168:176, :] for g in range(NB)]))
    sq = mem0[:, :512] * mem0[:, :512]
    over = jnp.max(jnp.max(sq, axis=1, keepdims=True) - jnp.sum(sq, axis=1, keepdims=True) / 8.0)
    return functools.reduce(jnp.logical_and, ok + [tokens, top <= lo / 8.0, over <= 0.0])


def _b_direct(b_ref, raw, mem0, x_tile, emit):
    def split(i, carry):
        for m in range(3):
            _interleave(_b_split_heads(raw.at[pl.ds(pl.multiple_of(RAW * m + i * 16 * H, 16), 16 * H)],
                                       b_ref.at[pl.ds(pl.multiple_of(i * 8, 8), O2), :],
                                       288 * m, 288 * (3 + m), 6 * 288))

    lax.fori_loop(0, D // 16, split, None)
    row = lax.broadcasted_iota(I32, (L, L + 8), 0)
    col = lax.broadcasted_iota(I32, (L, L + 8), 1)

    def segment(u, mem):
        x = pltpu.bitcast(_cat576(lambda n: b_ref[pl.ds(pl.multiple_of(TK + 128 * n + SEG * u, SEG), SEG), :]), F32)
        h = jnp.concatenate([mem, x, jnp.zeros((8, D), F32)], 0).astype(BF16)

        def head(i, acc):
            q, k, v = [_dot(h, pltpu.bitcast(b_ref[pl.ds(pl.multiple_of(288 * (3 * i + m), 8), 288), :], BF16))
                       for m in range(3)]
            s = jnp.where((row < M) | (row >= col), _dot_nt(q[:L], k.astype(BF16)) * DH ** -0.5, NEG)
            s = jnp.where(col < L, s, -jnp.inf)
            e = jnp.exp(s - jnp.max(s, axis=1, keepdims=True))
            o = _dot(e / jnp.sum(e, axis=1, keepdims=True), v.astype(BF16))
            return acc + _dot_nt(o, raw[pl.ds(pl.multiple_of(3 * RAW + D * i, 16), D), :])

        out = lax.fori_loop(0, H, head, jnp.zeros((L, D), F32))
        for n in range(5):
            c = min(128 * n, D - 128)
            b_ref[pl.ds(pl.multiple_of(RE + 128 * n + SEG * u, 8), SEG), :] = pltpu.bitcast(out[M:, c:c + 128], I32)
        return out[:M]

    def block(j, mem):
        for n in range(5):
            _Arena(b_ref).stf(TK + 128 * n, x_tile(j, n).T.astype(F32))
        mem = lax.fori_loop(0, U, segment, mem)
        for n in range(5):
            emit(j, n, _Arena(b_ref).ldf(RE + 128 * n, 128).T[64 * (n // 4):])
        return mem

    lax.fori_loop(0, NB, block, mem0)


def _kernel(xt_hbm, wqkv_hbm, wo_hbm, mem_hbm, gate_hbm, wq_hbm, wk_hbm, wv_hbm, wot_hbm,
            out_hbm,
            xt, wqkv, wo, mem_ref, gate_ref, raw, a_ref, b_ref, qkv_all, o_all, o_last, ga_all, omg, out_buf,
            norms, offs, sem_in, sem_w, sem_out):
    A, B = _Arena(a_ref), _Arena(b_ref)
    wot = raw.at[pl.ds(3 * RAW, H * D)]

    def cols(src, dst, c0, c1, sem):
        return pltpu.make_async_copy(src.at[:, pl.ds(c0, c1 - c0)], dst.at[:, pl.ds(c0, c1 - c0)], sem_in.at[sem])

    def rows(r0, r1, sem):
        return [pltpu.make_async_copy(w.at[pl.ds(r0 * H, (r1 - r0) * H)],
                                      raw.at[pl.ds(RAW * m + r0 * H, (r1 - r0) * H)], sem_w.at[sem])
                for m, w in enumerate((wq_hbm, wk_hbm, wv_hbm))]

    def x_stage(j, slot):
        A.stb(AX + 288 * slot, xt[:, pl.ds(pl.multiple_of(j * 128, 128), 128)])

    def x_tile(j, n):
        block = pl.ds(pl.multiple_of(j * 128, 128), 128)
        return xt[128 * n:128 * n + 128, block] if n < 4 else jnp.concatenate([xt[512:D, block]] * 2, 0)

    def x_transpose(j):
        sq = []
        for n in range(5):
            t = x_tile(j, n)
            B.stb(XN + 64 * n, t.T)
            if n < 4:
                parts = _squares(t)
                sq += [part[i:i + 8] for i in range(0, 64, 8) for part in parts]
        norms[j, 160:168, :] = functools.reduce(jnp.add, sq)
        norms[j, 168:176, :] = functools.reduce(jnp.maximum, sq)

    def x_tail(u):
        B.stf(_lh(u, 0) + M, B.ldb(XN + 256 + 16 * u, 16).astype(F32))

    def tick_raw(r):
        raw[D * H:D * H + 8, :] = r[:8].astype(BF16)

    def proj(j):
        if isinstance(j, int):
            return _Arena(qkv_all.at[pl.ds((j + 1) % 5 * SLOT, SLOT)])
        return _Arena(qkv_all.at[pl.ds(pl.multiple_of(offs[lax.rem(j + 1, 5)], 8), SLOT)])

    def raw_from(i, n):
        return raw.at[pl.ds(pl.multiple_of(offs[5 + i], 16), 2 * RAW + n * H)]

    x_copy = [cols(xt_hbm, xt, c0, c1, i) for i, (c0, c1) in enumerate(((0, 256), (256, 768), (768, S)))]
    w_copy = [cols(wqkv_hbm, wqkv, c0, c1, 3 + i) for i, (c0, c1) in
              enumerate(((512, 896), (896, 1152), (0, 512), (1152, 3 * D)))]
    wo_copy = pltpu.make_async_copy(wo_hbm, wo, sem_in.at[7])
    mem_copy = pltpu.make_async_copy(mem_hbm, mem_ref, sem_in.at[8])
    gate_copy = pltpu.make_async_copy(gate_hbm, gate_ref, sem_in.at[9])
    tail_copies, main_copies = rows(512, D, 0), rows(0, 512, 1)
    wot_copy = pltpu.make_async_copy(wot_hbm, wot, sem_w.at[2])
    for c in (w_copy[0], gate_copy, mem_copy, w_copy[1], x_copy[0], w_copy[2], w_copy[3], wo_copy):
        c.start()

    for i in range(5):
        offs[i] = i * SLOT
    for i in range(18):
        offs[5 + i] = 32 * H * i
    for i in range(NB):
        offs[23 + i] = 3 * RAW + 2 * D * i
    A.stb(SUMS, _b_sum_matrix())
    B.stf(OF + H * SEG, jnp.zeros((B_ROWS - OF - H * SEG, 128), F32))
    B.stf(AC, jnp.zeros((NPR * SEG, 128), F32))
    w_copy[0].wait()
    gate_copy.wait()
    mem_copy.wait()
    gate = jnp.broadcast_to(gate_ref[...].astype(F32)[None, :], (8, D))
    mem0 = mem_ref[...].astype(F32)
    for k in range(4):
        A.stf(GW + 8 * k, gate[:, 128 * k:128 * k + 128])
    A.stf(GW + 32, jnp.concatenate([gate[:, 512:]] * 2, 1))
    _b_place_memory(B, 0, [mem0[:, 128 * k:128 * k + 128] for k in range(4)]
                    + [jnp.concatenate([mem0[:, 512:]] * 2, 1)])

    def project(j, *parts):
        return _a_qkv(A, AX + 288 * j, proj(j), parts, first=j == 0)

    _a_transpose_w(A, wqkv, range(4, 7))
    w_copy[1].wait()
    _a_transpose_w(A, wqkv, range(7, 9))
    x_copy[0].wait()
    x_stage(0, 0)
    x_stage(1, 1)
    _interleave(project(0, 3, 1))
    x_transpose(0)
    for u in range(U):
        x_tail(u)
        _b_place_tokens(B, u)
    x_transpose(1)
    w_copy[2].wait()
    x_copy[1].start()
    _a_transpose_w(A, wqkv, range(0, 4))
    _interleave(_chain(project(1, 3, 1), project(0, 0)))
    w_copy[3].wait()
    x_copy[2].start()
    _a_transpose_w(A, wqkv, range(9, 14))
    _interleave(_chain(project(1, 0), project(0, 2)))
    wo_copy.wait()
    for c in tail_copies:
        c.start()
    _interleave(project(1, 2))
    _a_transpose_wo(A, wo)
    qkv_all[AK:AG, :] = jnp.broadcast_to(qkv_all[SLOT + AK:SLOT + AG, :1], (AG - AK, 128))

    def project_out(j0, n, tick=lambda r: None):
        return _chain(*[_a_out(A, o_all.at[j0 + b], ga_all.at[j0 + b], tick) for b in range(n)])

    def attend_trip(t, carry):
        @pl.when(t == 1)
        def _():
            x_copy[2].wait()
            wot_copy.start()

        _interleave(
            _chain(*[_chain(_a_qkv(A, AX + 288 * i, proj(2 * t + 2 + i)),
                            _once(x_stage, jnp.minimum(2 * t + 4 + i, NB - 1), i)) for i in range(2)]),
            _chain(*[_a_attend(j, proj(j), proj(j - 1), o_all.at[j], omg) for j in (2 * t, 2 * t + 1)]),
            span=(-0.04, 0.87))

    x_copy[1].wait()
    for c in main_copies:
        c.start()
    x_stage(2, 0)
    x_stage(3, 1)
    lax.fori_loop(0, NB // 2 - 1, attend_trip, None)

    def last_trip(t, carry):
        def tick(r):
            qkv_all[TICK:TICK + 8, :] = pltpu.bitcast(r[:8], I32)
            tick_raw(r)

        j = NB - 2 + t
        src, dst = raw_from(16 + t, 32), b_ref.at[pl.ds(pl.multiple_of(t * 16, 16), O2), :]
        _interleave(
            project_out(3 * t, 3, tick), _a_attend(j, proj(j), proj(j - 1), o_last.at[t], omg),
            _chain(*[_b_split_heads(src.at[pl.ds(RAW * m, 32 * H)], dst, even, odd) for m, (even, odd) in
                     enumerate(((Q2, Q2 + 32), (K2 + 32, K2), (V2, V2 + 32)))]),
            span=(-0.08, 0.82))

    for c in tail_copies:
        c.wait()
    lax.fori_loop(0, 2, last_trip, None)
    o_all[NB - 2:, :288, :] = o_last[:, :288, :]

    def prepare_trip(t, carry):
        src, dst = raw_from(t, 416), b_ref.at[pl.ds(pl.multiple_of(t * 16, 16), O2), :]
        _interleave(project_out(6 + 2 * t, 2), _chain(*[
            _b_product_tiles(A, src.at[pl.ds(RAW * m, 416 * H)], dst, m * NPR * 64) for m in range(3)]),
            span=(-0.04, 0.93))

    for c in main_copies:
        c.wait()
    lax.fori_loop(0, 4, prepare_trip, None)
    wot_copy.wait()
    _interleave(
        _chain(project_out(NB - 2, 2),
               *[_once(_b_project, B, U - 1, mat, g, 0) for mat in range(3) for g in range(NG)]),
        _b_transpose_wo(B, wot))

    def tail_sum(last, first_steps):
        lane = lax.broadcasted_iota(I32, (64, 128), 1)
        return functools.reduce(jnp.add, [B.ldf(B2 + 64 * last, 64)] + [
            jnp.where(lane < SEG * (u + 1) if first_steps else lane >= SEG * (u + 1), B.ldf(B2 + 64 * u, 64), 0.0)
            for u in range(U - 1)])

    def mix(j, n, bt):
        part = slice(128 * n, 128 * n + bt.shape[0])
        w = jnp.concatenate([omg[j]] * (bt.shape[0] // 8), 0)
        out_buf[j, part, :] = (ga_all[j, part, :] + w * bt).astype(BF16)

    def out_copy(j):
        return pltpu.make_async_copy(
            out_buf.at[j], out_hbm.at[:, pl.ds(pl.multiple_of(j * 128, 128), 128)], sem_out)

    def b_body(g, carry):
        done = jnp.maximum(g - 1, 0)
        B.stf(B2 + 64 * U, tail_sum(U - 1, True))
        weights = _b_norms(raw_from(g, 32), raw.at[pl.ds(pl.multiple_of(offs[23 + g], 16), 2 * D)], norms.at[g])

        def spare(r):
            tick_raw(r)
            next(weights)

        for u in range(U):
            def emit(stage):
                if u == 1:
                    for n in range(4):
                        if stage:
                            mix(done, n, B.ldf(PS + 128 * n, 128))
                        else:
                            B.stf(PS + 128 * n, B.ldf(BO + 128 * n, 128).T)
                if u == U - 1 and stage:
                    mix(done, 4, tail_sum(U, False))

            def after_use():
                x_tail(u)
                if u == 0:
                    _b_place_tokens(B, U - 1)
                if u < U - 1:
                    _b_place_tokens(B, u)
                else:
                    x_transpose(jnp.minimum(g + 2, NB - 1))

            _b_step(B, u, emit, after_use, spare)
        assert next(weights, "end") == "end"

        @pl.when(g > 0)
        def _():
            out_copy(done).start()

        return carry

    lax.fori_loop(0, NB, b_body, 0)
    acc = {}
    for g in range(NG):
        for p in TURN[1]:
            _b_out_product(B, 0, p, g, acc, 0)
    _b_out_collect(B, 0)
    B.stf(B2 + 64 * U, tail_sum(U - 1, True))
    for u in range(U - 1):
        _b_out_tail(B, u)
    for n in range(4):
        mix(NB - 1, n, B.ldf(BO + 128 * n, 128).T)
    mix(NB - 1, 4, tail_sum(U, False))
    out_copy(NB - 1).start()
    one_scale = _b_one_scale(norms, mem_ref[...].astype(F32))
    for j in range(NB):
        out_copy(j).wait()

    @pl.when(jnp.logical_not(one_scale))
    def _():
        _b_direct(b_ref, raw, mem_ref[...].astype(F32), x_tile, mix)
        copies = [out_copy(j) for j in range(NB)]
        for c in copies:
            c.start()
        for c in copies:
            c.wait()


@functools.partial(jax.jit, static_argnames=("B_seg_len",))
def pallas_gated_mix__sliding_local_dilated__memory_aug_recurrent_mem_tr__prompt_kernel(
    A_x: jax.Array,
    A_wqkv: jax.Array,
    A_wo: jax.Array,
    B_x: jax.Array,
    B_mem0: jax.Array,
    B_Wq: jax.Array,
    B_Wk: jax.Array,
    B_Wv: jax.Array,
    B_Wo: jax.Array,
    B_seg_len: int,
    gate_w: jax.Array,
):
    del B_x
    assert A_x.shape == (1, S, D) and B_mem0.shape == (1, M, D) and B_Wq.shape == (D, H, DH)
    assert B_seg_len == SEG
    hbm = pl.BlockSpec(memory_space=pl.ANY)
    out_t = pl.pallas_call(
        _kernel,
        out_shape=jax.ShapeDtypeStruct((D, S), BF16),
        in_specs=[hbm] * 9,
        out_specs=hbm,
        scratch_shapes=[
            pltpu.VMEM((D, S), BF16),
            pltpu.VMEM((D, 3 * D), BF16),
            pltpu.VMEM((D, D), BF16),
            pltpu.VMEM((M, D), BF16),
            pltpu.VMEM((D,), BF16),
            pltpu.VMEM((4 * RAW, DH), BF16),
            pltpu.VMEM((A_ROWS, 128), I32),
            pltpu.VMEM((B_ROWS, 128), I32),
            pltpu.VMEM((5 * SLOT, 128), I32),
            pltpu.VMEM((NB, 296, 128), I32),
            pltpu.VMEM((2, 296, 128), I32),
            pltpu.VMEM((NB, D, 128), F32),
            pltpu.VMEM((NB, 8, 128), F32),
            pltpu.VMEM((NB, D, 128), BF16),
            pltpu.VMEM((NB, 176, 128), F32),
            pltpu.SMEM((39,), I32),
            pltpu.SemaphoreType.DMA((10,)),
            pltpu.SemaphoreType.DMA((3,)),
            pltpu.SemaphoreType.DMA,
        ],
        compiler_params=pltpu.CompilerParams(vmem_limit_bytes=110 * 1024 * 1024),
    )(
        A_x.reshape(S, D).T, A_wqkv, A_wo, B_mem0.reshape(M, D), gate_w,
        B_Wq.reshape(D * H, DH), B_Wk.reshape(D * H, DH), B_Wv.reshape(D * H, DH),
        B_Wo.transpose(0, 2, 1).reshape(H * D, DH),
    )
    return out_t.T.reshape(1, S, D)
```

```python
import functools

import jax
import jax.numpy as jnp
import numpy as np
from jax import lax
import jax.experimental.pallas as pl
import jax.experimental.pallas.tpu as pltpu

F32, BF16, I32 = jnp.float32, jnp.bfloat16, jnp.int32

S, D = 2048, 576
NB = S // 128
DA, WIN, DIL = 18, 8, 2
H, DH, M, SEG = 32, 128, 8, 32
L = M + SEG
NP = H // 2
NG = H // 4
U = 128 // SEG
NEG = -1000000000.0

PRODUCTS = tuple(tuple({(int(t[1]), int(t[2])): int(t[0] + "1") for t in form.split()} for form in p) for p in (
    ("+00 -10", "-03 +30 -10 +00 -02", "+00"),
    ("+10", "+03 -30 +00 -01 -20", "+00 +10"),
    ("+03 -13", "-13 -32 +33", "+03"),
    ("+13", "-23 -31 +33", "+03 +13"),
    ("+02 +10", "-02 +20", "+00 -12"),
    ("+02", "-02 -21 +22 -32", "+02 +12"),
    ("+02 -12", "-12 -20 +22 -23", "-12"),
    ("+00 +02", "+02", "+00 +02"),
    ("+10 +12", "+20", "+10 +12"),
    ("+02 +13", "+23 -32", "+03 -12"),
    ("+02 +03", "+32", "+02 +03"),
    ("+12 +13", "+23", "+12 +13"),
    ("+00 +01 -10", "+03 -30 +10 -01", "+00 +10 +11"),
    ("+01", "+03 -01 +11 -12 -31", "+01"),
    ("+11", "+10 -30 -11 +13 +21", "-11"),
    ("+00 +01", "-03 +01", "+00 +01 +10 +11"),
    ("+11 +12", "+21", "+01 +02 +11 +12"),
    ("-02 +11 +12", "+12 -21", "+01 +02 +12"),
    ("+01 +03", "-03 +31", "+01 +03 +11 +13"),
    ("+10 +11 +13", "+30", "+10 +11 +13"),
    ("+01 +03 -13", "-13 +31", "-03 -11 -13"),
    ("+00 +01 +03", "+03", "+00 +01 +03"),
    ("+00 +01 -10 -11", "+10 -30", "-10 -11"),
    ("+01 +02 -11 -12", "+12", "+01 +02"),
    ("+01 +03 -11 -13", "-30 +13", "-11 -13"),
    ("+01 +03 +10", "-03 +30", "+00 -11 -13"),
))
NPR = len(PRODUCTS)
TURN = tuple(tuple(p for p, (a, _, c) in enumerate(PRODUCTS)
                   if any(k[0] == r for k in a) and any(k[0] == r for k in c)) for r in range(2))
ORDER = ((2, 9, 5, 10, 17, 23, 7, 4, 21, 20, 18, 25, 15, 0, 13, 12),
         (17, 16, 14, 4, 1, 22, 12, 8, 19, 25, 24, 20, 11, 3, 9, 6))
LONG = tuple(p for p in range(NPR) if len(PRODUCTS[p][1]) == 5)


def _is_matrix_product():
    t = np.zeros((2, 4, 4, 4, 2, 4), int)
    for a, w, c in PRODUCTS:
        for i in a:
            for j in w:
                for k in c:
                    t[i + j + k] += a[i] * w[j] * c[k]
    return (t == np.einsum("rs,kl,nm->rklnsm", np.eye(2), np.eye(4), np.eye(4))).all()


assert _is_matrix_product() and len(set(TURN[0] + TURN[1])) == NPR
assert all(sorted(ORDER[r]) == list(TURN[r]) for r in range(2))

GSTRIDE = 3 * NPR * 64 + 4
Q2 = NG * GSTRIDE
K2 = Q2 + 64
V2 = K2 + 64
PSTRIDE = 192 + 4
OA = Q2 + NP * PSTRIDE
O2 = OA + NG * NPR * 64
O2T = O2 + NP * 64
LH = O2T + H * 32
GS = LH + U * 18 * L
TK = GS + 64
MQ = TK + 3 * H * 128
VS = MQ + H * M
KS = VS + H * 40
RE = KS + NP * 64
PS = RE + H * L
RS = PS + NP * L
AC = RS + NP * L
XN = AC + NPR * SEG
OM = XN + 320
OF = OM + H * M
BO = OF + (U + 1) * H * SEG
B2 = BO + 512
B_ROWS = B2 + 64 * (U + 1)

RAW = D * H + 16

WT = 0
GW = WT + 5 * 1728
WP = GW + 40
WOT = WP + 27 * 160
AX = WOT + 5 * 288
SUMS = AX + 2 * 288
A_ROWS = SUMS + 4 * len(LONG) + 24
AQ, AK, AV, AG, TICK, SLOT = 0, 576, 864, 1152, 1160, 1168


def _dot(a, b):
    return lax.dot_general(a, b, (((1,), (0,)), ((), ())), preferred_element_type=F32)


def _dot_nt(a, b):
    return lax.dot_general(a, b, (((1,), (1,)), ((), ())), preferred_element_type=F32)


class _Arena:
    def __init__(self, ref):
        self.r = ref

    def ldi(self, o, n):
        return self.r[o:o + n, :]

    def ldf(self, o, n):
        return pltpu.bitcast(self.r[o:o + n, :], F32)

    def ldb(self, o, n):
        return pltpu.bitcast(self.r[o:o + n, :], BF16)

    def stf(self, o, v):
        self.r[o:o + v.shape[0], :] = pltpu.bitcast(v, I32)

    def stb(self, o, v):
        self.r[o:o + v.shape[0] // 2, :] = pltpu.bitcast(v.astype(BF16), I32)


def _signed_sum(terms):
    sign, acc = terms[0]
    for c, t in terms[1:]:
        if c == sign:
            acc = acc + t
        else:
            sign, acc = 1, acc - t if sign > 0 else t - acc
    return acc if sign > 0 else -acc


def _interleave(main, *side, span=(0.0, 0.9)):
    jobs = (main,) + side
    order = [((i + 1) / main[0], 0) for i in range(main[0])]
    order += [(span[0] + (span[1] - span[0]) * i / n, k + 1) for k, (n, _) in enumerate(side) for i in range(n)]
    for _, k in sorted(order):
        next(jobs[k][1])
    for _, gen in jobs:
        assert next(gen, "end") == "end"


def _once(fn, *args):
    def gen():
        fn(*args)
        yield
    return 1, gen()


def _chain(*jobs):
    def gen():
        for _, g in jobs:
            yield from g
    return sum(n for n, _ in jobs), gen()


def _tile_t(w_ref, k, c):
    t = w_ref[128 * k:min(128 * k + 128, w_ref.shape[0]), 128 * c:min(128 * c + 128, w_ref.shape[1])]
    nk, nc = t.shape
    if nc < 128:
        t = jnp.concatenate([t, jnp.zeros((nk, 128 - nc), t.dtype)], 1)
    if nk < 128:
        t = jnp.concatenate([t, jnp.zeros((128 - nk, 128), t.dtype)], 0)
    return t.T[:nc]


def _a_transpose_w(A, w_ref, cblocks):
    for c in cblocks:
        for k in range(5):
            A.stf(WT + 1728 * k + 128 * c, _tile_t(w_ref, k, c).astype(F32))


def _a_transpose_wo(A, w_ref):
    for c in range(5):
        for k in range(5):
            A.stb(WOT + 288 * k + 64 * c, _tile_t(w_ref, k, c))


def _cat576(chunk):
    ch = [chunk(k) for k in range(5)]
    return jnp.concatenate(ch[:4] + [ch[4][:, :64]], 1)


def _a_qkv(A, x_off, dst, parts=(3, 1, 0, 2), first=False):
    def gen():
        for part in parts:
            if part == 3:
                dst.stf(AG, jax.nn.sigmoid(_dot(_cat576(lambda k: A.ldf(GW + 8 * k, 8)), A.ldb(x_off, 288))))
                continue
            for d0 in range(0, DA, 2):
                def weights(k):
                    packed = WP + 160 * (9 * part + d0 // 2) + 32 * k
                    if not first:
                        return A.ldb(packed, 32)
                    w = jnp.concatenate([
                        pltpu.bitcast(A.r[pl.ds(WT + 1728 * k + D * part + 8 * DA * hg + d, 8, stride=DA), :], F32)
                        for hg in range(4) for d in (d0, d0 + 1)], 0)
                    A.stb(packed, w)
                    return w

                r = _dot(_cat576(weights), A.ldb(x_off, 288))
                for i in range(0, 64, 16):
                    if part == 0:
                        dst.stf(AQ + 32 * d0 + i, r[i:i + 16])
                    else:
                        dst.stb((AK if part == 1 else AV) + 16 * d0 + i // 2, r[i:i + 16])
                    yield
    return sum(2 * DA for p in parts if p < 3), gen()


def _a_attend(j, cur, old, o_ref, omg_ref):
    lane = lax.broadcasted_iota(I32, (8, 128), 1)
    wraps = {w: lane >= 128 - DIL * w for w in range(1, WIN)}

    def window(o):
        c, p = cur.ldi(o, 8), old.ldi(o, 8)
        out = []
        for w in range(WIN):
            t = pltpu.roll(lax.select(wraps[w], p, c), DIL * w, 1) if w else c
            out.append(pltpu.bitcast(t, BF16).astype(F32))
        return out

    def gen():
        pos = j * 128 + lane
        for hg in range(4):
            lg = None
            for d in range(0, DA, 2):
                q = cur.ldf(AQ + 32 * d + 16 * hg, 16)
                pr = [q * kw for kw in window(AK + 16 * d + 8 * hg)]
                pr = [t[:8] + t[8:] for t in pr]
                lg = pr if d == 0 else [a + b for a, b in zip(lg, pr)]
                yield
            lg = [jnp.where(pos >= DIL * w, t * DA ** -0.5, NEG) for w, t in enumerate(lg)]
            mx = functools.reduce(jnp.maximum, lg)
            e = [jnp.exp(t - mx) for t in lg]
            g = cur.ldf(AG, 8)
            if hg == 0:
                omg_ref[j] = 1.0 - g
            r = g / functools.reduce(jnp.add, e)
            p = [jnp.concatenate([t * r] * 2, 0) for t in e]
            yield
            for d in range(0, DA, 2):
                o = functools.reduce(jnp.add, [a * b for a, b in zip(p, window(AV + 16 * d + 8 * hg))])
                o = pltpu.bitcast(o.astype(BF16).astype(F32), I32)
                o_ref[pl.ds(4 * DA * hg + d // 2, 8, stride=DA // 2), :] = (
                    lax.shift_right_logical(o[:8], 16) | o[8:])
                yield
    return 4 * DA + 4, gen()


def _a_out(A, o_ref, ga_ref, tick):
    def gen():
        for r0 in range(0, D, 96):
            r = _dot(_cat576(lambda k: A.ldb(WOT + 288 * k + r0 // 2, 48)), pltpu.bitcast(o_ref[:288, :], BF16))
            for i in range(0, 96, 32):
                tick(r[i:i + 32])
                ga_ref[r0 + i:r0 + i + 32, :] = r[i:i + 32]
                yield
    return D // 32, gen()


def _pairs(g):
    return g, g + NG


def _heads(g):
    return [2 * j + i for j in _pairs(g) for i in range(2)]


def _b_split_heads(raw, dst, even, odd, stride=PSTRIDE):
    def gen():
        for r in range(raw.shape[0] // 64):
            e = pltpu.bitcast(raw[64 * r:64 * r + 32, :], I32)
            o = pltpu.bitcast(raw[64 * r + 32:64 * r + 64, :], I32)
            dst[pl.ds(even + r, NP, stride=stride), :] = (e & 0xFFFF) | (o << 16)
            dst[pl.ds(odd + r, NP, stride=stride), :] = lax.shift_right_logical(e, 16) | (o & -65536)
            yield
    return raw.shape[0] // 64, gen()


def _b_sum_matrix():
    g = lax.broadcasted_iota(I32, (8, 128), 0)
    lane = lax.broadcasted_iota(I32, (8, 128), 1)
    return jnp.concatenate([functools.reduce(jnp.add, [
        jnp.where(lane == H * k + _heads(0)[n] + 2 * g, float(c), 0.0) for (k, n), c in PRODUCTS[p][1].items()])
        for p in LONG], 0)


def _b_product_tiles(A, raw, dst, off):
    def gen():
        for r in range(16):
            t = [jnp.concatenate([raw[o:o + H, :] for o in range(64 * r + H * i, 512 * H, 128 * H)], 0)
                 for i in range(2)]
            long = [_dot(A.ldb(SUMS, 4 * len(LONG)), v) for v in t]
            word = [pltpu.bitcast(v, I32) for v in t]

            @functools.cache
            def block(k, n, i):
                v = word[i][16 * k + 8 * (n // 2):16 * k + 8 * (n // 2) + 8]
                return pltpu.bitcast(v & -65536 if n % 2 else v << 16, F32)

            for p, (_, w, _) in enumerate(PRODUCTS):
                e, o = [pltpu.bitcast(
                    long[i][8 * LONG.index(p):8 * LONG.index(p) + 8] if p in LONG else
                    _signed_sum([(c, block(k, n, i)) for (k, n), c in w.items()]), I32) for i in range(2)]
                if len(w) > 1:
                    e, o = e + 0x8000, (o + 0x7FFF) & -65536
                dst[pl.ds(off + p * 64 + r, NG, stride=GSTRIDE), :] = lax.shift_right_logical(e, 16) | o
            yield
    return 16, gen()


def _b_transpose_wo(B, wot):
    def gen():
        for g in range(NG):
            for p, (_, w, _) in enumerate(PRODUCTS):
                t = [(c, wot[pl.ds(D * _heads(g)[k] + 128 * n, 128), :]) for (k, n), c in w.items()]
                if len(t) > 1 or t[0][0] < 0:
                    t = [(1, _signed_sum([(c, v.astype(F32)) for c, v in t]).astype(BF16))]
                B.stb(OA + (g * NPR + p) * 64, t[0][1].T)
                yield
            for j in _pairs(g):
                t = jnp.concatenate([wot[D * h + 512:D * h + D, :] for h in (2 * j, 2 * j + 1)], 0)
                B.stb(O2T + 64 * j, t)
                B.stb(O2 + 64 * j, t.T)
                B.stb(K2 + PSTRIDE * j, B.ldb(K2 + PSTRIDE * j, 64).T)
    return NG * NPR, gen()


def _turn(u):
    return 1 - u % 2


def _halves(p, r):
    return (r,) if p in TURN[1 - r] else (0, 1)


def _lh(u, i):
    return LH + L * (18 * (u % U) + i)


def _b_place_memory(B, u, mem):
    r = _turn(u)
    for i, p in enumerate(TURN[r]):
        B.stf(_lh(u, 2 + i), _signed_sum([(s, mem[k]) for (rr, k), s in PRODUCTS[p][0].items() if rr == r]))
    for i in range(2):
        B.stf(_lh(u, i), mem[4])


def _b_place_tokens(B, u):
    r = _turn(u)
    top = (u + 1 - r) % U

    def x(seg, n, half):
        return B.ldb(XN + 64 * n + 16 * seg + 8 * half, 8).astype(F32)

    for i, p in enumerate(TURN[r]):
        for at, half in enumerate(_halves(p, r)):
            B.stf(_lh(u, 2 + i) + M + 16 * at,
                  _signed_sum([(s, x(top + rr, k, half)) for (rr, k), s in PRODUCTS[p][0].items()]))
    for half in range(2):
        B.stf(_lh(u, 1) + M + 16 * half, x((u + 1) % U, 4, half))


def _b_project(B, u, mat, g, m=M, keep=()):
    r = _turn(u)
    top = (u + 1 - r) % U
    items = [(PRODUCTS[p][2], _halves(p, r),
              _dot(B.ldf(_lh(u, 2 + TURN[r].index(p)) + M - m, m + 16 * len(_halves(p, r))),
                   B.ldb(GSTRIDE * g + (mat * NPR + p) * 64, 64))) for p in ORDER[r]]
    if mat == 0:
        items += [({(r, n): 1}, (0, 1),
                   _dot(B.ldf(_lh(u, 1) + M - m, m + SEG)[:, :64],
                        B.ldb(Q2 + PSTRIDE * (h // 2) + 32 * (h % 2), 32))) for n, h in enumerate(_heads(g))]

    def at(n, seg, half):
        return TK + 128 * (H * mat + _heads(g)[n]) + SEG * seg + 16 * half

    mem, tok, kept = {}, {}, {}
    for c, halves, y in items:
        y_mem, y_tok = y[:m] if m else None, [y[o:o + 16] for o in range(m, y.shape[0], 16)]
        for (rr, n), s in c.items():
            if m and rr == r:
                mem.setdefault(n, []).append((s, y_mem))
            for half, t in zip(halves, y_tok):
                tok.setdefault((rr, n, half), []).append((s, t))
    for (rr, n, half), terms in sorted(tok.items()):
        if r == 1:
            terms.append((1, B.ldf(at(n, top + rr, half), 16)))
        if r == 1 and rr in keep:
            kept[n, top + rr, half] = _signed_sum(terms)
        else:
            B.stf(at(n, top + rr, half), _signed_sum(terms))
    assert len(tok) == 16

    def tokens(n, seg):
        return [kept[n, seg, i] if (n, seg, i) in kept else B.ldf(at(n, seg, i), 16) for i in range(2)]

    return [_signed_sum(mem[n]) for n in sorted(mem)], tokens


def _b_out_product(B, u, p, g, acc, m=M):
    r = _turn(u)
    top = (u - 1 - r) % U
    a = PRODUCTS[p][0].items()
    lhs = [_signed_sum([(s, B.ldf(OM + M * _heads(g)[k], M)) for (rr, k), s in a if rr == r])] if m else []
    both = [k for (rr, k), s in a if rr and PRODUCTS[p][0].get((0, k)) == -s]
    first, rows = 16 * _halves(p, r)[0], 16 * len(_halves(p, r))
    lhs.append(_signed_sum([(s, B.ldf(OF + SEG * (H * (U if k in both else top + rr) + _heads(g)[k]) + first, rows))
                            for (rr, k), s in a if not (rr and k in both)]))
    y = _dot(jnp.concatenate(lhs, 0), B.ldb(OA + (g * NPR + p) * 64, 64))
    acc[p] = acc[p] + y if g else y
    if g == NG - 1:
        B.stf(AC + SEG * p + first, acc[p][m:])
        for (rr, n), s in PRODUCTS[p][2].items():
            if m and rr == r:
                acc.setdefault(("mem", n), []).append((s, acc[p][:m]))


def _b_out_collect(B, u):
    for rr in range(2):
        for n in range(4):
            B.stf(BO + 128 * n + SEG * ((u - 2 + rr) % U), _signed_sum(
                [(c[rr, n], B.ldf(AC + SEG * p, SEG)) for p, (_, _, c) in enumerate(PRODUCTS) if (rr, n) in c]))


def _b_out_tail(B, u):
    B.stf(B2 + 64 * u, functools.reduce(jnp.add, [
        _dot_nt(B.ldb(O2T + 32 * h, 32),
                jnp.concatenate([B.ldf(OF + SEG * (H * i + h), SEG) for i in range(U)], 0).astype(BF16))
        for h in range(8 * u, 8 * u + 8)]))


def _b_step(B, u, emit, after_use, spare):
    row = lax.broadcasted_iota(I32, (L, 128), 0)
    lane = lax.broadcasted_iota(I32, (L, 128), 1)
    lo = lane < 64
    lo64 = lax.broadcasted_iota(I32, (64, 128), 1) < 64
    mask = (row < M) | ((lane & 63) >= SEG) | (row - M >= (lane & 63))
    in_a, in_b = lane < L, (lane >= 64) & (lane < 64 + L)
    z24 = jnp.zeros((24, 128), F32)
    pair = [j for g in range(NG) for j in _pairs(g)]

    def h2():
        return jnp.concatenate([B.ldf(_lh(u, 0) + M, SEG), B.ldf(_lh(u, 0), M)], 0)

    def t_k(g):
        mem, tokens = _b_project(B, u, 1, g, keep=(0,))
        spare(mem[0])
        for i, j in enumerate(_pairs(g)):
            k = jnp.concatenate([t for n in (2 * i, 2 * i + 1) for t in tokens(n, u) + [mem[n], z24]], 0)
            B.stb(KS + 64 * j, k.astype(BF16).T)

    def t_q(g):
        mem = _b_project(B, u, 0, g)[0]
        for h, t in zip(_heads(g), mem):
            B.stf(MQ + M * h, t)

    def t_v(g):
        mem, tokens = _b_project(B, u, 2, g, keep=(0, 1))
        for n, h in enumerate(_heads(g)):
            B.stb(VS + 40 * h + 32, jnp.concatenate([mem[n], z24[:8]], 0))
            if _turn(u):
                B.stb(VS + 40 * h, jnp.concatenate(tokens(n, u) + tokens(n, u + 1), 0))

    def t_s(i):
        j = pair[i]
        kt, w2 = B.ldi(KS + 64 * j, 64), B.ldi(K2 + PSTRIDE * j, 64)
        ya, yb = [_dot(jnp.concatenate([B.ldf(MQ + M * h, M), B.ldf(TK + 128 * h + SEG * u, SEG)], 0),
                       pltpu.bitcast(rhs, BF16))
                  for h, rhs in ((2 * j, jnp.where(lo64, kt, w2)), (2 * j + 1, jnp.where(lo64, w2, kt)))]
        B.stf(RE + L * i, jnp.where(lo, ya, yb))
        B.stf(RE + L * (NP + i), jnp.where(lo, yb, ya))

    def t_softmax(n):
        c4 = h2()
        y = _dot_nt(jnp.concatenate([jnp.where(lo, 0.0, c4), jnp.where(lo, c4, 0.0)], 0),
                    B.ldf(RE + L * NP + 128 * n, 128).astype(BF16))
        B.stf(RS + 128 * n, jnp.concatenate([y[:L], z24, y[L:], z24], 0).T)
        for i in range(128 * n // L, 128 * (n + 1) // L):
            s = jnp.where(mask, (B.ldf(RE + L * i, L) + B.ldf(RS + L * i, L)) * DH ** -0.5, NEG)
            ma = jnp.max(jnp.where(in_a, s, -jnp.inf), axis=1, keepdims=True)
            mb = jnp.max(jnp.where(in_b, s, -jnp.inf), axis=1, keepdims=True)
            e = jnp.exp(s - jnp.where(lo, ma, mb))
            B.stf(PS + L * i, jnp.where(in_a | in_b, e, 0.0))

    def t_pv(i):
        p, r = B.ldf(PS + L * i, L), B.ldf(RS + L * i, L)
        for b, lhs in enumerate((jnp.where(lo, p, r), jnp.where(lo, r, p))):
            h = 2 * pair[i] + b
            v = [B.ldi(VS + 40 * h + 16 * (u % 2), 16), B.ldi(VS + 40 * h + 32, 8), jnp.zeros((8, 128), I32)]
            w2 = [B.ldi(V2 + PSTRIDE * pair[i] + 32 * b, 32)]
            o = _dot(lhs, pltpu.bitcast(jnp.concatenate(w2 + v if b else v + w2, 0), BF16))
            l = jnp.broadcast_to(jnp.sum(jnp.where(in_b if b else in_a, p, 0.0), axis=1, keepdims=True), (L, 128))
            rc = pltpu.reciprocal(l, approx=True)
            o = o * (rc * (2.0 - l * rc))
            B.stf(OM + M * h, o[:M])
            B.stf(OF + SEG * (H * u + h), o[M:])
            if u % 2:
                B.stf(OF + SEG * (H * U + h), B.ldf(OF + SEG * (H * (u - 1) + h), SEG) - o[M:])

    acc = {}

    def t_mem_tail(i):
        y = _dot(B.ldf(OM + 2 * M * pair[i], 2 * M), B.ldb(O2 + 64 * pair[i], 64))
        acc["tail"] = acc["tail"] + y if i else y

    for g in range(NG):
        t_k(g)
        if g == 1 and u % 2:
            _b_out_collect(B, u - 1)
    c4 = h2()
    B.stb(GS, jnp.concatenate([jnp.where(lo, 0.0, c4), z24, jnp.where(lo, c4, 0.0), z24], 0))
    lag_s, lag_softmax = 2, 4
    softmax_at = [(128 * n + 127) // L + lag_s + lag_softmax for n in range(5)]
    for i in range(2 * NP - 2):
        if i % 2 == 0:
            t_q(i // 2) if i < NP else t_v((i - NP) // 2)
        if 0 <= i - lag_s < NP:
            t_s(i - lag_s)
        if i in (2, 6):
            emit(i // 4)
        if i in softmax_at:
            t_softmax(softmax_at.index(i))
        for j in range(4 * (i - 2 * NP + 6), 4 * (i - 2 * NP + 7)):
            if j >= 0:
                B.stf(RS + L * j, _dot(B.ldf(PS + L * j, L), B.ldb(GS, 64)))
    prods = TURN[_turn(u)]
    passes = (((14, 5, 0, 12, 10), (1, 3, 4, 15), (8, 9, 6, 11), (13, 7, 2)),
              ((15, 5, 0, 12, 10), (8, 3, 4, 6, 13), (1, 7, 11), (9, 2, 14)))[_turn(u)]

    def t_out(k, g):
        for i in passes[k]:
            _b_out_product(B, u, prods[i], g, acc)
        if k < 2:
            t_mem_tail(NG * k + g)

    for g in range(NG + 2):
        if g < NG:
            t_pv(2 * g)
            t_pv(2 * g + 1)
        elif g < NG + 1:
            t_out(1, g - NG)
        if g == 2:
            t_v(NG - 1)
        if g >= 2:
            t_out(0, g - 2)
    after_use()
    for k in range(1, len(passes)):
        for g in range(1 if k == 1 else 0, NG):
            t_out(k, g)
    tail = jnp.where(lo[:M], acc["tail"][:M], acc["tail"][M:])
    _b_place_memory(B, u + 1, [_signed_sum(acc["mem", n]) for n in range(4)] + [tail + pltpu.roll(tail, 64, 1)])
    _b_out_tail(B, u)


def _squares(t):
    t = pltpu.bitcast(t, I32)
    even, odd = pltpu.bitcast(t << 16, F32), pltpu.bitcast(t, F32)
    return even * even, odd * odd


def _b_norms(qkv, wot, out):
    for m in range(3):
        acc = None
        for d in range(32):
            sq = jnp.concatenate(_squares(qkv[RAW * m + H * d:RAW * m + H * d + H, :]), 0)
            acc = acc + sq if d else sq
            if d == 31:
                out[32 * m:32 * m + 32, :] = acc
            yield acc
    for i in range(8):
        for d in range(4):
            o = D * (i // 4) + 128 * (i % 4) + 32 * d
            sq = jnp.add(*_squares(wot[o:o + 32, :]))
            acc = acc + sq if d else sq
            if d == 3:
                out[96 + 8 * i:104 + 8 * i, :] = acc[:8] + acc[8:]
            yield acc


def _b_one_scale(norms, mem0):
    def close(ts):
        lo, hi = jnp.min(functools.reduce(jnp.minimum, ts)), jnp.max(functools.reduce(jnp.maximum, ts))
        return (hi <= 4.0 * lo) & (lo > 0.0) & (hi < jnp.inf), lo

    ok = [close([functools.reduce(jnp.add, [norms[4 * k + i, 32 * m:32 * m + 32, :] for i in range(4)])
                 for k in range(4)])[0] for m in range(3)]
    ok.append(close([jnp.sum(norms[g, o:o + 8, :], axis=0, keepdims=True)
                     for g in range(NB) for o in range(96, 160, 8)])[0])
    tokens, lo = close([jnp.sum(norms[g, 160:168, :], axis=0, keepdims=True) for g in range(NB)])
    top = jnp.max(functools.reduce(jnp.maximum, [norms[g, 168:176, :] for g in range(NB)]))
    sq = mem0[:, :512] * mem0[:, :512]
    over = jnp.max(jnp.max(sq, axis=1, keepdims=True) - jnp.sum(sq, axis=1, keepdims=True) / 8.0)
    return functools.reduce(jnp.logical_and, ok + [tokens, top <= lo / 8.0, over <= 0.0])


def _b_direct(b_ref, raw, mem0, x_tile, emit):
    def split(i, carry):
        for m in range(3):
            _interleave(_b_split_heads(raw.at[pl.ds(pl.multiple_of(RAW * m + i * 16 * H, 16), 16 * H)],
                                       b_ref.at[pl.ds(pl.multiple_of(i * 8, 8), O2), :],
                                       288 * m, 288 * (3 + m), 6 * 288))

    lax.fori_loop(0, D // 16, split, None)
    row = lax.broadcasted_iota(I32, (L, L + 8), 0)
    col = lax.broadcasted_iota(I32, (L, L + 8), 1)

    def segment(u, mem):
        x = pltpu.bitcast(_cat576(lambda n: b_ref[pl.ds(pl.multiple_of(TK + 128 * n + SEG * u, SEG), SEG), :]), F32)
        h = jnp.concatenate([mem, x, jnp.zeros((8, D), F32)], 0).astype(BF16)

        def head(i, acc):
            q, k, v = [_dot(h, pltpu.bitcast(b_ref[pl.ds(pl.multiple_of(288 * (3 * i + m), 8), 288), :], BF16))
                       for m in range(3)]
            s = jnp.where((row < M) | (row >= col), _dot_nt(q[:L], k.astype(BF16)) * DH ** -0.5, NEG)
            s = jnp.where(col < L, s, -jnp.inf)
            e = jnp.exp(s - jnp.max(s, axis=1, keepdims=True))
            o = _dot(e / jnp.sum(e, axis=1, keepdims=True), v.astype(BF16))
            return acc + _dot_nt(o, raw[pl.ds(pl.multiple_of(3 * RAW + D * i, 16), D), :])

        out = lax.fori_loop(0, H, head, jnp.zeros((L, D), F32))
        for n in range(5):
            c = min(128 * n, D - 128)
            b_ref[pl.ds(pl.multiple_of(RE + 128 * n + SEG * u, 8), SEG), :] = pltpu.bitcast(out[M:, c:c + 128], I32)
        return out[:M]

    def block(j, mem):
        for n in range(5):
            _Arena(b_ref).stf(TK + 128 * n, x_tile(j, n).T.astype(F32))
        mem = lax.fori_loop(0, U, segment, mem)
        for n in range(5):
            emit(j, n, _Arena(b_ref).ldf(RE + 128 * n, 128).T[64 * (n // 4):])
        return mem

    lax.fori_loop(0, NB, block, mem0)


def _kernel(xt_hbm, wqkv_hbm, wo_hbm, mem_hbm, gate_hbm, wq_hbm, wk_hbm, wv_hbm, wot_hbm,
            out_hbm,
            xt, wqkv, wo, mem_ref, gate_ref, raw, a_ref, b_ref, qkv_all, o_all, o_last, ga_all, omg, out_buf,
            norms, offs, sem_in, sem_w, sem_out):
    A, B = _Arena(a_ref), _Arena(b_ref)
    wot = raw.at[pl.ds(3 * RAW, H * D)]

    def cols(src, dst, c0, c1, sem):
        return pltpu.make_async_copy(src.at[:, pl.ds(c0, c1 - c0)], dst.at[:, pl.ds(c0, c1 - c0)], sem_in.at[sem])

    def rows(r0, r1, sem):
        return [pltpu.make_async_copy(w.at[pl.ds(r0 * H, (r1 - r0) * H)],
                                      raw.at[pl.ds(RAW * m + r0 * H, (r1 - r0) * H)], sem_w.at[sem])
                for m, w in enumerate((wq_hbm, wk_hbm, wv_hbm))]

    def x_stage(j, slot):
        A.stb(AX + 288 * slot, xt[:, pl.ds(pl.multiple_of(j * 128, 128), 128)])

    def x_tile(j, n):
        block = pl.ds(pl.multiple_of(j * 128, 128), 128)
        return xt[128 * n:128 * n + 128, block] if n < 4 else jnp.concatenate([xt[512:D, block]] * 2, 0)

    def x_transpose(j):
        sq = []
        for n in range(5):
            t = x_tile(j, n)
            B.stb(XN + 64 * n, t.T)
            if n < 4:
                parts = _squares(t)
                sq += [part[i:i + 8] for i in range(0, 64, 8) for part in parts]
        norms[j, 160:168, :] = functools.reduce(jnp.add, sq)
        norms[j, 168:176, :] = functools.reduce(jnp.maximum, sq)

    def x_tail(u):
        B.stf(_lh(u, 0) + M, B.ldb(XN + 256 + 16 * u, 16).astype(F32))

    def tick_raw(r):
        raw[D * H:D * H + 8, :] = r[:8].astype(BF16)

    def proj(j):
        if isinstance(j, int):
            return _Arena(qkv_all.at[pl.ds((j + 1) % 5 * SLOT, SLOT)])
        return _Arena(qkv_all.at[pl.ds(pl.multiple_of(offs[lax.rem(j + 1, 5)], 8), SLOT)])

    def raw_from(i, n):
        return raw.at[pl.ds(pl.multiple_of(offs[5 + i], 16), 2 * RAW + n * H)]

    x_copy = [cols(xt_hbm, xt, c0, c1, i) for i, (c0, c1) in enumerate(((0, 256), (256, 768), (768, S)))]
    w_copy = [cols(wqkv_hbm, wqkv, c0, c1, 3 + i) for i, (c0, c1) in
              enumerate(((512, 896), (896, 1152), (0, 512), (1152, 3 * D)))]
    wo_copy = pltpu.make_async_copy(wo_hbm, wo, sem_in.at[7])
    mem_copy = pltpu.make_async_copy(mem_hbm, mem_ref, sem_in.at[8])
    gate_copy = pltpu.make_async_copy(gate_hbm, gate_ref, sem_in.at[9])
    tail_copies, main_copies = rows(512, D, 0), rows(0, 512, 1)
    wot_copy = pltpu.make_async_copy(wot_hbm, wot, sem_w.at[2])
    for c in (w_copy[0], gate_copy, mem_copy, w_copy[1], x_copy[0], w_copy[2], w_copy[3], wo_copy):
        c.start()

    for i in range(5):
        offs[i] = i * SLOT
    for i in range(18):
        offs[5 + i] = 32 * H * i
    for i in range(NB):
        offs[23 + i] = 3 * RAW + 2 * D * i
    A.stb(SUMS, _b_sum_matrix())
    B.stf(OF + H * SEG, jnp.zeros((B_ROWS - OF - H * SEG, 128), F32))
    B.stf(AC, jnp.zeros((NPR * SEG, 128), F32))
    w_copy[0].wait()
    gate_copy.wait()
    mem_copy.wait()
    gate = jnp.broadcast_to(gate_ref[...].astype(F32)[None, :], (8, D))
    mem0 = mem_ref[...].astype(F32)
    for k in range(4):
        A.stf(GW + 8 * k, gate[:, 128 * k:128 * k + 128])
    A.stf(GW + 32, jnp.concatenate([gate[:, 512:]] * 2, 1))
    _b_place_memory(B, 0, [mem0[:, 128 * k:128 * k + 128] for k in range(4)]
                    + [jnp.concatenate([mem0[:, 512:]] * 2, 1)])

    def project(j, *parts):
        return _a_qkv(A, AX + 288 * j, proj(j), parts, first=j == 0)

    _a_transpose_w(A, wqkv, range(4, 7))
    w_copy[1].wait()
    _a_transpose_w(A, wqkv, range(7, 9))
    x_copy[0].wait()
    x_stage(0, 0)
    x_stage(1, 1)
    _interleave(project(0, 3, 1))
    x_transpose(0)
    for u in range(U):
        x_tail(u)
        _b_place_tokens(B, u)
    x_transpose(1)
    w_copy[2].wait()
    x_copy[1].start()
    _a_transpose_w(A, wqkv, range(0, 4))
    _interleave(_chain(project(1, 3, 1), project(0, 0)))
    w_copy[3].wait()
    x_copy[2].start()
    _a_transpose_w(A, wqkv, range(9, 14))
    _interleave(_chain(project(1, 0), project(0, 2)))
    wo_copy.wait()
    for c in tail_copies:
        c.start()
    _interleave(project(1, 2))
    _a_transpose_wo(A, wo)
    qkv_all[AK:AG, :] = jnp.broadcast_to(qkv_all[SLOT + AK:SLOT + AG, :1], (AG - AK, 128))

    def project_out(j0, n, tick=lambda r: None):
        return _chain(*[_a_out(A, o_all.at[j0 + b], ga_all.at[j0 + b], tick) for b in range(n)])

    def attend_trip(t, carry):
        @pl.when(t == 1)
        def _():
            x_copy[2].wait()
            wot_copy.start()

        _interleave(
            _chain(*[_chain(_a_qkv(A, AX + 288 * i, proj(2 * t + 2 + i)),
                            _once(x_stage, jnp.minimum(2 * t + 4 + i, NB - 1), i)) for i in range(2)]),
            _chain(*[_a_attend(j, proj(j), proj(j - 1), o_all.at[j], omg) for j in (2 * t, 2 * t + 1)]),
            span=(-0.04, 0.87))

    x_copy[1].wait()
    for c in main_copies:
        c.start()
    x_stage(2, 0)
    x_stage(3, 1)
    lax.fori_loop(0, NB // 2 - 1, attend_trip, None)

    def last_trip(t, carry):
        def tick(r):
            qkv_all[TICK:TICK + 8, :] = pltpu.bitcast(r[:8], I32)
            tick_raw(r)

        j = NB - 2 + t
        src, dst = raw_from(16 + t, 32), b_ref.at[pl.ds(pl.multiple_of(t * 16, 16), O2), :]
        _interleave(
            project_out(3 * t, 3, tick), _a_attend(j, proj(j), proj(j - 1), o_last.at[t], omg),
            _chain(*[_b_split_heads(src.at[pl.ds(RAW * m, 32 * H)], dst, even, odd) for m, (even, odd) in
                     enumerate(((Q2, Q2 + 32), (K2 + 32, K2), (V2, V2 + 32)))]),
            span=(-0.08, 0.82))

    for c in tail_copies:
        c.wait()
    lax.fori_loop(0, 2, last_trip, None)
    o_all[NB - 2:, :288, :] = o_last[:, :288, :]

    def prepare_trip(t, carry):
        src, dst = raw_from(t, 416), b_ref.at[pl.ds(pl.multiple_of(t * 16, 16), O2), :]
        _interleave(project_out(6 + 2 * t, 2), _chain(*[
            _b_product_tiles(A, src.at[pl.ds(RAW * m, 416 * H)], dst, m * NPR * 64) for m in range(3)]),
            span=(-0.04, 0.93))

    for c in main_copies:
        c.wait()
    lax.fori_loop(0, 4, prepare_trip, None)
    wot_copy.wait()
    _interleave(
        _chain(project_out(NB - 2, 2),
               *[_once(_b_project, B, U - 1, mat, g, 0) for mat in range(3) for g in range(NG)]),
        _b_transpose_wo(B, wot))

    def tail_sum(last, first_steps):
        lane = lax.broadcasted_iota(I32, (64, 128), 1)
        return functools.reduce(jnp.add, [B.ldf(B2 + 64 * last, 64)] + [
            jnp.where(lane < SEG * (u + 1) if first_steps else lane >= SEG * (u + 1), B.ldf(B2 + 64 * u, 64), 0.0)
            for u in range(U - 1)])

    def mix(j, n, bt):
        part = slice(128 * n, 128 * n + bt.shape[0])
        w = jnp.concatenate([omg[j]] * (bt.shape[0] // 8), 0)
        out_buf[j, part, :] = (ga_all[j, part, :] + w * bt).astype(BF16)

    def out_copy(j):
        return pltpu.make_async_copy(
            out_buf.at[j], out_hbm.at[:, pl.ds(pl.multiple_of(j * 128, 128), 128)], sem_out)

    def b_body(g, carry):
        done = jnp.maximum(g - 1, 0)
        B.stf(B2 + 64 * U, tail_sum(U - 1, True))
        weights = _b_norms(raw_from(g, 32), raw.at[pl.ds(pl.multiple_of(offs[23 + g], 16), 2 * D)], norms.at[g])

        def spare(r):
            t = [next(weights) for _ in range(4)][-1]
            tick_raw(functools.reduce(jnp.add, [r] + [t[i:i + 8] for i in range(0, t.shape[0], 8)]))

        for u in range(U):
            def emit(stage):
                if u == 1:
                    for n in range(4):
                        if stage:
                            mix(done, n, B.ldf(PS + 128 * n, 128))
                        else:
                            B.stf(PS + 128 * n, B.ldf(BO + 128 * n, 128).T)
                if u == U - 1 and stage:
                    mix(done, 4, tail_sum(U, False))

            def after_use():
                x_tail(u)
                if u == 0:
                    _b_place_tokens(B, U - 1)
                if u < U - 1:
                    _b_place_tokens(B, u)
                else:
                    x_transpose(jnp.minimum(g + 2, NB - 1))

            _b_step(B, u, emit, after_use, spare)
        assert next(weights, "end") == "end"

        @pl.when(g > 0)
        def _():
            out_copy(done).start()

        return carry

    lax.fori_loop(0, NB, b_body, 0)
    acc = {}
    for g in range(NG):
        for p in TURN[1]:
            _b_out_product(B, 0, p, g, acc, 0)
    _b_out_collect(B, 0)
    B.stf(B2 + 64 * U, tail_sum(U - 1, True))
    for u in range(U - 1):
        _b_out_tail(B, u)
    for n in range(4):
        mix(NB - 1, n, B.ldf(BO + 128 * n, 128).T)
    mix(NB - 1, 4, tail_sum(U, False))
    out_copy(NB - 1).start()
    one_scale = _b_one_scale(norms, mem_ref[...].astype(F32))
    for j in range(NB):
        out_copy(j).wait()

    @pl.when(jnp.logical_not(one_scale))
    def _():
        _b_direct(b_ref, raw, mem_ref[...].astype(F32), x_tile, mix)
        copies = [out_copy(j) for j in range(NB)]
        for c in copies:
            c.start()
        for c in copies:
            c.wait()


@functools.partial(jax.jit, static_argnames=("B_seg_len",))
def pallas_gated_mix__sliding_local_dilated__memory_aug_recurrent_mem_tr__prompt_kernel(
    A_x: jax.Array,
    A_wqkv: jax.Array,
    A_wo: jax.Array,
    B_x: jax.Array,
    B_mem0: jax.Array,
    B_Wq: jax.Array,
    B_Wk: jax.Array,
    B_Wv: jax.Array,
    B_Wo: jax.Array,
    B_seg_len: int,
    gate_w: jax.Array,
):
    del B_x
    assert A_x.shape == (1, S, D) and B_mem0.shape == (1, M, D) and B_Wq.shape == (D, H, DH)
    assert B_seg_len == SEG
    hbm = pl.BlockSpec(memory_space=pl.ANY)
    out_t = pl.pallas_call(
        _kernel,
        out_shape=jax.ShapeDtypeStruct((D, S), BF16),
        in_specs=[hbm] * 9,
        out_specs=hbm,
        scratch_shapes=[
            pltpu.VMEM((D, S), BF16),
            pltpu.VMEM((D, 3 * D), BF16),
            pltpu.VMEM((D, D), BF16),
            pltpu.VMEM((M, D), BF16),
            pltpu.VMEM((D,), BF16),
            pltpu.VMEM((4 * RAW, DH), BF16),
            pltpu.VMEM((A_ROWS, 128), I32),
            pltpu.VMEM((B_ROWS, 128), I32),
            pltpu.VMEM((5 * SLOT, 128), I32),
            pltpu.VMEM((NB, 296, 128), I32),
            pltpu.VMEM((2, 296, 128), I32),
            pltpu.VMEM((NB, D, 128), F32),
            pltpu.VMEM((NB, 8, 128), F32),
            pltpu.VMEM((NB, D, 128), BF16),
            pltpu.VMEM((NB, 176, 128), F32),
            pltpu.SMEM((39,), I32),
            pltpu.SemaphoreType.DMA((10,)),
            pltpu.SemaphoreType.DMA((3,)),
            pltpu.SemaphoreType.DMA,
        ],
        compiler_params=pltpu.CompilerParams(vmem_limit_bytes=110 * 1024 * 1024),
    )(
        A_x.reshape(S, D).T, A_wqkv, A_wo, B_mem0.reshape(M, D), gate_w,
        B_Wq.reshape(D * H, DH), B_Wk.reshape(D * H, DH), B_Wv.reshape(D * H, DH),
        B_Wo.transpose(0, 2, 1).reshape(H * D, DH),
    )
    return out_t.T.reshape(1, S, D)
```

```python
import functools

import jax
import jax.numpy as jnp
import numpy as np
from jax import lax
import jax.experimental.pallas as pl
import jax.experimental.pallas.tpu as pltpu

F32, BF16, I32 = jnp.float32, jnp.bfloat16, jnp.int32

S, D = 2048, 576
NB = S // 128
DA, WIN, DIL = 18, 8, 2
H, DH, M, SEG = 32, 128, 8, 32
L = M + SEG
NP = H // 2
NG = H // 4
U = 128 // SEG
NEG = -1000000000.0

PRODUCTS = tuple(tuple({(int(t[1]), int(t[2])): int(t[0] + "1") for t in form.split()} for form in p) for p in (
    ("+00 -10", "-03 +30 -10 +00 -02", "+00"),
    ("+10", "+03 -30 +00 -01 -20", "+00 +10"),
    ("+03 -13", "-13 -32 +33", "+03"),
    ("+13", "-23 -31 +33", "+03 +13"),
    ("+02 +10", "-02 +20", "+00 -12"),
    ("+02", "-02 -21 +22 -32", "+02 +12"),
    ("+02 -12", "-12 -20 +22 -23", "-12"),
    ("+00 +02", "+02", "+00 +02"),
    ("+10 +12", "+20", "+10 +12"),
    ("+02 +13", "+23 -32", "+03 -12"),
    ("+02 +03", "+32", "+02 +03"),
    ("+12 +13", "+23", "+12 +13"),
    ("+00 +01 -10", "+03 -30 +10 -01", "+00 +10 +11"),
    ("+01", "+03 -01 +11 -12 -31", "+01"),
    ("+11", "+10 -30 -11 +13 +21", "-11"),
    ("+00 +01", "-03 +01", "+00 +01 +10 +11"),
    ("+11 +12", "+21", "+01 +02 +11 +12"),
    ("-02 +11 +12", "+12 -21", "+01 +02 +12"),
    ("+01 +03", "-03 +31", "+01 +03 +11 +13"),
    ("+10 +11 +13", "+30", "+10 +11 +13"),
    ("+01 +03 -13", "-13 +31", "-03 -11 -13"),
    ("+00 +01 +03", "+03", "+00 +01 +03"),
    ("+00 +01 -10 -11", "+10 -30", "-10 -11"),
    ("+01 +02 -11 -12", "+12", "+01 +02"),
    ("+01 +03 -11 -13", "-30 +13", "-11 -13"),
    ("+01 +03 +10", "-03 +30", "+00 -11 -13"),
))
NPR = len(PRODUCTS)
TURN = tuple(tuple(p for p, (a, _, c) in enumerate(PRODUCTS)
                   if any(k[0] == r for k in a) and any(k[0] == r for k in c)) for r in range(2))
ORDER = ((2, 9, 5, 10, 17, 23, 7, 4, 21, 20, 18, 25, 15, 0, 13, 12),
         (17, 16, 14, 4, 1, 22, 12, 8, 19, 25, 24, 20, 11, 3, 9, 6))
LONG = tuple(p for p in range(NPR) if len(PRODUCTS[p][1]) == 5)


def _is_matrix_product():
    t = np.zeros((2, 4, 4, 4, 2, 4), int)
    for a, w, c in PRODUCTS:
        for i in a:
            for j in w:
                for k in c:
                    t[i + j + k] += a[i] * w[j] * c[k]
    return (t == np.einsum("rs,kl,nm->rklnsm", np.eye(2), np.eye(4), np.eye(4))).all()


assert _is_matrix_product() and len(set(TURN[0] + TURN[1])) == NPR
assert all(sorted(ORDER[r]) == list(TURN[r]) for r in range(2))

GSTRIDE = 3 * NPR * 64 + 4
Q2 = NG * GSTRIDE
K2 = Q2 + 64
V2 = K2 + 64
PSTRIDE = 192 + 4
OA = Q2 + NP * PSTRIDE
O2 = OA + NG * NPR * 64
O2T = O2 + NP * 64
LH = O2T + H * 32
GS = LH + U * 18 * L
TK = GS + 64
MQ = TK + 3 * H * 128
VS = MQ + H * M
KS = VS + H * 40
RE = KS + NP * 64
PS = RE + H * L
RS = PS + NP * L
AC = RS + NP * L
XN = AC + NPR * SEG
OM = XN + 320
OF = OM + H * M
BO = OF + (U + 1) * H * SEG
B2 = BO + 512
B_ROWS = B2 + 64 * (U + 1)

RAW = D * H + 16

WT = 0
GW = WT + 5 * 1728
WP = GW + 40
WOT = WP + 27 * 160
AX = WOT + 5 * 288
SUMS = AX + 2 * 288
A_ROWS = SUMS + 4 * len(LONG) + 24
AQ, AK, AV, AG, TICK, SLOT = 0, 576, 864, 1152, 1160, 1168


def _dot(a, b):
    return lax.dot_general(a, b, (((1,), (0,)), ((), ())), preferred_element_type=F32)


def _dot_nt(a, b):
    return lax.dot_general(a, b, (((1,), (1,)), ((), ())), preferred_element_type=F32)


class _Arena:
    def __init__(self, ref):
        self.r = ref

    def ldi(self, o, n):
        return self.r[o:o + n, :]

    def ldf(self, o, n):
        return pltpu.bitcast(self.r[o:o + n, :], F32)

    def ldb(self, o, n):
        return pltpu.bitcast(self.r[o:o + n, :], BF16)

    def stf(self, o, v):
        self.r[o:o + v.shape[0], :] = pltpu.bitcast(v, I32)

    def stb(self, o, v):
        self.r[o:o + v.shape[0] // 2, :] = pltpu.bitcast(v.astype(BF16), I32)


def _signed_sum(terms):
    sign, acc = terms[0]
    for c, t in terms[1:]:
        if c == sign:
            acc = acc + t
        else:
            sign, acc = 1, acc - t if sign > 0 else t - acc
    return acc if sign > 0 else -acc


def _interleave(main, *side, span=(0.0, 0.9)):
    jobs = (main,) + side
    order = [((i + 1) / main[0], 0) for i in range(main[0])]
    order += [(span[0] + (span[1] - span[0]) * i / n, k + 1) for k, (n, _) in enumerate(side) for i in range(n)]
    for _, k in sorted(order):
        next(jobs[k][1])
    for _, gen in jobs:
        assert next(gen, "end") == "end"


def _once(fn, *args):
    def gen():
        fn(*args)
        yield
    return 1, gen()


def _chain(*jobs):
    def gen():
        for _, g in jobs:
            yield from g
    return sum(n for n, _ in jobs), gen()


def _tile_t(w_ref, k, c):
    t = w_ref[128 * k:min(128 * k + 128, w_ref.shape[0]), 128 * c:min(128 * c + 128, w_ref.shape[1])]
    nk, nc = t.shape
    if nc < 128:
        t = jnp.concatenate([t, jnp.zeros((nk, 128 - nc), t.dtype)], 1)
    if nk < 128:
        t = jnp.concatenate([t, jnp.zeros((128 - nk, 128), t.dtype)], 0)
    return t.T[:nc]


def _a_transpose_w(A, w_ref, cblocks):
    for c in cblocks:
        for k in range(5):
            A.stf(WT + 1728 * k + 128 * c, _tile_t(w_ref, k, c).astype(F32))


def _a_transpose_wo(A, w_ref):
    for c in range(5):
        for k in range(5):
            A.stb(WOT + 288 * k + 64 * c, _tile_t(w_ref, k, c))


def _cat576(chunk):
    ch = [chunk(k) for k in range(5)]
    return jnp.concatenate(ch[:4] + [ch[4][:, :64]], 1)


def _a_qkv(A, x_off, dst, parts=(3, 1, 0, 2), first=False):
    def gen():
        for part in parts:
            if part == 3:
                dst.stf(AG, jax.nn.sigmoid(_dot(_cat576(lambda k: A.ldf(GW + 8 * k, 8)), A.ldb(x_off, 288))))
                continue
            for d0 in range(0, DA, 2):
                def weights(k):
                    packed = WP + 160 * (9 * part + d0 // 2) + 32 * k
                    if not first:
                        return A.ldb(packed, 32)
                    w = jnp.concatenate([
                        pltpu.bitcast(A.r[pl.ds(WT + 1728 * k + D * part + 8 * DA * hg + d, 8, stride=DA), :], F32)
                        for hg in range(4) for d in (d0, d0 + 1)], 0)
                    A.stb(packed, w)
                    return w

                r = _dot(_cat576(weights), A.ldb(x_off, 288))
                for i in range(0, 64, 16):
                    if part == 0:
                        dst.stf(AQ + 32 * d0 + i, r[i:i + 16])
                    else:
                        dst.stb((AK if part == 1 else AV) + 16 * d0 + i // 2, r[i:i + 16])
                    yield
    return sum(2 * DA for p in parts if p < 3), gen()


def _a_attend(j, cur, old, o_ref, omg_ref):
    lane = lax.broadcasted_iota(I32, (8, 128), 1)
    wraps = {w: lane >= 128 - DIL * w for w in range(1, WIN)}

    def window(o):
        c, p = cur.ldi(o, 8), old.ldi(o, 8)
        out = []
        for w in range(WIN):
            t = pltpu.roll(lax.select(wraps[w], p, c), DIL * w, 1) if w else c
            out.append(pltpu.bitcast(t, BF16).astype(F32))
        return out

    def gen():
        pos = j * 128 + lane
        for hg in range(4):
            lg = None
            for d in range(0, DA, 2):
                q = cur.ldf(AQ + 32 * d + 16 * hg, 16)
                pr = [q * kw for kw in window(AK + 16 * d + 8 * hg)]
                pr = [t[:8] + t[8:] for t in pr]
                lg = pr if d == 0 else [a + b for a, b in zip(lg, pr)]
                yield
            lg = [jnp.where(pos >= DIL * w, t * DA ** -0.5, NEG) for w, t in enumerate(lg)]
            mx = functools.reduce(jnp.maximum, lg)
            e = [jnp.exp(t - mx) for t in lg]
            g = cur.ldf(AG, 8)
            if hg == 0:
                omg_ref[j] = 1.0 - g
            r = g / functools.reduce(jnp.add, e)
            p = [jnp.concatenate([t * r] * 2, 0) for t in e]
            yield
            for d in range(0, DA, 2):
                o = functools.reduce(jnp.add, [a * b for a, b in zip(p, window(AV + 16 * d + 8 * hg))])
                o = pltpu.bitcast(o.astype(BF16).astype(F32), I32)
                o_ref[pl.ds(4 * DA * hg + d // 2, 8, stride=DA // 2), :] = (
                    lax.shift_right_logical(o[:8], 16) | o[8:])
                yield
    return 4 * DA + 4, gen()


def _a_out(A, o_ref, ga_ref, tick):
    def gen():
        for r0 in range(0, D, 96):
            r = _dot(_cat576(lambda k: A.ldb(WOT + 288 * k + r0 // 2, 48)), pltpu.bitcast(o_ref[:288, :], BF16))
            for i in range(0, 96, 32):
                tick(r[i:i + 32])
                ga_ref[r0 + i:r0 + i + 32, :] = r[i:i + 32]
                yield
    return D // 32, gen()


def _pairs(g):
    return g, g + NG


def _heads(g):
    return [2 * j + i for j in _pairs(g) for i in range(2)]


def _b_split_heads(raw, dst, even, odd, stride=PSTRIDE):
    def gen():
        for r in range(raw.shape[0] // 64):
            e = pltpu.bitcast(raw[64 * r:64 * r + 32, :], I32)
            o = pltpu.bitcast(raw[64 * r + 32:64 * r + 64, :], I32)
            dst[pl.ds(even + r, NP, stride=stride), :] = (e & 0xFFFF) | (o << 16)
            dst[pl.ds(odd + r, NP, stride=stride), :] = lax.shift_right_logical(e, 16) | (o & -65536)
            yield
    return raw.shape[0] // 64, gen()


def _b_sum_matrix():
    g = lax.broadcasted_iota(I32, (8, 128), 0)
    lane = lax.broadcasted_iota(I32, (8, 128), 1)
    return jnp.concatenate([functools.reduce(jnp.add, [
        jnp.where(lane == H * k + _heads(0)[n] + 2 * g, float(c), 0.0) for (k, n), c in PRODUCTS[p][1].items()])
        for p in LONG], 0)


def _b_product_tiles(A, raw, dst, off):
    def gen():
        for r in range(16):
            t = [jnp.concatenate([raw[o:o + H, :] for o in range(64 * r + H * i, 512 * H, 128 * H)], 0)
                 for i in range(2)]
            long = [_dot(A.ldb(SUMS, 4 * len(LONG)), v) for v in t]
            word = [pltpu.bitcast(v, I32) for v in t]

            @functools.cache
            def block(k, n, i):
                v = word[i][16 * k + 8 * (n // 2):16 * k + 8 * (n // 2) + 8]
                return pltpu.bitcast(v & -65536 if n % 2 else v << 16, F32)

            for p, (_, w, _) in enumerate(PRODUCTS):
                e, o = [pltpu.bitcast(
                    long[i][8 * LONG.index(p):8 * LONG.index(p) + 8] if p in LONG else
                    _signed_sum([(c, block(k, n, i)) for (k, n), c in w.items()]), I32) for i in range(2)]
                if len(w) > 1:
                    e, o = e + 0x8000, (o + 0x7FFF) & -65536
                dst[pl.ds(off + p * 64 + r, NG, stride=GSTRIDE), :] = lax.shift_right_logical(e, 16) | o
            yield
    return 16, gen()


def _b_transpose_wo(B, wot):
    def gen():
        for g in range(NG):
            for p, (_, w, _) in enumerate(PRODUCTS):
                t = [(c, wot[pl.ds(D * _heads(g)[k] + 128 * n, 128), :]) for (k, n), c in w.items()]
                if len(t) > 1 or t[0][0] < 0:
                    t = [(1, _signed_sum([(c, v.astype(F32)) for c, v in t]).astype(BF16))]
                B.stb(OA + (g * NPR + p) * 64, t[0][1].T)
                yield
            for j in _pairs(g):
                t = jnp.concatenate([wot[D * h + 512:D * h + D, :] for h in (2 * j, 2 * j + 1)], 0)
                B.stb(O2T + 64 * j, t)
                B.stb(O2 + 64 * j, t.T)
                B.stb(K2 + PSTRIDE * j, B.ldb(K2 + PSTRIDE * j, 64).T)
    return NG * NPR, gen()


def _turn(u):
    return 1 - u % 2


def _halves(p, r):
    return (r,) if p in TURN[1 - r] else (0, 1)


def _lh(u, i):
    return LH + L * (18 * (u % U) + i)


def _b_place_memory(B, u, mem):
    r = _turn(u)
    for i, p in enumerate(TURN[r]):
        B.stf(_lh(u, 2 + i), _signed_sum([(s, mem[k]) for (rr, k), s in PRODUCTS[p][0].items() if rr == r]))
    for i in range(2):
        B.stf(_lh(u, i), mem[4])


def _b_place_tokens(B, u):
    r = _turn(u)
    top = (u + 1 - r) % U

    def x(seg, n, half):
        return B.ldb(XN + 64 * n + 16 * seg + 8 * half, 8).astype(F32)

    for i, p in enumerate(TURN[r]):
        for at, half in enumerate(_halves(p, r)):
            B.stf(_lh(u, 2 + i) + M + 16 * at,
                  _signed_sum([(s, x(top + rr, k, half)) for (rr, k), s in PRODUCTS[p][0].items()]))
    for half in range(2):
        B.stf(_lh(u, 1) + M + 16 * half, x((u + 1) % U, 4, half))


def _b_project(B, u, mat, g, m=M, keep=()):
    r = _turn(u)
    top = (u + 1 - r) % U
    items = [(PRODUCTS[p][2], _halves(p, r),
              _dot(B.ldf(_lh(u, 2 + TURN[r].index(p)) + M - m, m + 16 * len(_halves(p, r))),
                   B.ldb(GSTRIDE * g + (mat * NPR + p) * 64, 64))) for p in ORDER[r]]
    if mat == 0:
        items += [({(r, n): 1}, (0, 1),
                   _dot(B.ldf(_lh(u, 1) + M - m, m + SEG)[:, :64],
                        B.ldb(Q2 + PSTRIDE * (h // 2) + 32 * (h % 2), 32))) for n, h in enumerate(_heads(g))]

    def at(n, seg, half):
        return TK + 128 * (H * mat + _heads(g)[n]) + SEG * seg + 16 * half

    mem, tok, kept = {}, {}, {}
    for c, halves, y in items:
        y_mem, y_tok = y[:m] if m else None, [y[o:o + 16] for o in range(m, y.shape[0], 16)]
        for (rr, n), s in c.items():
            if m and rr == r:
                mem.setdefault(n, []).append((s, y_mem))
            for half, t in zip(halves, y_tok):
                tok.setdefault((rr, n, half), []).append((s, t))
    for (rr, n, half), terms in sorted(tok.items()):
        if r == 1:
            terms.append((1, B.ldf(at(n, top + rr, half), 16)))
        if r == 1 and rr in keep:
            kept[n, top + rr, half] = _signed_sum(terms)
        else:
            B.stf(at(n, top + rr, half), _signed_sum(terms))
    assert len(tok) == 16

    def tokens(n, seg):
        return [kept[n, seg, i] if (n, seg, i) in kept else B.ldf(at(n, seg, i), 16) for i in range(2)]

    return [_signed_sum(mem[n]) for n in sorted(mem)], tokens


def _b_out_product(B, u, p, g, acc, m=M):
    r = _turn(u)
    top = (u - 1 - r) % U
    a = PRODUCTS[p][0].items()
    lhs = [_signed_sum([(s, B.ldf(OM + M * _heads(g)[k], M)) for (rr, k), s in a if rr == r])] if m else []
    both = [k for (rr, k), s in a if rr and PRODUCTS[p][0].get((0, k)) == -s]
    first, rows = 16 * _halves(p, r)[0], 16 * len(_halves(p, r))
    lhs.append(_signed_sum([(s, B.ldf(OF + SEG * (H * (U if k in both else top + rr) + _heads(g)[k]) + first, rows))
                            for (rr, k), s in a if not (rr and k in both)]))
    y = _dot(jnp.concatenate(lhs, 0), B.ldb(OA + (g * NPR + p) * 64, 64))
    acc[p] = acc[p] + y if g else y
    if g == NG - 1:
        B.stf(AC + SEG * p + first, acc[p][m:])
        for (rr, n), s in PRODUCTS[p][2].items():
            if m and rr == r:
                acc.setdefault(("mem", n), []).append((s, acc[p][:m]))


def _b_out_collect(B, u):
    for rr in range(2):
        for n in range(4):
            B.stf(BO + 128 * n + SEG * ((u - 2 + rr) % U), _signed_sum(
                [(c[rr, n], B.ldf(AC + SEG * p, SEG)) for p, (_, _, c) in enumerate(PRODUCTS) if (rr, n) in c]))


def _b_out_tail(B, u):
    B.stf(B2 + 64 * u, functools.reduce(jnp.add, [
        _dot_nt(B.ldb(O2T + 32 * h, 32),
                jnp.concatenate([B.ldf(OF + SEG * (H * i + h), SEG) for i in range(U)], 0).astype(BF16))
        for h in range(8 * u, 8 * u + 8)]))


def _b_step(B, u, emit, after_use, spare):
    row = lax.broadcasted_iota(I32, (L, 128), 0)
    lane = lax.broadcasted_iota(I32, (L, 128), 1)
    lo = lane < 64
    lo64 = lax.broadcasted_iota(I32, (64, 128), 1) < 64
    mask = (row < M) | ((lane & 63) >= SEG) | (row - M >= (lane & 63))
    in_a, in_b = lane < L, (lane >= 64) & (lane < 64 + L)
    z24 = jnp.zeros((24, 128), F32)
    pair = [j for g in range(NG) for j in _pairs(g)]

    def h2():
        return jnp.concatenate([B.ldf(_lh(u, 0) + M, SEG), B.ldf(_lh(u, 0), M)], 0)

    def t_k(g):
        mem, tokens = _b_project(B, u, 1, g, keep=(0,))
        spare(mem[1])
        for i, j in enumerate(_pairs(g)):
            k = jnp.concatenate([t for n in (2 * i, 2 * i + 1) for t in tokens(n, u) + [mem[n], z24]], 0)
            B.stb(KS + 64 * j, k.astype(BF16).T)

    def t_q(g):
        for h, t in zip(_heads(g), _b_project(B, u, 0, g)[0]):
            B.stf(MQ + M * h, t)

    def t_v(g):
        mem, tokens = _b_project(B, u, 2, g, keep=(0, 1))
        for n, h in enumerate(_heads(g)):
            B.stb(VS + 40 * h + 32, jnp.concatenate([mem[n], z24[:8]], 0))
            if _turn(u):
                B.stb(VS + 40 * h, jnp.concatenate(tokens(n, u) + tokens(n, u + 1), 0))

    def t_s(i):
        j = pair[i]
        kt, w2 = B.ldi(KS + 64 * j, 64), B.ldi(K2 + PSTRIDE * j, 64)
        ya, yb = [_dot(jnp.concatenate([B.ldf(MQ + M * h, M), B.ldf(TK + 128 * h + SEG * u, SEG)], 0),
                       pltpu.bitcast(rhs, BF16))
                  for h, rhs in ((2 * j, jnp.where(lo64, kt, w2)), (2 * j + 1, jnp.where(lo64, w2, kt)))]
        B.stf(RE + L * i, jnp.where(lo, ya, yb))
        B.stf(RE + L * (NP + i), jnp.where(lo, yb, ya))

    def t_softmax(n):
        c4 = h2()
        y = _dot_nt(jnp.concatenate([jnp.where(lo, 0.0, c4), jnp.where(lo, c4, 0.0)], 0),
                    B.ldf(RE + L * NP + 128 * n, 128).astype(BF16))
        B.stf(RS + 128 * n, jnp.concatenate([y[:L], z24, y[L:], z24], 0).T)
        for i in range(128 * n // L, 128 * (n + 1) // L):
            s = jnp.where(mask, (B.ldf(RE + L * i, L) + B.ldf(RS + L * i, L)) * DH ** -0.5, NEG)
            ma = jnp.max(jnp.where(in_a, s, -jnp.inf), axis=1, keepdims=True)
            mb = jnp.max(jnp.where(in_b, s, -jnp.inf), axis=1, keepdims=True)
            e = jnp.exp(s - jnp.where(lo, ma, mb))
            B.stf(PS + L * i, jnp.where(in_a | in_b, e, 0.0))

    def t_pv(i):
        p, r = B.ldf(PS + L * i, L), B.ldf(RS + L * i, L)
        for b, lhs in enumerate((jnp.where(lo, p, r), jnp.where(lo, r, p))):
            h = 2 * pair[i] + b
            v = [B.ldi(VS + 40 * h + 16 * (u % 2), 16), B.ldi(VS + 40 * h + 32, 8), jnp.zeros((8, 128), I32)]
            w2 = [B.ldi(V2 + PSTRIDE * pair[i] + 32 * b, 32)]
            o = _dot(lhs, pltpu.bitcast(jnp.concatenate(w2 + v if b else v + w2, 0), BF16))
            l = jnp.broadcast_to(jnp.sum(jnp.where(in_b if b else in_a, p, 0.0), axis=1, keepdims=True), (L, 128))
            rc = pltpu.reciprocal(l, approx=True)
            o = o * (rc * (2.0 - l * rc))
            B.stf(OM + M * h, o[:M])
            B.stf(OF + SEG * (H * u + h), o[M:])
            if u % 2:
                B.stf(OF + SEG * (H * U + h), B.ldf(OF + SEG * (H * (u - 1) + h), SEG) - o[M:])

    acc = {}

    def t_mem_tail(i):
        y = _dot(B.ldf(OM + 2 * M * pair[i], 2 * M), B.ldb(O2 + 64 * pair[i], 64))
        acc["tail"] = acc["tail"] + y if i else y

    for g in range(NG):
        t_k(g)
        if g == 1 and u % 2:
            _b_out_collect(B, u - 1)
    c4 = h2()
    B.stb(GS, jnp.concatenate([jnp.where(lo, 0.0, c4), z24, jnp.where(lo, c4, 0.0), z24], 0))
    lag_s, lag_softmax = 2, 4
    softmax_at = [(128 * n + 127) // L + lag_s + lag_softmax for n in range(5)]
    for i in range(2 * NP - 2):
        if i % 2 == 0:
            t_q(i // 2) if i < NP else t_v((i - NP) // 2)
        if 0 <= i - lag_s < NP:
            t_s(i - lag_s)
        if i in (2, 6):
            emit(i // 4)
        if i in softmax_at:
            t_softmax(softmax_at.index(i))
        for j in range(4 * (i - 2 * NP + 6), 4 * (i - 2 * NP + 7)):
            if j >= 0:
                B.stf(RS + L * j, _dot(B.ldf(PS + L * j, L), B.ldb(GS, 64)))
    prods = TURN[_turn(u)]
    passes = (((14, 5, 0, 12, 10), (1, 3, 4, 15), (8, 9, 6, 11), (13, 7, 2)),
              ((7, 5, 0, 12, 10), (8, 3, 4, 6, 13), (1, 15, 11), (9, 2, 14)))[_turn(u)]

    def t_out(k, g):
        for i in passes[k]:
            _b_out_product(B, u, prods[i], g, acc)
        if k < 2:
            t_mem_tail(NG * k + g)

    for g in range(NG + 2):
        if g < NG:
            t_pv(2 * g)
            t_pv(2 * g + 1)
        elif g == NG:
            t_out(1, 0)
        if g == 2:
            t_v(NG - 1)
        if g >= 2:
            t_out(0, g - 2)
    after_use()
    for k in range(1, len(passes)):
        for g in range(1 if k == 1 else 0, NG):
            t_out(k, g)
    tail = jnp.where(lo[:M], acc["tail"][:M], acc["tail"][M:])
    _b_place_memory(B, u + 1, [_signed_sum(acc["mem", n]) for n in range(4)] + [tail + pltpu.roll(tail, 64, 1)])
    _b_out_tail(B, u)


def _squares(t):
    t = pltpu.bitcast(t, I32)
    even, odd = pltpu.bitcast(t << 16, F32), pltpu.bitcast(t, F32)
    return even * even, odd * odd


def _b_norms(qkv, wot, out):
    for m in range(3):
        acc = None
        for d in range(32):
            sq = jnp.concatenate(_squares(qkv[RAW * m + H * d:RAW * m + H * d + H, :]), 0)
            acc = acc + sq if d else sq
            if d == 31:
                out[32 * m:32 * m + 32, :] = acc
            yield acc
    for i in range(8):
        for d in range(4):
            o = D * (i // 4) + 128 * (i % 4) + 32 * d
            sq = jnp.add(*_squares(wot[o:o + 32, :]))
            acc = acc + sq if d else sq
            if d == 3:
                out[96 + 8 * i:104 + 8 * i, :] = acc[:8] + acc[8:]
            yield acc


def _b_one_scale(norms, mem0):
    def close(ts):
        lo, hi = jnp.min(functools.reduce(jnp.minimum, ts)), jnp.max(functools.reduce(jnp.maximum, ts))
        return (hi <= 4.0 * lo) & (lo > 0.0) & (hi < jnp.inf), lo

    ok = [close([functools.reduce(jnp.add, [norms[4 * k + i, 32 * m:32 * m + 32, :] for i in range(4)])
                 for k in range(4)])[0] for m in range(3)]
    ok.append(close([jnp.sum(norms[g, o:o + 8, :], axis=0, keepdims=True)
                     for g in range(NB) for o in range(96, 160, 8)])[0])
    tokens, lo = close([jnp.sum(norms[g, 160:168, :], axis=0, keepdims=True) for g in range(NB)])
    top = jnp.max(functools.reduce(jnp.maximum, [norms[g, 168:176, :] for g in range(NB)]))
    sq = mem0[:, :512] * mem0[:, :512]
    over = jnp.max(jnp.max(sq, axis=1, keepdims=True) - jnp.sum(sq, axis=1, keepdims=True) / 8.0)
    return functools.reduce(jnp.logical_and, ok + [tokens, top <= lo / 8.0, over <= 0.0])


def _b_direct(b_ref, raw, mem0, x_tile, emit):
    def split(i, carry):
        for m in range(3):
            _interleave(_b_split_heads(raw.at[pl.ds(pl.multiple_of(RAW * m + i * 16 * H, 16), 16 * H)],
                                       b_ref.at[pl.ds(pl.multiple_of(i * 8, 8), O2), :],
                                       288 * m, 288 * (3 + m), 6 * 288))

    lax.fori_loop(0, D // 16, split, None)
    row = lax.broadcasted_iota(I32, (L, L + 8), 0)
    col = lax.broadcasted_iota(I32, (L, L + 8), 1)

    def segment(u, mem):
        x = pltpu.bitcast(_cat576(lambda n: b_ref[pl.ds(pl.multiple_of(TK + 128 * n + SEG * u, SEG), SEG), :]), F32)
        h = jnp.concatenate([mem, x, jnp.zeros((8, D), F32)], 0).astype(BF16)

        def head(i, acc):
            q, k, v = [_dot(h, pltpu.bitcast(b_ref[pl.ds(pl.multiple_of(288 * (3 * i + m), 8), 288), :], BF16))
                       for m in range(3)]
            s = jnp.where((row < M) | (row >= col), _dot_nt(q[:L], k.astype(BF16)) * DH ** -0.5, NEG)
            s = jnp.where(col < L, s, -jnp.inf)
            e = jnp.exp(s - jnp.max(s, axis=1, keepdims=True))
            o = _dot(e / jnp.sum(e, axis=1, keepdims=True), v.astype(BF16))
            return acc + _dot_nt(o, raw[pl.ds(pl.multiple_of(3 * RAW + D * i, 16), D), :])

        out = lax.fori_loop(0, H, head, jnp.zeros((L, D), F32))
        for n in range(5):
            c = min(128 * n, D - 128)
            b_ref[pl.ds(pl.multiple_of(RE + 128 * n + SEG * u, 8), SEG), :] = pltpu.bitcast(out[M:, c:c + 128], I32)
        return out[:M]

    def block(j, mem):
        for n in range(5):
            _Arena(b_ref).stf(TK + 128 * n, x_tile(j, n).T.astype(F32))
        mem = lax.fori_loop(0, U, segment, mem)
        for n in range(5):
            emit(j, n, _Arena(b_ref).ldf(RE + 128 * n, 128).T[64 * (n // 4):])
        return mem

    lax.fori_loop(0, NB, block, mem0)


def _kernel(xt_hbm, wqkv_hbm, wo_hbm, mem_hbm, gate_hbm, wq_hbm, wk_hbm, wv_hbm, wot_hbm,
            out_hbm,
            xt, wqkv, wo, mem_ref, gate_ref, raw, a_ref, b_ref, qkv_all, o_all, o_last, ga_all, omg, out_buf,
            norms, offs, sem_in, sem_w, sem_out):
    A, B = _Arena(a_ref), _Arena(b_ref)
    wot = raw.at[pl.ds(3 * RAW, H * D)]

    def cols(src, dst, c0, c1, sem):
        return pltpu.make_async_copy(src.at[:, pl.ds(c0, c1 - c0)], dst.at[:, pl.ds(c0, c1 - c0)], sem_in.at[sem])

    def rows(r0, r1, sem):
        return [pltpu.make_async_copy(w.at[pl.ds(r0 * H, (r1 - r0) * H)],
                                      raw.at[pl.ds(RAW * m + r0 * H, (r1 - r0) * H)], sem_w.at[sem])
                for m, w in enumerate((wq_hbm, wk_hbm, wv_hbm))]

    def x_stage(j, slot):
        A.stb(AX + 288 * slot, xt[:, pl.ds(pl.multiple_of(j * 128, 128), 128)])

    def x_tile(j, n):
        block = pl.ds(pl.multiple_of(j * 128, 128), 128)
        return xt[128 * n:128 * n + 128, block] if n < 4 else jnp.concatenate([xt[512:D, block]] * 2, 0)

    def x_transpose(j):
        sq = []
        for n in range(5):
            t = x_tile(j, n)
            B.stb(XN + 64 * n, t.T)
            if n < 4:
                parts = _squares(t)
                sq += [part[i:i + 8] for i in range(0, 64, 8) for part in parts]
        norms[j, 160:168, :] = functools.reduce(jnp.add, sq)
        norms[j, 168:176, :] = functools.reduce(jnp.maximum, sq)

    def x_tail(u):
        B.stf(_lh(u, 0) + M, B.ldb(XN + 256 + 16 * u, 16).astype(F32))

    def tick_raw(r):
        raw[D * H:D * H + 8, :] = r[:8].astype(BF16)

    def proj(j):
        if isinstance(j, int):
            return _Arena(qkv_all.at[pl.ds((j + 1) % 5 * SLOT, SLOT)])
        return _Arena(qkv_all.at[pl.ds(pl.multiple_of(offs[lax.rem(j + 1, 5)], 8), SLOT)])

    def raw_from(i, n):
        return raw.at[pl.ds(pl.multiple_of(offs[5 + i], 16), 2 * RAW + n * H)]

    x_copy = [cols(xt_hbm, xt, c0, c1, i) for i, (c0, c1) in enumerate(((0, 256), (256, 768), (768, S)))]
    w_copy = [cols(wqkv_hbm, wqkv, c0, c1, 3 + i) for i, (c0, c1) in
              enumerate(((512, 896), (896, 1152), (0, 512), (1152, 3 * D)))]
    wo_copy = pltpu.make_async_copy(wo_hbm, wo, sem_in.at[7])
    mem_copy = pltpu.make_async_copy(mem_hbm, mem_ref, sem_in.at[8])
    gate_copy = pltpu.make_async_copy(gate_hbm, gate_ref, sem_in.at[9])
    tail_copies, main_copies = rows(512, D, 0), rows(0, 512, 1)
    wot_copy = pltpu.make_async_copy(wot_hbm, wot, sem_w.at[2])
    for c in (w_copy[0], gate_copy, mem_copy, w_copy[1], x_copy[0], w_copy[2], w_copy[3], wo_copy):
        c.start()

    for i in range(5):
        offs[i] = i * SLOT
    for i in range(18):
        offs[5 + i] = 32 * H * i
    for i in range(NB):
        offs[23 + i] = 3 * RAW + 2 * D * i
    A.stb(SUMS, _b_sum_matrix())
    B.stf(OF + H * SEG, jnp.zeros((B_ROWS - OF - H * SEG, 128), F32))
    B.stf(AC, jnp.zeros((NPR * SEG, 128), F32))
    w_copy[0].wait()
    gate_copy.wait()
    mem_copy.wait()
    gate = jnp.broadcast_to(gate_ref[...].astype(F32)[None, :], (8, D))
    mem0 = mem_ref[...].astype(F32)
    for k in range(4):
        A.stf(GW + 8 * k, gate[:, 128 * k:128 * k + 128])
    A.stf(GW + 32, jnp.concatenate([gate[:, 512:]] * 2, 1))
    _b_place_memory(B, 0, [mem0[:, 128 * k:128 * k + 128] for k in range(4)]
                    + [jnp.concatenate([mem0[:, 512:]] * 2, 1)])

    def project(j, *parts):
        return _a_qkv(A, AX + 288 * j, proj(j), parts, first=j == 0)

    _a_transpose_w(A, wqkv, range(4, 7))
    w_copy[1].wait()
    _a_transpose_w(A, wqkv, range(7, 9))
    x_copy[0].wait()
    x_stage(0, 0)
    x_stage(1, 1)
    _interleave(project(0, 3, 1))
    x_transpose(0)
    for u in range(U):
        x_tail(u)
        _b_place_tokens(B, u)
    x_transpose(1)
    w_copy[2].wait()
    x_copy[1].start()
    _a_transpose_w(A, wqkv, range(0, 4))
    _interleave(_chain(project(1, 3, 1), project(0, 0)))
    w_copy[3].wait()
    x_copy[2].start()
    _a_transpose_w(A, wqkv, range(9, 14))
    _interleave(_chain(project(1, 0), project(0, 2)))
    wo_copy.wait()
    for c in tail_copies:
        c.start()
    _interleave(project(1, 2))
    _a_transpose_wo(A, wo)
    qkv_all[AK:AG, :] = jnp.broadcast_to(qkv_all[SLOT + AK:SLOT + AG, :1], (AG - AK, 128))

    def project_out(j0, n, tick=lambda r: None):
        return _chain(*[_a_out(A, o_all.at[j0 + b], ga_all.at[j0 + b], tick) for b in range(n)])

    def attend_trip(t, carry):
        @pl.when(t == 1)
        def _():
            x_copy[2].wait()
            wot_copy.start()

        _interleave(
            _chain(*[_chain(_a_qkv(A, AX + 288 * i, proj(2 * t + 2 + i)),
                            _once(x_stage, jnp.minimum(2 * t + 4 + i, NB - 1), i)) for i in range(2)]),
            _chain(*[_a_attend(j, proj(j), proj(j - 1), o_all.at[j], omg) for j in (2 * t, 2 * t + 1)]),
            span=(-0.04, 0.87))

    x_copy[1].wait()
    for c in main_copies:
        c.start()
    x_stage(2, 0)
    x_stage(3, 1)
    lax.fori_loop(0, NB // 2 - 1, attend_trip, None)

    def last_trip(t, carry):
        def tick(r):
            qkv_all[TICK:TICK + 8, :] = pltpu.bitcast(r[:8], I32)
            tick_raw(r)

        j = NB - 2 + t
        src, dst = raw_from(16 + t, 32), b_ref.at[pl.ds(pl.multiple_of(t * 16, 16), O2), :]
        _interleave(
            project_out(3 * t, 3, tick), _a_attend(j, proj(j), proj(j - 1), o_last.at[t], omg),
            _chain(*[_b_split_heads(src.at[pl.ds(RAW * m, 32 * H)], dst, even, odd) for m, (even, odd) in
                     enumerate(((Q2, Q2 + 32), (K2 + 32, K2), (V2, V2 + 32)))]),
            span=(-0.08, 0.82))

    for c in tail_copies:
        c.wait()
    lax.fori_loop(0, 2, last_trip, None)
    o_all[NB - 2:, :288, :] = o_last[:, :288, :]

    def prepare_trip(t, carry):
        src, dst = raw_from(t, 416), b_ref.at[pl.ds(pl.multiple_of(t * 16, 16), O2), :]
        _interleave(project_out(6 + 2 * t, 2), _chain(*[
            _b_product_tiles(A, src.at[pl.ds(RAW * m, 416 * H)], dst, m * NPR * 64) for m in range(3)]),
            span=(-0.04, 0.93))

    for c in main_copies:
        c.wait()
    lax.fori_loop(0, 4, prepare_trip, None)
    wot_copy.wait()
    _interleave(
        _chain(project_out(NB - 2, 2),
               *[_once(_b_project, B, U - 1, mat, g, 0) for mat in range(3) for g in range(NG)]),
        _b_transpose_wo(B, wot))

    def tail_sum(last, first_steps):
        lane = lax.broadcasted_iota(I32, (64, 128), 1)
        return functools.reduce(jnp.add, [B.ldf(B2 + 64 * last, 64)] + [
            jnp.where(lane < SEG * (u + 1) if first_steps else lane >= SEG * (u + 1), B.ldf(B2 + 64 * u, 64), 0.0)
            for u in range(U - 1)])

    def mix(j, n, bt):
        part = slice(128 * n, 128 * n + bt.shape[0])
        w = jnp.concatenate([omg[j]] * (bt.shape[0] // 8), 0)
        out_buf[j, part, :] = (ga_all[j, part, :] + w * bt).astype(BF16)

    def out_copy(j):
        return pltpu.make_async_copy(
            out_buf.at[j], out_hbm.at[:, pl.ds(pl.multiple_of(j * 128, 128), 128)], sem_out)

    def b_body(g, carry):
        done = jnp.maximum(g - 1, 0)
        B.stf(B2 + 64 * U, tail_sum(U - 1, True))
        weights = _b_norms(raw_from(g, 32), raw.at[pl.ds(pl.multiple_of(offs[23 + g], 16), 2 * D)], norms.at[g])

        def spare(r):
            t = [next(weights) for _ in range(4)][-1]
            tick_raw(functools.reduce(jnp.add, [r] + [t[i:i + 8] for i in range(0, t.shape[0], 8)]))

        for u in range(U):
            def emit(stage):
                if u == 1:
                    for n in range(4):
                        if stage:
                            mix(done, n, B.ldf(PS + 128 * n, 128))
                        else:
                            B.stf(PS + 128 * n, B.ldf(BO + 128 * n, 128).T)
                if u == U - 1 and stage:
                    mix(done, 4, tail_sum(U, False))

            def after_use():
                x_tail(u)
                if u == 0:
                    _b_place_tokens(B, U - 1)
                if u < U - 1:
                    _b_place_tokens(B, u)
                else:
                    x_transpose(jnp.minimum(g + 2, NB - 1))

            _b_step(B, u, emit, after_use, spare)
        assert next(weights, "end") == "end"

        @pl.when(g > 0)
        def _():
            out_copy(done).start()

        return carry

    lax.fori_loop(0, NB, b_body, 0)
    acc = {}
    for g in range(NG):
        for p in TURN[1]:
            _b_out_product(B, 0, p, g, acc, 0)
    _b_out_collect(B, 0)
    B.stf(B2 + 64 * U, tail_sum(U - 1, True))
    for u in range(U - 1):
        _b_out_tail(B, u)
    for n in range(4):
        mix(NB - 1, n, B.ldf(BO + 128 * n, 128).T)
    mix(NB - 1, 4, tail_sum(U, False))
    out_copy(NB - 1).start()
    one_scale = _b_one_scale(norms, mem_ref[...].astype(F32))
    for j in range(NB):
        out_copy(j).wait()

    @pl.when(jnp.logical_not(one_scale))
    def _():
        _b_direct(b_ref, raw, mem_ref[...].astype(F32), x_tile, mix)
        copies = [out_copy(j) for j in range(NB)]
        for c in copies:
            c.start()
        for c in copies:
            c.wait()


@functools.partial(jax.jit, static_argnames=("B_seg_len",))
def pallas_gated_mix__sliding_local_dilated__memory_aug_recurrent_mem_tr__prompt_kernel(
    A_x: jax.Array,
    A_wqkv: jax.Array,
    A_wo: jax.Array,
    B_x: jax.Array,
    B_mem0: jax.Array,
    B_Wq: jax.Array,
    B_Wk: jax.Array,
    B_Wv: jax.Array,
    B_Wo: jax.Array,
    B_seg_len: int,
    gate_w: jax.Array,
):
    del B_x
    assert A_x.shape == (1, S, D) and B_mem0.shape == (1, M, D) and B_Wq.shape == (D, H, DH)
    assert B_seg_len == SEG
    hbm = pl.BlockSpec(memory_space=pl.ANY)
    out_t = pl.pallas_call(
        _kernel,
        out_shape=jax.ShapeDtypeStruct((D, S), BF16),
        in_specs=[hbm] * 9,
        out_specs=hbm,
        scratch_shapes=[
            pltpu.VMEM((D, S), BF16),
            pltpu.VMEM((D, 3 * D), BF16),
            pltpu.VMEM((D, D), BF16),
            pltpu.VMEM((M, D), BF16),
            pltpu.VMEM((D,), BF16),
            pltpu.VMEM((4 * RAW, DH), BF16),
            pltpu.VMEM((A_ROWS, 128), I32),
            pltpu.VMEM((B_ROWS, 128), I32),
            pltpu.VMEM((5 * SLOT, 128), I32),
            pltpu.VMEM((NB, 296, 128), I32),
            pltpu.VMEM((2, 296, 128), I32),
            pltpu.VMEM((NB, D, 128), F32),
            pltpu.VMEM((NB, 8, 128), F32),
            pltpu.VMEM((NB, D, 128), BF16),
            pltpu.VMEM((NB, 176, 128), F32),
            pltpu.SMEM((39,), I32),
            pltpu.SemaphoreType.DMA((10,)),
            pltpu.SemaphoreType.DMA((3,)),
            pltpu.SemaphoreType.DMA,
        ],
        compiler_params=pltpu.CompilerParams(vmem_limit_bytes=110 * 1024 * 1024),
    )(
        A_x.reshape(S, D).T, A_wqkv, A_wo, B_mem0.reshape(M, D), gate_w,
        B_Wq.reshape(D * H, DH), B_Wk.reshape(D * H, DH), B_Wv.reshape(D * H, DH),
        B_Wo.transpose(0, 2, 1).reshape(H * D, DH),
    )
    return out_t.T.reshape(1, S, D)
```

```python
import functools

import jax
import jax.numpy as jnp
import numpy as np
from jax import lax
import jax.experimental.pallas as pl
import jax.experimental.pallas.tpu as pltpu

F32, BF16, I32 = jnp.float32, jnp.bfloat16, jnp.int32

S, D = 2048, 576
NB = S // 128
DA, WIN, DIL = 18, 8, 2
H, DH, M, SEG = 32, 128, 8, 32
L = M + SEG
NP = H // 2
NG = H // 4
U = 128 // SEG
NEG = -1000000000.0

PRODUCTS = tuple(tuple({(int(t[1]), int(t[2])): int(t[0] + "1") for t in form.split()} for form in p) for p in (
    ("+00 -10", "-03 +30 -10 +00 -02", "+00"),
    ("+10", "+03 -30 +00 -01 -20", "+00 +10"),
    ("+03 -13", "-13 -32 +33", "+03"),
    ("+13", "-23 -31 +33", "+03 +13"),
    ("+02 +10", "-02 +20", "+00 -12"),
    ("+02", "-02 -21 +22 -32", "+02 +12"),
    ("+02 -12", "-12 -20 +22 -23", "-12"),
    ("+00 +02", "+02", "+00 +02"),
    ("+10 +12", "+20", "+10 +12"),
    ("+02 +13", "+23 -32", "+03 -12"),
    ("+02 +03", "+32", "+02 +03"),
    ("+12 +13", "+23", "+12 +13"),
    ("+00 +01 -10", "+03 -30 +10 -01", "+00 +10 +11"),
    ("+01", "+03 -01 +11 -12 -31", "+01"),
    ("+11", "+10 -30 -11 +13 +21", "-11"),
    ("+00 +01", "-03 +01", "+00 +01 +10 +11"),
    ("+11 +12", "+21", "+01 +02 +11 +12"),
    ("-02 +11 +12", "+12 -21", "+01 +02 +12"),
    ("+01 +03", "-03 +31", "+01 +03 +11 +13"),
    ("+10 +11 +13", "+30", "+10 +11 +13"),
    ("+01 +03 -13", "-13 +31", "-03 -11 -13"),
    ("+00 +01 +03", "+03", "+00 +01 +03"),
    ("+00 +01 -10 -11", "+10 -30", "-10 -11"),
    ("+01 +02 -11 -12", "+12", "+01 +02"),
    ("+01 +03 -11 -13", "-30 +13", "-11 -13"),
    ("+01 +03 +10", "-03 +30", "+00 -11 -13"),
))
NPR = len(PRODUCTS)
TURN = tuple(tuple(p for p, (a, _, c) in enumerate(PRODUCTS)
                   if any(k[0] == r for k in a) and any(k[0] == r for k in c)) for r in range(2))
ORDER = ((2, 9, 5, 10, 17, 23, 7, 4, 21, 20, 18, 25, 15, 0, 13, 12),
         (17, 16, 14, 4, 1, 22, 12, 8, 19, 25, 24, 20, 11, 3, 9, 6))
LONG = tuple(p for p in range(NPR) if len(PRODUCTS[p][1]) == 5)


def _is_matrix_product():
    t = np.zeros((2, 4, 4, 4, 2, 4), int)
    for a, w, c in PRODUCTS:
        for i in a:
            for j in w:
                for k in c:
                    t[i + j + k] += a[i] * w[j] * c[k]
    return (t == np.einsum("rs,kl,nm->rklnsm", np.eye(2), np.eye(4), np.eye(4))).all()


assert _is_matrix_product() and len(set(TURN[0] + TURN[1])) == NPR
assert all(sorted(ORDER[r]) == list(TURN[r]) for r in range(2))

GSTRIDE = 3 * NPR * 64 + 4
Q2 = NG * GSTRIDE
K2 = Q2 + 64
V2 = K2 + 64
PSTRIDE = 192 + 4
OA = Q2 + NP * PSTRIDE
O2 = OA + NG * NPR * 64
O2T = O2 + NP * 64
LH = O2T + H * 32
GS = LH + U * 18 * L
TK = GS + 64
MQ = TK + 3 * H * 128
VS = MQ + H * M
KS = VS + H * 40
RE = KS + NP * 64
PS = RE + H * L
RS = PS + NP * L
AC = RS + NP * L
XN = AC + NPR * SEG
OM = XN + 320
OF = OM + H * M
BO = OF + (U + 1) * H * SEG
B2 = BO + 512
B_ROWS = B2 + 64 * (U + 1)

RAW = D * H + 16

WT = 0
GW = WT + 5 * 1728
WP = GW + 40
WOT = WP + 27 * 160
AX = WOT + 5 * 288
SUMS = AX + 2 * 288
A_ROWS = SUMS + 4 * len(LONG) + 24
AQ, AK, AV, AG, TICK, SLOT = 0, 576, 864, 1152, 1160, 1168


def _dot(a, b):
    return lax.dot_general(a, b, (((1,), (0,)), ((), ())), preferred_element_type=F32)


def _dot_nt(a, b):
    return lax.dot_general(a, b, (((1,), (1,)), ((), ())), preferred_element_type=F32)


class _Arena:
    def __init__(self, ref):
        self.r = ref

    def ldi(self, o, n):
        return self.r[o:o + n, :]

    def ldf(self, o, n):
        return pltpu.bitcast(self.r[o:o + n, :], F32)

    def ldb(self, o, n):
        return pltpu.bitcast(self.r[o:o + n, :], BF16)

    def stf(self, o, v):
        self.r[o:o + v.shape[0], :] = pltpu.bitcast(v, I32)

    def stb(self, o, v):
        self.r[o:o + v.shape[0] // 2, :] = pltpu.bitcast(v.astype(BF16), I32)


def _signed_sum(terms):
    sign, acc = terms[0]
    for c, t in terms[1:]:
        if c == sign:
            acc = acc + t
        else:
            sign, acc = 1, acc - t if sign > 0 else t - acc
    return acc if sign > 0 else -acc


def _interleave(main, *side, span=(0.0, 0.9)):
    jobs = (main,) + side
    order = [((i + 1) / main[0], 0) for i in range(main[0])]
    order += [(span[0] + (span[1] - span[0]) * i / n, k + 1) for k, (n, _) in enumerate(side) for i in range(n)]
    for _, k in sorted(order):
        next(jobs[k][1])
    for _, gen in jobs:
        assert next(gen, "end") == "end"


def _once(fn, *args):
    def gen():
        fn(*args)
        yield
    return 1, gen()


def _chain(*jobs):
    def gen():
        for _, g in jobs:
            yield from g
    return sum(n for n, _ in jobs), gen()


def _tile_t(w_ref, k, c):
    t = w_ref[128 * k:min(128 * k + 128, w_ref.shape[0]), 128 * c:min(128 * c + 128, w_ref.shape[1])]
    nk, nc = t.shape
    if nc < 128:
        t = jnp.concatenate([t, jnp.zeros((nk, 128 - nc), t.dtype)], 1)
    if nk < 128:
        t = jnp.concatenate([t, jnp.zeros((128 - nk, 128), t.dtype)], 0)
    return t.T[:nc]


def _a_transpose_w(A, w_ref, cblocks):
    for c in cblocks:
        for k in range(5):
            A.stf(WT + 1728 * k + 128 * c, _tile_t(w_ref, k, c).astype(F32))


def _a_transpose_wo(A, w_ref):
    for c in range(5):
        for k in range(5):
            A.stb(WOT + 288 * k + 64 * c, _tile_t(w_ref, k, c))


def _cat576(chunk):
    ch = [chunk(k) for k in range(5)]
    return jnp.concatenate(ch[:4] + [ch[4][:, :64]], 1)


def _a_qkv(A, x_off, dst, parts=(3, 1, 0, 2), first=False):
    def gen():
        for part in parts:
            if part == 3:
                dst.stf(AG, jax.nn.sigmoid(_dot(_cat576(lambda k: A.ldf(GW + 8 * k, 8)), A.ldb(x_off, 288))))
                continue
            for d0 in range(0, DA, 2):
                def weights(k):
                    packed = WP + 160 * (9 * part + d0 // 2) + 32 * k
                    if not first:
                        return A.ldb(packed, 32)
                    w = jnp.concatenate([
                        pltpu.bitcast(A.r[pl.ds(WT + 1728 * k + D * part + 8 * DA * hg + d, 8, stride=DA), :], F32)
                        for hg in range(4) for d in (d0, d0 + 1)], 0)
                    A.stb(packed, w)
                    return w

                r = _dot(_cat576(weights), A.ldb(x_off, 288))
                for i in range(0, 64, 16):
                    if part == 0:
                        dst.stf(AQ + 32 * d0 + i, r[i:i + 16])
                    else:
                        dst.stb((AK if part == 1 else AV) + 16 * d0 + i // 2, r[i:i + 16])
                    yield
    return sum(2 * DA for p in parts if p < 3), gen()


def _a_attend(j, cur, old, o_ref, omg_ref):
    lane = lax.broadcasted_iota(I32, (8, 128), 1)
    wraps = {w: lane >= 128 - DIL * w for w in range(1, WIN)}

    def window(o):
        c, p = cur.ldi(o, 8), old.ldi(o, 8)
        out = []
        for w in range(WIN):
            t = pltpu.roll(lax.select(wraps[w], p, c), DIL * w, 1) if w else c
            out.append(pltpu.bitcast(t, BF16).astype(F32))
        return out

    def gen():
        pos = j * 128 + lane
        for hg in range(4):
            lg = None
            for d in range(0, DA, 2):
                q = cur.ldf(AQ + 32 * d + 16 * hg, 16)
                pr = [q * kw for kw in window(AK + 16 * d + 8 * hg)]
                pr = [t[:8] + t[8:] for t in pr]
                lg = pr if d == 0 else [a + b for a, b in zip(lg, pr)]
                yield
            lg = [jnp.where(pos >= DIL * w, t * DA ** -0.5, NEG) for w, t in enumerate(lg)]
            mx = functools.reduce(jnp.maximum, lg)
            e = [jnp.exp(t - mx) for t in lg]
            g = cur.ldf(AG, 8)
            if hg == 0:
                omg_ref[j] = 1.0 - g
            r = g / functools.reduce(jnp.add, e)
            p = [jnp.concatenate([t * r] * 2, 0) for t in e]
            yield
            for d in range(0, DA, 2):
                o = functools.reduce(jnp.add, [a * b for a, b in zip(p, window(AV + 16 * d + 8 * hg))])
                o = pltpu.bitcast(o.astype(BF16).astype(F32), I32)
                o_ref[pl.ds(4 * DA * hg + d // 2, 8, stride=DA // 2), :] = (
                    lax.shift_right_logical(o[:8], 16) | o[8:])
                yield
    return 4 * DA + 4, gen()


def _a_out(A, o_ref, ga_ref, tick):
    def gen():
        for r0 in range(0, D, 96):
            r = _dot(_cat576(lambda k: A.ldb(WOT + 288 * k + r0 // 2, 48)), pltpu.bitcast(o_ref[:288, :], BF16))
            for i in range(0, 96, 32):
                tick(r[i:i + 32])
                ga_ref[r0 + i:r0 + i + 32, :] = r[i:i + 32]
                yield
    return D // 32, gen()


def _pairs(g):
    return g, g + NG


def _heads(g):
    return [2 * j + i for j in _pairs(g) for i in range(2)]


def _b_split_heads(raw, dst, even, odd, stride=PSTRIDE):
    def gen():
        for r in range(raw.shape[0] // 64):
            e = pltpu.bitcast(raw[64 * r:64 * r + 32, :], I32)
            o = pltpu.bitcast(raw[64 * r + 32:64 * r + 64, :], I32)
            dst[pl.ds(even + r, NP, stride=stride), :] = (e & 0xFFFF) | (o << 16)
            dst[pl.ds(odd + r, NP, stride=stride), :] = lax.shift_right_logical(e, 16) | (o & -65536)
            yield
    return raw.shape[0] // 64, gen()


def _b_sum_matrix():
    g = lax.broadcasted_iota(I32, (8, 128), 0)
    lane = lax.broadcasted_iota(I32, (8, 128), 1)
    return jnp.concatenate([functools.reduce(jnp.add, [
        jnp.where(lane == H * k + _heads(0)[n] + 2 * g, float(c), 0.0) for (k, n), c in PRODUCTS[p][1].items()])
        for p in LONG], 0)


def _b_product_tiles(A, raw, dst, off):
    def gen():
        for r in range(16):
            t = [jnp.concatenate([raw[o:o + H, :] for o in range(64 * r + H * i, 512 * H, 128 * H)], 0)
                 for i in range(2)]
            long = [_dot(A.ldb(SUMS, 4 * len(LONG)), v) for v in t]
            word = [pltpu.bitcast(v, I32) for v in t]

            @functools.cache
            def block(k, n, i):
                v = word[i][16 * k + 8 * (n // 2):16 * k + 8 * (n // 2) + 8]
                return pltpu.bitcast(v & -65536 if n % 2 else v << 16, F32)

            for p, (_, w, _) in enumerate(PRODUCTS):
                e, o = [pltpu.bitcast(
                    long[i][8 * LONG.index(p):8 * LONG.index(p) + 8] if p in LONG else
                    _signed_sum([(c, block(k, n, i)) for (k, n), c in w.items()]), I32) for i in range(2)]
                if len(w) > 1:
                    e, o = e + 0x8000, (o + 0x7FFF) & -65536
                dst[pl.ds(off + p * 64 + r, NG, stride=GSTRIDE), :] = lax.shift_right_logical(e, 16) | o
            yield
    return 16, gen()


def _b_transpose_wo(B, wot):
    def gen():
        for g in range(NG):
            for p, (_, w, _) in enumerate(PRODUCTS):
                t = [(c, wot[pl.ds(D * _heads(g)[k] + 128 * n, 128), :]) for (k, n), c in w.items()]
                if len(t) > 1 or t[0][0] < 0:
                    t = [(1, _signed_sum([(c, v.astype(F32)) for c, v in t]).astype(BF16))]
                B.stb(OA + (g * NPR + p) * 64, t[0][1].T)
                yield
            for j in _pairs(g):
                t = jnp.concatenate([wot[D * h + 512:D * h + D, :] for h in (2 * j, 2 * j + 1)], 0)
                B.stb(O2T + 64 * j, t)
                B.stb(O2 + 64 * j, t.T)
                B.stb(K2 + PSTRIDE * j, B.ldb(K2 + PSTRIDE * j, 64).T)
    return NG * NPR, gen()


def _turn(u):
    return 1 - u % 2


def _halves(p, r):
    return (r,) if p in TURN[1 - r] else (0, 1)


def _lh(u, i):
    return LH + L * (18 * (u % U) + i)


def _b_place_memory(B, u, mem):
    r = _turn(u)
    for i, p in enumerate(TURN[r]):
        B.stf(_lh(u, 2 + i), _signed_sum([(s, mem[k]) for (rr, k), s in PRODUCTS[p][0].items() if rr == r]))
    for i in range(2):
        B.stf(_lh(u, i), mem[4])


def _b_place_tokens(B, u):
    r = _turn(u)
    top = (u + 1 - r) % U

    def x(seg, n, half):
        return B.ldb(XN + 64 * n + 16 * seg + 8 * half, 8).astype(F32)

    for i, p in enumerate(TURN[r]):
        for at, half in enumerate(_halves(p, r)):
            B.stf(_lh(u, 2 + i) + M + 16 * at,
                  _signed_sum([(s, x(top + rr, k, half)) for (rr, k), s in PRODUCTS[p][0].items()]))
    for half in range(2):
        B.stf(_lh(u, 1) + M + 16 * half, x((u + 1) % U, 4, half))


def _b_project(B, u, mat, g, m=M, keep=()):
    r = _turn(u)
    top = (u + 1 - r) % U
    items = [(PRODUCTS[p][2], _halves(p, r),
              _dot(B.ldf(_lh(u, 2 + TURN[r].index(p)) + M - m, m + 16 * len(_halves(p, r))),
                   B.ldb(GSTRIDE * g + (mat * NPR + p) * 64, 64))) for p in ORDER[r]]
    if mat == 0:
        items += [({(r, n): 1}, (0, 1),
                   _dot(B.ldf(_lh(u, 1) + M - m, m + SEG)[:, :64],
                        B.ldb(Q2 + PSTRIDE * (h // 2) + 32 * (h % 2), 32))) for n, h in enumerate(_heads(g))]

    def at(n, seg, half):
        return TK + 128 * (H * mat + _heads(g)[n]) + SEG * seg + 16 * half

    mem, tok, kept = {}, {}, {}
    for c, halves, y in items:
        y_mem, y_tok = y[:m] if m else None, [y[o:o + 16] for o in range(m, y.shape[0], 16)]
        for (rr, n), s in c.items():
            if m and rr == r:
                mem.setdefault(n, []).append((s, y_mem))
            for half, t in zip(halves, y_tok):
                tok.setdefault((rr, n, half), []).append((s, t))
    for (rr, n, half), terms in sorted(tok.items()):
        if r == 1:
            terms.append((1, B.ldf(at(n, top + rr, half), 16)))
        if r == 1 and rr in keep:
            kept[n, top + rr, half] = _signed_sum(terms)
        else:
            B.stf(at(n, top + rr, half), _signed_sum(terms))
    assert len(tok) == 16

    def tokens(n, seg):
        return [kept[n, seg, i] if (n, seg, i) in kept else B.ldf(at(n, seg, i), 16) for i in range(2)]

    return [_signed_sum(mem[n]) for n in sorted(mem)], tokens


def _b_out_product(B, u, p, g, acc, m=M):
    r = _turn(u)
    top = (u - 1 - r) % U
    a = PRODUCTS[p][0].items()
    lhs = [_signed_sum([(s, B.ldf(OM + M * _heads(g)[k], M)) for (rr, k), s in a if rr == r])] if m else []
    both = [k for (rr, k), s in a if rr and PRODUCTS[p][0].get((0, k)) == -s]
    first, rows = 16 * _halves(p, r)[0], 16 * len(_halves(p, r))
    lhs.append(_signed_sum([(s, B.ldf(OF + SEG * (H * (U if k in both else top + rr) + _heads(g)[k]) + first, rows))
                            for (rr, k), s in a if not (rr and k in both)]))
    y = _dot(jnp.concatenate(lhs, 0), B.ldb(OA + (g * NPR + p) * 64, 64))
    acc[p] = acc[p] + y if g else y
    if g == NG - 1:
        B.stf(AC + SEG * p + first, acc[p][m:])
        for (rr, n), s in PRODUCTS[p][2].items():
            if m and rr == r:
                acc.setdefault(("mem", n), []).append((s, acc[p][:m]))


def _b_out_collect(B, u):
    for rr in range(2):
        for n in range(4):
            B.stf(BO + 128 * n + SEG * ((u - 2 + rr) % U), _signed_sum(
                [(c[rr, n], B.ldf(AC + SEG * p, SEG)) for p, (_, _, c) in enumerate(PRODUCTS) if (rr, n) in c]))


def _b_out_tail(B, u):
    B.stf(B2 + 64 * u, functools.reduce(jnp.add, [
        _dot_nt(B.ldb(O2T + 32 * h, 32),
                jnp.concatenate([B.ldf(OF + SEG * (H * i + h), SEG) for i in range(U)], 0).astype(BF16))
        for h in range(8 * u, 8 * u + 8)]))


def _b_step(B, u, emit, after_use, spare):
    row = lax.broadcasted_iota(I32, (L, 128), 0)
    lane = lax.broadcasted_iota(I32, (L, 128), 1)
    lo = lane < 64
    lo64 = lax.broadcasted_iota(I32, (64, 128), 1) < 64
    mask = (row < M) | ((lane & 63) >= SEG) | (row - M >= (lane & 63))
    in_a, in_b = lane < L, (lane >= 64) & (lane < 64 + L)
    z24 = jnp.zeros((24, 128), F32)
    pair = [j for g in range(NG) for j in _pairs(g)]

    def h2():
        return jnp.concatenate([B.ldf(_lh(u, 0) + M, SEG), B.ldf(_lh(u, 0), M)], 0)

    def t_k(g):
        mem, tokens = _b_project(B, u, 1, g, keep=(0,))
        spare(mem[0])
        for i, j in enumerate(_pairs(g)):
            k = jnp.concatenate([t for n in (2 * i, 2 * i + 1) for t in tokens(n, u) + [mem[n], z24]], 0)
            B.stb(KS + 64 * j, k.astype(BF16).T)

    def t_q(g):
        for h, t in zip(_heads(g), _b_project(B, u, 0, g)[0]):
            B.stf(MQ + M * h, t)

    def t_v(g):
        mem, tokens = _b_project(B, u, 2, g, keep=(0, 1))
        for n, h in enumerate(_heads(g)):
            B.stb(VS + 40 * h + 32, jnp.concatenate([mem[n], z24[:8]], 0))
            if _turn(u):
                B.stb(VS + 40 * h, jnp.concatenate(tokens(n, u) + tokens(n, u + 1), 0))

    def t_s(i):
        j = pair[i]
        kt, w2 = B.ldi(KS + 64 * j, 64), B.ldi(K2 + PSTRIDE * j, 64)
        ya, yb = [_dot(jnp.concatenate([B.ldf(MQ + M * h, M), B.ldf(TK + 128 * h + SEG * u, SEG)], 0),
                       pltpu.bitcast(rhs, BF16))
                  for h, rhs in ((2 * j, jnp.where(lo64, kt, w2)), (2 * j + 1, jnp.where(lo64, w2, kt)))]
        B.stf(RE + L * i, jnp.where(lo, ya, yb))
        B.stf(RE + L * (NP + i), jnp.where(lo, yb, ya))

    def t_softmax(n):
        c4 = h2()
        y = _dot_nt(jnp.concatenate([jnp.where(lo, 0.0, c4), jnp.where(lo, c4, 0.0)], 0),
                    B.ldf(RE + L * NP + 128 * n, 128).astype(BF16))
        B.stf(RS + 128 * n, jnp.concatenate([y[:L], z24, y[L:], z24], 0).T)
        for i in range(128 * n // L, 128 * (n + 1) // L):
            s = jnp.where(mask, (B.ldf(RE + L * i, L) + B.ldf(RS + L * i, L)) * DH ** -0.5, NEG)
            ma = jnp.max(jnp.where(in_a, s, -jnp.inf), axis=1, keepdims=True)
            mb = jnp.max(jnp.where(in_b, s, -jnp.inf), axis=1, keepdims=True)
            e = jnp.exp(s - jnp.where(lo, ma, mb))
            B.stf(PS + L * i, jnp.where(in_a | in_b, e, 0.0))

    def t_pv(i):
        p, r = B.ldf(PS + L * i, L), B.ldf(RS + L * i, L)
        for b, lhs in enumerate((jnp.where(lo, p, r), jnp.where(lo, r, p))):
            h = 2 * pair[i] + b
            v = [B.ldi(VS + 40 * h + 16 * (u % 2), 16), B.ldi(VS + 40 * h + 32, 8), jnp.zeros((8, 128), I32)]
            w2 = [B.ldi(V2 + PSTRIDE * pair[i] + 32 * b, 32)]
            o = _dot(lhs, pltpu.bitcast(jnp.concatenate(w2 + v if b else v + w2, 0), BF16))
            l = jnp.broadcast_to(jnp.sum(jnp.where(in_b if b else in_a, p, 0.0), axis=1, keepdims=True), (L, 128))
            rc = pltpu.reciprocal(l, approx=True)
            o = o * (rc * (2.0 - l * rc))
            B.stf(OM + M * h, o[:M])
            B.stf(OF + SEG * (H * u + h), o[M:])
            if u % 2:
                B.stf(OF + SEG * (H * U + h), B.ldf(OF + SEG * (H * (u - 1) + h), SEG) - o[M:])

    acc = {}

    def t_mem_tail(i):
        y = _dot(B.ldf(OM + 2 * M * pair[i], 2 * M), B.ldb(O2 + 64 * pair[i], 64))
        acc["tail"] = acc["tail"] + y if i else y

    for g in range(NG):
        t_k(g)
        if g == 1 and u % 2:
            _b_out_collect(B, u - 1)
    c4 = h2()
    B.stb(GS, jnp.concatenate([jnp.where(lo, 0.0, c4), z24, jnp.where(lo, c4, 0.0), z24], 0))
    lag_s, lag_softmax = 2, 4
    softmax_at = [(128 * n + 127) // L + lag_s + lag_softmax for n in range(5)]
    for i in range(2 * NP - 2):
        if i % 2 == 0:
            t_q(i // 2) if i < NP else t_v((i - NP) // 2)
        if 0 <= i - lag_s < NP:
            t_s(i - lag_s)
        if i in (2, 6):
            emit(i // 4)
        if i in softmax_at:
            t_softmax(softmax_at.index(i))
        for j in range(4 * (i - 2 * NP + 6), 4 * (i - 2 * NP + 7)):
            if j >= 0:
                B.stf(RS + L * j, _dot(B.ldf(PS + L * j, L), B.ldb(GS, 64)))
    prods = TURN[_turn(u)]
    passes = (((14, 5, 0, 12, 10), (1, 3, 4, 15), (8, 9, 6, 11), (13, 7, 2)),
              ((7, 5, 0, 12, 10), (8, 3, 4, 6, 13), (1, 15, 11), (9, 2, 14)))[_turn(u)]

    def t_out(k, g):
        for i in passes[k]:
            _b_out_product(B, u, prods[i], g, acc)
        if k < 2:
            t_mem_tail(NG * k + g)

    for g in range(NG + 2):
        if g < NG:
            t_pv(2 * g)
            t_pv(2 * g + 1)
        elif g == NG:
            t_out(1, 0)
        if g == 2:
            t_v(NG - 1)
        if g >= 2:
            t_out(0, g - 2)
    after_use()
    for k in range(1, len(passes)):
        for g in range(1 if k == 1 else 0, NG):
            t_out(k, g)
    tail = jnp.where(lo[:M], acc["tail"][:M], acc["tail"][M:])
    _b_place_memory(B, u + 1, [_signed_sum(acc["mem", n]) for n in range(4)] + [tail + pltpu.roll(tail, 64, 1)])
    _b_out_tail(B, u)


def _squares(t):
    t = pltpu.bitcast(t, I32)
    even, odd = pltpu.bitcast(t << 16, F32), pltpu.bitcast(t, F32)
    return even * even, odd * odd


def _b_norms(qkv, wot, out):
    for m in range(3):
        acc = None
        for d in range(32):
            sq = jnp.concatenate(_squares(qkv[RAW * m + H * d:RAW * m + H * d + H, :]), 0)
            acc = acc + sq if d else sq
            row = jnp.broadcast_to(jnp.sum(sq[:8] + sq[8:16] + sq[16:24] + sq[24:], axis=1, keepdims=True), (8, 128))
            lo, hi = (jnp.minimum(lo, row), jnp.maximum(hi, row)) if d else (row, row)
            if d == 31:
                out[32 * m:32 * m + 32, :] = acc
                out[168 + 16 * m:184 + 16 * m, :] = jnp.concatenate([lo, hi], 0)
            yield acc
    for i in range(8):
        for d in range(4):
            o = D * (i // 4) + 128 * (i % 4) + 32 * d
            sq = jnp.add(*_squares(wot[o:o + 32, :]))
            acc = acc + sq if d else sq
            if d == 3:
                out[96 + 8 * i:104 + 8 * i, :] = acc[:8] + acc[8:]
            yield acc


def _b_one_scale(norms):
    kinds = [[functools.reduce(jnp.add, [norms[4 * k + i, 32 * m:32 * m + 32, :] for i in range(4)])
              for k in range(4)] for m in range(3)]
    kinds += [[norms[g, 168 + 16 * m:184 + 16 * m, :] for g in range(NB)] for m in range(3)]
    kinds += [[jnp.sum(norms[g, o:o + 8, :], axis=0, keepdims=True) for g in range(NB) for o in offsets]
              for offsets in (range(96, 160, 8), (160,))]
    ok = []
    for ts in kinds:
        lo, hi = jnp.min(functools.reduce(jnp.minimum, ts)), jnp.max(functools.reduce(jnp.maximum, ts))
        ok += [hi <= 4.0 * lo, lo > 0.0, hi < jnp.inf]
    return functools.reduce(jnp.logical_and, ok)


def _b_direct(b_ref, raw, mem0, x_tile, emit):
    def split(i, carry):
        for m in range(3):
            _interleave(_b_split_heads(raw.at[pl.ds(pl.multiple_of(RAW * m + i * 16 * H, 16), 16 * H)],
                                       b_ref.at[pl.ds(pl.multiple_of(i * 8, 8), O2), :],
                                       288 * m, 288 * (3 + m), 6 * 288))

    lax.fori_loop(0, D // 16, split, None)
    row = lax.broadcasted_iota(I32, (L, L + 8), 0)
    col = lax.broadcasted_iota(I32, (L, L + 8), 1)

    def segment(u, mem):
        x = pltpu.bitcast(_cat576(lambda n: b_ref[pl.ds(pl.multiple_of(TK + 128 * n + SEG * u, SEG), SEG), :]), F32)
        h = jnp.concatenate([mem, x, jnp.zeros((8, D), F32)], 0).astype(BF16)

        def head(i, acc):
            q, k, v = [_dot(h, pltpu.bitcast(b_ref[pl.ds(pl.multiple_of(288 * (3 * i + m), 8), 288), :], BF16))
                       for m in range(3)]
            s = jnp.where((row < M) | (row >= col), _dot_nt(q[:L], k.astype(BF16)) * DH ** -0.5, NEG)
            s = jnp.where(col < L, s, -jnp.inf)
            e = jnp.exp(s - jnp.max(s, axis=1, keepdims=True))
            o = _dot(e / jnp.sum(e, axis=1, keepdims=True), v.astype(BF16))
            return acc + _dot_nt(o, raw[pl.ds(pl.multiple_of(3 * RAW + D * i, 16), D), :])

        out = lax.fori_loop(0, H, head, jnp.zeros((L, D), F32))
        for n in range(5):
            c = min(128 * n, D - 128)
            b_ref[pl.ds(pl.multiple_of(RE + 128 * n + SEG * u, 8), SEG), :] = pltpu.bitcast(out[M:, c:c + 128], I32)
        return out[:M]

    def block(j, mem):
        for n in range(5):
            _Arena(b_ref).stf(TK + 128 * n, x_tile(j, n).T.astype(F32))
        mem = lax.fori_loop(0, U, segment, mem)
        for n in range(5):
            emit(j, n, _Arena(b_ref).ldf(RE + 128 * n, 128).T[64 * (n // 4):])
        return mem

    lax.fori_loop(0, NB, block, mem0)


def _kernel(xt_hbm, wqkv_hbm, wo_hbm, mem_hbm, gate_hbm, wq_hbm, wk_hbm, wv_hbm, wot_hbm,
            out_hbm,
            xt, wqkv, wo, mem_ref, gate_ref, raw, a_ref, b_ref, qkv_all, o_all, o_last, ga_all, omg, out_buf,
            norms, offs, sem_in, sem_w, sem_out):
    A, B = _Arena(a_ref), _Arena(b_ref)
    wot = raw.at[pl.ds(3 * RAW, H * D)]

    def cols(src, dst, c0, c1, sem):
        return pltpu.make_async_copy(src.at[:, pl.ds(c0, c1 - c0)], dst.at[:, pl.ds(c0, c1 - c0)], sem_in.at[sem])

    def rows(r0, r1, sem):
        return [pltpu.make_async_copy(w.at[pl.ds(r0 * H, (r1 - r0) * H)],
                                      raw.at[pl.ds(RAW * m + r0 * H, (r1 - r0) * H)], sem_w.at[sem])
                for m, w in enumerate((wq_hbm, wk_hbm, wv_hbm))]

    def x_stage(j, slot):
        A.stb(AX + 288 * slot, xt[:, pl.ds(pl.multiple_of(j * 128, 128), 128)])

    def x_tile(j, n):
        block = pl.ds(pl.multiple_of(j * 128, 128), 128)
        return xt[128 * n:128 * n + 128, block] if n < 4 else jnp.concatenate([xt[512:D, block]] * 2, 0)

    def x_transpose(j):
        sq = []
        for n in range(5):
            t = x_tile(j, n)
            B.stb(XN + 64 * n, t.T)
            if n < 4:
                parts = _squares(t)
                sq += [part[i:i + 8] for i in range(0, 64, 8) for part in parts]
        norms[j, 160:168, :] = functools.reduce(jnp.add, sq)

    def x_tail(u):
        B.stf(_lh(u, 0) + M, B.ldb(XN + 256 + 16 * u, 16).astype(F32))

    def tick_raw(r):
        raw[D * H:D * H + 8, :] = r[:8].astype(BF16)

    def proj(j):
        if isinstance(j, int):
            return _Arena(qkv_all.at[pl.ds((j + 1) % 5 * SLOT, SLOT)])
        return _Arena(qkv_all.at[pl.ds(pl.multiple_of(offs[lax.rem(j + 1, 5)], 8), SLOT)])

    def raw_from(i, n):
        return raw.at[pl.ds(pl.multiple_of(offs[5 + i], 16), 2 * RAW + n * H)]

    x_copy = [cols(xt_hbm, xt, c0, c1, i) for i, (c0, c1) in enumerate(((0, 256), (256, 768), (768, S)))]
    w_copy = [cols(wqkv_hbm, wqkv, c0, c1, 3 + i) for i, (c0, c1) in
              enumerate(((512, 896), (896, 1152), (0, 512), (1152, 3 * D)))]
    wo_copy = pltpu.make_async_copy(wo_hbm, wo, sem_in.at[7])
    mem_copy = pltpu.make_async_copy(mem_hbm, mem_ref, sem_in.at[8])
    gate_copy = pltpu.make_async_copy(gate_hbm, gate_ref, sem_in.at[9])
    tail_copies, main_copies = rows(512, D, 0), rows(0, 512, 1)
    wot_copy = pltpu.make_async_copy(wot_hbm, wot, sem_w.at[2])
    for c in (w_copy[0], gate_copy, mem_copy, w_copy[1], x_copy[0], w_copy[2], w_copy[3], wo_copy):
        c.start()

    for i in range(5):
        offs[i] = i * SLOT
    for i in range(18):
        offs[5 + i] = 32 * H * i
    for i in range(NB):
        offs[23 + i] = 3 * RAW + 2 * D * i
    A.stb(SUMS, _b_sum_matrix())
    B.stf(OF + H * SEG, jnp.zeros((B_ROWS - OF - H * SEG, 128), F32))
    B.stf(AC, jnp.zeros((NPR * SEG, 128), F32))
    w_copy[0].wait()
    gate_copy.wait()
    mem_copy.wait()
    gate = jnp.broadcast_to(gate_ref[...].astype(F32)[None, :], (8, D))
    mem0 = mem_ref[...].astype(F32)
    for k in range(4):
        A.stf(GW + 8 * k, gate[:, 128 * k:128 * k + 128])
    A.stf(GW + 32, jnp.concatenate([gate[:, 512:]] * 2, 1))
    _b_place_memory(B, 0, [mem0[:, 128 * k:128 * k + 128] for k in range(4)]
                    + [jnp.concatenate([mem0[:, 512:]] * 2, 1)])

    def project(j, *parts):
        return _a_qkv(A, AX + 288 * j, proj(j), parts, first=j == 0)

    _a_transpose_w(A, wqkv, range(4, 7))
    w_copy[1].wait()
    _a_transpose_w(A, wqkv, range(7, 9))
    x_copy[0].wait()
    x_stage(0, 0)
    x_stage(1, 1)
    _interleave(project(0, 3, 1))
    x_transpose(0)
    for u in range(U):
        x_tail(u)
        _b_place_tokens(B, u)
    x_transpose(1)
    w_copy[2].wait()
    x_copy[1].start()
    _a_transpose_w(A, wqkv, range(0, 4))
    _interleave(_chain(project(1, 3, 1), project(0, 0)))
    w_copy[3].wait()
    x_copy[2].start()
    _a_transpose_w(A, wqkv, range(9, 14))
    _interleave(_chain(project(1, 0), project(0, 2)))
    wo_copy.wait()
    for c in tail_copies:
        c.start()
    _interleave(project(1, 2))
    _a_transpose_wo(A, wo)
    qkv_all[AK:AG, :] = jnp.broadcast_to(qkv_all[SLOT + AK:SLOT + AG, :1], (AG - AK, 128))

    def project_out(j0, n, tick=lambda r: None):
        return _chain(*[_a_out(A, o_all.at[j0 + b], ga_all.at[j0 + b], tick) for b in range(n)])

    def attend_trip(t, carry):
        @pl.when(t == 1)
        def _():
            x_copy[2].wait()
            wot_copy.start()

        _interleave(
            _chain(*[_chain(_a_qkv(A, AX + 288 * i, proj(2 * t + 2 + i)),
                            _once(x_stage, jnp.minimum(2 * t + 4 + i, NB - 1), i)) for i in range(2)]),
            _chain(*[_a_attend(j, proj(j), proj(j - 1), o_all.at[j], omg) for j in (2 * t, 2 * t + 1)]),
            span=(-0.04, 0.87))

    x_copy[1].wait()
    for c in main_copies:
        c.start()
    x_stage(2, 0)
    x_stage(3, 1)
    lax.fori_loop(0, NB // 2 - 1, attend_trip, None)

    def last_trip(t, carry):
        def tick(r):
            qkv_all[TICK:TICK + 8, :] = pltpu.bitcast(r[:8], I32)
            tick_raw(r)

        j = NB - 2 + t
        src, dst = raw_from(16 + t, 32), b_ref.at[pl.ds(pl.multiple_of(t * 16, 16), O2), :]
        _interleave(
            project_out(3 * t, 3, tick), _a_attend(j, proj(j), proj(j - 1), o_last.at[t], omg),
            _chain(*[_b_split_heads(src.at[pl.ds(RAW * m, 32 * H)], dst, even, odd) for m, (even, odd) in
                     enumerate(((Q2, Q2 + 32), (K2 + 32, K2), (V2, V2 + 32)))]),
            span=(-0.08, 0.82))

    for c in tail_copies:
        c.wait()
    lax.fori_loop(0, 2, last_trip, None)
    o_all[NB - 2:, :288, :] = o_last[:, :288, :]

    def prepare_trip(t, carry):
        src, dst = raw_from(t, 416), b_ref.at[pl.ds(pl.multiple_of(t * 16, 16), O2), :]
        _interleave(project_out(6 + 2 * t, 2), _chain(*[
            _b_product_tiles(A, src.at[pl.ds(RAW * m, 416 * H)], dst, m * NPR * 64) for m in range(3)]),
            span=(-0.04, 0.93))

    for c in main_copies:
        c.wait()
    lax.fori_loop(0, 4, prepare_trip, None)
    wot_copy.wait()
    _interleave(
        _chain(project_out(NB - 2, 2),
               *[_once(_b_project, B, U - 1, mat, g, 0) for mat in range(3) for g in range(NG)]),
        _b_transpose_wo(B, wot))

    def tail_sum(last, first_steps):
        lane = lax.broadcasted_iota(I32, (64, 128), 1)
        return functools.reduce(jnp.add, [B.ldf(B2 + 64 * last, 64)] + [
            jnp.where(lane < SEG * (u + 1) if first_steps else lane >= SEG * (u + 1), B.ldf(B2 + 64 * u, 64), 0.0)
            for u in range(U - 1)])

    def mix(j, n, bt):
        part = slice(128 * n, 128 * n + bt.shape[0])
        w = jnp.concatenate([omg[j]] * (bt.shape[0] // 8), 0)
        out_buf[j, part, :] = (ga_all[j, part, :] + w * bt).astype(BF16)

    def out_copy(j):
        return pltpu.make_async_copy(
            out_buf.at[j], out_hbm.at[:, pl.ds(pl.multiple_of(j * 128, 128), 128)], sem_out)

    def b_body(g, carry):
        done = jnp.maximum(g - 1, 0)
        B.stf(B2 + 64 * U, tail_sum(U - 1, True))
        weights = _b_norms(raw_from(g, 32), raw.at[pl.ds(pl.multiple_of(offs[23 + g], 16), 2 * D)], norms.at[g])

        def spare(r):
            t = [next(weights) for _ in range(4)][-1]
            tick_raw(functools.reduce(jnp.add, [r] + [t[i:i + 8] for i in range(0, t.shape[0], 8)]))

        for u in range(U):
            def emit(stage):
                if u == 1:
                    for n in range(4):
                        if stage:
                            mix(done, n, B.ldf(PS + 128 * n, 128))
                        else:
                            B.stf(PS + 128 * n, B.ldf(BO + 128 * n, 128).T)
                if u == U - 1 and stage:
                    mix(done, 4, tail_sum(U, False))

            def after_use():
                x_tail(u)
                if u == 0:
                    _b_place_tokens(B, U - 1)
                if u < U - 1:
                    _b_place_tokens(B, u)
                else:
                    x_transpose(jnp.minimum(g + 2, NB - 1))

            _b_step(B, u, emit, after_use, spare)
        assert next(weights, "end") == "end"

        @pl.when(g > 0)
        def _():
            out_copy(done).start()

        return carry

    lax.fori_loop(0, NB, b_body, 0)
    acc = {}
    for g in range(NG):
        for p in TURN[1]:
            _b_out_product(B, 0, p, g, acc, 0)
    _b_out_collect(B, 0)
    B.stf(B2 + 64 * U, tail_sum(U - 1, True))
    for u in range(U - 1):
        _b_out_tail(B, u)
    for n in range(4):
        mix(NB - 1, n, B.ldf(BO + 128 * n, 128).T)
    mix(NB - 1, 4, tail_sum(U, False))
    out_copy(NB - 1).start()
    one_scale = _b_one_scale(norms)
    for j in range(NB):
        out_copy(j).wait()

    @pl.when(jnp.logical_not(one_scale))
    def _():
        _b_direct(b_ref, raw, mem_ref[...].astype(F32), x_tile, mix)
        copies = [out_copy(j) for j in range(NB)]
        for c in copies:
            c.start()
        for c in copies:
            c.wait()


@functools.partial(jax.jit, static_argnames=("B_seg_len",))
def pallas_gated_mix__sliding_local_dilated__memory_aug_recurrent_mem_tr__prompt_kernel(
    A_x: jax.Array,
    A_wqkv: jax.Array,
    A_wo: jax.Array,
    B_x: jax.Array,
    B_mem0: jax.Array,
    B_Wq: jax.Array,
    B_Wk: jax.Array,
    B_Wv: jax.Array,
    B_Wo: jax.Array,
    B_seg_len: int,
    gate_w: jax.Array,
):
    del B_x
    assert A_x.shape == (1, S, D) and B_mem0.shape == (1, M, D) and B_Wq.shape == (D, H, DH)
    assert B_seg_len == SEG
    hbm = pl.BlockSpec(memory_space=pl.ANY)
    out_t = pl.pallas_call(
        _kernel,
        out_shape=jax.ShapeDtypeStruct((D, S), BF16),
        in_specs=[hbm] * 9,
        out_specs=hbm,
        scratch_shapes=[
            pltpu.VMEM((D, S), BF16),
            pltpu.VMEM((D, 3 * D), BF16),
            pltpu.VMEM((D, D), BF16),
            pltpu.VMEM((M, D), BF16),
            pltpu.VMEM((D,), BF16),
            pltpu.VMEM((4 * RAW, DH), BF16),
            pltpu.VMEM((A_ROWS, 128), I32),
            pltpu.VMEM((B_ROWS, 128), I32),
            pltpu.VMEM((5 * SLOT, 128), I32),
            pltpu.VMEM((NB, 296, 128), I32),
            pltpu.VMEM((2, 296, 128), I32),
            pltpu.VMEM((NB, D, 128), F32),
            pltpu.VMEM((NB, 8, 128), F32),
            pltpu.VMEM((NB, D, 128), BF16),
            pltpu.VMEM((NB, 216, 128), F32),
            pltpu.SMEM((39,), I32),
            pltpu.SemaphoreType.DMA((10,)),
            pltpu.SemaphoreType.DMA((3,)),
            pltpu.SemaphoreType.DMA,
        ],
        compiler_params=pltpu.CompilerParams(vmem_limit_bytes=110 * 1024 * 1024),
    )(
        A_x.reshape(S, D).T, A_wqkv, A_wo, B_mem0.reshape(M, D), gate_w,
        B_Wq.reshape(D * H, DH), B_Wk.reshape(D * H, DH), B_Wv.reshape(D * H, DH),
        B_Wo.transpose(0, 2, 1).reshape(H * D, DH),
    )
    return out_t.T.reshape(1, S, D)
```
